```python
import jax
import jax.numpy as jnp

def _softmax(x, axis=-1):
    return jax.nn.softmax(x, axis=axis)

def _gelu(x):
    return jax.nn.gelu(x, approximate=True)

def _silu(x):
    return jax.nn.silu(x)

def _sigmoid(x):
    return jax.nn.sigmoid(x)

def _layernorm(x, axis=-1, eps=1e-05):
    m = jnp.mean(x, axis=axis, keepdims=True)
    v = jnp.var(x, axis=axis, keepdims=True)
    return (x - m) / jnp.sqrt(v + eps)

def _scatter_add(tgt, idx, src, axis=0):
    return tgt.at[idx].add(src)

def _segment_sum(src, seg, n):
    return jax.ops.segment_sum(src, seg, n)

class _Rng:

    def __init__(self, key):
        self._k = key

    def _next(self):
        self._k, sub = jax.random.split(self._k)
        return sub

    def normal(self, shape):
        return jax.random.normal(self._next(), shape, dtype=jnp.bfloat16)

    def randint(self, lo, hi, shape):
        return jax.random.randint(self._next(), shape, lo, hi, dtype=jnp.int32)

    def uniform(self, shape, lo=0.0, hi=1.0):
        return jax.random.uniform(self._next(), shape, jnp.bfloat16, lo, hi)

    def permutation(self, n):
        return jax.random.permutation(self._next(), n)
kernel_name = 'recurrent_scan__ssm_conv_h3__mixer_gmlp__prompt'

def setup_inputs():
    _rng = _Rng(jax.random.key(int.from_bytes(__import__("os").urandom(4), "little")))
    _w = lambda a: (lambda t: t.astype(jnp.bfloat16) if jnp.issubdtype(t.dtype, jnp.floating) else t)(jnp.asarray(a))

    def _A_setup():
        B, S, D = (1, 2048, 640)
        ks = 4
        return {'q': _w((lambda *s: _rng.normal(s) * 0.05)(B, S, D)), 'k': _w((lambda *s: _rng.normal(s) * 0.05)(B, S, D)), 'v': _w((lambda *s: _rng.normal(s) * 0.05)(B, S, D)), 'shift_k': _w((lambda *s: _rng.normal(s) * 0.05)(D, ks) * 0.5), 'ssm_k': _w((lambda *s: _rng.normal(s) * 0.05)(D, S) * (1.0 / S ** 0.5)), 'ssm_D': _w((lambda *s: _rng.normal(s) * 0.05)(D))}
    _A_in = _A_setup()

    def _B_setup():
        B, S, D, F = (1, 2048, 640, 1536)
        Fh = F // 2
        return {'x': _w((lambda *s: _rng.normal(s) * 0.05)(B, S, D)), 'w_in': _w((lambda *s: _rng.normal(s) * 0.05)(D, 2 * Fh)), 'w_sp': _w(0.01 * (lambda *s: _rng.normal(s) * 0.05)(S, S)), 'b_sp': _w(1.0 + 0.01 * (lambda *s: _rng.normal(s) * 0.05)(S)), 'w_out': _w((lambda *s: _rng.normal(s) * 0.05)(Fh, D))}
    _B_in = _B_setup()
    return {'A_q': _A_in['q'], 'A_k': _A_in['k'], 'A_v': _A_in['v'], 'A_shift_k': _A_in['shift_k'], 'A_ssm_k': _A_in['ssm_k'], 'A_ssm_D': _A_in['ssm_D'], 'B_x': _B_in['x'], 'B_w_in': _B_in['w_in'], 'B_w_sp': _B_in['w_sp'], 'B_b_sp': _B_in['b_sp'], 'B_w_out': _B_in['w_out']}

def reference(A_q, A_k, A_v, A_shift_k, A_ssm_k, A_ssm_D, B_x, B_w_in, B_w_sp, B_b_sp, B_w_out):

    def _A_ref(q, k, v, shift_k, ssm_k, ssm_D):
        B, S, D = q.shape
        ks = shift_k.shape[-1]
        k_pad = jnp.pad(k, ((0, 0), (ks - 1, 0), (0, 0)))
        k_shift = jnp.zeros_like(k)
        for t in range(ks):
            k_shift = k_shift + k_pad[:, t:t + S, :] * shift_k[:, ks - 1 - t][None, None, :]
        kv = k_shift * v
        L = 2 * S
        kv_pad = jnp.pad(kv, ((0, 0), (0, S), (0, 0)))
        kf_pad = jnp.pad(ssm_k, ((0, 0), (0, S)))
        kv_f = (lambda x, axes=(-2, -1): jnp.fft.rfft2(x.astype(jnp.float32), axes=axes))(kv_pad[:, None, :, :], axes=(1, 2))
        kf_f = (lambda x, axes=(-2, -1): jnp.fft.rfft2(x.astype(jnp.float32), axes=axes))(kf_pad[:, None, :], axes=(1, 2))
        kf_f = (lambda x, *d: x.transpose(*d))(kf_f, 1, 2, 0)
        y_f = kv_f * kf_f[None, :, :, :]
        y = (lambda x, s, axes=(-2, -1): jnp.fft.irfft2(x, s=s, axes=axes).astype(jnp.bfloat16))(y_f, (1, L), axes=(1, 2))[:, 0, :S, :]
        y = y + kv * ssm_D[None, None, :]
        return q * y

    def _B_ref(x, w_in, w_sp, b_sp, w_out):
        B, S, D = x.shape
        F = w_in.shape[-1]
        Fh = F // 2
        z = _gelu(jnp.einsum('bsd,df->bsf', x, w_in))
        z1 = z[..., :Fh].copy()
        z2 = _layernorm(z[..., Fh:], axis=-1)
        g = jnp.einsum('ts,bsf->btf', w_sp, z2) + b_sp[None, :, None]
        return jnp.einsum('bsf,fd->bsd', z1 * g, w_out)
    x = A_q
    xn = _layernorm(x, axis=-1)
    s = _A_ref(xn, A_k, A_v, A_shift_k, A_ssm_k, A_ssm_D)
    g = _silu(_B_ref(xn, B_w_in, B_w_sp, B_b_sp, B_w_out))
    return x + s * g
```

```python
import functools

import jax
import jax.numpy as jnp
import numpy as np
import jax.experimental.pallas as pl
import jax.experimental.pallas.tpu as pltpu

F32 = jnp.float32
BF16 = jnp.bfloat16

S = 2048
D = 640
FH = 768
KS = 4
BLK = 128
NB = S // BLK
NC = D // 128
NF = FH // 128
RT = 256
NR = S // RT
EPS = 1e-5

_GELU_C0 = float(np.sqrt(2.0 / np.pi))
_GELU_C1 = _GELU_C0 * 0.044715


def _dft_tables():
    m = np.arange(BLK)[:, None]
    n = np.arange(BLK)[None, :]
    ang = 2.0 * np.pi * (((4 * m + 1) * n) % (4 * BLK)) / (4 * BLK)
    fwd = np.concatenate([np.cos(ang), -np.sin(ang)], axis=0)
    inv = fwd.T / (2.0 * BLK)
    return fwd.astype(np.float32), inv.astype(np.float32)


def _layernorm(x, eps):
    m = jnp.mean(x, axis=-1, keepdims=True)
    d = x - m
    v = jnp.mean(d * d, axis=-1, keepdims=True)
    return d * jax.lax.rsqrt(v + eps)


def _gelu2(x):
    u = x * (x * x * _GELU_C1 + _GELU_C0)
    return x * (1.0 + jnp.tanh(u))


def _kernel(x_hbm, k_hbm, v_hbm, skt_ref, h_hbm, dv_ref, win_hbm, wsp_hbm, b_ref,
            wout_hbm, f_ref, g_ref, out_hbm,
            x_v, win_v, wsp_v, wout_v, k_v, v_v, h_v, xn_v, z1_v, z2_v, p_v, y_v,
            kf_v, ua_v, ub_v, us_v, hp_v, hq_v, hr_v, zz_v, bcol_v, sk_v, dd_v,
            o_v, sem_x, sem_w, sem_c, sem_o):
    def x_cp(j):
        return pltpu.make_async_copy(
            x_hbm.at[0, pl.ds(j * RT, RT), :], x_v.at[pl.ds(j * RT, RT), :], sem_x.at[j])

    win_cp = pltpu.make_async_copy(win_hbm, win_v, sem_w.at[0])
    wsp_cp = pltpu.make_async_copy(wsp_hbm, wsp_v, sem_w.at[1])
    wout_cp = pltpu.make_async_copy(wout_hbm, wout_v, sem_w.at[2])

    def k_cp(c):
        return pltpu.make_async_copy(
            k_hbm.at[0, :, pl.ds(c * 128, 128)], k_v.at[c], sem_c.at[3 * c])

    def v_cp(c):
        return pltpu.make_async_copy(
            v_hbm.at[0, :, pl.ds(c * 128, 128)], v_v.at[c], sem_c.at[3 * c + 1])

    def h_cp(c):
        return pltpu.make_async_copy(
            h_hbm.at[pl.ds(c * 128, 128), :], h_v.at[c], sem_c.at[3 * c + 2])

    def o_cp(j, slot):
        return pltpu.make_async_copy(
            o_v.at[slot], out_hbm.at[0, pl.ds(j * RT, RT), :], sem_o.at[slot])

    x_cp(0).start()
    win_cp.start()
    for j in range(1, NR):
        x_cp(j).start()

    skt = skt_ref[...].astype(F32)
    dv = dv_ref[...].astype(F32).reshape(1, D)
    for c in range(NC):
        sk_v[c] = skt[:, c * 128:(c + 1) * 128]
        dd_v[c] = dv[:, c * 128:(c + 1) * 128]
    brow = b_ref[...].astype(F32).reshape(1, S)
    bcol_v[...] = jnp.broadcast_to(brow, (128, S)).T
    kf_v[0:8, :] = jnp.zeros((8, 128), F32)

    win_cp.wait()
    wsp_cp.start()
    for c in range(NC):
        k_cp(c).start()
        v_cp(c).start()
        h_cp(c).start()
    wout_cp.start()

    def p1(j, carry):
        r0 = pl.multiple_of(j * RT, RT)
        x_cp(j).wait()
        x = x_v[pl.ds(r0, RT), :].astype(F32)
        xn = _layernorm(x, EPS).astype(BF16)
        xn_v[pl.ds(r0, RT), :] = xn
        z = _gelu2(jnp.dot(xn, win_v[...], preferred_element_type=F32))
        z1 = z[:, :FH].astype(BF16)
        z2 = _layernorm(z[:, FH:], 4.0 * EPS).astype(BF16)
        for n in range(NF):
            z1_v[n, pl.ds(r0, RT), :] = z1[:, n * 128:(n + 1) * 128]
            z2_v[n, pl.ds(r0, RT), :] = z2[:, n * 128:(n + 1) * 128]
        return carry

    jax.lax.fori_loop(0, NR, p1, 0)

    wsp_cp.wait()

    def p2(n, carry):
        k_cp(n).wait()
        v_cp(n).wait()
        h_cp(n).wait()
        kf_v[8:8 + S, :] = k_v[n].astype(F32)
        sk = sk_v[n]
        fwd = f_ref[...]
        for i in range(NB):
            r = 8 + i * BLK
            ks = kf_v[r:r + BLK, :] * sk[0:1, :]
            for t in range(1, KS):
                ks = ks + kf_v[r - t:r - t + BLK, :] * sk[t:t + 1, :]
            kv = (ks * v_v[n, i * BLK:(i + 1) * BLK, :].astype(F32)).astype(BF16)
            u = jnp.dot(fwd, kv, preferred_element_type=F32)
            a, b = u[:BLK], u[BLK:]
            ua_v[i] = a
            ub_v[i] = b
            us_v[i] = a + b
        dd = dd_v[n]
        cp = dp = None
        for i in range(NB):
            hb = h_v[n, :, i * BLK:(i + 1) * BLK]
            hf = jax.lax.dot_general(fwd, hb, (((1,), (1,)), ((), ())),
                                     preferred_element_type=F32)
            c, d = hf[:BLK], hf[BLK:]
            if i == 0:
                c2, d2 = c + dd, d
            else:
                c2, d2 = c - dp, d + cp
            cp, dp = c, d
            hr_v[i] = c2
            hp_v[i] = d2 - c2
            hq_v[i] = c2 + d2
        for f in range(BLK // 16):
            res = []
            for half in range(2):
                rows = slice(f * 16 + half * 8, f * 16 + half * 8 + 8)
                re_l, im_l = [], []
                GRP = 4
                for g0 in range(0, NB, GRP):
                    outs = range(g0, g0 + GRP)
                    planes = []
                    for xv, hv in ((us_v, hr_v), (ua_v, hp_v), (ub_v, hq_v)):
                        top = g0 + GRP
                        hs = [hv[t, rows, :] for t in range(top)]
                        acc = {o: None for o in outs}
                        for jj in range(top):
                            xj = xv[jj, rows, :]
                            for o in outs:
                                if o - jj >= 0:
                                    t = xj * hs[o - jj]
                                    acc[o] = t if acc[o] is None else acc[o] + t
                        planes.append(acc)
                    for o in outs:
                        re_l.append(planes[0][o] - planes[2][o])
                        im_l.append(planes[0][o] + planes[1][o])
                res.append((re_l, im_l))
            for o in range(NB):
                zz_v[o, f * 16:(f + 1) * 16, :] = jnp.concatenate(
                    [res[0][0][o], res[1][0][o]], axis=0).astype(BF16)
                zz_v[o, BLK + f * 16:BLK + (f + 1) * 16, :] = jnp.concatenate(
                    [res[0][1][o], res[1][1][o]], axis=0).astype(BF16)
        inv = g_ref[...]
        for i in range(NB):
            y_v[n, i * BLK:(i + 1) * BLK, :] = jnp.dot(
                inv, zz_v[i], preferred_element_type=F32)
        z2 = z2_v[n]
        for r in range(NR):
            rs = slice(r * RT, (r + 1) * RT)
            g = jnp.dot(wsp_v[rs, :], z2, preferred_element_type=F32) + bcol_v[rs, :]
            p_v[n, rs, :] = (z1_v[n, rs, :].astype(F32) * g).astype(BF16)
        return carry

    jax.lax.fori_loop(0, NC, p2, 0)

    wout_cp.wait()

    def p3(j, carry):
        r0 = pl.multiple_of(j * RT, RT)
        rs = pl.ds(r0, RT)
        slot = j % 2
        g = jnp.dot(wsp_v[rs, :], z2_v[NF - 1], preferred_element_type=F32) + bcol_v[rs, :]
        p5 = (z1_v[NF - 1, rs, :].astype(F32) * g).astype(BF16)
        p = jnp.concatenate([p_v[n, rs, :] for n in range(NF - 1)] + [p5], axis=1)
        o = jnp.dot(p, wout_v[...], preferred_element_type=F32)
        sig = 1.0 / (1.0 + jnp.exp(-0.5 * o))
        y = jnp.concatenate([y_v[c, rs, :] for c in range(NC)], axis=1)
        x = x_v[rs, :].astype(F32)
        xn = xn_v[rs, :].astype(F32)
        res = x + (xn * y) * (o * sig)

        @pl.when(j >= 2)
        def _():
            o_cp(j - 2, slot).wait()

        o_v[slot] = res.astype(BF16)
        o_cp(j, slot).start()
        return carry

    jax.lax.fori_loop(0, NR, p3, 0)
    o_cp(NR - 2, 0).wait()
    o_cp(NR - 1, 1).wait()


@jax.jit
def pallas_recurrent_scan__ssm_conv_h3__mixer_gmlp__prompt_kernel(
    A_q: jax.Array,
    A_k: jax.Array,
    A_v: jax.Array,
    A_shift_k: jax.Array,
    A_ssm_k: jax.Array,
    A_ssm_D: jax.Array,
    B_x: jax.Array,
    B_w_in: jax.Array,
    B_w_sp: jax.Array,
    B_b_sp: jax.Array,
    B_w_out: jax.Array,
):
    del B_x
    fwd, inv = _dft_tables()
    fwd = jnp.asarray(fwd, dtype=BF16)
    inv = jnp.asarray(inv, dtype=BF16)

    any_spec = pl.BlockSpec(memory_space=pl.ANY)
    vmem_spec = pl.BlockSpec(memory_space=pltpu.VMEM)
    plane = pltpu.VMEM((NB, BLK, 128), F32)
    return pl.pallas_call(
        _kernel,
        out_shape=jax.ShapeDtypeStruct((1, S, D), BF16),
        in_specs=[any_spec, any_spec, any_spec, vmem_spec, any_spec, vmem_spec,
                  any_spec, any_spec, vmem_spec, any_spec, vmem_spec, vmem_spec],
        out_specs=any_spec,
        scratch_shapes=[
            pltpu.VMEM((S, D), BF16),
            pltpu.VMEM((D, 2 * FH), BF16),
            pltpu.VMEM((S, S), BF16),
            pltpu.VMEM((FH, D), BF16),
            pltpu.VMEM((NC, S, 128), BF16),
            pltpu.VMEM((NC, S, 128), BF16),
            pltpu.VMEM((NC, 128, S), BF16),
            pltpu.VMEM((S, D), BF16),
            pltpu.VMEM((NF, S, 128), BF16),
            pltpu.VMEM((NF, S, 128), BF16),
            pltpu.VMEM((NF - 1, S, 128), BF16),
            pltpu.VMEM((NC, S, 128), F32),
            pltpu.VMEM((S + 8, 128), F32),
            plane, plane, plane, plane, plane, plane,
            pltpu.VMEM((NB, 2 * BLK, 128), BF16),
            pltpu.VMEM((S, 128), F32),
            pltpu.VMEM((NC, KS, 128), F32),
            pltpu.VMEM((NC, 1, 128), F32),
            pltpu.VMEM((2, RT, D), BF16),
            pltpu.SemaphoreType.DMA((NR,)),
            pltpu.SemaphoreType.DMA((3,)),
            pltpu.SemaphoreType.DMA((3 * NC,)),
            pltpu.SemaphoreType.DMA((2,)),
        ],
        compiler_params=pltpu.CompilerParams(vmem_limit_bytes=100 * 1024 * 1024),
    )(A_q, A_k, A_v, A_shift_k.T, A_ssm_k, A_ssm_D, B_w_in, B_w_sp, B_b_sp, B_w_out,
      fwd, inv)
```

```python
import jax
import jax.numpy as jnp
import numpy as np
import jax.experimental.pallas as pl
import jax.experimental.pallas.tpu as pltpu

F32 = jnp.float32
BF16 = jnp.bfloat16
U32 = jnp.uint32

S = 2048
D = 640
FH = 768
KS = 4
BLK = 128
NB = S // BLK
NC = D // 128
NF = FH // 128
RT = 256
NR = S // RT
SUB = 128
NSUB = RT // SUB
CH = 128
EPS = 1e-5
UA, UB, US, HP, HQ, HR, TOK = (i * NB for i in range(7))
import os
GRP = int(os.environ.get('GRP', 4))
TAP0 = int(os.environ.get('TAP0', 0))
TAP1 = int(os.environ.get('TAP1', 1000))

_GELU_C0 = float(np.sqrt(2.0 / np.pi))
_GELU_C1 = _GELU_C0 * 0.044715


def _dft_tables():
    m = np.arange(BLK)[:, None]
    n = np.arange(BLK)[None, :]
    ang = 2.0 * np.pi * (((4 * m + 1) * n) % (4 * BLK)) / (4 * BLK)
    fwd = np.concatenate([np.cos(ang), -np.sin(ang)], axis=0)
    inv = fwd.T / (4.0 * BLK)
    return fwd.astype(np.float32), inv.astype(np.float32)


def _layernorm(x, eps):
    m = jnp.mean(x, axis=-1, keepdims=True)
    d = x - m
    v = jnp.mean(d * d, axis=-1, keepdims=True)
    return d * jax.lax.rsqrt(v + eps)


def _gelu2(x):
    u = x * (x * x * _GELU_C1 + _GELU_C0)
    return x * (1.0 + jnp.tanh(u))


def _pk(x):
    return pltpu.bitcast(x, U32)


def _up(x):
    return pltpu.bitcast(x, BF16)


def _kernel(x_hbm, k_hbm, v_hbm, skt_ref, h_hbm, dv_ref, win_hbm, wsp_hbm, b_ref,
            wout_hbm, f_ref, g_ref, out_hbm,
            x_v, win_v, wsp_v, wout_v, k_v, v_v, h_v, xn_v, z1_v, z2_v, p_v,
            kf_v, pl_v, zz_v, bcol_v, sk_v, dd_v,
            o_v, zt0_v, zt1_v, fg_v, zero_s, sem_x, sem_w, sem_c, sem_o):
    zt_v = (zt0_v, zt1_v)

    def x_cp(j):
        return pltpu.make_async_copy(
            x_hbm.at[0, pl.ds(j * RT, RT), :], x_v.at[pl.ds(j * RT, RT), :], sem_x.at[j])

    win_cp = pltpu.make_async_copy(win_hbm, win_v.bitcast(BF16), sem_w.at[0])
    wsp_cp = pltpu.make_async_copy(wsp_hbm, wsp_v.bitcast(BF16), sem_w.at[1])
    wout_cp = pltpu.make_async_copy(wout_hbm, wout_v.bitcast(BF16), sem_w.at[2])

    def k_cp(c):
        return pltpu.make_async_copy(
            k_hbm.at[0, :, pl.ds(c * 128, 128)], k_v.at[c], sem_c.at[3 * c])

    def v_cp(c):
        return pltpu.make_async_copy(
            v_hbm.at[0, :, pl.ds(c * 128, 128)], v_v.at[c], sem_c.at[3 * c + 1])

    def h_cp(c):
        return pltpu.make_async_copy(
            h_hbm.at[pl.ds(c * 128, 128), :], h_v.bitcast(BF16).at[c], sem_c.at[3 * c + 2])

    def o_cp(j, slot):
        return pltpu.make_async_copy(
            o_v.at[slot], out_hbm.at[0, pl.ds(j * RT, RT), :], sem_o.at[slot])

    x_cp(0).start()
    win_cp.start()
    for j in range(1, NR):
        x_cp(j).start()

    zero_s[0] = 0
    skt = skt_ref[...].astype(F32)
    dv = dv_ref[...].astype(F32).reshape(1, D)
    for c in range(NC):
        sk_v[c] = skt[:, c * 128:(c + 1) * 128]
        dd_v[c] = dv[:, c * 128:(c + 1) * 128]
    brow = b_ref[...].astype(F32).reshape(1, S)
    bcol_v[...] = jnp.broadcast_to(brow, (128, S)).T
    kf_v[0:8, :] = jnp.zeros((8, 128), F32)
    fg_v[0] = _pk(f_ref[...])
    fg_v[1, 0:64, :] = _pk(g_ref[:, 0:128])
    fg_v[1, 64:128, :] = _pk(g_ref[:, 128:256])

    def ln_x(j):
        x = x_v[pl.ds(pl.multiple_of(j * RT, RT), RT), :].astype(F32)
        xn_v[pl.ds(pl.multiple_of(j * RT, RT), RT), :] = _layernorm(x, EPS).astype(BF16)

    x_cp(0).wait()
    ln_x(0)

    win_cp.wait()
    wsp_cp.start()
    for c in range(NC):
        k_cp(c).start()
        v_cp(c).start()
        h_cp(c).start()
    wout_cp.start()

    def p1(j, carry):
        jn = jnp.minimum(j + 1, NR - 1)
        zero = pl.multiple_of(zero_s[0], 8)

        @pl.when(j + 1 < NR)
        def _():
            x_cp(jn).wait()

        for sub in range(NSUB):
            hs = pl.ds(pl.multiple_of((j * RT + sub * SUB) // 2, SUB // 2), SUB // 2)
            rs = pl.ds(pl.multiple_of(j * RT + sub * SUB, SUB), SUB)
            xn = xn_v[rs, :]
            zt_v[sub][...] = _gelu2(
                jnp.dot(xn, _up(win_v[:, FH:]), preferred_element_type=F32))
            z1 = _gelu2(jnp.dot(xn, _up(win_v[:, :FH]),
                                preferred_element_type=F32)).astype(BF16)
            for n in range(NF):
                z1_v[n, rs, :] = z1[:, n * 128:(n + 1) * 128]
            z2 = _pk(_layernorm(zt_v[sub][pl.ds(zero, SUB), :], 4.0 * EPS).astype(BF16))
            for n in range(NF):
                z2_v[n, hs, :] = z2[:, n * 128:(n + 1) * 128]
        ln_x(jn)
        return carry

    jax.lax.fori_loop(0, NR, p1, 0)

    wsp_cp.wait()

    def p2(n, carry):
        k_cp(n).wait()
        v_cp(n).wait()
        h_cp(n).wait()
        zero = zero_s[0]
        fwd = _up(fg_v[0])
        dd = dd_v[n]
        cp = dp = None
        for i in range(NB):
            hb = _up(h_v[n, :, i * BLK:(i + 1) * BLK])
            hf = jax.lax.dot_general(fwd, hb, (((1,), (1,)), ((), ())),
                                     preferred_element_type=F32)
            c, d = hf[:BLK], hf[BLK:]
            if i == 0:
                c2, d2 = c + dd, d
            else:
                c2, d2 = c - dp, d + cp
            cp, dp = c, d
            pl_v[:, HR + i] = (c2).reshape(BLK // 8, 8, 128)
            pl_v[:, HP + i] = (d2 - c2).reshape(BLK // 8, 8, 128)
            pl_v[:, HQ + i] = (c2 + d2).reshape(BLK // 8, 8, 128)
        kf_v[8:8 + S, :] = k_v[n].astype(F32)
        sk = sk_v[n]
        for i in range(NB):
            r = 8 + i * BLK
            ks = kf_v[r:r + BLK, :] * sk[0:1, :]
            for t in range(1, KS):
                ks = ks + kf_v[r - t:r - t + BLK, :] * sk[t:t + 1, :]
            kv = (ks * v_v[n, i * BLK:(i + 1) * BLK, :].astype(F32)).astype(BF16)
            u = jnp.dot(fwd, kv, preferred_element_type=F32)
            a, b = u[:BLK], u[BLK:]
            pl_v[:, UA + i] = a.reshape(BLK // 8, 8, 128)
            pl_v[:, UB + i] = b.reshape(BLK // 8, 8, 128)
            pl_v[:, US + i] = (a + b).reshape(BLK // 8, 8, 128)

        items = []
        state = {}

        def mac_item(pos, g0, pi):
            xv, hv = ((US, HR), (UA, HP), (UB, HQ))[pi]
            outs = range(g0, g0 + GRP)
            top = g0 + GRP

            def run():
                pz = zero + pos
                hs = [pl_v[pz, hv + t] for t in range(top)]
                acc = {o: None for o in outs}
                for jj in range(top):
                    xj = pl_v[pz, xv + jj]
                    for o in outs:
                        if o - jj >= 0:
                            t = xj * hs[o - jj]
                            acc[o] = t if acc[o] is None else acc[o] + t
                r0 = pos * 8
                if pi == 0:
                    state['k1'] = acc
                elif pi == 1:
                    for o in outs:
                        zz_v[n, o, BLK + r0:BLK + r0 + 8, :] = (state['k1'][o] + acc[o]).astype(BF16)
                else:
                    for o in outs:
                        zz_v[n, o, r0:r0 + 8, :] = (state['k1'][o] - acc[o]).astype(BF16)

            nmac = sum(o + 1 for o in outs)
            return (2 * nmac - GRP + (2 * GRP if pi else 0), run)

        for pos in range(BLK // 8):
            for g0 in range(0, NB, GRP):
                for pi in range(3):
                    items.append(mac_item(pos, g0, pi))

        KG = 512
        nq = S // KG
        vpc = CH // 8
        ntap = (S // CH) * nq * vpc
        total = sum(c for c, _ in items)
        tap_of = []
        cum = 0
        for c, _ in items:
            tap_of.append(TAP0 + int(cum * (TAP1 - TAP0) / total))
            cum += c
        nxt = 0
        for r in range(S // CH):
            rs = slice(r * CH, (r + 1) * CH)
            hs = slice(r * CH // 2, (r + 1) * CH // 2)
            acc = None
            for q in range(nq):
                part = jnp.dot(_up(wsp_v[hs, q * KG:(q + 1) * KG]),
                               _up(z2_v[n, q * KG // 2:(q + 1) * KG // 2, :]),
                               preferred_element_type=F32)
                acc = part if acc is None else acc + part
                t0 = (r * nq + q) * vpc
                while nxt < len(items) and tap_of[nxt] < t0 + vpc:
                    i = tap_of[nxt] - t0
                    pl_v[0, TOK] = acc[i * 8:(i + 1) * 8, :]
                    items[nxt][1]()
                    nxt += 1
            g = acc + bcol_v[rs, :]
            p_v[n, rs, :] = (z1_v[n, rs, :].astype(F32) * g).astype(BF16)
        assert nxt == len(items)
        return carry

    jax.lax.fori_loop(0, NC, p2, 0)

    wout_cp.wait()

    def p3(j, carry):
        slot = j % 2

        @pl.when(j >= 2)
        def _():
            o_cp(j - 2, slot).wait()

        inv = jnp.concatenate([_up(fg_v[1, 0:64, :]), _up(fg_v[1, 64:128, :])], axis=1)
        p5s = []
        for sub in range(NSUB):
            rs = pl.ds(pl.multiple_of(j * RT + sub * SUB, SUB), SUB)
            hs = pl.ds(pl.multiple_of((j * RT + sub * SUB) // 2, SUB // 2), SUB // 2)
            g = jnp.dot(_up(wsp_v[hs, :]), _up(z2_v[NF - 1]),
                        preferred_element_type=F32) + bcol_v[rs, :]
            p5s.append((z1_v[NF - 1, rs, :].astype(F32) * g).astype(BF16))
        for sub in range(NSUB):
            rs = pl.ds(pl.multiple_of(j * RT + sub * SUB, SUB), SUB)
            hs = pl.ds(pl.multiple_of((j * RT + sub * SUB) // 2, SUB // 2), SUB // 2)
            zz = jnp.concatenate(
                [zz_v[c, j * NSUB + sub] for c in range(NC)], axis=1)
            y = jnp.dot(inv, zz, preferred_element_type=F32)
            p = jnp.concatenate(
                [p_v[n, rs, :] for n in range(NF - 1)] + [p5s[sub]], axis=1)
            o = jnp.dot(p, _up(wout_v[...]), preferred_element_type=F32)
            gate = o * (1.0 + jnp.tanh(0.25 * o))
            x = x_v[rs, :].astype(F32)
            xn = xn_v[rs, :].astype(F32)
            res = x + (xn * y) * gate
            o_v[slot, sub * SUB:(sub + 1) * SUB, :] = res.astype(BF16)
        o_cp(j, slot).start()
        return carry

    jax.lax.fori_loop(0, NR, p3, 0)
    o_cp(NR - 2, 0).wait()
    o_cp(NR - 1, 1).wait()


@jax.jit
def pallas_recurrent_scan__ssm_conv_h3__mixer_gmlp__prompt_kernel(
    A_q: jax.Array,
    A_k: jax.Array,
    A_v: jax.Array,
    A_shift_k: jax.Array,
    A_ssm_k: jax.Array,
    A_ssm_D: jax.Array,
    B_x: jax.Array,
    B_w_in: jax.Array,
    B_w_sp: jax.Array,
    B_b_sp: jax.Array,
    B_w_out: jax.Array,
):
    del B_x
    fwd, inv = _dft_tables()
    fwd = jnp.asarray(fwd, dtype=BF16)
    inv = jnp.asarray(inv, dtype=BF16)

    any_spec = pl.BlockSpec(memory_space=pl.ANY)
    vmem_spec = pl.BlockSpec(memory_space=pltpu.VMEM)
    return pl.pallas_call(
        _kernel,
        out_shape=jax.ShapeDtypeStruct((1, S, D), BF16),
        in_specs=[any_spec, any_spec, any_spec, vmem_spec, any_spec, vmem_spec,
                  any_spec, any_spec, vmem_spec, any_spec, vmem_spec, vmem_spec],
        out_specs=any_spec,
        scratch_shapes=[
            pltpu.VMEM((S, D), BF16),
            pltpu.VMEM((D // 2, 2 * FH), U32),
            pltpu.VMEM((S // 2, S), U32),
            pltpu.VMEM((FH // 2, D), U32),
            pltpu.VMEM((NC, S, 128), BF16),
            pltpu.VMEM((NC, S, 128), BF16),
            pltpu.VMEM((NC, 64, S), U32),
            pltpu.VMEM((S, D), BF16),
            pltpu.VMEM((NF, S, 128), BF16),
            pltpu.VMEM((NF, S // 2, 128), U32),
            pltpu.VMEM((NF - 1, S, 128), BF16),
            pltpu.VMEM((S + 8, 128), F32),
            pltpu.VMEM((BLK // 8, 6 * NB + 1, 8, 128), F32),
            pltpu.VMEM((NC, NB, 2 * BLK, 128), BF16),
            pltpu.VMEM((S, 128), F32),
            pltpu.VMEM((NC, KS, 128), F32),
            pltpu.VMEM((NC, 1, 128), F32),
            pltpu.VMEM((2, RT, D), BF16),
            pltpu.VMEM((SUB, FH), F32),
            pltpu.VMEM((SUB, FH), F32),
            pltpu.VMEM((2, 128, 128), U32),
            pltpu.SMEM((1,), jnp.int32),
            pltpu.SemaphoreType.DMA((NR,)),
            pltpu.SemaphoreType.DMA((3,)),
            pltpu.SemaphoreType.DMA((3 * NC,)),
            pltpu.SemaphoreType.DMA((2,)),
        ],
        compiler_params=pltpu.CompilerParams(vmem_limit_bytes=100 * 1024 * 1024),
    )(A_q, A_k, A_v, A_shift_k.T, A_ssm_k, A_ssm_D, B_w_in, B_w_sp, B_b_sp, B_w_out,
      fwd, inv)
```

```python
import os

import jax
import jax.numpy as jnp
import numpy as np
import jax.experimental.pallas as pl
import jax.experimental.pallas.tpu as pltpu

F32 = jnp.float32
BF16 = jnp.bfloat16
U32 = jnp.uint32

S = 2048
D = 640
FH = 768
KS = 4
BLK = 128
NB = S // BLK
NC = D // 128
NF = FH // 128
T = 128
NT = S // T
EPS = 1e-5
GRP = 4
KG = 512
UA, UB, US, HP, HQ, HR, TOK = (i * NB for i in range(7))
TB = int(os.environ.get('TB', 5))
P3I = int(os.environ.get('P3I', 4))
LAG = int(os.environ.get('LAG', 4))
TAP1 = int(os.environ.get('TAP1', 1000))

_GELU_C0 = float(np.sqrt(2.0 / np.pi))
_GELU_C1 = _GELU_C0 * 0.044715


def _dft_tables():
    m = np.arange(BLK)[:, None]
    n = np.arange(BLK)[None, :]
    ang = 2.0 * np.pi * (((4 * m + 1) * n) % (4 * BLK)) / (4 * BLK)
    fwd = np.concatenate([np.cos(ang), -np.sin(ang)], axis=0)
    inv = fwd.T / (4.0 * BLK)
    return np.concatenate([fwd, inv[:, :BLK], inv[:, BLK:]], axis=0).astype(np.float32)


def _layernorm(x, eps):
    m = jnp.mean(x, axis=-1, keepdims=True)
    d = x - m
    v = jnp.mean(d * d, axis=-1, keepdims=True)
    return d * jax.lax.rsqrt(v + eps)


def _gelu2(x):
    u = x * (x * x * _GELU_C1 + _GELU_C0)
    return x * (1.0 + jnp.tanh(u))


def _pk(x):
    return pltpu.bitcast(x, U32)


def _up(x):
    return pltpu.bitcast(x, BF16)


def _dot(a, b):
    return jnp.dot(a, b, preferred_element_type=F32)


def _spread(items, taps):
    total = sum(c for c, _, _ in items)
    cum = 0
    for c, gate, run in items:
        gate(taps[int(cum * len(taps) / total)]())
        run()
        cum += c


def _kernel(x_hbm, k_hbm, v_hbm, skt_hbm, h_hbm, dv_hbm, win_hbm, wsp_hbm, b_hbm,
            wout_hbm, tab_hbm, out_hbm,
            x_v, win_v, wsp_v, wout_v, kv_v, h_v, xn_v, z1_v, z2_v, p_v,
            kf_v, kvb_v, pl_v, zz_v, bcol_v, sk_v, dd_v, o_v, zta_v, ztb_v, tab_v,
            skt_v, dv_v, b_v, zero_s, sem):
    cp = pltpu.make_async_copy
    x16 = x_v.bitcast(BF16)
    win16 = win_v.bitcast(BF16)
    kv16 = kv_v.bitcast(BF16)
    h16 = h_v.bitcast(BF16)

    def x_cp(lo, hi, s):
        return cp(x_hbm.at[0, lo:hi, :], x16.at[lo:hi, :], sem.at[s])

    def win_cp(lo, hi, s):
        return cp(win_hbm.at[:, lo:hi], win16.at[0:D, lo:hi], sem.at[s])

    def k_cp(c, s):
        return cp(k_hbm.at[0, :, pl.ds(c * 128, 128)], kv16.at[2 * c, 0:S, :], sem.at[s])

    def v_cp(c, s):
        return cp(v_hbm.at[0, :, pl.ds(c * 128, 128)], kv16.at[2 * c + 1, 0:S, :], sem.at[s])

    def h_cp(c, s):
        return cp(h_hbm.at[pl.ds(c * 128, 128), :], h16.at[c], sem.at[s])

    H = FH // 2
    groups = [
        [cp(b_hbm, b_v, sem.at[0]), cp(skt_hbm, skt_v, sem.at[0]), cp(dv_hbm, dv_v, sem.at[0])],
        [x_cp(0, 256, 1)],
        [win_cp(FH, FH + H, 2)],
        [win_cp(FH + H, 2 * FH, 3)],
        [win_cp(0, H, 4)],
        [win_cp(H, FH, 5), x_cp(256, 512, 5)],
        [x_cp(512, 1024, 6)],
        [x_cp(1024, S, 7), k_cp(0, 7), v_cp(0, 7)],
        [cp(tab_hbm, tab_v.bitcast(BF16), sem.at[8]), h_cp(0, 8),
         cp(wsp_hbm, wsp_v.bitcast(BF16), sem.at[8])],
    ]
    for g in groups:
        for c in g:
            c.start()

    def tile_cps(c):
        return [k_cp(c, 8 + c), v_cp(c, 8 + c), h_cp(c, 8 + c)]

    for c in range(1, NC):
        for d in tile_cps(c):
            d.start()
    wout_cp = cp(wout_hbm, wout_v.bitcast(BF16), sem.at[13])
    wout_cp.start()

    def wait(i):
        for c in groups[i]:
            c.wait()

    zero_s[0] = 0
    kf_v[0:8, :] = jnp.zeros((8, 128), F32)
    wait(0)
    skt = skt_v[...].astype(F32)
    dv = dv_v[...].astype(F32).reshape(1, D)
    for c in range(NC):
        sk_v[c] = skt[:, c * 128:(c + 1) * 128]
        dd_v[c] = dv[:, c * 128:(c + 1) * 128]
    brow = b_v[...].astype(F32).reshape(1, S)
    bcol_v[...] = jnp.broadcast_to(brow, (128, S)).T

    def gate_x(tok):
        x_v[S // 2:S // 2 + 8, 0:128] = pltpu.bitcast(tok, U32)

    zt_v = (zta_v, ztb_v)

    def gate_zt(t):
        def gate(tok):
            zt_v[t % 2][T:T + 8, 0:128] = tok
        return gate

    def gate_kv(tok):
        kv_v[0, S // 2:S // 2 + 8, :] = pltpu.bitcast(tok, U32)

    def gate_pl(tok):
        pl_v[0, TOK] = tok

    ndone = [0]

    def done(val):
        c = (ndone[0] % (2 * NF)) * 128
        ndone[0] += 1
        win_v[D // 2:D // 2 + 8, c:c + 128] = val

    def lnx_items(t, zero, mark=True):
        def item(r0):
            def run():
                xw = x_v[pl.ds(pl.multiple_of(zero + r0 // 2, 8), 8), :]
                xn = _layernorm(_up(xw).astype(F32), EPS)
                xn_v[r0:r0 + 16, :] = xn.astype(BF16)
                if mark:
                    done(pltpu.bitcast(xn[0:8, 0:128], U32))
                    done(pltpu.bitcast(xn[8:16, 0:128], U32))
            return (1, gate_x, run)
        return [item(t * T + g * 16) for g in range(T // 16)]

    def lnz_items(t, zero):
        def item(g):
            def run():
                z = zt_v[t % 2][pl.ds(pl.multiple_of(zero + g * 16, 8), 16), :]
                z2 = _pk(_layernorm(z, 4.0 * EPS).astype(BF16))
                done(z2[:, 0:128])
                r0 = (t * T + g * 16) // 2
                for n in range(NF):
                    z2_v[n, r0:r0 + 8, :] = z2[:, n * 128:(n + 1) * 128]
            return (1, gate_zt(t), run)
        return [item(g) for g in range(T // 16)]

    KR = 32

    def kv_items(c):
        sk = sk_v[c]

        def item(r0):
            def run():
                hs = slice(r0 // 2, (r0 + KR) // 2)
                r = 8 + r0
                kf_v[r:r + KR, :] = _up(kv_v[2 * c, hs, :]).astype(F32)
                ks = kf_v[r:r + KR, :] * sk[0:1, :]
                for t in range(1, KS):
                    ks = ks + kf_v[r - t:r - t + KR, :] * sk[t:t + 1, :]
                kvb_v[r0:r0 + KR, :] = (
                    ks * _up(kv_v[2 * c + 1, hs, :]).astype(F32)).astype(BF16)
            return (11 * KR // 8, gate_kv, run)
        return [item(r0) for r0 in range(0, S, KR)]

    def taps_of(val):
        rows, cols = val.shape
        return [(lambda i=i, n=n: val[i * 8:(i + 1) * 8, n * 128:(n + 1) * 128])
                for n in range(cols // 128) for i in range(rows // 8)]

    def piece(kind, t, n, zero):
        rows = slice(0, D // 2) if zero is None else pl.ds(pl.multiple_of(zero, 8), D // 2)
        col = n * 128 + (FH if kind == 2 else 0)
        z = _dot(xn_v[t * T:(t + 1) * T, :], _up(win_v[rows, col:col + 128]))
        if kind == 2:
            zt_v[t % 2][0:T, n * 128:(n + 1) * 128] = _gelu2(z)
        else:
            z1_v[n, t * T:(t + 1) * T, :] = _gelu2(z).astype(BF16)
        return taps_of(z)

    def block(pieces, work):
        zero = zero_s[0]
        rel = [[] for _ in pieces]
        for mk, lo, hi in work:
            items = mk(zero)
            for i, it in enumerate(items):
                tau = (lo * 16) + (i * (hi - lo) * 16) // len(items)
                rel[tau // 16].append((tau % 16, it))
        taps = []
        gated = False
        for k in range(len(pieces) + LAG):
            if k < len(pieces):
                taps.append(piece(*pieces[k], zero if gated else None))
            if k >= LAG:
                for i, (_, gate, run) in sorted(rel[k - LAG], key=lambda e: e[0]):
                    gate(taps[k - LAG][i]())
                    run()
                    gated = True

    def cols(kind, t, lo=0, hi=NF):
        return [(kind, t, n) for n in range(lo, hi)]

    def lnx(t):
        return lambda zero: lnx_items(t, zero)

    def lnz(t):
        return lambda zero: lnz_items(t, zero)

    wait(1)
    for it in lnx_items(0, 0, False) + lnx_items(1, 0, False):
        it[2]()
    HN = NF // 2
    wait(2)
    block(cols(2, 0, 0, HN) + cols(2, 1, 0, HN), [])
    wait(3)
    block(cols(2, 0, HN) + cols(2, 1, HN), [])
    wait(4)
    block(cols(1, 0, 0, HN) + cols(1, 1, 0, HN), [(lnz(0), 0, 1)])
    wait(5)
    block(cols(1, 0, HN) + cols(1, 1, HN), [(lnx(2), 0, 1)])

    def big_block(first, last, extra):
        pieces, work = [], list(extra)
        for t in range(first, last - 1):
            k = len(pieces)
            pieces += cols(2, t) + cols(1, t)
            if t + 1 < last - 1:
                work += [(lnx(t + 1), k, k + 11 - LAG), (lnz(t), k + 6, k + 18)]
            else:
                work += [(lnx(t + 1), k, k + 11 - LAG), (lnx(t + 2), k + 11 - LAG, k + 17 - LAG),
                         (lnz(t), k + 6, k + 17 - LAG)]
        a, b = last - 1, last
        k = len(pieces)
        pieces += cols(2, a) + cols(2, b) + cols(1, a) + cols(1, b)
        work += [(lnz(a), k + 6, k + 12), (lnz(b), k + 12, k + 23 - LAG)]
        if b + 1 < NT:
            work += [(lnx(b + 1), k + 2, k + 12)]
        else:
            work += [(kv_items, k - 24, k + 24)]
        block(pieces, work)

    wait(6)
    big_block(2, TB, [(lnz(1), 0, 11 - LAG)])
    wait(7)
    big_block(TB + 1, NT - 1, [])

    wait(8)

    def p2(n, carry):
        nn = jnp.minimum(n + 1, NC - 1)

        @pl.when(n + 1 < NC)
        def _():
            for d in tile_cps(nn):
                d.wait()

        zero = zero_s[0]
        fwd = _up(tab_v[0:128, :])
        dd = dd_v[n]
        cp_ = dp_ = None

        def put(slot, val):
            pl_v[:, slot] = val.reshape(BLK // 8, 8, 128)

        for i in range(NB):
            hb = _up(h_v[n, :, i * BLK:(i + 1) * BLK])
            hf = jax.lax.dot_general(fwd, hb, (((1,), (1,)), ((), ())),
                                     preferred_element_type=F32)
            c, d = hf[:BLK], hf[BLK:]
            if i == 0:
                c2, d2 = c + dd, d
            else:
                c2, d2 = c - dp_, d + cp_
            cp_, dp_ = c, d
            put(HR + i, c2)
            put(HP + i, d2 - c2)
            put(HQ + i, c2 + d2)
        for i in range(NB):
            u = _dot(fwd, kvb_v[i * BLK:(i + 1) * BLK, :])
            a, b = u[:BLK], u[BLK:]
            put(UA + i, a)
            put(UB + i, b)
            put(US + i, a + b)

        state = {}

        def mac_item(pos, g0, pi):
            xv, hv = ((US, HR), (UA, HP), (UB, HQ))[pi]
            outs = range(g0, g0 + GRP)
            top = g0 + GRP

            def run():
                pz = zero + pos
                hs = [pl_v[pz, hv + t] for t in range(top)]
                acc = {o: None for o in outs}
                for jj in range(top):
                    xj = pl_v[pz, xv + jj]
                    for o in outs:
                        if o - jj >= 0:
                            t = xj * hs[o - jj]
                            acc[o] = t if acc[o] is None else acc[o] + t
                r0 = pos * 8
                if pi == 0:
                    state['k1'] = acc
                elif pi == 1:
                    for o in outs:
                        zz_v[n, o, BLK + r0:BLK + r0 + 8, :] = (state['k1'][o] + acc[o]).astype(BF16)
                else:
                    for o in outs:
                        zz_v[n, o, r0:r0 + 8, :] = (state['k1'][o] - acc[o]).astype(BF16)

            nmac = sum(o + 1 for o in outs)
            return (2 * nmac - GRP + (2 * GRP if pi else 0), gate_pl, run)

        kvi = kv_items(nn)
        items = []
        for pos in range(BLK // 8):
            for g0 in range(0, NB, GRP):
                for pi in range(3):
                    items.append(mac_item(pos, g0, pi))
                items.append(kvi[pos * (NB // GRP) + g0 // GRP])

        nq = S // KG
        vpc = T // 8
        total = sum(c for c, _, _ in items)
        tap_of = []
        cum = 0
        for c, _, _ in items:
            tap_of.append(int(cum * TAP1 / total))
            cum += c
        nxt = 0
        for r in range(NT):
            rs = slice(r * T, (r + 1) * T)
            hs = slice(r * T // 2, (r + 1) * T // 2)
            acc = None
            for q in range(nq):
                part = _dot(_up(wsp_v[hs, q * KG:(q + 1) * KG]),
                            _up(z2_v[n, q * KG // 2:(q + 1) * KG // 2, :]))
                acc = part if acc is None else acc + part
                t0 = (r * nq + q) * vpc
                while nxt < len(items) and tap_of[nxt] < t0 + vpc:
                    i = tap_of[nxt] - t0
                    items[nxt][1](acc[i * 8:(i + 1) * 8, :])
                    items[nxt][2]()
                    nxt += 1
            g = acc + bcol_v[rs, :]
            p_v[n, rs, :] = (z1_v[n, rs, :].astype(F32) * g).astype(BF16)
        assert nxt == len(items)
        return carry

    jax.lax.fori_loop(0, NC, p2, 0)

    wout_cp.wait()

    TPI = NT // P3I

    def p3(j, carry):
        inv = jnp.concatenate([_up(tab_v[128:192, :]), _up(tab_v[192:256, :])], axis=1)

        def rows(t):
            r0 = (j * TPI + t) * T
            return (pl.ds(pl.multiple_of(r0, T), T),
                    pl.ds(pl.multiple_of(r0 // 2, T // 2), T // 2))

        def g5(t):
            rs, hs = rows(t)
            g = _dot(_up(wsp_v[hs, :]), _up(z2_v[NF - 1])) + bcol_v[rs, :]
            return (z1_v[NF - 1, rs, :].astype(F32) * g).astype(BF16)

        p5 = g5(0)
        for t in range(TPI):
            rs, hs = rows(t)
            p = jnp.concatenate([p_v[n, rs, :] for n in range(NF - 1)] + [p5], axis=1)
            if t + 1 < TPI:
                p5 = g5(t + 1)
            for c in range(NC):
                cs = slice(c * 128, (c + 1) * 128)
                y = _dot(inv, zz_v[c, j * TPI + t])
                o = _dot(p, _up(wout_v[:, cs]))
                gate = o * (1.0 + jnp.tanh(0.25 * o))
                x = _up(x_v[hs, cs]).astype(F32)
                xn = xn_v[rs, cs].astype(F32)
                o_v[rs, cs] = (x + (xn * y) * gate).astype(BF16)
            cp(o_v.at[rs, :], out_hbm.at[0, rs, :], sem.at[14]).start()
        return carry

    jax.lax.fori_loop(0, P3I, p3, 0)
    cp(o_v, out_hbm.at[0], sem.at[14]).wait()


@jax.jit
def pallas_recurrent_scan__ssm_conv_h3__mixer_gmlp__prompt_kernel(
    A_q: jax.Array,
    A_k: jax.Array,
    A_v: jax.Array,
    A_shift_k: jax.Array,
    A_ssm_k: jax.Array,
    A_ssm_D: jax.Array,
    B_x: jax.Array,
    B_w_in: jax.Array,
    B_w_sp: jax.Array,
    B_b_sp: jax.Array,
    B_w_out: jax.Array,
):
    del B_x
    tab = jnp.asarray(_dft_tables(), dtype=BF16)

    any_spec = pl.BlockSpec(memory_space=pl.ANY)
    return pl.pallas_call(
        _kernel,
        out_shape=jax.ShapeDtypeStruct((1, S, D), BF16),
        in_specs=[any_spec] * 11,
        out_specs=any_spec,
        scratch_shapes=[
            pltpu.VMEM((S // 2 + 8, D), U32),
            pltpu.VMEM((D // 2 + 8, 2 * FH), U32),
            pltpu.VMEM((S // 2, S), U32),
            pltpu.VMEM((FH // 2, D), U32),
            pltpu.VMEM((2 * NC, S // 2 + 8, 128), U32),
            pltpu.VMEM((NC, 64, S), U32),
            pltpu.VMEM((S, D), BF16),
            pltpu.VMEM((NF, S, 128), BF16),
            pltpu.VMEM((NF, S // 2, 128), U32),
            pltpu.VMEM((NF - 1, S, 128), BF16),
            pltpu.VMEM((S + 8, 128), F32),
            pltpu.VMEM((S, 128), BF16),
            pltpu.VMEM((BLK // 8, 6 * NB + 1, 8, 128), F32),
            pltpu.VMEM((NC, NB, 2 * BLK, 128), BF16),
            pltpu.VMEM((S, 128), F32),
            pltpu.VMEM((NC, KS, 128), F32),
            pltpu.VMEM((NC, 1, 128), F32),
            pltpu.VMEM((S, D), BF16),
            pltpu.VMEM((T + 8, FH), F32),
            pltpu.VMEM((T + 8, FH), F32),
            pltpu.VMEM((256, 128), U32),
            pltpu.VMEM((KS, D), BF16),
            pltpu.VMEM((D,), BF16),
            pltpu.VMEM((S,), BF16),
            pltpu.SMEM((1,), jnp.int32),
            pltpu.SemaphoreType.DMA((15,)),
        ],
        compiler_params=pltpu.CompilerParams(
            vmem_limit_bytes=100 * 1024 * 1024, disable_bounds_checks=True),
    )(A_q, A_k, A_v, A_shift_k.T, A_ssm_k, A_ssm_D, B_w_in, B_w_sp, B_b_sp, B_w_out, tab)
```

```python
import os

import jax
import jax.numpy as jnp
import numpy as np
import jax.experimental.pallas as pl
import jax.experimental.pallas.tpu as pltpu

F32 = jnp.float32
BF16 = jnp.bfloat16
U32 = jnp.uint32

S = 2048
D = 640
FH = 768
KS = 4
BLK = 128
NB = S // BLK
NC = D // 128
NF = FH // 128
T = 128
NT = S // T
EPS = 1e-5
GRP = 4
KG = 512
UA, UB, US, HP, HQ, HR, TOK = (i * NB for i in range(7))
TB = int(os.environ.get('TB', 5))
P3I = int(os.environ.get('P3I', 4))
LAG = int(os.environ.get('LAG', 4))
TAP1 = int(os.environ.get('TAP1', 1000))

_GELU_C0 = float(np.sqrt(2.0 / np.pi))
_GELU_C1 = _GELU_C0 * 0.044715


def _dft_tables():
    m = np.arange(BLK)[:, None]
    n = np.arange(BLK)[None, :]
    ang = 2.0 * np.pi * (((4 * m + 1) * n) % (4 * BLK)) / (4 * BLK)
    fwd = np.concatenate([np.cos(ang), -np.sin(ang)], axis=0)
    inv = fwd.T / (4.0 * BLK)
    return np.concatenate([fwd, inv[:, :BLK], inv[:, BLK:]], axis=0).astype(np.float32)


def _layernorm(x, eps):
    m = jnp.mean(x, axis=-1, keepdims=True)
    d = x - m
    v = jnp.mean(d * d, axis=-1, keepdims=True)
    return d * jax.lax.rsqrt(v + eps)


def _gelu2(x):
    u = x * (x * x * _GELU_C1 + _GELU_C0)
    return x * (1.0 + jnp.tanh(u))


def _pk(x):
    return pltpu.bitcast(x, U32)


def _up(x):
    return pltpu.bitcast(x, BF16)


def _dot(a, b):
    return jnp.dot(a, b, preferred_element_type=F32)


def _spread(items, taps):
    total = sum(c for c, _, _ in items)
    cum = 0
    for c, gate, run in items:
        gate(taps[int(cum * len(taps) / total)]())
        run()
        cum += c


def _kernel(x_hbm, k_hbm, v_hbm, skt_hbm, h_hbm, dv_hbm, win_hbm, wsp_hbm, b_hbm,
            wout_hbm, tab_hbm, out_hbm,
            x_v, win_v, wsp_v, wout_v, kv_v, h_v, xn_v, z1_v, z2_v, p_v,
            kvb_v, pl_v, zz_v, bcol_v, sk_v, dd_v, o_v, zta_v, ztb_v, tab_v,
            skt_v, dv_v, b_v, zero_s, sem):
    cp = pltpu.make_async_copy
    x16 = x_v.bitcast(BF16)
    win16 = win_v.bitcast(BF16)
    kv16 = kv_v.bitcast(BF16)
    h16 = h_v.bitcast(BF16)

    xn32, z232, p32, kvb32, zz32 = (
        r.bitcast(U32) for r in (xn_v, z2_v, p_v, kvb_v, zz_v))

    def x_cp(lo, hi, s):
        return cp(x_hbm.at[0, lo:hi, :], x16.at[lo:hi, :], sem.at[s])

    def win_cp(lo, hi, s):
        return cp(win_hbm.at[:, lo:hi], win16.at[0:D, lo:hi], sem.at[s])

    def k_cp(c, s):
        return cp(k_hbm.at[0, :, pl.ds(c * 128, 128)], kv16.at[2 * c, 0:S, :], sem.at[s])

    def v_cp(c, s):
        return cp(v_hbm.at[0, :, pl.ds(c * 128, 128)], kv16.at[2 * c + 1, 0:S, :], sem.at[s])

    def h_cp(c, s):
        return cp(h_hbm.at[pl.ds(c * 128, 128), :], h16.at[c], sem.at[s])

    H = FH // 2
    groups = [
        [cp(b_hbm, b_v, sem.at[0]), cp(skt_hbm, skt_v, sem.at[0]), cp(dv_hbm, dv_v, sem.at[0])],
        [x_cp(0, 256, 1)],
        [win_cp(FH, FH + H, 2)],
        [win_cp(FH + H, 2 * FH, 3)],
        [win_cp(0, H, 4)],
        [win_cp(H, FH, 5), x_cp(256, 512, 5)],
        [x_cp(512, 1024, 6)],
        [x_cp(1024, S, 7), k_cp(0, 7), v_cp(0, 7)],
        [cp(tab_hbm, tab_v.bitcast(BF16), sem.at[8]), h_cp(0, 8),
         cp(wsp_hbm, wsp_v.bitcast(BF16), sem.at[8])],
    ]
    for g in groups:
        for c in g:
            c.start()

    def tile_cps(c):
        return [k_cp(c, 8 + c), v_cp(c, 8 + c), h_cp(c, 8 + c)]

    for c in range(1, NC):
        for d in tile_cps(c):
            d.start()
    wout_cp = cp(wout_hbm, wout_v.bitcast(BF16), sem.at[13])
    wout_cp.start()

    def wait(i):
        for c in groups[i]:
            c.wait()

    zero_s[0] = 0
    wait(0)
    skt = skt_v[...].astype(F32)
    dv = dv_v[...].astype(F32).reshape(1, D)
    for c in range(NC):
        sk_v[c] = skt[:, c * 128:(c + 1) * 128]
        dd_v[c] = dv[:, c * 128:(c + 1) * 128]
    brow = b_v[...].astype(F32).reshape(1, S)
    bcol_v[...] = jnp.broadcast_to(brow, (128, S)).T

    def gate_x(tok):
        x_v[S // 2:S // 2 + 8, 0:128] = pltpu.bitcast(tok, U32)

    zt_v = (zta_v, ztb_v)

    def gate_zt(t):
        def gate(tok):
            zt_v[t % 2][T:T + 8, 0:128] = tok
        return gate

    def gate_kv(tok):
        kv_v[0, S // 2:S // 2 + 8, :] = pltpu.bitcast(tok, U32)

    def gate_pl(tok):
        pl_v[0, TOK] = tok

    ndone = [0]

    def done(val):
        c = (ndone[0] % (2 * NF)) * 128
        ndone[0] += 1
        win_v[D // 2:D // 2 + 8, c:c + 128] = val

    def lnx_items(t, zero, mark=True):
        def item(r0):
            def run():
                xw = x_v[pl.ds(pl.multiple_of(zero + r0 // 2, 8), 8), :]
                xn = _layernorm(_up(xw).astype(F32), EPS)
                for c in range(NC):
                    xn_v[c, r0:r0 + 16, :] = xn[:, c * 128:(c + 1) * 128].astype(BF16)
                if mark:
                    done(pltpu.bitcast(xn[0:8, 0:128], U32))
                    done(pltpu.bitcast(xn[8:16, 0:128], U32))
            return (1, gate_x, run)
        return [item(t * T + g * 16) for g in range(T // 16)]

    def lnz_items(t, zero):
        def item(g):
            def run():
                z = zt_v[t % 2][pl.ds(pl.multiple_of(zero + g * 16, 8), 16), :]
                z = _layernorm(z, 4.0 * EPS)
                done(pltpu.bitcast(z[0:8, 0:128], U32))
                done(pltpu.bitcast(z[8:16, 0:128], U32))
                r0 = t * T + g * 16
                for n in range(NF):
                    z2_v[n, r0:r0 + 16, :] = z[:, n * 128:(n + 1) * 128].astype(BF16)
            return (1, gate_zt(t), run)
        return [item(g) for g in range(T // 16)]

    KR = 32

    def kv_items(c):
        sk = sk_v[c]

        def item(r0):
            def run():
                hs = slice(r0 // 2, (r0 + KR) // 2)
                if r0 == 0:
                    kw = jnp.concatenate(
                        [jnp.zeros((8, 128), F32), _up(kv_v[2 * c, hs, :]).astype(F32)], axis=0)
                else:
                    kw = _up(kv_v[2 * c, r0 // 2 - 8:(r0 + KR) // 2, :]).astype(F32)[8:]
                ks = kw[8:] * sk[0:1, :]
                for t in range(1, KS):
                    ks = ks + pltpu.roll(kw, t, 0)[8:] * sk[t:t + 1, :]
                kvb_v[r0:r0 + KR, :] = (
                    ks * _up(kv_v[2 * c + 1, hs, :]).astype(F32)).astype(BF16)
            return (14 * KR // 8, gate_kv, run)
        return [item(r0) for r0 in range(0, S, KR)]

    def taps_of(val):
        rows, cols = val.shape
        return [(lambda i=i, n=n: val[i * 8:(i + 1) * 8, n * 128:(n + 1) * 128])
                for n in range(cols // 128) for i in range(rows // 8)]

    def piece(kind, t, n, zero):
        rows = slice(0, D // 2) if zero is None else pl.ds(pl.multiple_of(zero, 8), D // 2)
        col = n * 128 + (FH if kind == 2 else 0)
        xn = jnp.concatenate(
            [_up(xn32[c, t * T // 2:(t + 1) * T // 2, :]) for c in range(NC)], axis=1)
        z = _dot(xn, _up(win_v[rows, col:col + 128]))
        if kind == 2:
            zt_v[t % 2][0:T, n * 128:(n + 1) * 128] = _gelu2(z)
        else:
            z1_v[n, t * T:(t + 1) * T, :] = _gelu2(z).astype(BF16)
        return taps_of(z)

    def block(pieces, work):
        zero = zero_s[0]
        rel = [[] for _ in pieces]
        for mk, lo, hi in work:
            items = mk(zero)
            for i, it in enumerate(items):
                tau = (lo * 16) + (i * (hi - lo) * 16) // len(items)
                rel[tau // 16].append((tau % 16, it))
        taps = []
        gated = False
        for k in range(len(pieces) + LAG):
            if k < len(pieces):
                taps.append(piece(*pieces[k], zero if gated else None))
            if k >= LAG:
                for i, (_, gate, run) in sorted(rel[k - LAG], key=lambda e: e[0]):
                    gate(taps[k - LAG][i]())
                    run()
                    gated = True

    def cols(kind, t, lo=0, hi=NF):
        return [(kind, t, n) for n in range(lo, hi)]

    def lnx(t):
        return lambda zero: lnx_items(t, zero)

    def lnz(t):
        return lambda zero: lnz_items(t, zero)

    wait(1)
    for it in lnx_items(0, 0, False) + lnx_items(1, 0, False):
        it[2]()
    HN = NF // 2
    wait(2)
    block(cols(2, 0, 0, HN) + cols(2, 1, 0, HN), [])
    wait(3)
    block(cols(2, 0, HN) + cols(2, 1, HN), [])
    wait(4)
    block(cols(1, 0, 0, HN) + cols(1, 1, 0, HN), [(lnz(0), 0, 1)])
    wait(5)
    block(cols(1, 0, HN) + cols(1, 1, HN), [(lnx(2), 0, 1)])

    def big_block(first, last, extra):
        pieces, work = [], list(extra)
        for t in range(first, last - 1):
            k = len(pieces)
            pieces += cols(2, t) + cols(1, t)
            if t + 1 < last - 1:
                work += [(lnx(t + 1), k, k + 11 - LAG), (lnz(t), k + 6, k + 18)]
            else:
                work += [(lnx(t + 1), k, k + 11 - LAG), (lnx(t + 2), k + 11 - LAG, k + 17 - LAG),
                         (lnz(t), k + 6, k + 17 - LAG)]
        a, b = last - 1, last
        k = len(pieces)
        pieces += cols(2, a) + cols(2, b) + cols(1, a) + cols(1, b)
        work += [(lnz(a), k + 6, k + 12), (lnz(b), k + 12, k + 23 - LAG)]
        if b + 1 < NT:
            work += [(lnx(b + 1), k + 2, k + 12)]
        else:
            work += [(kv_items, k - 24, k + 24)]
        block(pieces, work)

    wait(6)
    big_block(2, TB, [(lnz(1), 0, 11 - LAG)])
    wait(7)
    big_block(TB + 1, NT - 1, [])

    wait(8)

    def p2(n, carry):
        nn = jnp.minimum(n + 1, NC - 1)

        @pl.when(n + 1 < NC)
        def _():
            for d in tile_cps(nn):
                d.wait()

        zero = zero_s[0]
        fwd = _up(tab_v[0:128, :])
        dd = dd_v[n]
        cp_ = dp_ = None

        def put(slot, val):
            pl_v[:, slot] = val.reshape(BLK // 8, 8, 128)

        for i in range(NB):
            hb = _up(h_v[n, :, i * BLK:(i + 1) * BLK])
            hf = jax.lax.dot_general(fwd, hb, (((1,), (1,)), ((), ())),
                                     preferred_element_type=F32)
            c, d = hf[:BLK], hf[BLK:]
            if i == 0:
                c2, d2 = c + dd, d
            else:
                c2, d2 = c - dp_, d + cp_
            cp_, dp_ = c, d
            put(HR + i, c2)
            put(HP + i, d2 - c2)
            put(HQ + i, c2 + d2)
        for i in range(NB):
            u = _dot(fwd, _up(kvb32[i * BLK // 2:(i + 1) * BLK // 2, :]))
            a, b = u[:BLK], u[BLK:]
            put(UA + i, a)
            put(UB + i, b)
            put(US + i, a + b)

        state = {}

        def mac_item(pos, g0, pi):
            xv, hv = ((US, HR), (UA, HP), (UB, HQ))[pi]
            outs = range(g0, g0 + GRP)
            top = g0 + GRP

            def run():
                pz = zero + pos
                hs = [pl_v[pz, hv + t] for t in range(top)]
                acc = {o: None for o in outs}
                for jj in range(top):
                    xj = pl_v[pz, xv + jj]
                    for o in outs:
                        if o - jj >= 0:
                            t = xj * hs[o - jj]
                            acc[o] = t if acc[o] is None else acc[o] + t
                r0 = pos * 8
                if pi == 0:
                    state['k1'] = acc
                elif pi == 1:
                    for o in outs:
                        zz_v[n, o, BLK + r0:BLK + r0 + 8, :] = (state['k1'][o] + acc[o]).astype(BF16)
                else:
                    for o in outs:
                        zz_v[n, o, r0:r0 + 8, :] = (state['k1'][o] - acc[o]).astype(BF16)

            nmac = sum(o + 1 for o in outs)
            return (2 * nmac - GRP + (2 * GRP if pi else 0), gate_pl, run)

        kvi = kv_items(nn)
        items = []
        for pos in range(BLK // 8):
            for g0 in range(0, NB, GRP):
                for pi in range(3):
                    items.append(mac_item(pos, g0, pi))
                items.append(kvi[pos * (NB // GRP) + g0 // GRP])

        nq = S // KG
        vpc = T // 8
        total = sum(c for c, _, _ in items)
        tap_of = []
        cum = 0
        for c, _, _ in items:
            tap_of.append(int(cum * TAP1 / total))
            cum += c
        nxt = 0
        for r in range(NT):
            rs = slice(r * T, (r + 1) * T)
            hs = slice(r * T // 2, (r + 1) * T // 2)
            acc = None
            for q in range(nq):
                part = _dot(_up(wsp_v[hs, q * KG:(q + 1) * KG]),
                            _up(z232[n, q * KG // 2:(q + 1) * KG // 2, :]))
                acc = part if acc is None else acc + part
                t0 = (r * nq + q) * vpc
                while nxt < len(items) and tap_of[nxt] < t0 + vpc:
                    i = tap_of[nxt] - t0
                    items[nxt][1](acc[i * 8:(i + 1) * 8, :])
                    items[nxt][2]()
                    nxt += 1
            g = acc + bcol_v[rs, :]
            p_v[n, rs, :] = (z1_v[n, rs, :].astype(F32) * g).astype(BF16)
        assert nxt == len(items)
        return carry

    jax.lax.fori_loop(0, NC, p2, 0)

    wout_cp.wait()

    TPI = NT // P3I

    def p3(j, carry):
        inv = jnp.concatenate([_up(tab_v[128:192, :]), _up(tab_v[192:256, :])], axis=1)

        def rows(t):
            r0 = (j * TPI + t) * T
            return (pl.ds(pl.multiple_of(r0, T), T),
                    pl.ds(pl.multiple_of(r0 // 2, T // 2), T // 2))

        def g5(t):
            rs, hs = rows(t)
            g = _dot(_up(wsp_v[hs, :]), _up(z232[NF - 1])) + bcol_v[rs, :]
            return (z1_v[NF - 1, rs, :].astype(F32) * g).astype(BF16)

        p5 = g5(0)
        for t in range(TPI):
            rs, hs = rows(t)
            p = jnp.concatenate([_up(p32[n, hs, :]) for n in range(NF - 1)] + [p5], axis=1)
            if t + 1 < TPI:
                p5 = g5(t + 1)
            for c in range(NC):
                cs = slice(c * 128, (c + 1) * 128)
                y = _dot(inv, _up(zz32[c, j * TPI + t]))
                o = _dot(p, _up(wout_v[:, cs]))
                gate = o * (1.0 + jnp.tanh(0.25 * o))
                x = _up(x_v[hs, cs]).astype(F32)
                xn = xn_v[c, rs, :].astype(F32)
                o_v[rs, cs] = (x + (xn * y) * gate).astype(BF16)
            cp(o_v.at[rs, :], out_hbm.at[0, rs, :], sem.at[14]).start()
        return carry

    jax.lax.fori_loop(0, P3I, p3, 0)
    cp(o_v, out_hbm.at[0], sem.at[14]).wait()


@jax.jit
def pallas_recurrent_scan__ssm_conv_h3__mixer_gmlp__prompt_kernel(
    A_q: jax.Array,
    A_k: jax.Array,
    A_v: jax.Array,
    A_shift_k: jax.Array,
    A_ssm_k: jax.Array,
    A_ssm_D: jax.Array,
    B_x: jax.Array,
    B_w_in: jax.Array,
    B_w_sp: jax.Array,
    B_b_sp: jax.Array,
    B_w_out: jax.Array,
):
    del B_x
    tab = jnp.asarray(_dft_tables(), dtype=BF16)

    any_spec = pl.BlockSpec(memory_space=pl.ANY)
    return pl.pallas_call(
        _kernel,
        out_shape=jax.ShapeDtypeStruct((1, S, D), BF16),
        in_specs=[any_spec] * 11,
        out_specs=any_spec,
        scratch_shapes=[
            pltpu.VMEM((S // 2 + 8, D), U32),
            pltpu.VMEM((D // 2 + 8, 2 * FH), U32),
            pltpu.VMEM((S // 2, S), U32),
            pltpu.VMEM((FH // 2, D), U32),
            pltpu.VMEM((2 * NC, S // 2 + 8, 128), U32),
            pltpu.VMEM((NC, 64, S), U32),
            pltpu.VMEM((NC, S, 128), BF16),
            pltpu.VMEM((NF, S, 128), BF16),
            pltpu.VMEM((NF, S, 128), BF16),
            pltpu.VMEM((NF - 1, S, 128), BF16),
            pltpu.VMEM((S, 128), BF16),
            pltpu.VMEM((BLK // 8, 6 * NB + 1, 8, 128), F32),
            pltpu.VMEM((NC, NB, 2 * BLK, 128), BF16),
            pltpu.VMEM((S, 128), F32),
            pltpu.VMEM((NC, KS, 128), F32),
            pltpu.VMEM((NC, 1, 128), F32),
            pltpu.VMEM((S, D), BF16),
            pltpu.VMEM((T + 8, FH), F32),
            pltpu.VMEM((T + 8, FH), F32),
            pltpu.VMEM((256, 128), U32),
            pltpu.VMEM((KS, D), BF16),
            pltpu.VMEM((D,), BF16),
            pltpu.VMEM((S,), BF16),
            pltpu.SMEM((1,), jnp.int32),
            pltpu.SemaphoreType.DMA((15,)),
        ],
        compiler_params=pltpu.CompilerParams(
            vmem_limit_bytes=100 * 1024 * 1024, disable_bounds_checks=True),
    )(A_q, A_k, A_v, A_shift_k.T, A_ssm_k, A_ssm_D, B_w_in, B_w_sp, B_b_sp, B_w_out, tab)
```

```python
import os

import jax
import jax.numpy as jnp
import numpy as np
import jax.experimental.pallas as pl
import jax.experimental.pallas.tpu as pltpu

F32 = jnp.float32
BF16 = jnp.bfloat16
U32 = jnp.uint32

S = 2048
D = 640
FH = 768
KS = 4
BLK = 128
NB = S // BLK
NC = D // 128
NF = FH // 128
T = 128
NT = S // T
EPS = 1e-5
GRP = 4
KG = 512
UA, UB, US, HP, HQ, HR, TOK = (i * NB for i in range(7))
TB = int(os.environ.get('TB', 5))
P3I = int(os.environ.get('P3I', 4))
LAG = int(os.environ.get('LAG', 4))
TAP1 = int(os.environ.get('TAP1', 1000))

_GELU_C0 = float(np.sqrt(2.0 / np.pi))
_GELU_C1 = _GELU_C0 * 0.044715


def _dft_tables():
    m = np.arange(BLK)[:, None]
    n = np.arange(BLK)[None, :]
    th = 2.0 * np.pi * (((4 * m + 1) * n) % (4 * BLK)) / (4 * BLK)
    ph = 2.0 * np.pi * (((4 * m + 1) * (2 * n + 1)) % (8 * BLK)) / (8 * BLK)
    fu = np.concatenate([np.cos(ph), -np.sin(ph)], axis=0)
    fh = np.concatenate([np.cos(th) + np.sin(th), np.cos(th) - np.sin(th)], axis=0)
    cp = (np.cos(ph) + np.sin(ph)).T[:BLK // 2] / (8.0 * BLK)
    cm = (np.cos(ph) - np.sin(ph)).T[:BLK // 2] / (8.0 * BLK)
    return np.concatenate([fu, fh, cp, cm], axis=0).astype(np.float32)


def _layernorm(x, eps):
    m = jnp.mean(x, axis=-1, keepdims=True)
    d = x - m
    v = jnp.mean(d * d, axis=-1, keepdims=True)
    return d * jax.lax.rsqrt(v + eps)


def _gelu2(x):
    u = x * (x * x * _GELU_C1 + _GELU_C0)
    return x * (1.0 + jnp.tanh(u))


def _pk(x):
    return pltpu.bitcast(x, U32)


def _up(x):
    return pltpu.bitcast(x, BF16)


def _dot(a, b):
    return jnp.dot(a, b, preferred_element_type=F32)


def _spread(items, taps):
    total = sum(c for c, _, _ in items)
    cum = 0
    for c, gate, run in items:
        gate(taps[int(cum * len(taps) / total)]())
        run()
        cum += c


def _kernel(x_hbm, k_hbm, v_hbm, skt_hbm, h_hbm, dv_hbm, win_hbm, wsp_hbm, b_hbm,
            wout_hbm, tab_hbm, out_hbm,
            x_v, win_v, wsp_v, wout_v, kv_v, h_v, xn_v, z1_v, z2_v, p_v,
            kvb_v, pl_v, zz_v, bcol_v, sk_v, dd_v, o_v, zta_v, ztb_v, tab_v,
            skt_v, dv_v, b_v, zero_s, sem):
    cp = pltpu.make_async_copy
    x16 = x_v.bitcast(BF16)
    win16 = win_v.bitcast(BF16)
    kv16 = kv_v.bitcast(BF16)
    h16 = h_v.bitcast(BF16)

    xn32, z232, p32, kvb32, zz32 = (
        r.bitcast(U32) for r in (xn_v, z2_v, p_v, kvb_v, zz_v))

    def x_cp(lo, hi, s):
        return cp(x_hbm.at[0, lo:hi, :], x16.at[lo:hi, :], sem.at[s])

    def win_cp(lo, hi, s):
        return cp(win_hbm.at[:, lo:hi], win16.at[0:D, lo:hi], sem.at[s])

    def k_cp(c, s):
        return cp(k_hbm.at[0, :, pl.ds(c * 128, 128)], kv16.at[2 * c, 0:S, :], sem.at[s])

    def v_cp(c, s):
        return cp(v_hbm.at[0, :, pl.ds(c * 128, 128)], kv16.at[2 * c + 1, 0:S, :], sem.at[s])

    def h_cp(c, s):
        return cp(h_hbm.at[pl.ds(c * 128, 128), :], h16.at[c], sem.at[s])

    H = FH // 2
    groups = [
        [cp(b_hbm, b_v, sem.at[0]), cp(skt_hbm, skt_v, sem.at[0]), cp(dv_hbm, dv_v, sem.at[0])],
        [x_cp(0, 256, 1)],
        [win_cp(FH, FH + H, 2)],
        [win_cp(FH + H, 2 * FH, 3)],
        [win_cp(0, H, 4)],
        [win_cp(H, FH, 5), x_cp(256, 512, 5)],
        [x_cp(512, 1024, 6)],
        [x_cp(1024, S, 7), k_cp(0, 7), v_cp(0, 7)],
        [cp(tab_hbm, tab_v.bitcast(BF16), sem.at[8]), h_cp(0, 8),
         cp(wsp_hbm, wsp_v.bitcast(BF16), sem.at[8])],
    ]
    for g in groups:
        for c in g:
            c.start()

    def tile_cps(c):
        return [k_cp(c, 8 + c), v_cp(c, 8 + c), h_cp(c, 8 + c)]

    for c in range(1, NC):
        for d in tile_cps(c):
            d.start()
    wout_cp = cp(wout_hbm, wout_v.bitcast(BF16), sem.at[13])
    wout_cp.start()

    def wait(i):
        for c in groups[i]:
            c.wait()

    zero_s[0] = 0
    wait(0)
    skt = skt_v[...].astype(F32)
    dv = dv_v[...].astype(F32).reshape(1, D)
    for c in range(NC):
        sk_v[c] = skt[:, c * 128:(c + 1) * 128]
        dd_v[c] = dv[:, c * 128:(c + 1) * 128]
    brow = b_v[...].astype(F32).reshape(1, S)
    bcol_v[...] = jnp.broadcast_to(brow, (128, S)).T

    def gate_x(tok):
        x_v[S // 2:S // 2 + 8, 0:128] = pltpu.bitcast(tok, U32)

    zt_v = (zta_v, ztb_v)

    def gate_zt(t):
        def gate(tok):
            zt_v[t % 2][T:T + 8, 0:128] = tok
        return gate

    def gate_kv(tok):
        kv_v[0, S // 2:S // 2 + 8, :] = pltpu.bitcast(tok, U32)

    def gate_pl(tok):
        pl_v[0, TOK] = tok

    ndone = [0]

    def done(val):
        c = (ndone[0] % (2 * NF)) * 128
        ndone[0] += 1
        win_v[D // 2:D // 2 + 8, c:c + 128] = val

    def lnx_items(t, zero, mark=True):
        def item(r0):
            def run():
                xw = x_v[pl.ds(pl.multiple_of(zero + r0 // 2, 8), 8), :]
                xn = _layernorm(_up(xw).astype(F32), EPS)
                for c in range(NC):
                    xn_v[c, r0:r0 + 16, :] = xn[:, c * 128:(c + 1) * 128].astype(BF16)
                if mark:
                    done(pltpu.bitcast(xn[0:8, 0:128], U32))
                    done(pltpu.bitcast(xn[8:16, 0:128], U32))
            return (1, gate_x, run)
        return [item(t * T + g * 16) for g in range(T // 16)]

    def lnz_items(t, zero):
        def item(g):
            def run():
                z = zt_v[t % 2][pl.ds(pl.multiple_of(zero + g * 16, 8), 16), :]
                z = _layernorm(z, 4.0 * EPS)
                done(pltpu.bitcast(z[0:8, 0:128], U32))
                done(pltpu.bitcast(z[8:16, 0:128], U32))
                r0 = t * T + g * 16
                for n in range(NF):
                    z2_v[n, r0:r0 + 16, :] = z[:, n * 128:(n + 1) * 128].astype(BF16)
            return (1, gate_zt(t), run)
        return [item(g) for g in range(T // 16)]

    KR = 32

    def kv_items(c):
        sk = sk_v[c]

        def item(r0):
            def run():
                hs = slice(r0 // 2, (r0 + KR) // 2)
                if r0 == 0:
                    kw = jnp.concatenate(
                        [jnp.zeros((8, 128), F32), _up(kv_v[2 * c, hs, :]).astype(F32)], axis=0)
                else:
                    kw = _up(kv_v[2 * c, r0 // 2 - 8:(r0 + KR) // 2, :]).astype(F32)[8:]
                ks = kw[8:] * sk[0:1, :]
                for t in range(1, KS):
                    ks = ks + pltpu.roll(kw, t, 0)[8:] * sk[t:t + 1, :]
                kvb_v[r0:r0 + KR, :] = (
                    ks * _up(kv_v[2 * c + 1, hs, :]).astype(F32)).astype(BF16)
            return (14 * KR // 8, gate_kv, run)
        return [item(r0) for r0 in range(0, S, KR)]

    def taps_of(val):
        rows, cols = val.shape
        return [(lambda i=i, n=n: val[i * 8:(i + 1) * 8, n * 128:(n + 1) * 128])
                for n in range(cols // 128) for i in range(rows // 8)]

    def piece(kind, t, n, zero):
        rows = slice(0, D // 2) if zero is None else pl.ds(pl.multiple_of(zero, 8), D // 2)
        col = n * 128 + (FH if kind == 2 else 0)
        xn = jnp.concatenate(
            [_up(xn32[c, t * T // 2:(t + 1) * T // 2, :]) for c in range(NC)], axis=1)
        z = _dot(xn, _up(win_v[rows, col:col + 128]))
        if kind == 2:
            zt_v[t % 2][0:T, n * 128:(n + 1) * 128] = _gelu2(z)
        else:
            z1_v[n, t * T:(t + 1) * T, :] = _gelu2(z).astype(BF16)
        return taps_of(z)

    def block(pieces, work):
        zero = zero_s[0]
        rel = [[] for _ in pieces]
        for mk, lo, hi in work:
            items = mk(zero)
            for i, it in enumerate(items):
                tau = (lo * 16) + (i * (hi - lo) * 16) // len(items)
                rel[tau // 16].append((tau % 16, it))
        taps = []
        gated = False
        for k in range(len(pieces) + LAG):
            if k < len(pieces):
                taps.append(piece(*pieces[k], zero if gated else None))
            if k >= LAG:
                for i, (_, gate, run) in sorted(rel[k - LAG], key=lambda e: e[0]):
                    gate(taps[k - LAG][i]())
                    run()
                    gated = True

    def cols(kind, t, lo=0, hi=NF):
        return [(kind, t, n) for n in range(lo, hi)]

    def lnx(t):
        return lambda zero: lnx_items(t, zero)

    def lnz(t):
        return lambda zero: lnz_items(t, zero)

    wait(1)
    for it in lnx_items(0, 0, False) + lnx_items(1, 0, False):
        it[2]()
    HN = NF // 2
    wait(2)
    block(cols(2, 0, 0, HN) + cols(2, 1, 0, HN), [])
    wait(3)
    block(cols(2, 0, HN) + cols(2, 1, HN), [])
    wait(4)
    block(cols(1, 0, 0, HN) + cols(1, 1, 0, HN), [(lnz(0), 0, 1)])
    wait(5)
    block(cols(1, 0, HN) + cols(1, 1, HN), [(lnx(2), 0, 1)])

    def big_block(first, last, extra):
        pieces, work = [], list(extra)
        for t in range(first, last - 1):
            k = len(pieces)
            pieces += cols(2, t) + cols(1, t)
            if t + 1 < last - 1:
                work += [(lnx(t + 1), k, k + 11 - LAG), (lnz(t), k + 6, k + 18)]
            else:
                work += [(lnx(t + 1), k, k + 11 - LAG), (lnx(t + 2), k + 11 - LAG, k + 17 - LAG),
                         (lnz(t), k + 6, k + 17 - LAG)]
        a, b = last - 1, last
        k = len(pieces)
        pieces += cols(2, a) + cols(2, b) + cols(1, a) + cols(1, b)
        work += [(lnz(a), k + 6, k + 12), (lnz(b), k + 12, k + 23 - LAG)]
        if b + 1 < NT:
            work += [(lnx(b + 1), k + 2, k + 12)]
        else:
            work += [(kv_items, k - 24, k + 24)]
        block(pieces, work)

    wait(6)
    big_block(2, TB, [(lnz(1), 0, 11 - LAG)])
    wait(7)
    big_block(TB + 1, NT - 1, [])

    wait(8)

    def p2(n, carry):
        nn = jnp.minimum(n + 1, NC - 1)

        @pl.when(n + 1 < NC)
        def _():
            for d in tile_cps(nn):
                d.wait()

        zero = zero_s[0]
        fwd_u = _up(tab_v[0:128, :])
        fwd_h = _up(tab_v[128:256, :])
        dd = dd_v[n]
        cp_ = dp_ = None

        def put(slot, val):
            pl_v[:, slot] = val.reshape(BLK // 8, 8, 128)

        for i in range(NB):
            hb = _up(h_v[n, :, i * BLK:(i + 1) * BLK])
            hf = jax.lax.dot_general(fwd_h, hb, (((1,), (1,)), ((), ())),
                                     preferred_element_type=F32)
            c, d = hf[:BLK], hf[BLK:]
            if i == 0:
                c2, d2 = c + dd, d + dd
            else:
                c2, d2 = c - dp_, d + cp_
            cp_, dp_ = c, d
            put(HR + i, c2)
            put(HP + i, d2 - c2)
            put(HQ + i, c2 + d2)
        for i in range(NB):
            u = _dot(fwd_u, _up(kvb32[i * BLK // 2:(i + 1) * BLK // 2, :]))
            a, b = u[:BLK], u[BLK:]
            put(UA + i, a)
            put(UB + i, b)
            put(US + i, a + b)

        state = {}

        def mac_item(pos, g0, pi):
            xv, hv = ((US, HR), (UA, HP), (UB, HQ))[pi]
            outs = range(g0, g0 + GRP)
            top = g0 + GRP

            def run():
                pz = zero + pos
                hs = [pl_v[pz, hv + t] for t in range(top)]
                acc = {o: None for o in outs}
                for jj in range(top):
                    xj = pl_v[pz, xv + jj]
                    for o in outs:
                        if o - jj >= 0:
                            t = xj * hs[o - jj]
                            acc[o] = t if acc[o] is None else acc[o] + t
                r0 = pos * 8
                if pi == 0:
                    state['k1'] = acc
                elif pi == 1:
                    for o in outs:
                        zz_v[n, o, BLK + r0:BLK + r0 + 8, :] = (state['k1'][o] + acc[o]).astype(BF16)
                else:
                    for o in outs:
                        zz_v[n, o, r0:r0 + 8, :] = (state['k1'][o] - acc[o]).astype(BF16)

            nmac = sum(o + 1 for o in outs)
            return (2 * nmac - GRP + (2 * GRP if pi else 0), gate_pl, run)

        kvi = kv_items(nn)
        items = []
        for pos in range(BLK // 8):
            for g0 in range(0, NB, GRP):
                for pi in range(3):
                    items.append(mac_item(pos, g0, pi))
                items.append(kvi[pos * (NB // GRP) + g0 // GRP])

        nq = S // KG
        vpc = T // 8
        total = sum(c for c, _, _ in items)
        tap_of = []
        cum = 0
        for c, _, _ in items:
            tap_of.append(int(cum * TAP1 / total))
            cum += c
        nxt = 0
        for r in range(NT):
            rs = slice(r * T, (r + 1) * T)
            hs = slice(r * T // 2, (r + 1) * T // 2)
            acc = None
            for q in range(nq):
                part = _dot(_up(wsp_v[hs, q * KG:(q + 1) * KG]),
                            _up(z232[n, q * KG // 2:(q + 1) * KG // 2, :]))
                acc = part if acc is None else acc + part
                t0 = (r * nq + q) * vpc
                while nxt < len(items) and tap_of[nxt] < t0 + vpc:
                    i = tap_of[nxt] - t0
                    items[nxt][1](acc[i * 8:(i + 1) * 8, :])
                    items[nxt][2]()
                    nxt += 1
            g = acc + bcol_v[rs, :]
            p_v[n, rs, :] = (z1_v[n, rs, :].astype(F32) * g).astype(BF16)
        assert nxt == len(items)
        return carry

    jax.lax.fori_loop(0, NC, p2, 0)

    wout_cp.wait()

    TPI = NT // P3I

    def p3(j, carry):
        inv_p = _up(tab_v[256:288, :])
        inv_m = _up(tab_v[288:320, :])
        rev = 7 - jax.lax.broadcasted_iota(jnp.int32, (8, 128), 0)

        def rows(t):
            r0 = (j * TPI + t) * T
            return (pl.ds(pl.multiple_of(r0, T), T),
                    pl.ds(pl.multiple_of(r0 // 2, T // 2), T // 2))

        def g5(t):
            rs, hs = rows(t)
            g = _dot(_up(wsp_v[hs, :]), _up(z232[NF - 1])) + bcol_v[rs, :]
            return (z1_v[NF - 1, rs, :].astype(F32) * g).astype(BF16)

        p5 = g5(0)
        for t in range(TPI):
            rs, hs = rows(t)
            p = jnp.concatenate([_up(p32[n, hs, :]) for n in range(NF - 1)] + [p5], axis=1)
            if t + 1 < TPI:
                p5 = g5(t + 1)
            for c in range(NC):
                cs = slice(c * 128, (c + 1) * 128)
                ye = _dot(inv_p, _up(zz32[c, j * TPI + t, 0:64, :]))
                yo = _dot(inv_m, _up(zz32[c, j * TPI + t, 64:128, :]))
                yd = ye - yo
                y = jnp.concatenate(
                    [ye + yo] + [
                        jnp.take_along_axis(yd[i * 8:(i + 1) * 8], rev, axis=0,
                                            mode="promise_in_bounds")
                        for i in reversed(range(BLK // 16))], axis=0)
                o = _dot(p, _up(wout_v[:, cs]))
                gate = o * (1.0 + jnp.tanh(0.25 * o))
                x = _up(x_v[hs, cs]).astype(F32)
                xn = xn_v[c, rs, :].astype(F32)
                o_v[rs, cs] = (x + (xn * y) * gate).astype(BF16)
            cp(o_v.at[rs, :], out_hbm.at[0, rs, :], sem.at[14]).start()
        return carry

    jax.lax.fori_loop(0, P3I, p3, 0)
    cp(o_v, out_hbm.at[0], sem.at[14]).wait()


@jax.jit
def pallas_recurrent_scan__ssm_conv_h3__mixer_gmlp__prompt_kernel(
    A_q: jax.Array,
    A_k: jax.Array,
    A_v: jax.Array,
    A_shift_k: jax.Array,
    A_ssm_k: jax.Array,
    A_ssm_D: jax.Array,
    B_x: jax.Array,
    B_w_in: jax.Array,
    B_w_sp: jax.Array,
    B_b_sp: jax.Array,
    B_w_out: jax.Array,
):
    del B_x
    tab = jnp.asarray(_dft_tables(), dtype=BF16)

    any_spec = pl.BlockSpec(memory_space=pl.ANY)
    return pl.pallas_call(
        _kernel,
        out_shape=jax.ShapeDtypeStruct((1, S, D), BF16),
        in_specs=[any_spec] * 11,
        out_specs=any_spec,
        scratch_shapes=[
            pltpu.VMEM((S // 2 + 8, D), U32),
            pltpu.VMEM((D // 2 + 8, 2 * FH), U32),
            pltpu.VMEM((S // 2, S), U32),
            pltpu.VMEM((FH // 2, D), U32),
            pltpu.VMEM((2 * NC, S // 2 + 8, 128), U32),
            pltpu.VMEM((NC, 64, S), U32),
            pltpu.VMEM((NC, S, 128), BF16),
            pltpu.VMEM((NF, S, 128), BF16),
            pltpu.VMEM((NF, S, 128), BF16),
            pltpu.VMEM((NF - 1, S, 128), BF16),
            pltpu.VMEM((S, 128), BF16),
            pltpu.VMEM((BLK // 8, 6 * NB + 1, 8, 128), F32),
            pltpu.VMEM((NC, NB, 2 * BLK, 128), BF16),
            pltpu.VMEM((S, 128), F32),
            pltpu.VMEM((NC, KS, 128), F32),
            pltpu.VMEM((NC, 1, 128), F32),
            pltpu.VMEM((S, D), BF16),
            pltpu.VMEM((T + 8, FH), F32),
            pltpu.VMEM((T + 8, FH), F32),
            pltpu.VMEM((320, 128), U32),
            pltpu.VMEM((KS, D), BF16),
            pltpu.VMEM((D,), BF16),
            pltpu.VMEM((S,), BF16),
            pltpu.SMEM((1,), jnp.int32),
            pltpu.SemaphoreType.DMA((15,)),
        ],
        compiler_params=pltpu.CompilerParams(
            vmem_limit_bytes=100 * 1024 * 1024, disable_bounds_checks=True),
    )(A_q, A_k, A_v, A_shift_k.T, A_ssm_k, A_ssm_D, B_w_in, B_w_sp, B_b_sp, B_w_out, tab)
```

```python
import os

import jax
import jax.numpy as jnp
import numpy as np
import jax.experimental.pallas as pl
import jax.experimental.pallas.tpu as pltpu

F32 = jnp.float32
BF16 = jnp.bfloat16
U32 = jnp.uint32

S = 2048
D = 640
FH = 768
KS = 4
BLK = 128
NB = S // BLK
NC = D // 128
NF = FH // 128
T = 128
NT = S // T
EPS = 1e-5
GRP = 4
KG = 512
UA, UB, US, HP, HQ, HR, TOK = (i * NB for i in range(7))
TB = int(os.environ.get('TB', 5))
P3I = int(os.environ.get('P3I', 4))
LAG = int(os.environ.get('LAG', 4))
TAP1 = int(os.environ.get('TAP1', 1000))

_GELU_C0 = float(np.sqrt(2.0 / np.pi))
_GELU_C1 = _GELU_C0 * 0.044715


def _dft_tables():
    m = np.arange(BLK)[:, None]
    n = np.arange(BLK)[None, :]
    th = 2.0 * np.pi * (((4 * m + 1) * n) % (4 * BLK)) / (4 * BLK)
    ph = 2.0 * np.pi * (((4 * m + 1) * (2 * n + 1)) % (8 * BLK)) / (8 * BLK)
    fu = np.concatenate([np.cos(ph), -np.sin(ph)], axis=0)
    fh = np.concatenate([np.cos(th) + np.sin(th), np.cos(th) - np.sin(th)], axis=0)
    cp = (np.cos(ph) + np.sin(ph)).T[:BLK // 2] / (8.0 * BLK)
    cm = (np.cos(ph) - np.sin(ph)).T[:BLK // 2] / (8.0 * BLK)
    return np.concatenate([fu, fh, cp, cm], axis=0).astype(np.float32)


def _layernorm(x, eps):
    m = jnp.mean(x, axis=-1, keepdims=True)
    d = x - m
    v = jnp.mean(d * d, axis=-1, keepdims=True)
    return d * jax.lax.rsqrt(v + eps)


def _gelu2(x):
    u = x * (x * x * _GELU_C1 + _GELU_C0)
    return x * (1.0 + jnp.tanh(u))


def _pk(x):
    return pltpu.bitcast(x, U32)


def _up(x):
    return pltpu.bitcast(x, BF16)


def _dot(a, b):
    return jnp.dot(a, b, preferred_element_type=F32)


def _spread(items, taps):
    total = sum(c for c, _, _ in items)
    cum = 0
    for c, gate, run in items:
        gate(taps[int(cum * len(taps) / total)]())
        run()
        cum += c


def _kernel(x_hbm, k_hbm, v_hbm, skt_hbm, h_hbm, dv_hbm, win_hbm, wsp_hbm, b_hbm,
            wout_hbm, tab_hbm, out_hbm,
            x_v, win_v, wsp_v, wout_v, kv_v, h_v, xn_v, z1_v, z2_v, p_v,
            kvb_v, pl_v, zz_v, bcol_v, o_v, zta_v, ztb_v, tab_v,
            sk_v, dd_v, skt_v, dv_v, b_v, zero_s, sem):
    cp = pltpu.make_async_copy
    x16 = x_v.bitcast(BF16)
    win16 = win_v.bitcast(BF16)
    kv16 = kv_v.bitcast(BF16)
    h16 = h_v.bitcast(BF16)

    xn32, z232, p32, kvb32, zz32 = (
        r.bitcast(U32) for r in (xn_v, z2_v, p_v, kvb_v, zz_v))

    def x_cp(lo, hi, s):
        return cp(x_hbm.at[0, lo:hi, :], x16.at[0, lo:hi, :], sem.at[s])

    def win_cp(lo, hi, s):
        return cp(win_hbm.at[:, lo:hi], win16.at[0, 0:D, lo:hi], sem.at[s])

    def k_cp(c, s):
        return cp(k_hbm.at[0, :, pl.ds(c * 128, 128)], kv16.at[2 * c, 0:S, :], sem.at[s])

    def v_cp(c, s):
        return cp(v_hbm.at[0, :, pl.ds(c * 128, 128)], kv16.at[2 * c + 1, 0:S, :], sem.at[s])

    def h_cp(c, s):
        return cp(h_hbm.at[pl.ds(c * 128, 128), :], h16.at[c], sem.at[s])

    H = FH // 2
    groups = [
        [cp(b_hbm, b_v, sem.at[0]), cp(skt_hbm, skt_v, sem.at[0]), cp(dv_hbm, dv_v, sem.at[0])],
        [x_cp(0, 256, 1)],
        [win_cp(FH, FH + H, 2)],
        [win_cp(FH + H, 2 * FH, 3)],
        [win_cp(0, H, 4)],
        [win_cp(H, FH, 5), x_cp(256, 512, 5)],
        [x_cp(512, 1024, 6)],
        [x_cp(1024, S, 7), k_cp(0, 7), v_cp(0, 7)],
        [cp(tab_hbm, tab_v.bitcast(BF16), sem.at[8]), h_cp(0, 8),
         cp(wsp_hbm, wsp_v.bitcast(BF16), sem.at[8])],
    ]
    for g in groups:
        for c in g:
            c.start()

    def tile_cps(c):
        return [k_cp(c, 8 + c), v_cp(c, 8 + c), h_cp(c, 8 + c)]

    for c in range(1, NC):
        for d in tile_cps(c):
            d.start()
    wout_cp = cp(wout_hbm, wout_v.bitcast(BF16), sem.at[13])
    wout_cp.start()

    def wait(i):
        for c in groups[i]:
            c.wait()

    zero_s[0] = 0
    wait(0)
    skt = skt_v[...].astype(F32)
    dv = dv_v[...].astype(F32).reshape(1, D)
    for c in range(NC):
        sk_v[c] = skt[:, c * 128:(c + 1) * 128]
        dd_v[c] = dv[:, c * 128:(c + 1) * 128]
    brow = b_v[...].astype(F32).reshape(1, S)
    bcol_v[...] = jnp.broadcast_to(brow, (128, S)).T

    def gate_x(tok):
        x_v[0, S // 2:S // 2 + 8, 0:128] = pltpu.bitcast(tok, U32)

    zt_v = (zta_v, ztb_v)

    def gate_zt(t):
        def gate(tok):
            zt_v[t % 2][0, T:T + 8, 0:128] = tok
        return gate

    def gate_kv(tok):
        kv_v[0, S // 2:S // 2 + 8, :] = pltpu.bitcast(tok, U32)

    def gate_pl(tok):
        pl_v[0, TOK] = tok

    ndone = [0]

    def done(val):
        c = (ndone[0] % (2 * NF)) * 128
        ndone[0] += 1
        win_v[0, D // 2:D // 2 + 8, c:c + 128] = val

    def lnx_items(t, zero, mark=True):
        def item(r0):
            def run():
                xw = x_v[zero, r0 // 2:r0 // 2 + 8, :]
                xn = _layernorm(_up(xw).astype(F32), EPS)
                for c in range(NC):
                    xn_v[c, r0:r0 + 16, :] = xn[:, c * 128:(c + 1) * 128].astype(BF16)
                if mark:
                    done(pltpu.bitcast(xn[0:8, 0:128], U32))
                    done(pltpu.bitcast(xn[8:16, 0:128], U32))
            return (1, gate_x, run)
        return [item(t * T + g * 16) for g in range(T // 16)]

    def lnz_items(t, zero):
        def item(g):
            def run():
                z = zt_v[t % 2][zero, g * 16:(g + 1) * 16, :]
                z = _layernorm(z, 4.0 * EPS)
                done(pltpu.bitcast(z[0:8, 0:128], U32))
                done(pltpu.bitcast(z[8:16, 0:128], U32))
                r0 = t * T + g * 16
                for n in range(NF):
                    z2_v[n, r0:r0 + 16, :] = z[:, n * 128:(n + 1) * 128].astype(BF16)
            return (1, gate_zt(t), run)
        return [item(g) for g in range(T // 16)]

    KR = 32

    def kv_items(c):
        sk = sk_v[c]

        def item(r0):
            def run():
                hs = slice(r0 // 2, (r0 + KR) // 2)
                if r0 == 0:
                    kw = jnp.concatenate(
                        [jnp.zeros((8, 128), F32), _up(kv_v[2 * c, hs, :]).astype(F32)], axis=0)
                else:
                    kw = _up(kv_v[2 * c, r0 // 2 - 8:(r0 + KR) // 2, :]).astype(F32)[8:]
                ks = kw[8:] * sk[0:1, :]
                for t in range(1, KS):
                    ks = ks + pltpu.roll(kw, t, 0)[8:] * sk[t:t + 1, :]
                kvb_v[r0:r0 + KR, :] = (
                    ks * _up(kv_v[2 * c + 1, hs, :]).astype(F32)).astype(BF16)
            return (14 * KR // 8, gate_kv, run)
        return [item(r0) for r0 in range(0, S, KR)]

    def taps_of(val):
        rows, cols = val.shape
        return [(lambda i=i, n=n: val[i * 8:(i + 1) * 8, n * 128:(n + 1) * 128])
                for n in range(cols // 128) for i in range(rows // 8)]

    def piece(kind, t, n, zero):
        col = n * 128 + (FH if kind == 2 else 0)
        xn = jnp.concatenate(
            [_up(xn32[c, t * T // 2:(t + 1) * T // 2, :]) for c in range(NC)], axis=1)
        z = _dot(xn, _up(win_v[0 if zero is None else zero, 0:D // 2, col:col + 128]))
        if kind == 2:
            zt_v[t % 2][0, 0:T, n * 128:(n + 1) * 128] = _gelu2(z)
        else:
            z1_v[n, t * T:(t + 1) * T, :] = _gelu2(z).astype(BF16)
        return taps_of(z)

    def block(pieces, work):
        zero = zero_s[0]
        rel = [[] for _ in pieces]
        for mk, lo, hi in work:
            items = mk(zero)
            for i, it in enumerate(items):
                tau = (lo * 16) + (i * (hi - lo) * 16) // len(items)
                rel[tau // 16].append((tau % 16, it))
        taps = []
        gated = False
        for k in range(len(pieces) + LAG):
            if k < len(pieces):
                taps.append(piece(*pieces[k], zero if gated else None))
            if k >= LAG:
                for i, (_, gate, run) in sorted(rel[k - LAG], key=lambda e: e[0]):
                    gate(taps[k - LAG][i]())
                    run()
                    gated = True

    def cols(kind, t, lo=0, hi=NF):
        return [(kind, t, n) for n in range(lo, hi)]

    def lnx(t):
        return lambda zero: lnx_items(t, zero)

    def lnz(t):
        return lambda zero: lnz_items(t, zero)

    wait(1)
    for it in lnx_items(0, 0, False) + lnx_items(1, 0, False):
        it[2]()
    HN = NF // 2
    wait(2)
    block(cols(2, 0, 0, HN) + cols(2, 1, 0, HN), [])
    wait(3)
    block(cols(2, 0, HN) + cols(2, 1, HN), [])
    wait(4)
    block(cols(1, 0, 0, HN) + cols(1, 1, 0, HN), [(lnz(0), 0, 1)])
    wait(5)
    block(cols(1, 0, HN) + cols(1, 1, HN), [(lnx(2), 0, 1)])

    def big_block(first, last, extra):
        pieces, work = [], list(extra)
        for t in range(first, last - 1):
            k = len(pieces)
            pieces += cols(2, t) + cols(1, t)
            if t + 1 < last - 1:
                work += [(lnx(t + 1), k, k + 11 - LAG), (lnz(t), k + 6, k + 18)]
            else:
                work += [(lnx(t + 1), k, k + 11 - LAG), (lnx(t + 2), k + 11 - LAG, k + 17 - LAG),
                         (lnz(t), k + 6, k + 17 - LAG)]
        a, b = last - 1, last
        k = len(pieces)
        pieces += cols(2, a) + cols(2, b) + cols(1, a) + cols(1, b)
        work += [(lnz(a), k + 6, k + 12), (lnz(b), k + 12, k + 23 - LAG)]
        if b + 1 < NT:
            work += [(lnx(b + 1), k + 2, k + 12)]
        else:
            work += [(kv_items, k - 24, k + 24)]
        block(pieces, work)

    wait(6)
    big_block(2, TB, [(lnz(1), 0, 11 - LAG)])
    wait(7)
    big_block(TB + 1, NT - 1, [])

    wait(8)

    def p2(n, carry):
        nn = jnp.minimum(n + 1, NC - 1)

        @pl.when(n + 1 < NC)
        def _():
            for d in tile_cps(nn):
                d.wait()

        zero = zero_s[0]
        fwd_u = _up(tab_v[0:128, :])
        fwd_h = _up(tab_v[128:256, :])
        dd = dd_v[n]
        cp_ = dp_ = None

        def put(slot, val):
            pl_v[:, slot] = val.reshape(BLK // 8, 8, 128)

        for i in range(NB):
            hb = _up(h_v[n, :, i * BLK:(i + 1) * BLK])
            hf = jax.lax.dot_general(fwd_h, hb, (((1,), (1,)), ((), ())),
                                     preferred_element_type=F32)
            c, d = hf[:BLK], hf[BLK:]
            if i == 0:
                c2, d2 = c + dd, d + dd
            else:
                c2, d2 = c - dp_, d + cp_
            cp_, dp_ = c, d
            put(HR + i, c2)
            put(HP + i, d2 - c2)
            put(HQ + i, c2 + d2)
        for i in range(NB):
            u = _dot(fwd_u, _up(kvb32[i * BLK // 2:(i + 1) * BLK // 2, :]))
            a, b = u[:BLK], u[BLK:]
            put(UA + i, a)
            put(UB + i, b)
            put(US + i, a + b)

        state = {}

        def mac_item(pos, g0, pi):
            xv, hv = ((US, HR), (UA, HP), (UB, HQ))[pi]
            outs = range(g0, g0 + GRP)
            top = g0 + GRP

            def run():
                pz = zero + pos
                hs = [pl_v[pz, hv + t] for t in range(top)]
                acc = {o: None for o in outs}
                for jj in range(top):
                    xj = pl_v[pz, xv + jj]
                    for o in outs:
                        if o - jj >= 0:
                            t = xj * hs[o - jj]
                            acc[o] = t if acc[o] is None else acc[o] + t
                r0 = pos * 8
                if pi == 0:
                    state['k1'] = acc
                elif pi == 1:
                    for o in outs:
                        zz_v[n, o, BLK + r0:BLK + r0 + 8, :] = (state['k1'][o] + acc[o]).astype(BF16)
                else:
                    for o in outs:
                        zz_v[n, o, r0:r0 + 8, :] = (state['k1'][o] - acc[o]).astype(BF16)

            nmac = sum(o + 1 for o in outs)
            return (2 * nmac - GRP + (2 * GRP if pi else 0), gate_pl, run)

        kvi = kv_items(nn)
        items = []
        for pos in range(BLK // 8):
            for g0 in range(0, NB, GRP):
                for pi in range(3):
                    items.append(mac_item(pos, g0, pi))
                items.append(kvi[pos * (NB // GRP) + g0 // GRP])

        nq = S // KG
        vpc = T // 8
        total = sum(c for c, _, _ in items)
        tap_of = []
        cum = 0
        for c, _, _ in items:
            tap_of.append(int(cum * TAP1 / total))
            cum += c
        nxt = 0
        for r in range(NT):
            rs = slice(r * T, (r + 1) * T)
            hs = slice(r * T // 2, (r + 1) * T // 2)
            acc = None
            for q in range(nq):
                part = _dot(_up(wsp_v[hs, q * KG:(q + 1) * KG]),
                            _up(z232[n, q * KG // 2:(q + 1) * KG // 2, :]))
                acc = part if acc is None else acc + part
                t0 = (r * nq + q) * vpc
                while nxt < len(items) and tap_of[nxt] < t0 + vpc:
                    i = tap_of[nxt] - t0
                    items[nxt][1](acc[i * 8:(i + 1) * 8, :])
                    items[nxt][2]()
                    nxt += 1
            g = acc + bcol_v[rs, :]
            p_v[n, rs, :] = (z1_v[n, rs, :].astype(F32) * g).astype(BF16)
        assert nxt == len(items)
        return carry

    jax.lax.fori_loop(0, NC, p2, 0)

    wout_cp.wait()

    TPI = NT // P3I

    def p3(j, carry):
        inv_p = _up(tab_v[256:288, :])
        inv_m = _up(tab_v[288:320, :])
        rev = 7 - jax.lax.broadcasted_iota(jnp.int32, (8, 128), 0)

        def rows(t):
            r0 = (j * TPI + t) * T
            return (pl.ds(pl.multiple_of(r0, T), T),
                    pl.ds(pl.multiple_of(r0 // 2, T // 2), T // 2))

        def g5(t):
            rs, hs = rows(t)
            g = _dot(_up(wsp_v[hs, :]), _up(z232[NF - 1])) + bcol_v[rs, :]
            return (z1_v[NF - 1, rs, :].astype(F32) * g).astype(BF16)

        p5 = g5(0)
        for t in range(TPI):
            rs, hs = rows(t)
            p = jnp.concatenate([_up(p32[n, hs, :]) for n in range(NF - 1)] + [p5], axis=1)
            if t + 1 < TPI:
                p5 = g5(t + 1)
            for c in range(NC):
                cs = slice(c * 128, (c + 1) * 128)
                ye = _dot(inv_p, _up(zz32[c, j * TPI + t, 0:64, :]))
                yo = _dot(inv_m, _up(zz32[c, j * TPI + t, 64:128, :]))
                yd = ye - yo
                y = jnp.concatenate(
                    [ye + yo] + [
                        jnp.take_along_axis(yd[i * 8:(i + 1) * 8], rev, axis=0,
                                            mode="promise_in_bounds")
                        for i in reversed(range(BLK // 16))], axis=0)
                o = _dot(p, _up(wout_v[:, cs]))
                gate = o * (1.0 + jnp.tanh(0.25 * o))
                x = _up(x_v[0, hs, cs]).astype(F32)
                xn = xn_v[c, rs, :].astype(F32)
                o_v[rs, cs] = (x + (xn * y) * gate).astype(BF16)
            cp(o_v.at[rs, :], out_hbm.at[0, rs, :], sem.at[14]).start()
        return carry

    jax.lax.fori_loop(0, P3I, p3, 0)
    cp(o_v, out_hbm.at[0], sem.at[14]).wait()


@jax.jit
def pallas_recurrent_scan__ssm_conv_h3__mixer_gmlp__prompt_kernel(
    A_q: jax.Array,
    A_k: jax.Array,
    A_v: jax.Array,
    A_shift_k: jax.Array,
    A_ssm_k: jax.Array,
    A_ssm_D: jax.Array,
    B_x: jax.Array,
    B_w_in: jax.Array,
    B_w_sp: jax.Array,
    B_b_sp: jax.Array,
    B_w_out: jax.Array,
):
    del B_x
    tab = jnp.asarray(_dft_tables(), dtype=BF16)

    any_spec = pl.BlockSpec(memory_space=pl.ANY)
    return pl.pallas_call(
        _kernel,
        out_shape=jax.ShapeDtypeStruct((1, S, D), BF16),
        in_specs=[any_spec] * 11,
        out_specs=any_spec,
        scratch_shapes=[
            pltpu.VMEM((1, S // 2 + 32, D), U32),
            pltpu.VMEM((1, D // 2 + 8, 2 * FH), U32),
            pltpu.VMEM((S // 2, S), U32),
            pltpu.VMEM((FH // 2, D), U32),
            pltpu.VMEM((2 * NC, S // 2 + 32, 128), U32),
            pltpu.VMEM((NC, 64, S), U32),
            pltpu.VMEM((NC, S, 128), BF16),
            pltpu.VMEM((NF, S, 128), BF16),
            pltpu.VMEM((NF, S, 128), BF16),
            pltpu.VMEM((NF - 1, S, 128), BF16),
            pltpu.VMEM((S, 128), BF16),
            pltpu.VMEM((BLK // 8, 6 * NB + 1, 8, 128), F32),
            pltpu.VMEM((NC, NB, 2 * BLK, 128), BF16),
            pltpu.VMEM((S, 128), F32),
            pltpu.VMEM((S, D), BF16),
            pltpu.VMEM((1, T + 16, FH), F32),
            pltpu.VMEM((1, T + 16, FH), F32),
            pltpu.VMEM((320, 128), U32),
            pltpu.VMEM((NC, KS, 128), F32),
            pltpu.VMEM((NC + 2, 1, 128), F32),
            pltpu.VMEM((KS, D), BF16),
            pltpu.VMEM((D,), BF16),
            pltpu.VMEM((S,), BF16),
            pltpu.SMEM((1,), jnp.int32),
            pltpu.SemaphoreType.DMA((15,)),
        ],
        compiler_params=pltpu.CompilerParams(
            vmem_limit_bytes=100 * 1024 * 1024, disable_bounds_checks=True),
    )(A_q, A_k, A_v, A_shift_k.T, A_ssm_k, A_ssm_D, B_w_in, B_w_sp, B_b_sp, B_w_out, tab)
```

```python
import os

import jax
import jax.numpy as jnp
import numpy as np
import jax.experimental.pallas as pl
import jax.experimental.pallas.tpu as pltpu

F32 = jnp.float32
BF16 = jnp.bfloat16
U32 = jnp.uint32

S = 2048
D = 640
FH = 768
KS = 4
BLK = 128
NB = S // BLK
NC = D // 128
NF = FH // 128
T = 128
NT = S // T
EPS = 1e-5
GRP = 4
KG = 512
UA, UB, US, HP, HQ, HR, TOK = (i * NB for i in range(7))
TB = int(os.environ.get('TB', 5))
P3I = int(os.environ.get('P3I', 4))
LAG = int(os.environ.get('LAG', 4))
TAP1 = int(os.environ.get('TAP1', 1000))

_GELU_C0 = float(np.sqrt(2.0 / np.pi))
_GELU_C1 = _GELU_C0 * 0.044715


def _dft_tables():
    m = np.arange(BLK)[:, None]
    n = np.arange(BLK)[None, :]
    th = 2.0 * np.pi * (((4 * m + 1) * n) % (4 * BLK)) / (4 * BLK)
    ph = 2.0 * np.pi * (((4 * m + 1) * (2 * n + 1)) % (8 * BLK)) / (8 * BLK)
    fu = np.concatenate([np.cos(ph), -np.sin(ph)], axis=0)
    fh = np.concatenate([np.cos(th) + np.sin(th), np.cos(th) - np.sin(th)], axis=0)
    fu, fh = (f.reshape(2, BLK // 8, 8, BLK).transpose(1, 0, 2, 3).reshape(2 * BLK, BLK)
              for f in (fu, fh))
    cp = (np.cos(ph) + np.sin(ph)).T[:BLK // 2] / (8.0 * BLK)
    cm = (np.cos(ph) - np.sin(ph)).T[:BLK // 2] / (8.0 * BLK)
    return np.concatenate([fu, fh, cp, cm], axis=0).astype(np.float32)


def _layernorm(x, eps):
    m = jnp.mean(x, axis=-1, keepdims=True)
    d = x - m
    v = jnp.mean(d * d, axis=-1, keepdims=True)
    return d * jax.lax.rsqrt(v + eps)


def _gelu2(x):
    u = x * (x * x * _GELU_C1 + _GELU_C0)
    return x * (1.0 + jnp.tanh(u))


def _pk(x):
    return pltpu.bitcast(x, U32)


def _up(x):
    return pltpu.bitcast(x, BF16)


def _dot(a, b):
    return jnp.dot(a, b, preferred_element_type=F32)


def _spread(items, taps):
    total = sum(c for c, _, _ in items)
    cum = 0
    for c, gate, run in items:
        gate(taps[int(cum * len(taps) / total)]())
        run()
        cum += c


def _kernel(x_hbm, k_hbm, v_hbm, skt_hbm, h_hbm, dv_hbm, win_hbm, wsp_hbm, b_hbm,
            wout_hbm, tab_hbm, out_hbm,
            x_v, win_v, wsp_v, wout_v, kv_v, h_v, xn_v, z1_v, z2_v, p_v,
            kvb_v, pl_v, zz_v, bcol_v, o_v, zta_v, ztb_v, tab_v,
            sk_v, dd_v, skt_v, dv_v, b_v, zero_s, sem):
    cp = pltpu.make_async_copy
    x16 = x_v.bitcast(BF16)
    win16 = win_v.bitcast(BF16)
    kv16 = kv_v.bitcast(BF16)
    h16 = h_v.bitcast(BF16)

    xn32, z232, p32, kvb32, zz32 = (
        r.bitcast(U32) for r in (xn_v, z2_v, p_v, kvb_v, zz_v))

    def x_cp(lo, hi, s):
        return cp(x_hbm.at[0, lo:hi, :], x16.at[0, lo:hi, :], sem.at[s])

    def win_cp(lo, hi, s):
        return cp(win_hbm.at[:, lo:hi], win16.at[0, 0:D, lo:hi], sem.at[s])

    def k_cp(c, s):
        return cp(k_hbm.at[0, :, pl.ds(c * 128, 128)], kv16.at[2 * c, 0:S, :], sem.at[s])

    def v_cp(c, s):
        return cp(v_hbm.at[0, :, pl.ds(c * 128, 128)], kv16.at[2 * c + 1, 0:S, :], sem.at[s])

    def h_cp(c, s):
        return cp(h_hbm.at[pl.ds(c * 128, 128), :], h16.at[c], sem.at[s])

    H = FH // 2
    groups = [
        [cp(b_hbm, b_v, sem.at[0]), cp(skt_hbm, skt_v, sem.at[0]), cp(dv_hbm, dv_v, sem.at[0])],
        [x_cp(0, 256, 1)],
        [win_cp(FH, FH + H, 2)],
        [win_cp(FH + H, 2 * FH, 3)],
        [win_cp(0, H, 4)],
        [win_cp(H, FH, 5), x_cp(256, 512, 5)],
        [x_cp(512, 1024, 6)],
        [x_cp(1024, S, 7), k_cp(0, 7), v_cp(0, 7)],
        [cp(tab_hbm, tab_v.bitcast(BF16), sem.at[8]), h_cp(0, 8),
         cp(wsp_hbm, wsp_v.bitcast(BF16), sem.at[8])],
    ]
    for g in groups:
        for c in g:
            c.start()

    def tile_cps(c):
        return [k_cp(c, 8 + c), v_cp(c, 8 + c), h_cp(c, 8 + c)]

    for c in range(1, NC):
        for d in tile_cps(c):
            d.start()
    wout_cp = cp(wout_hbm, wout_v.bitcast(BF16), sem.at[13])
    wout_cp.start()

    def wait(i):
        for c in groups[i]:
            c.wait()

    zero_s[0] = 0
    wait(0)
    skt = skt_v[...].astype(F32)
    dv = dv_v[...].astype(F32).reshape(1, D)
    for c in range(NC):
        sk_v[c] = skt[:, c * 128:(c + 1) * 128]
        dd_v[c] = dv[:, c * 128:(c + 1) * 128]
    brow = b_v[...].astype(F32).reshape(1, S)
    bcol_v[...] = jnp.broadcast_to(brow, (128, S)).T

    def gate_x(tok):
        x_v[0, S // 2:S // 2 + 8, 0:128] = pltpu.bitcast(tok, U32)

    zt_v = (zta_v, ztb_v)

    def gate_zt(t):
        def gate(tok):
            zt_v[t % 2][0, T:T + 8, 0:128] = tok
        return gate

    def gate_kv(tok):
        kv_v[0, S // 2:S // 2 + 8, :] = pltpu.bitcast(tok, U32)

    def gate_pl(tok):
        pl_v[0, TOK] = tok

    ndone = [0]

    def done(val):
        c = (ndone[0] % (2 * NF)) * 128
        ndone[0] += 1
        win_v[0, D // 2:D // 2 + 8, c:c + 128] = val

    def lnx_items(t, zero, mark=True):
        def item(r0):
            def run():
                xw = x_v[zero, r0 // 2:r0 // 2 + 8, :]
                xn = _layernorm(_up(xw).astype(F32), EPS)
                for c in range(NC):
                    xn_v[c, r0:r0 + 16, :] = xn[:, c * 128:(c + 1) * 128].astype(BF16)
                if mark:
                    done(pltpu.bitcast(xn[0:8, 0:128], U32))
                    done(pltpu.bitcast(xn[8:16, 0:128], U32))
            return (1, gate_x, run)
        return [item(t * T + g * 16) for g in range(T // 16)]

    def lnz_items(t, zero):
        def item(g):
            def run():
                z = zt_v[t % 2][zero, g * 16:(g + 1) * 16, :]
                z = _layernorm(z, 4.0 * EPS)
                done(pltpu.bitcast(z[0:8, 0:128], U32))
                done(pltpu.bitcast(z[8:16, 0:128], U32))
                r0 = t * T + g * 16
                for n in range(NF):
                    z2_v[n, r0:r0 + 16, :] = z[:, n * 128:(n + 1) * 128].astype(BF16)
            return (1, gate_zt(t), run)
        return [item(g) for g in range(T // 16)]

    KR = 32

    def kv_items(c):
        sk = sk_v[c]

        def item(r0):
            def run():
                hs = slice(r0 // 2, (r0 + KR) // 2)
                if r0 == 0:
                    kw = jnp.concatenate(
                        [jnp.zeros((8, 128), F32), _up(kv_v[2 * c, hs, :]).astype(F32)], axis=0)
                else:
                    kw = _up(kv_v[2 * c, r0 // 2 - 8:(r0 + KR) // 2, :]).astype(F32)[8:]
                ks = kw[8:] * sk[0:1, :]
                for t in range(1, KS):
                    ks = ks + pltpu.roll(kw, t, 0)[8:] * sk[t:t + 1, :]
                kvb_v[r0:r0 + KR, :] = (
                    ks * _up(kv_v[2 * c + 1, hs, :]).astype(F32)).astype(BF16)
            return (14 * KR // 8, gate_kv, run)
        return [item(r0) for r0 in range(0, S, KR)]

    def taps_of(val):
        rows, cols = val.shape
        return [(lambda i=i, n=n: val[i * 8:(i + 1) * 8, n * 128:(n + 1) * 128])
                for n in range(cols // 128) for i in range(rows // 8)]

    def piece(kind, t, n, zero):
        col = n * 128 + (FH if kind == 2 else 0)
        xn = jnp.concatenate(
            [_up(xn32[c, t * T // 2:(t + 1) * T // 2, :]) for c in range(NC)], axis=1)
        z = _dot(xn, _up(win_v[0 if zero is None else zero, 0:D // 2, col:col + 128]))
        if kind == 2:
            zt_v[t % 2][0, 0:T, n * 128:(n + 1) * 128] = _gelu2(z)
        else:
            z1_v[n, t * T:(t + 1) * T, :] = _gelu2(z).astype(BF16)
        return taps_of(z)

    def block(pieces, work):
        zero = zero_s[0]
        rel = [[] for _ in pieces]
        for mk, lo, hi in work:
            items = mk(zero)
            for i, it in enumerate(items):
                tau = (lo * 16) + (i * (hi - lo) * 16) // len(items)
                rel[tau // 16].append((tau % 16, it))
        taps = []
        gated = False
        for k in range(len(pieces) + LAG):
            if k < len(pieces):
                taps.append(piece(*pieces[k], zero if gated else None))
            if k >= LAG:
                for i, (_, gate, run) in sorted(rel[k - LAG], key=lambda e: e[0]):
                    gate(taps[k - LAG][i]())
                    run()
                    gated = True

    def cols(kind, t, lo=0, hi=NF):
        return [(kind, t, n) for n in range(lo, hi)]

    def lnx(t):
        return lambda zero: lnx_items(t, zero)

    def lnz(t):
        return lambda zero: lnz_items(t, zero)

    wait(1)
    for it in lnx_items(0, 0, False) + lnx_items(1, 0, False):
        it[2]()
    HN = NF // 2
    wait(2)
    block(cols(2, 0, 0, HN) + cols(2, 1, 0, HN), [])
    wait(3)
    block(cols(2, 0, HN) + cols(2, 1, HN), [])
    wait(4)
    block(cols(1, 0, 0, HN) + cols(1, 1, 0, HN), [(lnz(0), 0, 1)])
    wait(5)
    block(cols(1, 0, HN) + cols(1, 1, HN), [(lnx(2), 0, 1)])

    def big_block(first, last, extra):
        pieces, work = [], list(extra)
        for t in range(first, last - 1):
            k = len(pieces)
            pieces += cols(2, t) + cols(1, t)
            if t + 1 < last - 1:
                work += [(lnx(t + 1), k, k + 11 - LAG), (lnz(t), k + 6, k + 18)]
            else:
                work += [(lnx(t + 1), k, k + 11 - LAG), (lnx(t + 2), k + 11 - LAG, k + 17 - LAG),
                         (lnz(t), k + 6, k + 17 - LAG)]
        a, b = last - 1, last
        k = len(pieces)
        pieces += cols(2, a) + cols(2, b) + cols(1, a) + cols(1, b)
        work += [(lnz(a), k + 6, k + 12), (lnz(b), k + 12, k + 23 - LAG)]
        if b + 1 < NT:
            work += [(lnx(b + 1), k + 2, k + 12)]
        else:
            work += [(kv_items, k - 24, k + 24)]
        block(pieces, work)

    wait(6)
    big_block(2, TB, [(lnz(1), 0, 11 - LAG)])
    wait(7)
    big_block(TB + 1, NT - 1, [])

    wait(8)

    def p2(n, carry):
        nn = jnp.minimum(n + 1, NC - 1)

        @pl.when(n + 1 < NC)
        def _():
            for d in tile_cps(nn):
                d.wait()

        zero = zero_s[0]
        fwd_u = _up(tab_v[0:128, :])
        fwd_h = _up(tab_v[128:256, :])
        dd = dd_v[n]

        def put(slot, val):
            pl_v[:, slot] = val

        def re_im(val):
            val = val.reshape(BLK // 8, 2, 8, 128)
            return val[:, 0], val[:, 1]

        kvi = kv_items(nn)

        def pace_kv(d, val):
            if d % 4 == 3:
                for j in range(8):
                    _, gate, run = kvi[(d // 4) * 8 + j]
                    gate(val[j * 32:j * 32 + 8, :])
                    run()

        for i in range(NB):
            u = _dot(fwd_u, _up(kvb32[i * BLK // 2:(i + 1) * BLK // 2, :]))
            a, b = re_im(u)
            put(UA + i, a)
            put(UB + i, b)
            put(US + i, a + b)
            pace_kv(i, u)
        for i in range(NB):
            hb = _up(h_v[n, :, i * BLK:(i + 1) * BLK])
            hf = jax.lax.dot_general(fwd_h, hb, (((1,), (1,)), ((), ())),
                                     preferred_element_type=F32)
            c, d = re_im(hf)
            if i == 0:
                c, d = c + dd, d + dd
            put(HR + i, c)
            put(HP + i, d - c)
            put(HQ + i, c + d)
            pace_kv(NB + i, hf)

        state = {}

        def mac_item(pos, g0, pi):
            xv, hv = ((US, HR), (UA, HP), (UB, HQ))[pi]
            outs = range(g0, g0 + GRP)
            top = g0 + GRP

            def run():
                pz = zero + pos
                hs = [pl_v[pz, hv + t] for t in range(top)]
                acc = {o: None for o in outs}
                for jj in range(top):
                    xj = pl_v[pz, xv + jj]
                    for o in outs:
                        if o - jj >= 0:
                            t = xj * hs[o - jj]
                            acc[o] = t if acc[o] is None else acc[o] + t
                r0 = pos * 8
                if pi == 0:
                    state['k1'] = acc
                elif pi == 1:
                    state['im'] = {o: state['k1'][o] + acc[o] for o in outs}
                else:
                    for o in outs:
                        re, im = state['k1'][o] - acc[o], state['im'][o]
                        zr, zi = re, im
                        if o > 0:
                            zr, zi = re - state['prev'][1], im + state['prev'][0]
                        state['prev'] = (re, im)
                        zz_v[n, o, r0:r0 + 8, :] = zr.astype(BF16)
                        zz_v[n, o, BLK + r0:BLK + r0 + 8, :] = zi.astype(BF16)

            nmac = sum(o + 1 for o in outs)
            return (2 * nmac - GRP + (0, GRP, 5 * GRP)[pi], gate_pl, run)

        items = []
        for pos in range(BLK // 8):
            for g0 in range(0, NB, GRP):
                for pi in range(3):
                    items.append(mac_item(pos, g0, pi))

        nq = S // KG
        vpc = T // 8
        total = sum(c for c, _, _ in items)
        tap_of = []
        cum = 0
        for c, _, _ in items:
            tap_of.append(int(cum * TAP1 / total))
            cum += c
        nxt = 0
        for r in range(NT):
            rs = slice(r * T, (r + 1) * T)
            hs = slice(r * T // 2, (r + 1) * T // 2)
            acc = None
            for q in range(nq):
                part = _dot(_up(wsp_v[hs, q * KG:(q + 1) * KG]),
                            _up(z232[n, q * KG // 2:(q + 1) * KG // 2, :]))
                acc = part if acc is None else acc + part
                t0 = (r * nq + q) * vpc
                while nxt < len(items) and tap_of[nxt] < t0 + vpc:
                    i = tap_of[nxt] - t0
                    items[nxt][1](acc[i * 8:(i + 1) * 8, :])
                    items[nxt][2]()
                    nxt += 1
            g = acc + bcol_v[rs, :]
            p_v[n, rs, :] = (z1_v[n, rs, :].astype(F32) * g).astype(BF16)
        assert nxt == len(items)
        return carry

    jax.lax.fori_loop(0, NC, p2, 0)

    wout_cp.wait()

    TPI = NT // P3I

    def p3(j, carry):
        inv_p = _up(tab_v[256:288, :])
        inv_m = _up(tab_v[288:320, :])
        rev = 7 - jax.lax.broadcasted_iota(jnp.int32, (8, 128), 0)

        def rows(t):
            r0 = (j * TPI + t) * T
            return (pl.ds(pl.multiple_of(r0, T), T),
                    pl.ds(pl.multiple_of(r0 // 2, T // 2), T // 2))

        def g5(t):
            rs, hs = rows(t)
            g = _dot(_up(wsp_v[hs, :]), _up(z232[NF - 1])) + bcol_v[rs, :]
            return (z1_v[NF - 1, rs, :].astype(F32) * g).astype(BF16)

        p5 = g5(0)
        for t in range(TPI):
            rs, hs = rows(t)
            p = jnp.concatenate([_up(p32[n, hs, :]) for n in range(NF - 1)] + [p5], axis=1)
            if t + 1 < TPI:
                p5 = g5(t + 1)
            for c in range(NC):
                cs = slice(c * 128, (c + 1) * 128)
                ye = _dot(inv_p, _up(zz32[c, j * TPI + t, 0:64, :]))
                yo = _dot(inv_m, _up(zz32[c, j * TPI + t, 64:128, :]))
                yd = ye - yo
                y = jnp.concatenate(
                    [ye + yo] + [
                        jnp.take_along_axis(yd[i * 8:(i + 1) * 8], rev, axis=0,
                                            mode="promise_in_bounds")
                        for i in reversed(range(BLK // 16))], axis=0)
                o = _dot(p, _up(wout_v[:, cs]))
                gate = o * (1.0 + jnp.tanh(0.25 * o))
                x = _up(x_v[0, hs, cs]).astype(F32)
                xn = xn_v[c, rs, :].astype(F32)
                o_v[rs, cs] = (x + (xn * y) * gate).astype(BF16)
            cp(o_v.at[rs, :], out_hbm.at[0, rs, :], sem.at[14]).start()
        return carry

    jax.lax.fori_loop(0, P3I, p3, 0)
    cp(o_v, out_hbm.at[0], sem.at[14]).wait()


@jax.jit
def pallas_recurrent_scan__ssm_conv_h3__mixer_gmlp__prompt_kernel(
    A_q: jax.Array,
    A_k: jax.Array,
    A_v: jax.Array,
    A_shift_k: jax.Array,
    A_ssm_k: jax.Array,
    A_ssm_D: jax.Array,
    B_x: jax.Array,
    B_w_in: jax.Array,
    B_w_sp: jax.Array,
    B_b_sp: jax.Array,
    B_w_out: jax.Array,
):
    del B_x
    tab = jnp.asarray(_dft_tables(), dtype=BF16)

    any_spec = pl.BlockSpec(memory_space=pl.ANY)
    return pl.pallas_call(
        _kernel,
        out_shape=jax.ShapeDtypeStruct((1, S, D), BF16),
        in_specs=[any_spec] * 11,
        out_specs=any_spec,
        scratch_shapes=[
            pltpu.VMEM((1, S // 2 + 32, D), U32),
            pltpu.VMEM((1, D // 2 + 8, 2 * FH), U32),
            pltpu.VMEM((S // 2, S), U32),
            pltpu.VMEM((FH // 2, D), U32),
            pltpu.VMEM((2 * NC, S // 2 + 32, 128), U32),
            pltpu.VMEM((NC, 64, S), U32),
            pltpu.VMEM((NC, S, 128), BF16),
            pltpu.VMEM((NF, S, 128), BF16),
            pltpu.VMEM((NF, S, 128), BF16),
            pltpu.VMEM((NF - 1, S, 128), BF16),
            pltpu.VMEM((S, 128), BF16),
            pltpu.VMEM((BLK // 8, 6 * NB + 1, 8, 128), F32),
            pltpu.VMEM((NC, NB, 2 * BLK, 128), BF16),
            pltpu.VMEM((S, 128), F32),
            pltpu.VMEM((S, D), BF16),
            pltpu.VMEM((1, T + 16, FH), F32),
            pltpu.VMEM((1, T + 16, FH), F32),
            pltpu.VMEM((320, 128), U32),
            pltpu.VMEM((NC, KS, 128), F32),
            pltpu.VMEM((NC + 2, 1, 128), F32),
            pltpu.VMEM((KS, D), BF16),
            pltpu.VMEM((D,), BF16),
            pltpu.VMEM((S,), BF16),
            pltpu.SMEM((1,), jnp.int32),
            pltpu.SemaphoreType.DMA((15,)),
        ],
        compiler_params=pltpu.CompilerParams(
            vmem_limit_bytes=100 * 1024 * 1024, disable_bounds_checks=True),
    )(A_q, A_k, A_v, A_shift_k.T, A_ssm_k, A_ssm_D, B_w_in, B_w_sp, B_b_sp, B_w_out, tab)
```

```python
import os

import jax
import jax.numpy as jnp
import numpy as np
import jax.experimental.pallas as pl
import jax.experimental.pallas.tpu as pltpu

F32 = jnp.float32
BF16 = jnp.bfloat16
U32 = jnp.uint32

S = 2048
D = 640
FH = 768
KS = 4
BLK = 128
NB = S // BLK
NC = D // 128
NF = FH // 128
T = 128
NT = S // T
EPS = 1e-5
GRP = int(os.environ.get('GRP', 4))
KG = 512
UA, UB, US, HP, HQ, HR, TOK = (i * NB for i in range(7))
TB = int(os.environ.get('TB', 4))
P3I = int(os.environ.get('P3I', 2))
LAG = int(os.environ.get('LAG', 4))
TAP1 = int(os.environ.get('TAP1', 1016))

_GELU_C0 = float(np.sqrt(2.0 / np.pi))
_GELU_C1 = _GELU_C0 * 0.044715
_A = _GELU_C1 ** (1.0 / 3.0)
_K = _GELU_C0 / _A


def _dft_tables():
    m = np.arange(BLK)[:, None]
    n = np.arange(BLK)[None, :]
    th = 2.0 * np.pi * (((4 * m + 1) * n) % (4 * BLK)) / (4 * BLK)
    ph = 2.0 * np.pi * (((4 * m + 1) * (2 * n + 1)) % (8 * BLK)) / (8 * BLK)
    fu = np.concatenate([np.cos(ph), -np.sin(ph)], axis=0)
    fh = np.concatenate([np.cos(th) + np.sin(th), np.cos(th) - np.sin(th)], axis=0)
    fu, fh = (f.reshape(2, BLK // 8, 8, BLK).transpose(1, 0, 2, 3).reshape(2 * BLK, BLK)
              for f in (fu, fh))
    cp = (np.cos(ph) + np.sin(ph)).T[:BLK // 2] / (8.0 * BLK * _A * _A)
    cm = (np.cos(ph) - np.sin(ph)).T[:BLK // 2] / (8.0 * BLK * _A * _A)
    return np.concatenate([fu, fh, cp, cm], axis=0).astype(np.float32)


def _layernorm(x, eps, scale=1.0):
    m = jnp.mean(x, axis=-1, keepdims=True)
    d = x - m
    v = jnp.sum(d * d, axis=-1, keepdims=True) * (1.0 / (x.shape[-1] * scale * scale))
    return d * jax.lax.rsqrt(v + eps / (scale * scale))


def _gelu2(y):
    return y * (1.0 + jnp.tanh(y * (y * y + _K)))


def _pk(x):
    return pltpu.bitcast(x, U32)


def _up(x):
    return pltpu.bitcast(x, BF16)


def _dot(a, b):
    return jnp.dot(a, b, preferred_element_type=F32)


def _spread(items, taps):
    total = sum(c for c, _, _ in items)
    cum = 0
    for c, gate, run in items:
        gate(taps[int(cum * len(taps) / total)]())
        run()
        cum += c


def _kernel(x_hbm, k_hbm, v_hbm, skt_hbm, h_hbm, dv_hbm, win_hbm, wsp_hbm, b_hbm,
            wout_hbm, tab_hbm, out_hbm,
            x_v, win_v, wsp_v, wout_v, kv_v, h_v, xn_v, z1_v, z2_v, p_v,
            kvb_v, pl_v, zz_v, bcol_v, o_v, zta_v, ztb_v, raw_v, tab_v,
            sk_v, dd_v, skt_v, dv_v, b_v, zero_s, sem):
    cp = pltpu.make_async_copy
    x16 = x_v.bitcast(BF16)
    win16 = win_v.bitcast(BF16)
    kv16 = kv_v.bitcast(BF16)
    h16 = h_v.bitcast(BF16)

    xn32, z232, p32, kvb32, zz32 = (
        r.bitcast(U32) for r in (xn_v, z2_v, p_v, kvb_v, zz_v))

    def x_cp(lo, hi, s):
        return cp(x_hbm.at[0, lo:hi, :], x16.at[0, lo:hi, :], sem.at[s])

    def win_cp(lo, hi, s):
        return cp(win_hbm.at[:, lo:hi], win16.at[0, 0:D, lo:hi], sem.at[s])

    def k_cp(c, s):
        return cp(k_hbm.at[0, :, pl.ds(c * 128, 128)], kv16.at[2 * c, 0:S, :], sem.at[s])

    def v_cp(c, s):
        return cp(v_hbm.at[0, :, pl.ds(c * 128, 128)], kv16.at[2 * c + 1, 0:S, :], sem.at[s])

    def h_cp(c, s):
        return cp(h_hbm.at[pl.ds(c * 128, 128), :], h16.at[c], sem.at[s])

    groups = [
        [cp(b_hbm, b_v, sem.at[0]), cp(skt_hbm, skt_v, sem.at[0]), cp(dv_hbm, dv_v, sem.at[0])],
        [x_cp(0, 256, 1)],
        [win_cp(FH, FH + 256, 2)],
        [win_cp(FH + 256, 2 * FH, 3)],
        [win_cp(0, 512, 4)],
        [win_cp(512, FH, 5), x_cp(256, 384, 5)],
        [x_cp(384, (TB + 2) * T, 6)],
        [x_cp((TB + 2) * T, S, 7), k_cp(0, 7), v_cp(0, 7)],
        [cp(tab_hbm, tab_v.bitcast(BF16), sem.at[8]), h_cp(0, 8),
         cp(wsp_hbm, wsp_v.bitcast(BF16), sem.at[8])],
    ]
    for g in groups:
        for c in g:
            c.start()

    def tile_cps(c):
        return [k_cp(c, 8 + c), v_cp(c, 8 + c), h_cp(c, 8 + c)]

    for c in range(1, NC):
        for d in tile_cps(c):
            d.start()
    wout_cp = cp(wout_hbm, wout_v.bitcast(BF16), sem.at[13])
    wout_cp.start()

    def wait(i):
        for c in groups[i]:
            c.wait()

    zero_s[0] = 0
    wait(0)
    skt = skt_v[...].astype(F32)
    dv = dv_v[...].astype(F32).reshape(1, D)
    for c in range(NC):
        sk_v[c] = skt[:, c * 128:(c + 1) * 128]
        dd_v[c] = dv[:, c * 128:(c + 1) * 128]
    brow = b_v[...].astype(F32).reshape(1, S)
    bcol_v[...] = jnp.broadcast_to(brow, (128, S)).T

    def gate_x(tok):
        x_v[0, S // 2:S // 2 + 8, 0:128] = pltpu.bitcast(tok, U32)

    zt_v = (zta_v, ztb_v)

    def gate_zt(t):
        def gate(tok):
            zt_v[t % 2][0, T:T + 8, 0:128] = tok
        return gate

    def gate_kv(tok):
        kv_v[0, S // 2:S // 2 + 8, :] = pltpu.bitcast(tok, U32)

    def gate_pl(tok):
        pl_v[0, TOK] = tok

    ndone = [0]

    def done(val):
        c = (ndone[0] % (2 * NF)) * 128
        ndone[0] += 1
        win_v[0, D // 2:D // 2 + 8, c:c + 128] = val

    def lnx_items(t, zero, mark=True):
        def item(r0):
            def run():
                xw = x_v[zero, r0 // 2:r0 // 2 + 8, :]
                xn = _layernorm(_up(xw).astype(F32), EPS, _A)
                for c in range(NC):
                    xn_v[c, r0:r0 + 16, :] = xn[:, c * 128:(c + 1) * 128].astype(BF16)
                if mark:
                    done(pltpu.bitcast(xn[0:8, 0:128], U32))
                    done(pltpu.bitcast(xn[8:16, 0:128], U32))
            return (1, gate_x, run)
        return [item(t * T + g * 16) for g in range(T // 16)]

    def lnz_items(t, zero):
        def item(g):
            def run():
                z = zt_v[t % 2][zero, g * 16:(g + 1) * 16, :]
                z = _layernorm(z, 4.0 * _A * _A * EPS)
                done(pltpu.bitcast(z[0:8, 0:128], U32))
                done(pltpu.bitcast(z[8:16, 0:128], U32))
                r0 = t * T + g * 16
                for n in range(NF):
                    z2_v[n, r0:r0 + 16, :] = z[:, n * 128:(n + 1) * 128].astype(BF16)
            return (1, gate_zt(t), run)
        return [item(g) for g in range(T // 16)]

    KR = 32

    def kv_items(c):
        sk = sk_v[c]

        def item(r0):
            def run():
                hs = slice(r0 // 2, (r0 + KR) // 2)
                if r0 == 0:
                    kw = jnp.concatenate(
                        [jnp.zeros((8, 128), F32), _up(kv_v[2 * c, hs, :]).astype(F32)], axis=0)
                else:
                    kw = _up(kv_v[2 * c, r0 // 2 - 8:(r0 + KR) // 2, :]).astype(F32)[8:]
                ks = kw[8:] * sk[0:1, :]
                for t in range(1, KS):
                    ks = ks + pltpu.roll(kw, t, 0)[8:] * sk[t:t + 1, :]
                kvb_v[r0:r0 + KR, :] = (
                    ks * _up(kv_v[2 * c + 1, hs, :]).astype(F32)).astype(BF16)
            return (14 * KR // 8, gate_kv, run)
        return [item(r0) for r0 in range(0, S, KR)]

    def taps_of(val):
        rows, cols = val.shape
        return [(lambda i=i, n=n: val[i * 8:(i + 1) * 8, n * 128:(n + 1) * 128])
                for n in range(cols // 128) for i in range(rows // 8)]

    def activate(kind, t, n, z):
        if kind == 2:
            zt_v[t % 2][0, 0:T, n * 128:(n + 1) * 128] = _gelu2(z)
        else:
            z1_v[n, t * T:(t + 1) * T, :] = _gelu2(z).astype(BF16)

    def piece(kind, t, n, zero, defer=False):
        col = n * 128 + (FH if kind == 2 else 0)
        xn = jnp.concatenate(
            [_up(xn32[c, t * T // 2:(t + 1) * T // 2, :]) for c in range(NC)], axis=1)
        z = _dot(xn, _up(win_v[0 if zero is None else zero, 0:D // 2, col:col + 128]))
        if defer:
            raw_v[...] = z
        else:
            activate(kind, t, n, z)
        return taps_of(z)

    pending = []

    def block(pieces, work, defer=True, free=None):
        zero = zero_s[0]
        if pending:
            activate(*pending.pop(), raw_v[...])
        rel = [[] for _ in pieces]
        for mk, lo, hi in work:
            items = mk(zero)
            for i, it in enumerate(items):
                tau = (lo * 16) + (i * (hi - lo) * 16) // len(items)
                rel[tau // 16].append((tau % 16, it))
        taps = []
        gated = False
        for k in range(len(pieces) + LAG):
            if free is not None and k == len(pieces) - 1:
                for _, _, run in free(zero):
                    run()
                gated = True
            if k < len(pieces):
                last = defer and k == len(pieces) - 1
                taps.append(piece(*pieces[k], zero if gated else None, last))
                if last:
                    pending.append(pieces[k])
            if k >= LAG:
                for i, (_, gate, run) in sorted(rel[k - LAG], key=lambda e: e[0]):
                    gate(taps[k - LAG][i]())
                    run()
                    gated = True

    def cols(kind, t, lo=0, hi=NF):
        return [(kind, t, n) for n in range(lo, hi)]

    def lnx(t):
        return lambda zero: lnx_items(t, zero)

    def lnz(t):
        return lambda zero: lnz_items(t, zero)

    wait(1)
    for it in lnx_items(0, 0, False) + lnx_items(1, 0, False):
        it[2]()
    wait(2)
    block(cols(2, 0, 0, 2) + cols(2, 1, 0, 2), [])
    wait(3)
    block(cols(2, 0, 2) + cols(2, 1, 2), [])
    wait(4)
    block(cols(1, 0, 0, 4) + cols(1, 1, 0, 4), [(lnz(0), 0, 3)])
    wait(5)
    block(cols(1, 0, 4) + cols(1, 1, 4), [], free=lnx(2))

    def big_block(first, last, extra):
        pieces, work = [], [(lnx(first + 1), 0, 11 - LAG)] + list(extra)
        for t in range(first, last - 1):
            k = len(pieces)
            pieces += cols(2, t) + cols(1, t)
            lo = k + (4 if t == first else 0)
            if t + 1 < last - 1:
                work += [(lnx(t + 2), lo, k + 12), (lnz(t), k + 6, k + 18)]
            else:
                work += [(lnx(t + 2), lo, k + 12), (lnz(t), k + 6, k + 17 - LAG)]
        a, b = last - 1, last
        k = len(pieces)
        pieces += cols(2, a) + cols(2, b) + cols(1, a) + cols(1, b)
        work += [(lnz(a), k + 6, k + 13), (lnz(b), k + 12, k + 23 - LAG)]
        if b + 1 < NT:
            work += [(lnx(b + 1), k, k + 8)]
        else:
            work += [(kv_items, 0, k + 24)]
        block(pieces, work, b + 1 < NT)

    wait(6)
    big_block(2, TB, [(lnz(1), 0, 11 - LAG)])
    wait(7)
    big_block(TB + 1, NT - 1, [])

    wait(8)

    def p2(n, carry):
        nn = jnp.minimum(n + 1, NC - 1)

        @pl.when(n + 1 < NC)
        def _():
            for d in tile_cps(nn):
                d.wait()

        zero = zero_s[0]
        fwd_u = _up(tab_v[0:128, :])
        fwd_h = _up(tab_v[128:256, :])
        dd = dd_v[n]

        def put(slot, val):
            pl_v[:, slot] = val

        def re_im(val):
            val = val.reshape(BLK // 8, 2, 8, 128)
            return val[:, 0], val[:, 1]

        kvi = kv_items(nn)

        def pace_kv(d, val):
            if d % 4 == 3:
                for j in range(8):
                    _, gate, run = kvi[(d // 4) * 8 + j]
                    gate(val[j * 32:j * 32 + 8, :])
                    run()

        for i in range(NB):
            u = _dot(fwd_u, _up(kvb32[i * BLK // 2:(i + 1) * BLK // 2, :]))
            a, b = re_im(u)
            put(UA + i, a)
            put(UB + i, b)
            put(US + i, a + b)
            pace_kv(i, u)
        for i in range(NB):
            hb = _up(h_v[n, :, i * BLK:(i + 1) * BLK])
            hf = jax.lax.dot_general(fwd_h, hb, (((1,), (1,)), ((), ())),
                                     preferred_element_type=F32)
            c, d = re_im(hf)
            if i == 0:
                c, d = c + dd, d + dd
            put(HR + i, c)
            put(HP + i, d - c)
            put(HQ + i, c + d)
            pace_kv(NB + i, hf)

        state = {}

        def mac_item(pos, g0, pi):
            xv, hv = ((US, HR), (UA, HP), (UB, HQ))[pi]
            outs = range(g0, g0 + GRP)
            top = g0 + GRP

            def run():
                pz = zero + pos
                hs = [pl_v[pz, hv + t] for t in range(top)]
                acc = {o: None for o in outs}
                for jj in range(top):
                    xj = pl_v[pz, xv + jj]
                    for o in outs:
                        if o - jj >= 0:
                            t = xj * hs[o - jj]
                            acc[o] = t if acc[o] is None else acc[o] + t
                r0 = pos * 8
                if pi == 0:
                    state['k1'] = acc
                elif pi == 1:
                    state['im'] = {o: state['k1'][o] + acc[o] for o in outs}
                else:
                    for o in outs:
                        re, im = state['k1'][o] - acc[o], state['im'][o]
                        zr, zi = re, im
                        if o > 0:
                            zr, zi = re - state['prev'][1], im + state['prev'][0]
                        state['prev'] = (re, im)
                        zz_v[n, o, r0:r0 + 8, :] = zr.astype(BF16)
                        zz_v[n, o, BLK + r0:BLK + r0 + 8, :] = zi.astype(BF16)

            nmac = sum(o + 1 for o in outs)
            return (2 * nmac - GRP + (0, GRP, 5 * GRP)[pi], gate_pl, run)

        items = []
        for pos in range(BLK // 8):
            for g0 in range(0, NB, GRP):
                for pi in range(3):
                    items.append(mac_item(pos, g0, pi))

        nq = S // KG
        vpc = T // 8
        total = sum(c for c, _, _ in items)
        tap_of = []
        cum = 0
        for c, _, _ in items:
            tap_of.append(int(cum * TAP1 / total))
            cum += c
        nxt = 0
        for r in range(NT):
            rs = slice(r * T, (r + 1) * T)
            hs = slice(r * T // 2, (r + 1) * T // 2)
            acc = None
            for q in range(nq):
                part = _dot(_up(wsp_v[hs, q * KG:(q + 1) * KG]),
                            _up(z232[n, q * KG // 2:(q + 1) * KG // 2, :]))
                acc = part if acc is None else acc + part
                t0 = (r * nq + q) * vpc
                while nxt < len(items) and tap_of[nxt] < t0 + vpc:
                    i = tap_of[nxt] - t0
                    items[nxt][1](acc[i * 8:(i + 1) * 8, :])
                    items[nxt][2]()
                    nxt += 1
            g = acc + bcol_v[rs, :]
            p_v[n, rs, :] = (z1_v[n, rs, :].astype(F32) * g).astype(BF16)
        assert nxt == len(items)
        return carry

    jax.lax.fori_loop(0, NC, p2, 0)

    wout_cp.wait()

    TPI = NT // P3I

    def p3(j, carry):
        inv_p = _up(tab_v[256:288, :])
        inv_m = _up(tab_v[288:320, :])
        rev = 7 - jax.lax.broadcasted_iota(jnp.int32, (8, 128), 0)

        def rows(t):
            r0 = (j * TPI + t) * T
            return (pl.ds(pl.multiple_of(r0, T), T),
                    pl.ds(pl.multiple_of(r0 // 2, T // 2), T // 2))

        def g5(t):
            rs, hs = rows(t)
            g = _dot(_up(wsp_v[hs, :]), _up(z232[NF - 1])) + bcol_v[rs, :]
            return (z1_v[NF - 1, rs, :].astype(F32) * g).astype(BF16)

        p5 = g5(0)
        for t in range(TPI):
            rs, hs = rows(t)
            p = jnp.concatenate([_up(p32[n, hs, :]) for n in range(NF - 1)] + [p5], axis=1)
            if t + 1 < TPI:
                p5 = g5(t + 1)
            for c in range(NC):
                cs = slice(c * 128, (c + 1) * 128)
                ye = _dot(inv_p, _up(zz32[c, j * TPI + t, 0:64, :]))
                yo = _dot(inv_m, _up(zz32[c, j * TPI + t, 64:128, :]))
                yd = ye - yo
                y = jnp.concatenate(
                    [ye + yo] + [
                        jnp.take_along_axis(yd[i * 8:(i + 1) * 8], rev, axis=0,
                                            mode="promise_in_bounds")
                        for i in reversed(range(BLK // 16))], axis=0)
                o = _dot(p, _up(wout_v[:, cs]))
                gate = o * (1.0 + jnp.tanh((0.25 / _A) * o))
                x = _up(x_v[0, hs, cs]).astype(F32)
                xn = xn_v[c, rs, :].astype(F32)
                o_v[rs, cs] = (x + (xn * y) * gate).astype(BF16)
                if t == TPI - 1 and c == NC - 2:
                    cp(o_v.at[rs, 0:512], out_hbm.at[0, rs, 0:512], sem.at[14]).start()
            if t == TPI - 1:
                cp(o_v.at[rs, 512:D], out_hbm.at[0, rs, 512:D], sem.at[14]).start()
            else:
                cp(o_v.at[rs, :], out_hbm.at[0, rs, :], sem.at[14]).start()
        return carry

    jax.lax.fori_loop(0, P3I, p3, 0)
    cp(o_v, out_hbm.at[0], sem.at[14]).wait()


@jax.jit
def pallas_recurrent_scan__ssm_conv_h3__mixer_gmlp__prompt_kernel(
    A_q: jax.Array,
    A_k: jax.Array,
    A_v: jax.Array,
    A_shift_k: jax.Array,
    A_ssm_k: jax.Array,
    A_ssm_D: jax.Array,
    B_x: jax.Array,
    B_w_in: jax.Array,
    B_w_sp: jax.Array,
    B_b_sp: jax.Array,
    B_w_out: jax.Array,
):
    del B_x
    tab = jnp.asarray(_dft_tables(), dtype=BF16)

    any_spec = pl.BlockSpec(memory_space=pl.ANY)
    return pl.pallas_call(
        _kernel,
        out_shape=jax.ShapeDtypeStruct((1, S, D), BF16),
        in_specs=[any_spec] * 11,
        out_specs=any_spec,
        scratch_shapes=[
            pltpu.VMEM((1, S // 2 + 32, D), U32),
            pltpu.VMEM((1, D // 2 + 8, 2 * FH), U32),
            pltpu.VMEM((S // 2, S), U32),
            pltpu.VMEM((FH // 2, D), U32),
            pltpu.VMEM((2 * NC, S // 2 + 32, 128), U32),
            pltpu.VMEM((NC, 64, S), U32),
            pltpu.VMEM((NC, S, 128), BF16),
            pltpu.VMEM((NF, S, 128), BF16),
            pltpu.VMEM((NF, S, 128), BF16),
            pltpu.VMEM((NF - 1, S, 128), BF16),
            pltpu.VMEM((S, 128), BF16),
            pltpu.VMEM((BLK // 8, 6 * NB + 1, 8, 128), F32),
            pltpu.VMEM((NC, NB, 2 * BLK, 128), BF16),
            pltpu.VMEM((S, 128), F32),
            pltpu.VMEM((S, D), BF16),
            pltpu.VMEM((1, T + 16, FH), F32),
            pltpu.VMEM((1, T + 16, FH), F32),
            pltpu.VMEM((T, 128), F32),
            pltpu.VMEM((320, 128), U32),
            pltpu.VMEM((NC, KS, 128), F32),
            pltpu.VMEM((NC + 2, 1, 128), F32),
            pltpu.VMEM((KS, D), BF16),
            pltpu.VMEM((D,), BF16),
            pltpu.VMEM((S,), BF16),
            pltpu.SMEM((1,), jnp.int32),
            pltpu.SemaphoreType.DMA((15,)),
        ],
        compiler_params=pltpu.CompilerParams(
            vmem_limit_bytes=100 * 1024 * 1024, disable_bounds_checks=True),
    )(A_q, A_k, A_v, A_shift_k.T, A_ssm_k, A_ssm_D, B_w_in, B_w_sp, B_b_sp, B_w_out, tab)
```

```python
import os

import jax
import jax.numpy as jnp
import numpy as np
import jax.experimental.pallas as pl
import jax.experimental.pallas.tpu as pltpu

F32 = jnp.float32
BF16 = jnp.bfloat16
U32 = jnp.uint32

S = 2048
D = 640
FH = 768
KS = 4
BLK = 128
NB = S // BLK
NC = D // 128
NF = FH // 128
T = 128
NT = S // T
EPS = 1e-5
GRP = int(os.environ.get('GRP', 4))
KG = 512
UA, UB, US, HP, HQ, HR, TOK = (i * NB for i in range(7))
TB = int(os.environ.get('TB', 4))
P3I = int(os.environ.get('P3I', 2))
LAG = int(os.environ.get('LAG', 4))
GC = int(os.environ.get('GC', 0))
TAP1 = int(os.environ.get('TAP1', 1016))

_GELU_C0 = float(np.sqrt(2.0 / np.pi))
_GELU_C1 = _GELU_C0 * 0.044715
_A = _GELU_C1 ** (1.0 / 3.0)
_K = _GELU_C0 / _A


def _dft_tables():
    m = np.arange(BLK)[:, None]
    n = np.arange(BLK)[None, :]
    th = 2.0 * np.pi * (((4 * m + 1) * n) % (4 * BLK)) / (4 * BLK)
    ph = 2.0 * np.pi * (((4 * m + 1) * (2 * n + 1)) % (8 * BLK)) / (8 * BLK)
    fu = np.concatenate([np.cos(ph), -np.sin(ph)], axis=0)
    fh = np.concatenate([np.cos(th) + np.sin(th), np.cos(th) - np.sin(th)], axis=0)
    fu, fh = (f.reshape(2, BLK // 8, 8, BLK).transpose(1, 0, 2, 3).reshape(2 * BLK, BLK)
              for f in (fu, fh))
    cp = (np.cos(ph) + np.sin(ph)).T[:BLK // 2] / (8.0 * BLK * _A * _A)
    cm = (np.cos(ph) - np.sin(ph)).T[:BLK // 2] / (8.0 * BLK * _A * _A)
    return np.concatenate([fu, fh, cp, cm], axis=0).astype(np.float32)


def _layernorm(x, eps, scale=1.0):
    m = jnp.mean(x, axis=-1, keepdims=True)
    d = x - m
    v = jnp.sum(d * d, axis=-1, keepdims=True) * (1.0 / (x.shape[-1] * scale * scale))
    return d * jax.lax.rsqrt(v + eps / (scale * scale))


def _gelu2(y):
    return y * (1.0 + jnp.tanh(y * (y * y + _K)))


def _pk(x):
    return pltpu.bitcast(x, U32)


def _up(x):
    return pltpu.bitcast(x, BF16)


def _dot(a, b):
    return jnp.dot(a, b, preferred_element_type=F32)


def _spread(items, taps):
    total = sum(c for c, _, _ in items)
    cum = 0
    for c, gate, run in items:
        gate(taps[int(cum * len(taps) / total)]())
        run()
        cum += c


def _kernel(x_hbm, k_hbm, v_hbm, skt_hbm, h_hbm, dv_hbm, win_hbm, wsp_hbm, b_hbm,
            wout_hbm, tab_hbm, out_hbm,
            x_v, win_v, wsp_v, wout_v, kv_v, h_v, xn_v, z1_v, z2_v, p_v,
            kvb_v, pl_v, zz_v, bcol_v, o_v, zta_v, ztb_v, raw_v, tab_v,
            sk_v, dd_v, skt_v, dv_v, b_v, zero_s, sem):
    cp = pltpu.make_async_copy
    x16 = x_v.bitcast(BF16)
    win16 = win_v.bitcast(BF16)
    kv16 = kv_v.bitcast(BF16)
    h16 = h_v.bitcast(BF16)

    xn32, z232, p32, kvb32, zz32 = (
        r.bitcast(U32) for r in (xn_v, z2_v, p_v, kvb_v, zz_v))

    def x_cp(lo, hi, s):
        return cp(x_hbm.at[0, lo:hi, :], x16.at[0, lo:hi, :], sem.at[s])

    def win_cp(lo, hi, s):
        return cp(win_hbm.at[:, lo:hi], win16.at[:, lo:hi], sem.at[s])

    def k_cp(c, s):
        return cp(k_hbm.at[0, :, pl.ds(c * 128, 128)], kv16.at[2 * c, 0:S, :], sem.at[s])

    def v_cp(c, s):
        return cp(v_hbm.at[0, :, pl.ds(c * 128, 128)], kv16.at[2 * c + 1, 0:S, :], sem.at[s])

    def h_cp(c, s):
        return cp(h_hbm.at[pl.ds(c * 128, 128), :], h16.at[c], sem.at[s])

    groups = [
        [cp(b_hbm, b_v, sem.at[0]), cp(skt_hbm, skt_v, sem.at[0]), cp(dv_hbm, dv_v, sem.at[0])],
        [x_cp(0, 256, 1)],
        [win_cp(FH, FH + 256, 2)],
        [win_cp(FH + 256, 2 * FH, 3)],
        [win_cp(0, 512, 4)],
        [win_cp(512, FH, 5), x_cp(256, 384, 5)],
        [x_cp(384, (TB + 2) * T, 6)],
        [x_cp((TB + 2) * T, S, 7), k_cp(0, 7), v_cp(0, 7)],
        [cp(tab_hbm, tab_v.bitcast(BF16), sem.at[8]), h_cp(0, 8),
         cp(wsp_hbm, wsp_v.bitcast(BF16), sem.at[8])],
    ]
    for g in groups:
        for c in g:
            c.start()

    def tile_cps(c):
        return [k_cp(c, 8 + c), v_cp(c, 8 + c), h_cp(c, 8 + c)]

    for c in range(1, NC):
        for d in tile_cps(c):
            d.start()
    wout_cp = cp(wout_hbm, wout_v.bitcast(BF16), sem.at[13])
    wout_cp.start()

    def wait(i):
        for c in groups[i]:
            c.wait()

    zero_s[0] = 0
    wait(0)
    skt = skt_v[...].astype(F32)
    dv = dv_v[...].astype(F32).reshape(1, D)
    for c in range(NC):
        sk_v[c] = skt[:, c * 128:(c + 1) * 128]
        dd_v[c] = dv[:, c * 128:(c + 1) * 128]
    brow = b_v[...].astype(F32).reshape(1, S)
    bcol_v[...] = jnp.broadcast_to(brow, (128, S)).T

    def gate_x(tok):
        x_v[0, S // 2:S // 2 + 8, 0:128] = pltpu.bitcast(tok, U32)

    zt_v = (zta_v, ztb_v)

    def gate_zt(t):
        def gate(tok):
            zt_v[t % 2][0, T:T + 8, 0:128] = tok
        return gate

    def gate_kv(tok):
        kv_v[0, S // 2:S // 2 + 8, :] = pltpu.bitcast(tok, U32)

    def gate_pl(tok):
        pl_v[0, TOK] = tok

    ndone = [0]

    def done(val):
        r = S + (ndone[0] % 16) * 16
        ndone[0] += 1
        xn_v[0, r:r + 16, :] = val

    def lnx_items(t, zero):
        def item(r0):
            def run():
                xw = x_v[zero, r0 // 2:r0 // 2 + 8, :]
                xn = _layernorm(_up(xw).astype(F32), EPS, _A)
                for c in range(NC):
                    xn_v[c, r0:r0 + 16, :] = xn[:, c * 128:(c + 1) * 128].astype(BF16)
            return (1, gate_x, run)
        return [item(t * T + g * 16) for g in range(T // 16)]

    def lnz_items(t, zero):
        def item(g):
            def run():
                z = zt_v[t % 2][zero, g * 16:(g + 1) * 16, :]
                z = _layernorm(z, 4.0 * _A * _A * EPS)
                r0 = t * T + g * 16
                for n in range(NF):
                    zb = z[:, n * 128:(n + 1) * 128].astype(BF16)
                    z2_v[n, r0:r0 + 16, :] = zb
                    if n == 0:
                        done(zb)
            return (1, gate_zt(t), run)
        return [item(g) for g in range(T // 16)]

    KR = 32

    def kv_items(c):
        sk = sk_v[c]

        def item(r0):
            def run():
                hs = slice(r0 // 2, (r0 + KR) // 2)
                if r0 == 0:
                    kw = jnp.concatenate(
                        [jnp.zeros((8, 128), F32), _up(kv_v[2 * c, hs, :]).astype(F32)], axis=0)
                else:
                    kw = _up(kv_v[2 * c, r0 // 2 - 8:(r0 + KR) // 2, :]).astype(F32)[8:]
                ks = kw[8:] * sk[0:1, :]
                for t in range(1, KS):
                    ks = ks + pltpu.roll(kw, t, 0)[8:] * sk[t:t + 1, :]
                kvb_v[r0:r0 + KR, :] = (
                    ks * _up(kv_v[2 * c + 1, hs, :]).astype(F32)).astype(BF16)
            return (14 * KR // 8, gate_kv, run)
        return [item(r0) for r0 in range(0, S, KR)]

    def taps_of(val):
        rows, cols = val.shape
        return [(lambda i=i, n=n: val[i * 8:(i + 1) * 8, n * 128:(n + 1) * 128])
                for n in range(cols // 128) for i in range(rows // 8)]

    def activate(kind, t, n, z):
        if kind == 2:
            zt_v[t % 2][0, 0:T, n * 128:(n + 1) * 128] = _gelu2(z)
        else:
            z1_v[n, t * T:(t + 1) * T, :] = _gelu2(z).astype(BF16)

    def piece(kind, t, n, zero, defer=False):
        col = n * 128 + (FH if kind == 2 else 0)
        xn = jnp.concatenate(
            [_up(xn32[c + zero if zero is not None and c == GC else c,
                      t * T // 2:(t + 1) * T // 2, :]) for c in range(NC)], axis=1)
        z = _dot(xn, _up(win_v[:, col:col + 128]))
        if defer:
            raw_v[...] = z
        else:
            activate(kind, t, n, z)
        return taps_of(z)

    pending = []

    def block(pieces, work, defer=True, free=None):
        zero = zero_s[0]
        if pending:
            activate(*pending.pop(), raw_v[...])
        rel = [[] for _ in pieces]
        for mk, lo, hi in work:
            items = mk(zero)
            for i, it in enumerate(items):
                tau = (lo * 16) + (i * (hi - lo) * 16) // len(items)
                rel[tau // 16].append((tau % 16, it))
        taps = []
        gated = False
        for k in range(len(pieces) + LAG):
            if free is not None and k == len(pieces) - 1:
                for _, _, run in free(zero):
                    run()
                gated = True
            if k < len(pieces):
                last = defer and k == len(pieces) - 1
                taps.append(piece(*pieces[k], zero if gated else None, last))
                if last:
                    pending.append(pieces[k])
            if k >= LAG:
                for i, (_, gate, run) in sorted(rel[k - LAG], key=lambda e: e[0]):
                    gate(taps[k - LAG][i]())
                    run()
                    gated = True

    def cols(kind, t, lo=0, hi=NF):
        return [(kind, t, n) for n in range(lo, hi)]

    def lnx(t):
        return lambda zero: lnx_items(t, zero)

    def lnz(t):
        return lambda zero: lnz_items(t, zero)

    wait(1)
    for it in lnx_items(0, 0) + lnx_items(1, 0):
        it[2]()
    wait(2)
    block(cols(2, 0, 0, 2) + cols(2, 1, 0, 2), [])
    wait(3)
    block(cols(2, 0, 2) + cols(2, 1, 2), [])
    wait(4)
    block(cols(1, 0, 0, 4) + cols(1, 1, 0, 4), [(lnz(0), 0, 3)])
    wait(5)
    block(cols(1, 0, 4) + cols(1, 1, 4), [], free=lnx(2))

    def big_block(first, last, extra):
        pieces, work = [], [(lnx(first + 1), 0, 11 - LAG)] + list(extra)
        for t in range(first, last - 1):
            k = len(pieces)
            pieces += cols(2, t) + cols(1, t)
            lo = k + (4 if t == first else 0)
            if t + 1 < last - 1:
                work += [(lnx(t + 2), lo, k + 12), (lnz(t), k + 6, k + 18)]
            else:
                work += [(lnx(t + 2), lo, k + 12), (lnz(t), k + 6, k + 17 - LAG)]
        a, b = last - 1, last
        k = len(pieces)
        pieces += cols(2, a) + cols(2, b) + cols(1, a) + cols(1, b)
        work += [(lnz(a), k + 6, k + 13), (lnz(b), k + 12, k + 23 - LAG)]
        if b + 1 < NT:
            work += [(lnx(b + 1), k, k + 8)]
        else:
            work += [(kv_items, 0, k + 24)]
        block(pieces, work, b + 1 < NT)

    wait(6)
    big_block(2, TB, [(lnz(1), 0, 11 - LAG)])
    wait(7)
    big_block(TB + 1, NT - 1, [])

    wait(8)

    def p2(n, carry):
        nn = jnp.minimum(n + 1, NC - 1)

        @pl.when(n + 1 < NC)
        def _():
            for d in tile_cps(nn):
                d.wait()

        zero = zero_s[0]
        fwd_u = _up(tab_v[0:128, :])
        fwd_h = _up(tab_v[128:256, :])
        dd = dd_v[n]

        def put(slot, val):
            pl_v[:, slot] = val

        def re_im(val):
            val = val.reshape(BLK // 8, 2, 8, 128)
            return val[:, 0], val[:, 1]

        kvi = kv_items(nn)

        def pace_kv(d, val):
            if d % 4 == 3:
                for j in range(8):
                    _, gate, run = kvi[(d // 4) * 8 + j]
                    gate(val[j * 32:j * 32 + 8, :])
                    run()

        for i in range(NB):
            u = _dot(fwd_u, _up(kvb32[i * BLK // 2:(i + 1) * BLK // 2, :]))
            a, b = re_im(u)
            put(UA + i, a)
            put(UB + i, b)
            put(US + i, a + b)
            pace_kv(i, u)
        for i in range(NB):
            hb = _up(h_v[n, :, i * BLK:(i + 1) * BLK])
            hf = jax.lax.dot_general(fwd_h, hb, (((1,), (1,)), ((), ())),
                                     preferred_element_type=F32)
            c, d = re_im(hf)
            if i == 0:
                c, d = c + dd, d + dd
            put(HR + i, c)
            put(HP + i, d - c)
            put(HQ + i, c + d)
            pace_kv(NB + i, hf)

        state = {}

        def mac_item(pos, g0, pi):
            xv, hv = ((US, HR), (UA, HP), (UB, HQ))[pi]
            outs = range(g0, g0 + GRP)
            top = g0 + GRP

            def run():
                pz = zero + pos
                hs = [pl_v[pz, hv + t] for t in range(top)]
                acc = {o: None for o in outs}
                for jj in range(top):
                    xj = pl_v[pz, xv + jj]
                    for o in outs:
                        if o - jj >= 0:
                            t = xj * hs[o - jj]
                            acc[o] = t if acc[o] is None else acc[o] + t
                r0 = pos * 8
                if pi == 0:
                    state['k1'] = acc
                elif pi == 1:
                    state['im'] = {o: state['k1'][o] + acc[o] for o in outs}
                else:
                    for o in outs:
                        re, im = state['k1'][o] - acc[o], state['im'][o]
                        zr, zi = re, im
                        if o > 0:
                            zr, zi = re - state['prev'][1], im + state['prev'][0]
                        state['prev'] = (re, im)
                        zz_v[n, o, r0:r0 + 8, :] = zr.astype(BF16)
                        zz_v[n, o, BLK + r0:BLK + r0 + 8, :] = zi.astype(BF16)

            nmac = sum(o + 1 for o in outs)
            return (2 * nmac - GRP + (0, GRP, 5 * GRP)[pi], gate_pl, run)

        items = []
        for pos in range(BLK // 8):
            for g0 in range(0, NB, GRP):
                for pi in range(3):
                    items.append(mac_item(pos, g0, pi))

        nq = S // KG
        vpc = T // 8
        total = sum(c for c, _, _ in items)
        tap_of = []
        cum = 0
        for c, _, _ in items:
            tap_of.append(int(cum * TAP1 / total))
            cum += c
        nxt = 0
        for r in range(NT):
            rs = slice(r * T, (r + 1) * T)
            hs = slice(r * T // 2, (r + 1) * T // 2)
            acc = None
            for q in range(nq):
                part = _dot(_up(wsp_v[hs, q * KG:(q + 1) * KG]),
                            _up(z232[n, q * KG // 2:(q + 1) * KG // 2, :]))
                acc = part if acc is None else acc + part
                t0 = (r * nq + q) * vpc
                while nxt < len(items) and tap_of[nxt] < t0 + vpc:
                    i = tap_of[nxt] - t0
                    items[nxt][1](acc[i * 8:(i + 1) * 8, :])
                    items[nxt][2]()
                    nxt += 1
            g = acc + bcol_v[rs, :]
            p_v[n, rs, :] = (z1_v[n, rs, :].astype(F32) * g).astype(BF16)
        assert nxt == len(items)
        return carry

    jax.lax.fori_loop(0, NC, p2, 0)

    wout_cp.wait()

    TPI = NT // P3I

    def p3(j, carry):
        inv_p = _up(tab_v[256:288, :])
        inv_m = _up(tab_v[288:320, :])
        rev = 7 - jax.lax.broadcasted_iota(jnp.int32, (8, 128), 0)

        def rows(t):
            r0 = (j * TPI + t) * T
            return (pl.ds(pl.multiple_of(r0, T), T),
                    pl.ds(pl.multiple_of(r0 // 2, T // 2), T // 2))

        def g5(t):
            rs, hs = rows(t)
            g = _dot(_up(wsp_v[hs, :]), _up(z232[NF - 1])) + bcol_v[rs, :]
            return (z1_v[NF - 1, rs, :].astype(F32) * g).astype(BF16)

        p5 = g5(0)
        for t in range(TPI):
            rs, hs = rows(t)
            p = jnp.concatenate([_up(p32[n, hs, :]) for n in range(NF - 1)] + [p5], axis=1)
            if t + 1 < TPI:
                p5 = g5(t + 1)
            for c in range(NC):
                cs = slice(c * 128, (c + 1) * 128)
                ye = _dot(inv_p, _up(zz32[c, j * TPI + t, 0:64, :]))
                yo = _dot(inv_m, _up(zz32[c, j * TPI + t, 64:128, :]))
                yd = ye - yo
                y = jnp.concatenate(
                    [ye + yo] + [
                        jnp.take_along_axis(yd[i * 8:(i + 1) * 8], rev, axis=0,
                                            mode="promise_in_bounds")
                        for i in reversed(range(BLK // 16))], axis=0)
                o = _dot(p, _up(wout_v[:, cs]))
                gate = o * (1.0 + jnp.tanh((0.25 / _A) * o))
                x = _up(x_v[0, hs, cs]).astype(F32)
                xn = xn_v[c, rs, :].astype(F32)
                o_v[rs, cs] = (x + (xn * y) * gate).astype(BF16)
                if t == TPI - 1 and c == NC - 2:
                    cp(o_v.at[rs, 0:512], out_hbm.at[0, rs, 0:512], sem.at[14]).start()
            if t == TPI - 1:
                cp(o_v.at[rs, 512:D], out_hbm.at[0, rs, 512:D], sem.at[14]).start()
            else:
                cp(o_v.at[rs, :], out_hbm.at[0, rs, :], sem.at[14]).start()
        return carry

    jax.lax.fori_loop(0, P3I, p3, 0)
    cp(o_v, out_hbm.at[0], sem.at[14]).wait()


@jax.jit
def pallas_recurrent_scan__ssm_conv_h3__mixer_gmlp__prompt_kernel(
    A_q: jax.Array,
    A_k: jax.Array,
    A_v: jax.Array,
    A_shift_k: jax.Array,
    A_ssm_k: jax.Array,
    A_ssm_D: jax.Array,
    B_x: jax.Array,
    B_w_in: jax.Array,
    B_w_sp: jax.Array,
    B_b_sp: jax.Array,
    B_w_out: jax.Array,
):
    del B_x
    tab = jnp.asarray(_dft_tables(), dtype=BF16)

    any_spec = pl.BlockSpec(memory_space=pl.ANY)
    return pl.pallas_call(
        _kernel,
        out_shape=jax.ShapeDtypeStruct((1, S, D), BF16),
        in_specs=[any_spec] * 11,
        out_specs=any_spec,
        scratch_shapes=[
            pltpu.VMEM((1, S // 2 + 32, D), U32),
            pltpu.VMEM((D // 2, 2 * FH), U32),
            pltpu.VMEM((S // 2, S), U32),
            pltpu.VMEM((FH // 2, D), U32),
            pltpu.VMEM((2 * NC, S // 2 + 32, 128), U32),
            pltpu.VMEM((NC, 64, S), U32),
            pltpu.VMEM((NC, S + 256, 128), BF16),
            pltpu.VMEM((NF, S, 128), BF16),
            pltpu.VMEM((NF, S, 128), BF16),
            pltpu.VMEM((NF - 1, S, 128), BF16),
            pltpu.VMEM((S, 128), BF16),
            pltpu.VMEM((BLK // 8, 6 * NB + 1, 8, 128), F32),
            pltpu.VMEM((NC, NB, 2 * BLK, 128), BF16),
            pltpu.VMEM((S, 128), F32),
            pltpu.VMEM((S, D), BF16),
            pltpu.VMEM((1, T + 16, FH), F32),
            pltpu.VMEM((1, T + 16, FH), F32),
            pltpu.VMEM((T, 128), F32),
            pltpu.VMEM((320, 128), U32),
            pltpu.VMEM((NC, KS, 128), F32),
            pltpu.VMEM((NC + 2, 1, 128), F32),
            pltpu.VMEM((KS, D), BF16),
            pltpu.VMEM((D,), BF16),
            pltpu.VMEM((S,), BF16),
            pltpu.SMEM((1,), jnp.int32),
            pltpu.SemaphoreType.DMA((15,)),
        ],
        compiler_params=pltpu.CompilerParams(
            vmem_limit_bytes=100 * 1024 * 1024, disable_bounds_checks=True),
    )(A_q, A_k, A_v, A_shift_k.T, A_ssm_k, A_ssm_D, B_w_in, B_w_sp, B_b_sp, B_w_out, tab)
```

```python
import jax
import jax.numpy as jnp
import numpy as np
import jax.experimental.pallas as pl
import jax.experimental.pallas.tpu as pltpu

F32 = jnp.float32
BF16 = jnp.bfloat16
U32 = jnp.uint32

S = 2048
D = 640
FH = 768
KS = 4
BLK = 128
NB = S // BLK
NC = D // 128
NF = FH // 128
T = 128
NT = S // T
EPS = 1e-5
GRP = 4
KG = 512
KR = 32
UA, UB, US, HP, HQ, HR, TOK = (i * NB for i in range(7))
TB = 4
LAG = 4
NTAP = 1016
P3I = 2

_GELU_C0 = float(np.sqrt(2.0 / np.pi))
_GELU_C1 = _GELU_C0 * 0.044715
_A = _GELU_C1 ** (1.0 / 3.0)
_K = _GELU_C0 / _A


def _dft_tables():
    m = np.arange(BLK)[:, None]
    n = np.arange(BLK)[None, :]
    th = 2.0 * np.pi * (((4 * m + 1) * n) % (4 * BLK)) / (4 * BLK)
    ph = 2.0 * np.pi * (((4 * m + 1) * (2 * n + 1)) % (8 * BLK)) / (8 * BLK)
    fu = np.concatenate([np.cos(ph), -np.sin(ph)], axis=0)
    fh = np.concatenate([np.cos(th) + np.sin(th), np.cos(th) - np.sin(th)], axis=0)
    fu, fh = (f.reshape(2, BLK // 8, 8, BLK).transpose(1, 0, 2, 3).reshape(2 * BLK, BLK)
              for f in (fu, fh))
    cp = (np.cos(ph) + np.sin(ph)).T[:BLK // 2] / (8.0 * BLK * _A * _A)
    cm = (np.cos(ph) - np.sin(ph)).T[:BLK // 2] / (8.0 * BLK * _A * _A)
    return np.concatenate([fu, fh, cp, cm], axis=0).astype(np.float32)


def _layernorm(x, eps, scale=1.0):
    m = jnp.mean(x, axis=-1, keepdims=True)
    d = x - m
    v = jnp.sum(d * d, axis=-1, keepdims=True) * (1.0 / (x.shape[-1] * scale * scale))
    return d * jax.lax.rsqrt(v + eps / (scale * scale))


def _gelu2(y):
    return y * (1.0 + jnp.tanh(y * (y * y + _K)))


def _up(x):
    return pltpu.bitcast(x, BF16)


def _dot(a, b):
    return jnp.dot(a, b, preferred_element_type=F32)


def _kernel(x_hbm, k_hbm, v_hbm, skt_hbm, h_hbm, dv_hbm, win_hbm, wsp_hbm, b_hbm,
            wout_hbm, tab_hbm, out_hbm,
            x_v, win_v, wsp_v, wout_v, kv_v, h_v, xn_v, z1_v, z2_v, p_v,
            kvb_v, pl_v, zz_v, bcol_v, o_v, zta_v, ztb_v, raw_v, tab_v,
            sk_v, dd_v, skt_v, dv_v, b_v, zero_s, sem):
    cp = pltpu.make_async_copy
    x16 = x_v.bitcast(BF16)
    win16 = win_v.bitcast(BF16)
    kv16 = kv_v.bitcast(BF16)
    h16 = h_v.bitcast(BF16)

    xn32, z232, p32, kvb32, zz32 = (
        r.bitcast(U32) for r in (xn_v, z2_v, p_v, kvb_v, zz_v))

    def x_cp(lo, hi, s):
        return cp(x_hbm.at[0, lo:hi, :], x16.at[0, lo:hi, :], sem.at[s])

    def win_cp(lo, hi, s):
        return cp(win_hbm.at[:, lo:hi], win16.at[:, lo:hi], sem.at[s])

    def k_cp(c, s):
        return cp(k_hbm.at[0, :, pl.ds(c * 128, 128)], kv16.at[2 * c, 0:S, :], sem.at[s])

    def v_cp(c, s):
        return cp(v_hbm.at[0, :, pl.ds(c * 128, 128)], kv16.at[2 * c + 1, 0:S, :], sem.at[s])

    def h_cp(c, s):
        return cp(h_hbm.at[pl.ds(c * 128, 128), :], h16.at[c], sem.at[s])

    groups = [
        [cp(b_hbm, b_v, sem.at[0]), cp(skt_hbm, skt_v, sem.at[0]), cp(dv_hbm, dv_v, sem.at[0])],
        [x_cp(0, 256, 1)],
        [win_cp(FH, FH + 256, 2)],
        [win_cp(FH + 256, 2 * FH, 3)],
        [win_cp(0, 512, 4)],
        [win_cp(512, FH, 5), x_cp(256, 384, 5)],
        [x_cp(384, (TB + 2) * T, 6)],
        [x_cp((TB + 2) * T, S, 7), k_cp(0, 7), v_cp(0, 7)],
        [cp(tab_hbm, tab_v.bitcast(BF16), sem.at[8]), h_cp(0, 8),
         cp(wsp_hbm, wsp_v.bitcast(BF16), sem.at[8])],
    ]
    for g in groups:
        for c in g:
            c.start()

    def tile_cps(c):
        s = jnp.where(c == NC - 1, 9, c - 1) if isinstance(c, jax.Array) else (0, 1, 2, 9)[c - 1]
        return [k_cp(c, s), v_cp(c, s), h_cp(c, s)]

    wout_cp = cp(wout_hbm, wout_v.bitcast(BF16), sem.at[10])
    out_sem = sem.at[5]

    def wait(i):
        for c in groups[i]:
            c.wait()

    zero_s[0] = 0
    wait(0)
    skt = skt_v[...].astype(F32)
    dv = dv_v[...].astype(F32).reshape(1, D)
    for c in range(NC):
        sk_v[c] = skt[:, c * 128:(c + 1) * 128]
        dd_v[c] = dv[:, c * 128:(c + 1) * 128]
    brow = b_v[...].astype(F32).reshape(1, S)
    bcol_v[...] = jnp.broadcast_to(brow, (128, S)).T

    def gate_x(tok):
        x_v[0, S // 2:S // 2 + 8, 0:128] = pltpu.bitcast(tok, U32)

    zt_v = (zta_v, ztb_v)

    def gate_zt(t):
        def gate(tok):
            zt_v[t % 2][0, T:T + 8, 0:128] = tok
        return gate

    def gate_kv(tok):
        kv_v[0, S // 2:S // 2 + 8, :] = pltpu.bitcast(tok, U32)

    def gate_pl(tok):
        pl_v[0, TOK] = tok

    ndone = [0]

    def done(val):
        r = S + (ndone[0] % 16) * 16
        ndone[0] += 1
        xn_v[0, r:r + 16, :] = val

    def lnx_items(t, zero):
        def item(r0):
            def run():
                xw = x_v[zero, r0 // 2:r0 // 2 + 8, :]
                xn = _layernorm(_up(xw).astype(F32), EPS, _A)
                for c in range(NC):
                    xn_v[c, r0:r0 + 16, :] = xn[:, c * 128:(c + 1) * 128].astype(BF16)
            return (1, gate_x, run)
        return [item(t * T + g * 16) for g in range(T // 16)]

    def lnz_items(t, zero):
        def item(g):
            def run():
                z = zt_v[t % 2][zero, g * 16:(g + 1) * 16, :]
                z = _layernorm(z, 4.0 * _A * _A * EPS)
                r0 = t * T + g * 16
                for n in range(NF):
                    zb = z[:, n * 128:(n + 1) * 128].astype(BF16)
                    z2_v[n, r0:r0 + 16, :] = zb
                    if n == 0:
                        done(zb)
            return (1, gate_zt(t), run)
        return [item(g) for g in range(T // 16)]

    def kv_items(c):
        sk = sk_v[c]

        def item(r0):
            def run():
                hs = slice(r0 // 2, (r0 + KR) // 2)
                if r0 == 0:
                    kw = jnp.concatenate(
                        [jnp.zeros((8, 128), F32), _up(kv_v[2 * c, hs, :]).astype(F32)], axis=0)
                else:
                    kw = _up(kv_v[2 * c, r0 // 2 - 8:(r0 + KR) // 2, :]).astype(F32)[8:]
                ks = kw[8:] * sk[0:1, :]
                for t in range(1, KS):
                    ks = ks + pltpu.roll(kw, t, 0)[8:] * sk[t:t + 1, :]
                kvb_v[r0:r0 + KR, :] = (
                    ks * _up(kv_v[2 * c + 1, hs, :]).astype(F32)).astype(BF16)
            return (14 * KR // 8, gate_kv, run)
        return [item(r0) for r0 in range(0, S, KR)]

    def taps_of(val):
        rows, cols = val.shape
        return [(lambda i=i, n=n: val[i * 8:(i + 1) * 8, n * 128:(n + 1) * 128])
                for n in range(cols // 128) for i in range(rows // 8)]

    def activate(kind, t, n, z):
        if kind == 2:
            zt_v[t % 2][0, 0:T, n * 128:(n + 1) * 128] = _gelu2(z)
        else:
            z1_v[n, t * T:(t + 1) * T, :] = _gelu2(z).astype(BF16)

    def piece(kind, t, n, zero, defer=False):
        col = n * 128 + (FH if kind == 2 else 0)
        xn = jnp.concatenate(
            [_up(xn32[zero if zero is not None and c == 0 else c,
                      t * T // 2:(t + 1) * T // 2, :]) for c in range(NC)], axis=1)
        z = _dot(xn, _up(win_v[:, col:col + 128]))
        if defer:
            raw_v[...] = z
        else:
            activate(kind, t, n, z)
        return taps_of(z)

    pending = []

    def block(pieces, work, defer=True, free=None):
        zero = zero_s[0]
        if pending:
            activate(*pending.pop(), raw_v[...])
        rel = [[] for _ in pieces]
        for mk, lo, hi in work:
            items = mk(zero)
            for i, it in enumerate(items):
                tau = (lo * 16) + (i * (hi - lo) * 16) // len(items)
                rel[tau // 16].append((tau % 16, it))
        taps = []
        gated = False
        for k in range(len(pieces) + LAG):
            if free is not None and k == len(pieces) - 1:
                for _, _, run in free(zero):
                    run()
                gated = True
            if k < len(pieces):
                last = defer and k == len(pieces) - 1
                taps.append(piece(*pieces[k], zero if gated else None, last))
                if last:
                    pending.append(pieces[k])
            if k >= LAG:
                for i, (_, gate, run) in sorted(rel[k - LAG], key=lambda e: e[0]):
                    gate(taps[k - LAG][i]())
                    run()
                    gated = True

    def cols(kind, t, lo=0, hi=NF):
        return [(kind, t, n) for n in range(lo, hi)]

    def lnx(t):
        return lambda zero: lnx_items(t, zero)

    def lnz(t):
        return lambda zero: lnz_items(t, zero)

    wait(1)
    for it in lnx_items(0, 0) + lnx_items(1, 0):
        it[2]()
    wait(2)
    block(cols(2, 0, 0, 2) + cols(2, 1, 0, 2), [])
    for c in range(1, NC):
        for d in tile_cps(c):
            d.start()
    wout_cp.start()
    wait(3)
    block(cols(2, 0, 2) + cols(2, 1, 2), [])
    wait(4)
    block(cols(1, 0, 0, 4) + cols(1, 1, 0, 4), [(lnz(0), 0, 3)])
    wait(5)
    block(cols(1, 0, 4) + cols(1, 1, 4), [], free=lnx(2))

    def big_block(first, last, extra):
        pieces, work = [], [(lnx(first + 1), 0, 11 - LAG)] + list(extra)
        for t in range(first, last - 1):
            k = len(pieces)
            pieces += cols(2, t) + cols(1, t)
            lo = k + (7 if t == first else 0)
            if t + 1 < last - 1:
                work += [(lnx(t + 2), lo, k + (16 if t == first else 12)), (lnz(t), k + 6, k + 18)]
            else:
                work += [(lnx(t + 2), lo, k + 12), (lnz(t), k + 6, k + 17 - LAG)]
        a, b = last - 1, last
        k = len(pieces)
        pieces += cols(2, a) + cols(2, b) + cols(1, a) + cols(1, b)
        work += [(lnz(a), k + 6, k + 13), (lnz(b), k + 12, k + 23 - LAG)]
        if b + 1 < NT:
            work += [(lnx(b + 1), k, k + 8)]
        else:
            work += [(kv_items, 14, k + 24)]
        block(pieces, work, b + 1 < NT)

    wait(6)
    big_block(2, TB, [(lnz(1), 0, 11 - LAG)])
    wait(7)
    big_block(TB + 1, NT - 1, [])

    wait(8)

    def p2(n, carry):
        nn = jnp.minimum(n + 1, NC - 1)

        @pl.when(n + 1 < NC)
        def _():
            for d in tile_cps(nn):
                d.wait()

        zero = zero_s[0]
        fwd_u = _up(tab_v[0:128, :])
        fwd_h = _up(tab_v[128:256, :])
        dd = dd_v[n]

        def put(slot, val):
            pl_v[:, slot] = val

        def re_im(val):
            val = val.reshape(BLK // 8, 2, 8, 128)
            return val[:, 0], val[:, 1]

        kvi = kv_items(nn)

        def pace_kv(d, val):
            if d % 4 == 3:
                for j in range(8):
                    _, gate, run = kvi[(d // 4) * 8 + j]
                    gate(val[j * 32:j * 32 + 8, :])
                    run()

        for i in range(NB):
            u = _dot(fwd_u, _up(kvb32[i * BLK // 2:(i + 1) * BLK // 2, :]))
            a, b = re_im(u)
            put(UA + i, a)
            put(UB + i, b)
            put(US + i, a + b)
            pace_kv(i, u)
        for i in range(NB):
            hb = _up(h_v[n, :, i * BLK:(i + 1) * BLK])
            hf = jax.lax.dot_general(fwd_h, hb, (((1,), (1,)), ((), ())),
                                     preferred_element_type=F32)
            c, d = re_im(hf)
            if i == 0:
                c, d = c + dd, d + dd
            put(HR + i, c)
            put(HP + i, d - c)
            put(HQ + i, c + d)
            pace_kv(NB + i, hf)

        state = {}

        def mac_item(pos, g0, pi):
            xv, hv = ((US, HR), (UA, HP), (UB, HQ))[pi]
            outs = range(g0, g0 + GRP)
            top = g0 + GRP

            def run():
                pz = zero + pos
                hs = [pl_v[pz, hv + t] for t in range(top)]
                acc = {o: None for o in outs}
                for jj in range(top):
                    xj = pl_v[pz, xv + jj]
                    for o in outs:
                        if o - jj >= 0:
                            t = xj * hs[o - jj]
                            acc[o] = t if acc[o] is None else acc[o] + t
                r0 = pos * 8
                if pi == 0:
                    state['k1'] = acc
                elif pi == 1:
                    state['im'] = {o: state['k1'][o] + acc[o] for o in outs}
                else:
                    for o in outs:
                        re, im = state['k1'][o] - acc[o], state['im'][o]
                        zr, zi = re, im
                        if o > 0:
                            zr, zi = re - state['prev'][1], im + state['prev'][0]
                        state['prev'] = (re, im)
                        zz_v[n, o, r0:r0 + 8, :] = zr.astype(BF16)
                        zz_v[n, o, BLK + r0:BLK + r0 + 8, :] = zi.astype(BF16)

            nmac = sum(o + 1 for o in outs)
            return (2 * nmac - GRP + (0, GRP, 5 * GRP)[pi], gate_pl, run)

        items = []
        for pos in range(BLK // 8):
            for g0 in range(0, NB, GRP):
                for pi in range(3):
                    items.append(mac_item(pos, g0, pi))

        nq = S // KG
        vpc = T // 8
        total = sum(c for c, _, _ in items)
        tap_of = []
        cum = 0
        for c, _, _ in items:
            tap_of.append(int(cum * NTAP / total))
            cum += c
        nxt = 0
        for r in range(NT):
            rs = slice(r * T, (r + 1) * T)
            hs = slice(r * T // 2, (r + 1) * T // 2)
            acc = None
            for q in range(nq):
                part = _dot(_up(wsp_v[hs, q * KG:(q + 1) * KG]),
                            _up(z232[n, q * KG // 2:(q + 1) * KG // 2, :]))
                acc = part if acc is None else acc + part
                t0 = (r * nq + q) * vpc
                while nxt < len(items) and tap_of[nxt] < t0 + vpc:
                    i = tap_of[nxt] - t0
                    items[nxt][1](acc[i * 8:(i + 1) * 8, :])
                    items[nxt][2]()
                    nxt += 1
            g = acc + bcol_v[rs, :]
            p_v[n, rs, :] = (z1_v[n, rs, :].astype(F32) * g).astype(BF16)
        assert nxt == len(items)
        return carry

    jax.lax.fori_loop(0, NC, p2, 0)

    wout_cp.wait()

    TPI = NT // P3I

    def p3(j, carry):
        inv_p = _up(tab_v[256:288, :])
        inv_m = _up(tab_v[288:320, :])
        rev = 7 - jax.lax.broadcasted_iota(jnp.int32, (8, 128), 0)

        def rows(t):
            r0 = (j * TPI + t) * T
            return (pl.ds(pl.multiple_of(r0, T), T),
                    pl.ds(pl.multiple_of(r0 // 2, T // 2), T // 2))

        def g5(t):
            rs, hs = rows(t)
            g = _dot(_up(wsp_v[hs, :]), _up(z232[NF - 1])) + bcol_v[rs, :]
            return (z1_v[NF - 1, rs, :].astype(F32) * g).astype(BF16)

        p5 = g5(0)
        for t in range(TPI):
            rs, hs = rows(t)
            p = jnp.concatenate([_up(p32[n, hs, :]) for n in range(NF - 1)] + [p5], axis=1)
            if t + 1 < TPI:
                p5 = g5(t + 1)
            for c in range(NC):
                cs = slice(c * 128, (c + 1) * 128)
                ye = _dot(inv_p, _up(zz32[c, j * TPI + t, 0:64, :]))
                yo = _dot(inv_m, _up(zz32[c, j * TPI + t, 64:128, :]))
                yd = ye - yo
                y = jnp.concatenate(
                    [ye + yo] + [
                        jnp.take_along_axis(yd[i * 8:(i + 1) * 8], rev, axis=0,
                                            mode="promise_in_bounds")
                        for i in reversed(range(BLK // 16))], axis=0)
                o = _dot(p, _up(wout_v[:, cs]))
                gate = o * (1.0 + jnp.tanh((0.25 / _A) * o))
                x = _up(x_v[0, hs, cs]).astype(F32)
                xn = xn_v[c, rs, :].astype(F32)
                o_v[rs, cs] = (x + (xn * y) * gate).astype(BF16)
                if t == TPI - 1 and c == NC - 2:
                    cp(o_v.at[rs, 0:512], out_hbm.at[0, rs, 0:512], out_sem).start()
            if t == TPI - 1:
                cp(o_v.at[rs, 512:D], out_hbm.at[0, rs, 512:D], out_sem).start()
            else:
                cp(o_v.at[rs, :], out_hbm.at[0, rs, :], out_sem).start()
        return carry

    jax.lax.fori_loop(0, P3I, p3, 0)
    cp(o_v, out_hbm.at[0], out_sem).wait()


@jax.jit
def pallas_recurrent_scan__ssm_conv_h3__mixer_gmlp__prompt_kernel(
    A_q: jax.Array,
    A_k: jax.Array,
    A_v: jax.Array,
    A_shift_k: jax.Array,
    A_ssm_k: jax.Array,
    A_ssm_D: jax.Array,
    B_x: jax.Array,
    B_w_in: jax.Array,
    B_w_sp: jax.Array,
    B_b_sp: jax.Array,
    B_w_out: jax.Array,
):
    del B_x
    tab = jnp.asarray(_dft_tables(), dtype=BF16)

    any_spec = pl.BlockSpec(memory_space=pl.ANY)
    return pl.pallas_call(
        _kernel,
        out_shape=jax.ShapeDtypeStruct((1, S, D), BF16),
        in_specs=[any_spec] * 11,
        out_specs=any_spec,
        scratch_shapes=[
            pltpu.VMEM((1, S // 2 + 32, D), U32),
            pltpu.VMEM((D // 2, 2 * FH), U32),
            pltpu.VMEM((S // 2, S), U32),
            pltpu.VMEM((FH // 2, D), U32),
            pltpu.VMEM((2 * NC, S // 2 + 32, 128), U32),
            pltpu.VMEM((NC, 64, S), U32),
            pltpu.VMEM((NC, S + 256, 128), BF16),
            pltpu.VMEM((NF, S, 128), BF16),
            pltpu.VMEM((NF, S, 128), BF16),
            pltpu.VMEM((NF - 1, S, 128), BF16),
            pltpu.VMEM((S, 128), BF16),
            pltpu.VMEM((BLK // 8, 6 * NB + 1, 8, 128), F32),
            pltpu.VMEM((NC, NB, 2 * BLK, 128), BF16),
            pltpu.VMEM((S, 128), F32),
            pltpu.VMEM((S, D), BF16),
            pltpu.VMEM((1, T + 16, FH), F32),
            pltpu.VMEM((1, T + 16, FH), F32),
            pltpu.VMEM((T, 128), F32),
            pltpu.VMEM((320, 128), U32),
            pltpu.VMEM((NC, KS, 128), F32),
            pltpu.VMEM((NC + 2, 1, 128), F32),
            pltpu.VMEM((KS, D), BF16),
            pltpu.VMEM((D,), BF16),
            pltpu.VMEM((S,), BF16),
            pltpu.SMEM((1,), jnp.int32),
            pltpu.SemaphoreType.DMA((11,)),
        ],
        compiler_params=pltpu.CompilerParams(
            vmem_limit_bytes=100 * 1024 * 1024, disable_bounds_checks=True),
    )(A_q, A_k, A_v, A_shift_k.T, A_ssm_k, A_ssm_D, B_w_in, B_w_sp, B_b_sp, B_w_out, tab)
```

```python
import jax
import jax.numpy as jnp
import numpy as np
import jax.experimental.pallas as pl
import jax.experimental.pallas.tpu as pltpu

F32 = jnp.float32
BF16 = jnp.bfloat16
U32 = jnp.uint32

S = 2048
D = 640
FH = 768
KS = 4
BLK = 128
NB = S // BLK
NC = D // 128
NF = FH // 128
T = 128
NT = S // T
EPS = 1e-5
GRP = 4
SPLIT = 8
KG = 512
KR = 32
UA, UB, US, HP, HQ, HR, TOK = (i * NB for i in range(7))
TB = 4
LAG = 4
NTAP = 1016
P3I = 2

_GELU_C0 = float(np.sqrt(2.0 / np.pi))
_GELU_C1 = _GELU_C0 * 0.044715
_A = _GELU_C1 ** (1.0 / 3.0)
_K = _GELU_C0 / _A


def _dft_tables():
    m = np.arange(BLK)[:, None]
    n = np.arange(BLK)[None, :]
    th = 2.0 * np.pi * (((4 * m + 1) * n) % (4 * BLK)) / (4 * BLK)
    ph = 2.0 * np.pi * (((4 * m + 1) * (2 * n + 1)) % (8 * BLK)) / (8 * BLK)
    fu = np.concatenate([np.cos(ph), -np.sin(ph)], axis=0)
    fh = np.concatenate([np.cos(th) + np.sin(th), np.cos(th) - np.sin(th)], axis=0)
    fu, fh = (f.reshape(2, BLK // 8, 8, BLK).transpose(1, 0, 2, 3).reshape(2 * BLK, BLK)
              for f in (fu, fh))
    cp = (np.cos(ph) + np.sin(ph)).T[:BLK // 2] / (8.0 * BLK * _A * _A)
    cm = (np.cos(ph) - np.sin(ph)).T[:BLK // 2] / (8.0 * BLK * _A * _A)
    return np.concatenate([fu, fh, cp, cm], axis=0).astype(np.float32)


def _layernorm(x, eps, scale=1.0):
    m = jnp.mean(x, axis=-1, keepdims=True)
    d = x - m
    v = jnp.sum(d * d, axis=-1, keepdims=True) * (1.0 / (x.shape[-1] * scale * scale))
    return d * jax.lax.rsqrt(v + eps / (scale * scale))


def _gelu2(y):
    return y * (1.0 + jnp.tanh(y * (y * y + _K)))


def _up(x):
    return pltpu.bitcast(x, BF16)


def _dot(a, b):
    return jnp.dot(a, b, preferred_element_type=F32)


def _kernel(x_hbm, k_hbm, v_hbm, skt_hbm, h_hbm, dv_hbm, win_hbm, wsp_hbm, b_hbm,
            wout_hbm, tab_hbm, out_hbm,
            x_v, win_v, wsp_v, wout_v, kv_v, h_v, xn_v, z1_v, z2_v, p_v,
            kvb_v, pl_v, zz_v, bcol_v, o_v, zta_v, ztb_v, raw_v, tab_v,
            sk_v, dd_v, skt_v, dv_v, b_v, zero_s, sem):
    cp = pltpu.make_async_copy
    x16 = x_v.bitcast(BF16)
    win16 = win_v.bitcast(BF16)
    kv16 = kv_v.bitcast(BF16)
    h16 = h_v.bitcast(BF16)

    xn32, z232, p32, kvb32, zz32 = (
        r.bitcast(U32) for r in (xn_v, z2_v, p_v, kvb_v, zz_v))

    def x_cp(lo, hi, s):
        return cp(x_hbm.at[0, lo:hi, :], x16.at[0, lo:hi, :], sem.at[s])

    def win_cp(lo, hi, s):
        return cp(win_hbm.at[:, lo:hi], win16.at[:, lo:hi], sem.at[s])

    def k_cp(c, s):
        return cp(k_hbm.at[0, :, pl.ds(c * 128, 128)], kv16.at[2 * c, 0:S, :], sem.at[s])

    def v_cp(c, s):
        return cp(v_hbm.at[0, :, pl.ds(c * 128, 128)], kv16.at[2 * c + 1, 0:S, :], sem.at[s])

    def h_cp(c, s):
        return cp(h_hbm.at[pl.ds(c * 128, 128), :], h16.at[c], sem.at[s])

    groups = [
        [cp(b_hbm, b_v, sem.at[0]), cp(skt_hbm, skt_v, sem.at[0]), cp(dv_hbm, dv_v, sem.at[0])],
        [x_cp(0, 256, 1)],
        [win_cp(FH, FH + 256, 2)],
        [win_cp(FH + 256, 2 * FH, 3)],
        [win_cp(0, 512, 4)],
        [win_cp(512, FH, 5), x_cp(256, 384, 5)],
        [x_cp(384, (TB + 2) * T, 6)],
        [x_cp((TB + 2) * T, S, 7), k_cp(0, 7), v_cp(0, 7)],
        [cp(tab_hbm, tab_v.bitcast(BF16), sem.at[8]), h_cp(0, 8),
         cp(wsp_hbm, wsp_v.bitcast(BF16), sem.at[8])],
    ]
    for g in groups:
        for c in g:
            c.start()

    def tile_cps(c):
        s = jnp.where(c == NC - 1, 9, c - 1) if isinstance(c, jax.Array) else (0, 1, 2, 9)[c - 1]
        return [k_cp(c, s), v_cp(c, s), h_cp(c, s)]

    wout_cp = cp(wout_hbm, wout_v.bitcast(BF16), sem.at[10])
    out_sem = sem.at[5]

    def wait(i):
        for c in groups[i]:
            c.wait()

    zero_s[0] = 0
    wait(0)
    skt = skt_v[...].astype(F32)
    dv = dv_v[...].astype(F32).reshape(1, D)
    for c in range(NC):
        sk_v[c] = skt[:, c * 128:(c + 1) * 128]
        dd_v[c] = dv[:, c * 128:(c + 1) * 128]
    brow = b_v[...].astype(F32).reshape(1, S)
    bcol_v[...] = jnp.broadcast_to(brow, (128, S)).T

    def gate_x(tok):
        x_v[0, S // 2:S // 2 + 8, 0:128] = pltpu.bitcast(tok, U32)

    zt_v = (zta_v, ztb_v)

    def gate_zt(t):
        def gate(tok):
            zt_v[t % 2][0, T:T + 8, 0:128] = tok
        return gate

    def gate_kv(tok):
        kv_v[0, S // 2:S // 2 + 8, :] = pltpu.bitcast(tok, U32)

    def gate_pl(tok):
        pl_v[0, TOK] = tok

    ndone = [0]

    def done(val):
        r = S + (ndone[0] % 16) * 16
        ndone[0] += 1
        xn_v[0, r:r + 16, :] = val

    def lnx_items(t, zero):
        def item(r0):
            def run():
                xw = x_v[zero, r0 // 2:r0 // 2 + 8, :]
                xn = _layernorm(_up(xw).astype(F32), EPS, _A)
                for c in range(NC):
                    xn_v[c, r0:r0 + 16, :] = xn[:, c * 128:(c + 1) * 128].astype(BF16)
            return (1, gate_x, run)
        return [item(t * T + g * 16) for g in range(T // 16)]

    def lnz_items(t, zero):
        def item(g):
            def run():
                z = zt_v[t % 2][zero, g * 16:(g + 1) * 16, :]
                z = _layernorm(z, 4.0 * _A * _A * EPS)
                r0 = t * T + g * 16
                for n in range(NF):
                    zb = z[:, n * 128:(n + 1) * 128].astype(BF16)
                    z2_v[n, r0:r0 + 16, :] = zb
                    if n == 0:
                        done(zb)
            return (1, gate_zt(t), run)
        return [item(g) for g in range(T // 16)]

    def kv_items(c):
        sk = sk_v[c]

        def item(r0):
            def run():
                hs = slice(r0 // 2, (r0 + KR) // 2)
                if r0 == 0:
                    kw = jnp.concatenate(
                        [jnp.zeros((8, 128), F32), _up(kv_v[2 * c, hs, :]).astype(F32)], axis=0)
                else:
                    kw = _up(kv_v[2 * c, r0 // 2 - 8:(r0 + KR) // 2, :]).astype(F32)[8:]
                ks = kw[8:] * sk[0:1, :]
                for t in range(1, KS):
                    ks = ks + pltpu.roll(kw, t, 0)[8:] * sk[t:t + 1, :]
                kvb_v[r0:r0 + KR, :] = (
                    ks * _up(kv_v[2 * c + 1, hs, :]).astype(F32)).astype(BF16)
            return (14 * KR // 8, gate_kv, run)
        return [item(r0) for r0 in range(0, S, KR)]

    def taps_of(val):
        rows, cols = val.shape
        return [(lambda i=i, n=n: val[i * 8:(i + 1) * 8, n * 128:(n + 1) * 128])
                for n in range(cols // 128) for i in range(rows // 8)]

    def activate(kind, t, n, z):
        if kind == 2:
            zt_v[t % 2][0, 0:T, n * 128:(n + 1) * 128] = _gelu2(z)
        else:
            z1_v[n, t * T:(t + 1) * T, :] = _gelu2(z).astype(BF16)

    def piece(kind, t, n, zero, defer=False):
        col = n * 128 + (FH if kind == 2 else 0)
        xn = jnp.concatenate(
            [_up(xn32[zero if zero is not None and c == 0 else c,
                      t * T // 2:(t + 1) * T // 2, :]) for c in range(NC)], axis=1)
        z = _dot(xn, _up(win_v[:, col:col + 128]))
        if defer:
            raw_v[...] = z
        else:
            activate(kind, t, n, z)
        return taps_of(z)

    pending = []

    def block(pieces, work, defer=True, free=None):
        zero = zero_s[0]
        if pending:
            activate(*pending.pop(), raw_v[...])
        rel = [[] for _ in pieces]
        for mk, lo, hi in work:
            items = mk(zero)
            for i, it in enumerate(items):
                tau = (lo * 16) + (i * (hi - lo) * 16) // len(items)
                rel[tau // 16].append((tau % 16, it))
        taps = []
        gated = False
        for k in range(len(pieces) + LAG):
            if free is not None and k == len(pieces) - 1:
                for _, _, run in free(zero):
                    run()
                gated = True
            if k < len(pieces):
                last = defer and k == len(pieces) - 1
                taps.append(piece(*pieces[k], zero if gated else None, last))
                if last:
                    pending.append(pieces[k])
            if k >= LAG:
                for i, (_, gate, run) in sorted(rel[k - LAG], key=lambda e: e[0]):
                    gate(taps[k - LAG][i]())
                    run()
                    gated = True

    def cols(kind, t, lo=0, hi=NF):
        return [(kind, t, n) for n in range(lo, hi)]

    def lnx(t):
        return lambda zero: lnx_items(t, zero)

    def lnz(t):
        return lambda zero: lnz_items(t, zero)

    wait(1)
    for it in lnx_items(0, 0) + lnx_items(1, 0):
        it[2]()
    wait(2)
    block(cols(2, 0, 0, 2) + cols(2, 1, 0, 2), [])
    for c in range(1, NC):
        for d in tile_cps(c):
            d.start()
    wout_cp.start()
    wait(3)
    block(cols(2, 0, 2) + cols(2, 1, 2), [])
    wait(4)
    block(cols(1, 0, 0, 4) + cols(1, 1, 0, 4), [(lnz(0), 0, 3)])
    wait(5)
    block(cols(1, 0, 4) + cols(1, 1, 4), [], free=lnx(2))

    def big_block(first, last, extra):
        pieces, work = [], [(lnx(first + 1), 0, 11 - LAG)] + list(extra)
        for t in range(first, last - 1):
            k = len(pieces)
            pieces += cols(2, t) + cols(1, t)
            lo = k + (7 if t == first else 0)
            if t + 1 < last - 1:
                work += [(lnx(t + 2), lo, k + (16 if t == first else 12)), (lnz(t), k + 6, k + 18)]
            else:
                work += [(lnx(t + 2), lo, k + 12), (lnz(t), k + 6, k + 17 - LAG)]
        a, b = last - 1, last
        k = len(pieces)
        pieces += cols(2, a) + cols(2, b) + cols(1, a) + cols(1, b)
        work += [(lnz(a), k + 6, k + 13), (lnz(b), k + 12, k + 23 - LAG)]
        if b + 1 < NT:
            work += [(lnx(b + 1), k, k + 8)]
        else:
            work += [(kv_items, 14, k + 24)]
        block(pieces, work, b + 1 < NT)

    wait(6)
    big_block(2, TB, [(lnz(1), 0, 11 - LAG)])
    wait(7)
    big_block(TB + 1, NT - 1, [])

    wait(8)

    def p2(n, carry):
        nn = jnp.minimum(n + 1, NC - 1)

        @pl.when(n + 1 < NC)
        def _():
            for d in tile_cps(nn):
                d.wait()

        zero = zero_s[0]
        fwd_u = _up(tab_v[0:128, :])
        fwd_h = _up(tab_v[128:256, :])
        dd = dd_v[n]

        def put(slot, val):
            pl_v[:, slot] = val

        def re_im(val):
            val = val.reshape(BLK // 8, 2, 8, 128)
            return val[:, 0], val[:, 1]

        kvi = kv_items(nn)

        def pace_kv(d, val):
            if d % 4 == 3:
                for j in range(8):
                    _, gate, run = kvi[(d // 4) * 8 + j]
                    gate(val[j * 32:j * 32 + 8, :])
                    run()

        for i in range(NB):
            u = _dot(fwd_u, _up(kvb32[i * BLK // 2:(i + 1) * BLK // 2, :]))
            a, b = re_im(u)
            put(UA + i, a)
            put(UB + i, b)
            put(US + i, a + b)
            pace_kv(i, u)
        for i in range(NB):
            hb = _up(h_v[n, :, i * BLK:(i + 1) * BLK])
            hf = jax.lax.dot_general(fwd_h, hb, (((1,), (1,)), ((), ())),
                                     preferred_element_type=F32)
            c, d = re_im(hf)
            if i == 0:
                c, d = c + dd, d + dd
            put(HR + i, c)
            put(HP + i, d - c)
            put(HQ + i, c + d)
            pace_kv(NB + i, hf)

        state = {}

        def mac_item(pos, g0, pi, j0, j1):
            xv, hv = ((US, HR), (UA, HP), (UB, HQ))[pi]
            outs = range(g0, g0 + GRP)
            top = g0 + GRP

            def run():
                pz = zero + pos
                hs = {t: pl_v[pz, hv + t]
                      for t in range(max(g0 - j1 + 1, 0), top - j0)}
                acc = state['acc'] if j0 else {o: None for o in outs}
                for jj in range(j0, j1):
                    xj = pl_v[pz, xv + jj]
                    for o in outs:
                        if o - jj >= 0:
                            t = xj * hs[o - jj]
                            acc[o] = t if acc[o] is None else acc[o] + t
                if j1 < top:
                    state['acc'] = acc
                    return
                r0 = pos * 8
                if pi == 0:
                    state['k1'] = acc
                elif pi == 1:
                    state['im'] = {o: state['k1'][o] + acc[o] for o in outs}
                else:
                    for o in outs:
                        re, im = state['k1'][o] - acc[o], state['im'][o]
                        zr, zi = re, im
                        if o > 0:
                            zr, zi = re - state['prev'][1], im + state['prev'][0]
                        state['prev'] = (re, im)
                        zz_v[n, o, r0:r0 + 8, :] = zr.astype(BF16)
                        zz_v[n, o, BLK + r0:BLK + r0 + 8, :] = zi.astype(BF16)

            nmac = sum(1 for o in outs for jj in range(j0, j1) if o >= jj)
            return (2 * nmac + ((0, GRP, 5 * GRP)[pi] if j1 == top else 0), gate_pl, run)

        items = []
        for pos in range(BLK // 8):
            for g0 in range(0, NB, GRP):
                top = g0 + GRP
                cuts = [0, top] if top <= SPLIT else [0, (top - 1) // 2, top]
                for pi in range(3):
                    for j0, j1 in zip(cuts[:-1], cuts[1:]):
                        items.append(mac_item(pos, g0, pi, j0, j1))

        nq = S // KG
        vpc = T // 8
        total = sum(c for c, _, _ in items)
        tap_of = []
        cum = 0
        for c, _, _ in items:
            tap_of.append(int(cum * NTAP / total))
            cum += c
        nxt = 0
        for r in range(NT):
            rs = slice(r * T, (r + 1) * T)
            hs = slice(r * T // 2, (r + 1) * T // 2)
            acc = None
            for q in range(nq):
                part = _dot(_up(wsp_v[hs, q * KG:(q + 1) * KG]),
                            _up(z232[n, q * KG // 2:(q + 1) * KG // 2, :]))
                acc = part if acc is None else acc + part
                t0 = (r * nq + q) * vpc
                while nxt < len(items) and tap_of[nxt] < t0 + vpc:
                    i = tap_of[nxt] - t0
                    items[nxt][1](acc[i * 8:(i + 1) * 8, :])
                    items[nxt][2]()
                    nxt += 1
            g = acc + bcol_v[rs, :]
            p_v[n, rs, :] = (z1_v[n, rs, :].astype(F32) * g).astype(BF16)
        assert nxt == len(items)
        return carry

    jax.lax.fori_loop(0, NC, p2, 0)

    wout_cp.wait()

    TPI = NT // P3I

    def p3(j, carry):
        inv_p = _up(tab_v[256:288, :])
        inv_m = _up(tab_v[288:320, :])
        rev = 7 - jax.lax.broadcasted_iota(jnp.int32, (8, 128), 0)

        def rows(t):
            r0 = (j * TPI + t) * T
            return (pl.ds(pl.multiple_of(r0, T), T),
                    pl.ds(pl.multiple_of(r0 // 2, T // 2), T // 2))

        def g5(t):
            rs, hs = rows(t)
            g = _dot(_up(wsp_v[hs, :]), _up(z232[NF - 1])) + bcol_v[rs, :]
            return (z1_v[NF - 1, rs, :].astype(F32) * g).astype(BF16)

        p5 = g5(0)
        for t in range(TPI):
            rs, hs = rows(t)
            p = jnp.concatenate([_up(p32[n, hs, :]) for n in range(NF - 1)] + [p5], axis=1)
            if t + 1 < TPI:
                p5 = g5(t + 1)
            for c in range(NC):
                cs = slice(c * 128, (c + 1) * 128)
                ye = _dot(inv_p, _up(zz32[c, j * TPI + t, 0:64, :]))
                yo = _dot(inv_m, _up(zz32[c, j * TPI + t, 64:128, :]))
                yd = ye - yo
                y = jnp.concatenate(
                    [ye + yo] + [
                        jnp.take_along_axis(yd[i * 8:(i + 1) * 8], rev, axis=0,
                                            mode="promise_in_bounds")
                        for i in reversed(range(BLK // 16))], axis=0)
                o = _dot(p, _up(wout_v[:, cs]))
                gate = o * (1.0 + jnp.tanh((0.25 / _A) * o))
                x = _up(x_v[0, hs, cs]).astype(F32)
                xn = xn_v[c, rs, :].astype(F32)
                o_v[rs, cs] = (x + (xn * y) * gate).astype(BF16)
                if t == TPI - 1 and c == NC - 2:
                    cp(o_v.at[rs, 0:512], out_hbm.at[0, rs, 0:512], out_sem).start()
            if t == TPI - 1:
                cp(o_v.at[rs, 512:D], out_hbm.at[0, rs, 512:D], out_sem).start()
            else:
                cp(o_v.at[rs, :], out_hbm.at[0, rs, :], out_sem).start()
        return carry

    jax.lax.fori_loop(0, P3I, p3, 0)
    cp(o_v, out_hbm.at[0], out_sem).wait()


@jax.jit
def pallas_recurrent_scan__ssm_conv_h3__mixer_gmlp__prompt_kernel(
    A_q: jax.Array,
    A_k: jax.Array,
    A_v: jax.Array,
    A_shift_k: jax.Array,
    A_ssm_k: jax.Array,
    A_ssm_D: jax.Array,
    B_x: jax.Array,
    B_w_in: jax.Array,
    B_w_sp: jax.Array,
    B_b_sp: jax.Array,
    B_w_out: jax.Array,
):
    del B_x
    tab = jnp.asarray(_dft_tables(), dtype=BF16)

    any_spec = pl.BlockSpec(memory_space=pl.ANY)
    return pl.pallas_call(
        _kernel,
        out_shape=jax.ShapeDtypeStruct((1, S, D), BF16),
        in_specs=[any_spec] * 11,
        out_specs=any_spec,
        scratch_shapes=[
            pltpu.VMEM((1, S // 2 + 32, D), U32),
            pltpu.VMEM((D // 2, 2 * FH), U32),
            pltpu.VMEM((S // 2, S), U32),
            pltpu.VMEM((FH // 2, D), U32),
            pltpu.VMEM((2 * NC, S // 2 + 32, 128), U32),
            pltpu.VMEM((NC, 64, S), U32),
            pltpu.VMEM((NC, S + 256, 128), BF16),
            pltpu.VMEM((NF, S, 128), BF16),
            pltpu.VMEM((NF, S, 128), BF16),
            pltpu.VMEM((NF - 1, S, 128), BF16),
            pltpu.VMEM((S, 128), BF16),
            pltpu.VMEM((BLK // 8, 6 * NB + 1, 8, 128), F32),
            pltpu.VMEM((NC, NB, 2 * BLK, 128), BF16),
            pltpu.VMEM((S, 128), F32),
            pltpu.VMEM((S, D), BF16),
            pltpu.VMEM((1, T + 16, FH), F32),
            pltpu.VMEM((1, T + 16, FH), F32),
            pltpu.VMEM((T, 128), F32),
            pltpu.VMEM((320, 128), U32),
            pltpu.VMEM((NC, KS, 128), F32),
            pltpu.VMEM((NC + 2, 1, 128), F32),
            pltpu.VMEM((KS, D), BF16),
            pltpu.VMEM((D,), BF16),
            pltpu.VMEM((S,), BF16),
            pltpu.SMEM((1,), jnp.int32),
            pltpu.SemaphoreType.DMA((11,)),
        ],
        compiler_params=pltpu.CompilerParams(
            vmem_limit_bytes=100 * 1024 * 1024, disable_bounds_checks=True),
    )(A_q, A_k, A_v, A_shift_k.T, A_ssm_k, A_ssm_D, B_w_in, B_w_sp, B_b_sp, B_w_out, tab)
```

```python
import jax
import jax.numpy as jnp
import numpy as np
import jax.experimental.pallas as pl
import jax.experimental.pallas.tpu as pltpu

F32 = jnp.float32
BF16 = jnp.bfloat16
U32 = jnp.uint32

S = 2048
D = 640
FH = 768
KS = 4
BLK = 128
NB = S // BLK
NC = D // 128
NF = FH // 128
T = 128
NT = S // T
EPS = 1e-5
GRP = 4
SPLIT = 8
KG = 512
KR = 32
UA, UB, US, HP, HQ, HR, TOK = (i * NB for i in range(7))
TB = 4
LAG = 4
NTAP = 1016
P3I = 2

_GELU_C0 = float(np.sqrt(2.0 / np.pi))
_GELU_C1 = _GELU_C0 * 0.044715
_A = _GELU_C1 ** (1.0 / 3.0)
_K = _GELU_C0 / _A


def _dft_tables():
    m = np.arange(BLK)[:, None]
    n = np.arange(BLK)[None, :]
    th = 2.0 * np.pi * (((4 * m + 1) * n) % (4 * BLK)) / (4 * BLK)
    ph = 2.0 * np.pi * (((4 * m + 1) * (2 * n + 1)) % (8 * BLK)) / (8 * BLK)
    fu = np.concatenate([np.cos(ph), -np.sin(ph)], axis=0)
    fh = np.concatenate([np.cos(th) + np.sin(th), np.cos(th) - np.sin(th)], axis=0)
    fu, fh = (f.reshape(2, BLK // 8, 8, BLK).transpose(1, 0, 2, 3).reshape(2 * BLK, BLK)
              for f in (fu, fh))
    cp = (np.cos(ph) + np.sin(ph)).T[:BLK // 2] / (8.0 * BLK * _A * _A)
    cm = (np.cos(ph) - np.sin(ph)).T[:BLK // 2] / (8.0 * BLK * _A * _A)
    return np.concatenate([fu, fh, cp, cm], axis=0).astype(np.float32)


def _layernorm(x, eps, scale=1.0):
    m = jnp.mean(x, axis=-1, keepdims=True)
    d = x - m
    v = jnp.sum(d * d, axis=-1, keepdims=True) * (1.0 / (x.shape[-1] * scale * scale))
    return d * jax.lax.rsqrt(v + eps / (scale * scale))


def _gelu2(y):
    return y * (1.0 + jnp.tanh(y * (y * y + _K)))


def _up(x):
    return pltpu.bitcast(x, BF16)


def _dot(a, b):
    return jnp.dot(a, b, preferred_element_type=F32)


def _kernel(x_hbm, k_hbm, v_hbm, skt_hbm, h_hbm, dv_hbm, win_hbm, wsp_hbm, b_hbm,
            wout_hbm, tab_hbm, out_hbm,
            x_v, win_v, wsp_v, wout_v, kv_v, h_v, xn_v, z1_v, z2_v, p_v,
            kvb_v, pl_v, zz_v, bcol_v, o_v, zta_v, ztb_v, ztc_v, raw_v, tab_v,
            sk_v, dd_v, skt_v, dv_v, b_v, zero_s, sem):
    cp = pltpu.make_async_copy
    x16 = x_v.bitcast(BF16)
    win16 = win_v.bitcast(BF16)
    kv16 = kv_v.bitcast(BF16)
    h16 = h_v.bitcast(BF16)

    xn32, z232, p32, kvb32, zz32 = (
        r.bitcast(U32) for r in (xn_v, z2_v, p_v, kvb_v, zz_v))

    def x_cp(lo, hi, s):
        return cp(x_hbm.at[0, lo:hi, :], x16.at[0, lo:hi, :], sem.at[s])

    def win_cp(lo, hi, s):
        return cp(win_hbm.at[:, lo:hi], win16.at[:, lo:hi], sem.at[s])

    def k_cp(c, s):
        return cp(k_hbm.at[0, :, pl.ds(c * 128, 128)], kv16.at[2 * c, 0:S, :], sem.at[s])

    def v_cp(c, s):
        return cp(v_hbm.at[0, :, pl.ds(c * 128, 128)], kv16.at[2 * c + 1, 0:S, :], sem.at[s])

    def h_cp(c, s):
        return cp(h_hbm.at[pl.ds(c * 128, 128), :], h16.at[c], sem.at[s])

    groups = [
        [cp(b_hbm, b_v, sem.at[0]), cp(skt_hbm, skt_v, sem.at[0]), cp(dv_hbm, dv_v, sem.at[0])],
        [x_cp(0, 256, 1)],
        [win_cp(FH, FH + 256, 2)],
        [win_cp(FH + 256, 2 * FH, 3)],
        [win_cp(0, 512, 4)],
        [win_cp(512, FH, 5), x_cp(256, 384, 5)],
        [x_cp(384, (TB + 2) * T, 6)],
        [x_cp((TB + 2) * T, S, 7), k_cp(0, 7), v_cp(0, 7)],
        [cp(tab_hbm, tab_v.bitcast(BF16), sem.at[8]), h_cp(0, 8),
         cp(wsp_hbm, wsp_v.bitcast(BF16), sem.at[8])],
    ]
    for g in groups:
        for c in g:
            c.start()

    def tile_cps(c):
        s = jnp.where(c == NC - 1, 9, c - 1) if isinstance(c, jax.Array) else (0, 1, 2, 9)[c - 1]
        return [k_cp(c, s), v_cp(c, s), h_cp(c, s)]

    wout_cp = cp(wout_hbm, wout_v.bitcast(BF16), sem.at[10])
    out_sem = sem.at[5]

    def wait(i):
        for c in groups[i]:
            c.wait()

    zero_s[0] = 0
    wait(0)
    skt = skt_v[...].astype(F32)
    dv = dv_v[...].astype(F32).reshape(1, D)
    for c in range(NC):
        sk_v[c] = skt[:, c * 128:(c + 1) * 128]
        dd_v[c] = dv[:, c * 128:(c + 1) * 128]
    brow = b_v[...].astype(F32).reshape(1, S)
    bcol_v[...] = jnp.broadcast_to(brow, (128, S)).T

    def gate_x(tok):
        x_v[0, S // 2:S // 2 + 8, 0:128] = pltpu.bitcast(tok, U32)

    zt_v = (zta_v, ztb_v, ztc_v)

    def gate_zt(t):
        def gate(tok):
            zt_v[t % 3][0, T:T + 8, 0:128] = tok
        return gate

    def gate_kv(tok):
        kv_v[0, S // 2:S // 2 + 8, :] = pltpu.bitcast(tok, U32)

    def gate_pl(tok):
        pl_v[0, TOK] = tok

    ndone = [0]

    def done(val):
        r = S + (ndone[0] % 16) * 16
        ndone[0] += 1
        xn_v[0, r:r + 16, :] = val

    def lnx_items(t, zero):
        def item(r0):
            def run():
                xw = x_v[zero, r0 // 2:r0 // 2 + 8, :]
                xn = _layernorm(_up(xw).astype(F32), EPS, _A)
                for c in range(NC):
                    xn_v[c, r0:r0 + 16, :] = xn[:, c * 128:(c + 1) * 128].astype(BF16)
            return (1, gate_x, run)
        return [item(t * T + g * 16) for g in range(T // 16)]

    def lnz_items(t, zero):
        def item(g):
            def run():
                z = zt_v[t % 3][zero, g * 16:(g + 1) * 16, :]
                z = _layernorm(z, 4.0 * _A * _A * EPS)
                r0 = t * T + g * 16
                for n in range(NF):
                    zb = z[:, n * 128:(n + 1) * 128].astype(BF16)
                    z2_v[n, r0:r0 + 16, :] = zb
                    if n == 0:
                        done(zb)
            return (1, gate_zt(t), run)
        return [item(g) for g in range(T // 16)]

    def kv_items(c):
        sk = sk_v[c]

        def item(r0):
            def run():
                hs = slice(r0 // 2, (r0 + KR) // 2)
                if r0 == 0:
                    kw = jnp.concatenate(
                        [jnp.zeros((8, 128), F32), _up(kv_v[2 * c, hs, :]).astype(F32)], axis=0)
                else:
                    kw = _up(kv_v[2 * c, r0 // 2 - 8:(r0 + KR) // 2, :]).astype(F32)[8:]
                ks = kw[8:] * sk[0:1, :]
                for t in range(1, KS):
                    ks = ks + pltpu.roll(kw, t, 0)[8:] * sk[t:t + 1, :]
                kvb_v[r0:r0 + KR, :] = (
                    ks * _up(kv_v[2 * c + 1, hs, :]).astype(F32)).astype(BF16)
            return (14 * KR // 8, gate_kv, run)
        return [item(r0) for r0 in range(0, S, KR)]

    def taps_of(val):
        rows, cols = val.shape
        return [(lambda i=i, n=n: val[i * 8:(i + 1) * 8, n * 128:(n + 1) * 128])
                for n in range(cols // 128) for i in range(rows // 8)]

    def activate(kind, t, n, z):
        if kind == 2:
            zt_v[t % 3][0, 0:T, n * 128:(n + 1) * 128] = _gelu2(z)
        else:
            z1_v[n, t * T:(t + 1) * T, :] = _gelu2(z).astype(BF16)

    def piece(kind, t, n, zero, defer=False):
        col = n * 128 + (FH if kind == 2 else 0)
        xn = jnp.concatenate(
            [_up(xn32[zero if zero is not None and c == 0 else c,
                      t * T // 2:(t + 1) * T // 2, :]) for c in range(NC)], axis=1)
        z = _dot(xn, _up(win_v[:, col:col + 128]))
        if defer:
            raw_v[...] = z
        else:
            activate(kind, t, n, z)
        return taps_of(z)

    pending = []

    def block(pieces, work, defer=True, free=None):
        zero = zero_s[0]
        if pending:
            activate(*pending.pop(), raw_v[...])
        rel = [[] for _ in pieces]
        for mk, lo, hi in work:
            items = mk(zero)
            for i, it in enumerate(items):
                tau = (lo * 16) + (i * (hi - lo) * 16) // len(items)
                rel[tau // 16].append((tau % 16, it))
        taps = []
        gated = False
        for k in range(len(pieces) + LAG):
            if free is not None and k == len(pieces) - 1:
                for _, _, run in free(zero):
                    run()
                gated = True
            if k < len(pieces):
                last = defer and k == len(pieces) - 1
                taps.append(piece(*pieces[k], zero if gated else None, last))
                if last:
                    pending.append(pieces[k])
            if k >= LAG:
                for i, (_, gate, run) in sorted(rel[k - LAG], key=lambda e: e[0]):
                    gate(taps[k - LAG][i]())
                    run()
                    gated = True

    def cols(kind, t, lo=0, hi=NF):
        return [(kind, t, n) for n in range(lo, hi)]

    def lnx(t):
        return lambda zero: lnx_items(t, zero)

    def lnz(t):
        return lambda zero: lnz_items(t, zero)

    wait(1)
    for it in lnx_items(0, 0) + lnx_items(1, 0):
        it[2]()
    wait(2)
    block(cols(2, 0, 0, 2) + cols(2, 1, 0, 2), [])
    for c in range(1, NC):
        for d in tile_cps(c):
            d.start()
    wout_cp.start()
    wait(3)
    block(cols(2, 0, 2) + cols(2, 1, 2), [])
    wait(4)
    block(cols(1, 0, 0, 4) + cols(1, 1, 0, 4), [(lnz(0), 0, 3)])
    wait(5)
    block(cols(1, 0, 4) + cols(1, 1, 4), [], free=lnx(2))

    def end_pair(a):
        return cols(2, a) + cols(2, a + 1) + cols(1, a) + cols(1, a + 1)

    wait(6)
    block(cols(2, 2) + cols(1, 2) + end_pair(3),
          [(lnx(3), 0, 7), (lnz(1), 0, 12), (lnx(4), 7, 13), (lnz(2), 11, 20),
           (lnx(5), 13, 22), (lnz(3), 18, 26), (lnz(4), 24, 31)])
    wait(7)
    pieces, work = [], [(lnx(6), 0, 7)]
    for t in range(5, NT - 2):
        k = len(pieces)
        pieces += cols(2, t) + cols(1, t)
        work += [(lnx(t + 2), k + (7 if t == 5 else 3), k + (16 if t == 5 else 13 if t == NT - 3 else 15)),
                 (lnz(t), k + 6, k + 18)]
    k = len(pieces)
    pieces += end_pair(NT - 2)
    work += [(lnz(NT - 2), k + 6, k + 13), (lnz(NT - 1), k + 12, k + 19), (kv_items, 14, k + 24)]
    block(pieces, work, defer=False)

    wait(8)

    def p2(n, carry):
        nn = jnp.minimum(n + 1, NC - 1)

        @pl.when(n + 1 < NC)
        def _():
            for d in tile_cps(nn):
                d.wait()

        zero = zero_s[0]
        fwd_u = _up(tab_v[0:128, :])
        fwd_h = _up(tab_v[128:256, :])
        dd = dd_v[n]

        def put(slot, val):
            pl_v[:, slot] = val

        def re_im(val):
            val = val.reshape(BLK // 8, 2, 8, 128)
            return val[:, 0], val[:, 1]

        kvi = kv_items(nn)

        def pace_kv(d, val):
            if d % 4 == 3:
                for j in range(8):
                    _, gate, run = kvi[(d // 4) * 8 + j]
                    gate(val[j * 32:j * 32 + 8, :])
                    run()

        for i in range(NB):
            u = _dot(fwd_u, _up(kvb32[i * BLK // 2:(i + 1) * BLK // 2, :]))
            a, b = re_im(u)
            put(UA + i, a)
            put(UB + i, b)
            put(US + i, a + b)
            pace_kv(i, u)
        for i in range(NB):
            hb = _up(h_v[n, :, i * BLK:(i + 1) * BLK])
            hf = jax.lax.dot_general(fwd_h, hb, (((1,), (1,)), ((), ())),
                                     preferred_element_type=F32)
            c, d = re_im(hf)
            if i == 0:
                c, d = c + dd, d + dd
            put(HR + i, c)
            put(HP + i, d - c)
            put(HQ + i, c + d)
            pace_kv(NB + i, hf)

        state = {}

        def mac_item(pos, g0, pi, j0, j1):
            xv, hv = ((US, HR), (UA, HP), (UB, HQ))[pi]
            outs = range(g0, g0 + GRP)
            top = g0 + GRP

            def run():
                pz = zero + pos
                hs = {t: pl_v[pz, hv + t]
                      for t in range(max(g0 - j1 + 1, 0), top - j0)}
                acc = state['acc'] if j0 else {o: None for o in outs}
                for jj in range(j0, j1):
                    xj = pl_v[pz, xv + jj]
                    for o in outs:
                        if o - jj >= 0:
                            t = xj * hs[o - jj]
                            acc[o] = t if acc[o] is None else acc[o] + t
                if j1 < top:
                    state['acc'] = acc
                    return
                r0 = pos * 8
                if pi == 0:
                    state['k1'] = acc
                elif pi == 1:
                    state['im'] = {o: state['k1'][o] + acc[o] for o in outs}
                else:
                    for o in outs:
                        re, im = state['k1'][o] - acc[o], state['im'][o]
                        zr, zi = re, im
                        if o > 0:
                            zr, zi = re - state['prev'][1], im + state['prev'][0]
                        state['prev'] = (re, im)
                        zz_v[n, o, r0:r0 + 8, :] = zr.astype(BF16)
                        zz_v[n, o, BLK + r0:BLK + r0 + 8, :] = zi.astype(BF16)

            nmac = sum(1 for o in outs for jj in range(j0, j1) if o >= jj)
            return (2 * nmac + ((0, GRP, 5 * GRP)[pi] if j1 == top else 0), gate_pl, run)

        items = []
        for pos in range(BLK // 8):
            for g0 in range(0, NB, GRP):
                top = g0 + GRP
                cuts = [0, top] if top <= SPLIT else [0, (top - 1) // 2, top]
                for pi in range(3):
                    for j0, j1 in zip(cuts[:-1], cuts[1:]):
                        items.append(mac_item(pos, g0, pi, j0, j1))

        nq = S // KG
        vpc = T // 8
        total = sum(c for c, _, _ in items)
        tap_of = []
        cum = 0
        for c, _, _ in items:
            tap_of.append(int(cum * NTAP / total))
            cum += c
        nxt = 0
        for r in range(NT):
            rs = slice(r * T, (r + 1) * T)
            hs = slice(r * T // 2, (r + 1) * T // 2)
            acc = None
            for q in range(nq):
                part = _dot(_up(wsp_v[hs, q * KG:(q + 1) * KG]),
                            _up(z232[n, q * KG // 2:(q + 1) * KG // 2, :]))
                acc = part if acc is None else acc + part
                t0 = (r * nq + q) * vpc
                while nxt < len(items) and tap_of[nxt] < t0 + vpc:
                    i = tap_of[nxt] - t0
                    items[nxt][1](acc[i * 8:(i + 1) * 8, :])
                    items[nxt][2]()
                    nxt += 1
            g = acc + bcol_v[rs, :]
            p_v[n, rs, :] = (z1_v[n, rs, :].astype(F32) * g).astype(BF16)
        assert nxt == len(items)
        return carry

    jax.lax.fori_loop(0, NC, p2, 0)

    wout_cp.wait()

    TPI = NT // P3I

    def p3(j, carry):
        inv_p = _up(tab_v[256:288, :])
        inv_m = _up(tab_v[288:320, :])
        rev = 7 - jax.lax.broadcasted_iota(jnp.int32, (8, 128), 0)

        def rows(t):
            r0 = (j * TPI + t) * T
            return (pl.ds(pl.multiple_of(r0, T), T),
                    pl.ds(pl.multiple_of(r0 // 2, T // 2), T // 2))

        def g5(t):
            rs, hs = rows(t)
            g = _dot(_up(wsp_v[hs, :]), _up(z232[NF - 1])) + bcol_v[rs, :]
            return (z1_v[NF - 1, rs, :].astype(F32) * g).astype(BF16)

        p5 = g5(0)
        for t in range(TPI):
            rs, hs = rows(t)
            p = jnp.concatenate([_up(p32[n, hs, :]) for n in range(NF - 1)] + [p5], axis=1)
            if t + 1 < TPI:
                p5 = g5(t + 1)
            for c in range(NC):
                cs = slice(c * 128, (c + 1) * 128)
                ye = _dot(inv_p, _up(zz32[c, j * TPI + t, 0:64, :]))
                yo = _dot(inv_m, _up(zz32[c, j * TPI + t, 64:128, :]))
                yd = ye - yo
                y = jnp.concatenate(
                    [ye + yo] + [
                        jnp.take_along_axis(yd[i * 8:(i + 1) * 8], rev, axis=0,
                                            mode="promise_in_bounds")
                        for i in reversed(range(BLK // 16))], axis=0)
                o = _dot(p, _up(wout_v[:, cs]))
                gate = o * (1.0 + jnp.tanh((0.25 / _A) * o))
                x = _up(x_v[0, hs, cs]).astype(F32)
                xn = xn_v[c, rs, :].astype(F32)
                o_v[rs, cs] = (x + (xn * y) * gate).astype(BF16)
                if t == TPI - 1 and c == NC - 2:
                    cp(o_v.at[rs, 0:512], out_hbm.at[0, rs, 0:512], out_sem).start()
            if t == TPI - 1:
                cp(o_v.at[rs, 512:D], out_hbm.at[0, rs, 512:D], out_sem).start()
            else:
                cp(o_v.at[rs, :], out_hbm.at[0, rs, :], out_sem).start()
        return carry

    jax.lax.fori_loop(0, P3I, p3, 0)
    cp(o_v, out_hbm.at[0], out_sem).wait()


@jax.jit
def pallas_recurrent_scan__ssm_conv_h3__mixer_gmlp__prompt_kernel(
    A_q: jax.Array,
    A_k: jax.Array,
    A_v: jax.Array,
    A_shift_k: jax.Array,
    A_ssm_k: jax.Array,
    A_ssm_D: jax.Array,
    B_x: jax.Array,
    B_w_in: jax.Array,
    B_w_sp: jax.Array,
    B_b_sp: jax.Array,
    B_w_out: jax.Array,
):
    del B_x
    tab = jnp.asarray(_dft_tables(), dtype=BF16)

    any_spec = pl.BlockSpec(memory_space=pl.ANY)
    return pl.pallas_call(
        _kernel,
        out_shape=jax.ShapeDtypeStruct((1, S, D), BF16),
        in_specs=[any_spec] * 11,
        out_specs=any_spec,
        scratch_shapes=[
            pltpu.VMEM((1, S // 2 + 32, D), U32),
            pltpu.VMEM((D // 2, 2 * FH), U32),
            pltpu.VMEM((S // 2, S), U32),
            pltpu.VMEM((FH // 2, D), U32),
            pltpu.VMEM((2 * NC, S // 2 + 32, 128), U32),
            pltpu.VMEM((NC, 64, S), U32),
            pltpu.VMEM((NC, S + 256, 128), BF16),
            pltpu.VMEM((NF, S, 128), BF16),
            pltpu.VMEM((NF, S, 128), BF16),
            pltpu.VMEM((NF - 1, S, 128), BF16),
            pltpu.VMEM((S, 128), BF16),
            pltpu.VMEM((BLK // 8, 6 * NB + 1, 8, 128), F32),
            pltpu.VMEM((NC, NB, 2 * BLK, 128), BF16),
            pltpu.VMEM((S, 128), F32),
            pltpu.VMEM((S, D), BF16),
            pltpu.VMEM((1, T + 16, FH), F32),
            pltpu.VMEM((1, T + 16, FH), F32),
            pltpu.VMEM((1, T + 16, FH), F32),
            pltpu.VMEM((T, 128), F32),
            pltpu.VMEM((320, 128), U32),
            pltpu.VMEM((NC, KS, 128), F32),
            pltpu.VMEM((NC + 2, 1, 128), F32),
            pltpu.VMEM((KS, D), BF16),
            pltpu.VMEM((D,), BF16),
            pltpu.VMEM((S,), BF16),
            pltpu.SMEM((1,), jnp.int32),
            pltpu.SemaphoreType.DMA((11,)),
        ],
        compiler_params=pltpu.CompilerParams(
            vmem_limit_bytes=100 * 1024 * 1024, disable_bounds_checks=True),
    )(A_q, A_k, A_v, A_shift_k.T, A_ssm_k, A_ssm_D, B_w_in, B_w_sp, B_b_sp, B_w_out, tab)
```

```python
import jax
import jax.numpy as jnp
import numpy as np
import jax.experimental.pallas as pl
import jax.experimental.pallas.tpu as pltpu

F32 = jnp.float32
BF16 = jnp.bfloat16
U32 = jnp.uint32

S = 2048
D = 640
FH = 768
KS = 4
BLK = 128
NB = S // BLK
NC = D // 128
NF = FH // 128
T = 128
NT = S // T
EPS = 1e-5
GRP = 4
SPLIT = 8
KG = 512
KR = 32
UA, UB, US, HP, HQ, HR, TOK = (i * NB for i in range(7))
TB = 4
LAG = 4
NTAP = 1016
P3I = 2

_GELU_C0 = float(np.sqrt(2.0 / np.pi))
_GELU_C1 = _GELU_C0 * 0.044715
_A = _GELU_C1 ** (1.0 / 3.0)
_K = _GELU_C0 / _A


def _dft_tables():
    m = np.arange(BLK)[:, None]
    n = np.arange(BLK)[None, :]
    th = 2.0 * np.pi * (((4 * m + 1) * n) % (4 * BLK)) / (4 * BLK)
    ph = 2.0 * np.pi * (((4 * m + 1) * (2 * n + 1)) % (8 * BLK)) / (8 * BLK)
    fu = np.concatenate([np.cos(ph), -np.sin(ph)], axis=0)
    fh = np.concatenate([np.cos(th) + np.sin(th), np.cos(th) - np.sin(th)], axis=0)
    fu, fh = (f.reshape(2, BLK // 8, 8, BLK).transpose(1, 0, 2, 3).reshape(2 * BLK, BLK)
              for f in (fu, fh))
    cp = (np.cos(ph) + np.sin(ph)).T[:BLK // 2] / (8.0 * BLK * _A * _A)
    cm = (np.cos(ph) - np.sin(ph)).T[:BLK // 2] / (8.0 * BLK * _A * _A)
    return np.concatenate([fu, fh, cp, cm], axis=0).astype(np.float32)


def _layernorm(x, eps, scale=1.0):
    m = jnp.mean(x, axis=-1, keepdims=True)
    d = x - m
    v = jnp.sum(d * d, axis=-1, keepdims=True) * (1.0 / (x.shape[-1] * scale * scale))
    return d * jax.lax.rsqrt(v + eps / (scale * scale))


def _gelu2(y):
    return y * (1.0 + jnp.tanh(y * (y * y + _K)))


def _up(x):
    return pltpu.bitcast(x, BF16)


def _dot(a, b):
    return jnp.dot(a, b, preferred_element_type=F32)


def _kernel(x_hbm, k_hbm, v_hbm, skt_hbm, h_hbm, dv_hbm, win_hbm, wsp_hbm, b_hbm,
            wout_hbm, tab_hbm, out_hbm,
            x_v, win_v, wsp_v, wout_v, kv_v, h_v, xn_v, z1_v, z2_v, p_v,
            kvb_v, pl_v, zz_v, bcol_v, o_v, zta_v, ztb_v, ztc_v, raw_v, tab_v,
            sk_v, dd_v, skt_v, dv_v, b_v, zero_s, sem):
    cp = pltpu.make_async_copy
    x16 = x_v.bitcast(BF16)
    win16 = win_v.bitcast(BF16)
    kv16 = kv_v.bitcast(BF16)
    h16 = h_v.bitcast(BF16)

    xn32, z232, p32, kvb32, zz32 = (
        r.bitcast(U32) for r in (xn_v, z2_v, p_v, kvb_v, zz_v))

    def x_cp(lo, hi, s):
        return cp(x_hbm.at[0, lo:hi, :], x16.at[0, lo:hi, :], sem.at[s])

    def win_cp(lo, hi, s):
        return cp(win_hbm.at[:, lo:hi], win16.at[:, lo:hi], sem.at[s])

    def k_cp(c, s):
        return cp(k_hbm.at[0, :, pl.ds(c * 128, 128)], kv16.at[2 * c, 0:S, :], sem.at[s])

    def v_cp(c, s):
        return cp(v_hbm.at[0, :, pl.ds(c * 128, 128)], kv16.at[2 * c + 1, 0:S, :], sem.at[s])

    def h_cp(c, s):
        return cp(h_hbm.at[pl.ds(c * 128, 128), :], h16.at[c], sem.at[s])

    groups = [
        [cp(b_hbm, b_v, sem.at[0]), cp(skt_hbm, skt_v, sem.at[0]), cp(dv_hbm, dv_v, sem.at[0])],
        [x_cp(0, 256, 1)],
        [win_cp(FH, FH + 256, 2)],
        [win_cp(FH + 256, FH + 512, 3)],
        [win_cp(FH + 512, 2 * FH, 4), win_cp(0, 128, 4)],
        [win_cp(128, 512, 11)],
        [win_cp(512, FH, 5), x_cp(256, 384, 5)],
        [x_cp(384, (TB + 2) * T, 6)],
        [x_cp((TB + 2) * T, S, 7), k_cp(0, 7), v_cp(0, 7)],
        [cp(tab_hbm, tab_v.bitcast(BF16), sem.at[8]), h_cp(0, 8),
         cp(wsp_hbm, wsp_v.bitcast(BF16), sem.at[8])],
    ]
    for g in groups:
        for c in g:
            c.start()

    def tile_cps(c):
        s = jnp.where(c == NC - 1, 9, c - 1) if isinstance(c, jax.Array) else (0, 1, 2, 9)[c - 1]
        return [k_cp(c, s), v_cp(c, s), h_cp(c, s)]

    wout_cp = cp(wout_hbm, wout_v.bitcast(BF16), sem.at[10])
    out_sem = sem.at[5]

    def wait(i):
        for c in groups[i]:
            c.wait()

    zero_s[0] = 0
    wait(0)
    skt = skt_v[...].astype(F32)
    dv = dv_v[...].astype(F32).reshape(1, D)
    for c in range(NC):
        sk_v[c] = skt[:, c * 128:(c + 1) * 128]
        dd_v[c] = dv[:, c * 128:(c + 1) * 128]
    brow = b_v[...].astype(F32).reshape(1, S)
    bcol_v[...] = jnp.broadcast_to(brow, (128, S)).T

    def gate_x(tok):
        x_v[0, S // 2:S // 2 + 8, 0:128] = pltpu.bitcast(tok, U32)

    zt_v = (zta_v, ztb_v, ztc_v)

    def gate_zt(t):
        def gate(tok):
            zt_v[t % 3][0, T:T + 8, 0:128] = tok
        return gate

    def gate_kv(tok):
        kv_v[0, S // 2:S // 2 + 8, :] = pltpu.bitcast(tok, U32)

    def gate_pl(tok):
        pl_v[0, TOK] = tok

    ndone = [0]

    def done(val):
        r = S + (ndone[0] % 16) * 16
        ndone[0] += 1
        xn_v[0, r:r + 16, :] = val

    def lnx_items(t, zero):
        def item(r0):
            def run():
                xw = x_v[zero, r0 // 2:r0 // 2 + 8, :]
                xn = _layernorm(_up(xw).astype(F32), EPS, _A)
                for c in range(NC):
                    xn_v[c, r0:r0 + 16, :] = xn[:, c * 128:(c + 1) * 128].astype(BF16)
            return (1, gate_x, run)
        return [item(t * T + g * 16) for g in range(T // 16)]

    def lnz_items(t, zero):
        def item(g):
            def run():
                z = zt_v[t % 3][zero, g * 16:(g + 1) * 16, :]
                z = _layernorm(z, 4.0 * _A * _A * EPS)
                r0 = t * T + g * 16
                for n in range(NF):
                    zb = z[:, n * 128:(n + 1) * 128].astype(BF16)
                    z2_v[n, r0:r0 + 16, :] = zb
                    if n == 0:
                        done(zb)
            return (1, gate_zt(t), run)
        return [item(g) for g in range(T // 16)]

    def kv_items(c):
        sk = sk_v[c]

        def item(r0):
            def run():
                hs = slice(r0 // 2, (r0 + KR) // 2)
                if r0 == 0:
                    kw = jnp.concatenate(
                        [jnp.zeros((8, 128), F32), _up(kv_v[2 * c, hs, :]).astype(F32)], axis=0)
                else:
                    kw = _up(kv_v[2 * c, r0 // 2 - 8:(r0 + KR) // 2, :]).astype(F32)[8:]
                ks = kw[8:] * sk[0:1, :]
                for t in range(1, KS):
                    ks = ks + pltpu.roll(kw, t, 0)[8:] * sk[t:t + 1, :]
                kvb_v[r0:r0 + KR, :] = (
                    ks * _up(kv_v[2 * c + 1, hs, :]).astype(F32)).astype(BF16)
            return (14 * KR // 8, gate_kv, run)
        return [item(r0) for r0 in range(0, S, KR)]

    def taps_of(val):
        rows, cols = val.shape
        return [(lambda i=i, n=n: val[i * 8:(i + 1) * 8, n * 128:(n + 1) * 128])
                for n in range(cols // 128) for i in range(rows // 8)]

    def activate(kind, t, n, z):
        if kind == 2:
            zt_v[t % 3][0, 0:T, n * 128:(n + 1) * 128] = _gelu2(z)
        else:
            z1_v[n, t * T:(t + 1) * T, :] = _gelu2(z).astype(BF16)

    def piece(kind, t, n, zero, defer=False, halves=False):
        col = n * 128 + (FH if kind == 2 else 0)
        xn = jnp.concatenate(
            [_up(xn32[zero if zero is not None and c == 0 else c,
                      t * T // 2:(t + 1) * T // 2, :]) for c in range(NC)], axis=1)
        w = _up(win_v[:, col:col + 128])
        if halves:
            z = jnp.concatenate([_dot(xn[:T // 2], w), _dot(xn[T // 2:], w)], axis=0)
        else:
            z = _dot(xn, w)
        if defer:
            raw_v[...] = z
        else:
            activate(kind, t, n, z)
        return taps_of(z)

    pending = []

    def block(pieces, work, defer=True, free=None):
        zero = zero_s[0]
        if pending:
            activate(*pending.pop(), raw_v[...])
        rel = [[] for _ in pieces]
        for mk, lo, hi in work:
            items = mk(zero)
            for i, it in enumerate(items):
                tau = (lo * 16) + (i * (hi - lo) * 16) // len(items)
                rel[tau // 16].append((tau % 16, it))
        taps = []
        gated = False
        for k in range(len(pieces) + LAG):
            if free is not None and k == len(pieces) - 1:
                for _, _, run in free(zero):
                    run()
                gated = True
            if k < len(pieces):
                last = defer and k == len(pieces) - 1
                halves = len(pieces) % 4 == 2 and k == len(pieces) - 1
                taps.append(piece(*pieces[k], zero if gated else None, last, halves))
                if last:
                    pending.append(pieces[k])
            if k >= LAG:
                for i, (_, gate, run) in sorted(rel[k - LAG], key=lambda e: e[0]):
                    gate(taps[k - LAG][i]())
                    run()
                    gated = True

    def cols(kind, t, lo=0, hi=NF):
        return [(kind, t, n) for n in range(lo, hi)]

    def lnx(t):
        return lambda zero: lnx_items(t, zero)

    def lnz(t):
        return lambda zero: lnz_items(t, zero)

    wait(1)
    for it in lnx_items(0, 0) + lnx_items(1, 0):
        it[2]()
    wait(2)
    block(cols(2, 0, 0, 2) + cols(2, 1, 0, 2), [])
    for c in range(1, NC):
        for d in tile_cps(c):
            d.start()
    wout_cp.start()
    wait(3)
    block(cols(2, 0, 2, 4) + cols(2, 1, 2, 4), [])
    wait(4)
    block(cols(2, 0, 4) + cols(2, 1, 4) + cols(1, 0, 0, 1) + cols(1, 1, 0, 1), [])
    wait(5)
    block(cols(1, 0, 1, 4) + cols(1, 1, 1, 4), [(lnz(0), 0, 1)])
    wait(6)
    block(cols(1, 0, 4) + cols(1, 1, 4), [], free=lnx(2))

    def end_pair(a):
        return cols(2, a) + cols(2, a + 1) + cols(1, a) + cols(1, a + 1)

    wait(7)
    block(cols(2, 2) + cols(1, 2) + end_pair(3),
          [(lnx(3), 0, 7), (lnz(1), 0, 12), (lnx(4), 7, 13), (lnz(2), 11, 20),
           (lnx(5), 13, 22), (lnz(3), 18, 26), (lnz(4), 24, 31)])
    wait(8)
    pieces, work = [], [(lnx(6), 0, 7)]
    for t in range(5, NT - 2):
        k = len(pieces)
        pieces += cols(2, t) + cols(1, t)
        work += [(lnx(t + 2), k + (7 if t == 5 else 3), k + (16 if t == 5 else 13 if t == NT - 3 else 15)),
                 (lnz(t), k + 6, k + 18)]
    k = len(pieces)
    pieces += end_pair(NT - 2)
    work += [(lnz(NT - 2), k + 6, k + 13), (lnz(NT - 1), k + 12, k + 19), (kv_items, 14, k + 24)]
    block(pieces, work, defer=False)

    wait(9)

    def p2(n, carry):
        nn = jnp.minimum(n + 1, NC - 1)

        @pl.when(n + 1 < NC)
        def _():
            for d in tile_cps(nn):
                d.wait()

        zero = zero_s[0]
        fwd_u = _up(tab_v[0:128, :])
        fwd_h = _up(tab_v[128:256, :])
        dd = dd_v[n]

        def put(slot, val):
            pl_v[:, slot] = val

        def re_im(val):
            val = val.reshape(BLK // 8, 2, 8, 128)
            return val[:, 0], val[:, 1]

        kvi = kv_items(nn)

        def pace_kv(d, val):
            if d % 4 == 3:
                for j in range(8):
                    _, gate, run = kvi[(d // 4) * 8 + j]
                    gate(val[j * 32:j * 32 + 8, :])
                    run()

        for i in range(NB):
            u = _dot(fwd_u, _up(kvb32[i * BLK // 2:(i + 1) * BLK // 2, :]))
            a, b = re_im(u)
            put(UA + i, a)
            put(UB + i, b)
            put(US + i, a + b)
            pace_kv(i, u)
        for i in range(NB):
            hb = _up(h_v[n, :, i * BLK:(i + 1) * BLK])
            hf = jax.lax.dot_general(fwd_h, hb, (((1,), (1,)), ((), ())),
                                     preferred_element_type=F32)
            c, d = re_im(hf)
            if i == 0:
                c, d = c + dd, d + dd
            put(HR + i, c)
            put(HP + i, d - c)
            put(HQ + i, c + d)
            pace_kv(NB + i, hf)

        state = {}

        def mac_item(pos, g0, pi, j0, j1):
            xv, hv = ((US, HR), (UA, HP), (UB, HQ))[pi]
            outs = range(g0, g0 + GRP)
            top = g0 + GRP

            def run():
                pz = zero + pos
                hs = {t: pl_v[pz, hv + t]
                      for t in range(max(g0 - j1 + 1, 0), top - j0)}
                acc = state['acc'] if j0 else {o: None for o in outs}
                for jj in range(j0, j1):
                    xj = pl_v[pz, xv + jj]
                    for o in outs:
                        if o - jj >= 0:
                            t = xj * hs[o - jj]
                            acc[o] = t if acc[o] is None else acc[o] + t
                if j1 < top:
                    state['acc'] = acc
                    return
                r0 = pos * 8
                if pi == 0:
                    state['k1'] = acc
                elif pi == 1:
                    state['im'] = {o: state['k1'][o] + acc[o] for o in outs}
                else:
                    for o in outs:
                        re, im = state['k1'][o] - acc[o], state['im'][o]
                        zr, zi = re, im
                        if o > 0:
                            zr, zi = re - state['prev'][1], im + state['prev'][0]
                        state['prev'] = (re, im)
                        zz_v[n, o, r0:r0 + 8, :] = zr.astype(BF16)
                        zz_v[n, o, BLK + r0:BLK + r0 + 8, :] = zi.astype(BF16)

            nmac = sum(1 for o in outs for jj in range(j0, j1) if o >= jj)
            return (2 * nmac + ((0, GRP, 5 * GRP)[pi] if j1 == top else 0), gate_pl, run)

        items = []
        for pos in range(BLK // 8):
            for g0 in range(0, NB, GRP):
                top = g0 + GRP
                cuts = [0, top] if top <= SPLIT else [0, (top - 1) // 2, top]
                for pi in range(3):
                    for j0, j1 in zip(cuts[:-1], cuts[1:]):
                        items.append(mac_item(pos, g0, pi, j0, j1))

        nq = S // KG
        vpc = T // 8
        total = sum(c for c, _, _ in items)
        tap_of = []
        cum = 0
        for c, _, _ in items:
            tap_of.append(int(cum * NTAP / total))
            cum += c
        nxt = 0
        for r in range(NT):
            rs = slice(r * T, (r + 1) * T)
            hs = slice(r * T // 2, (r + 1) * T // 2)
            acc = None
            for q in range(nq):
                part = _dot(_up(wsp_v[hs, q * KG:(q + 1) * KG]),
                            _up(z232[n, q * KG // 2:(q + 1) * KG // 2, :]))
                acc = part if acc is None else acc + part
                t0 = (r * nq + q) * vpc
                while nxt < len(items) and tap_of[nxt] < t0 + vpc:
                    i = tap_of[nxt] - t0
                    items[nxt][1](acc[i * 8:(i + 1) * 8, :])
                    items[nxt][2]()
                    nxt += 1
            g = acc + bcol_v[rs, :]
            p_v[n, rs, :] = (z1_v[n, rs, :].astype(F32) * g).astype(BF16)
        assert nxt == len(items)
        return carry

    jax.lax.fori_loop(0, NC, p2, 0)

    wout_cp.wait()

    TPI = NT // P3I

    def p3(j, carry):
        inv_p = _up(tab_v[256:288, :])
        inv_m = _up(tab_v[288:320, :])
        rev = 7 - jax.lax.broadcasted_iota(jnp.int32, (8, 128), 0)

        def rows(t):
            r0 = (j * TPI + t) * T
            return (pl.ds(pl.multiple_of(r0, T), T),
                    pl.ds(pl.multiple_of(r0 // 2, T // 2), T // 2))

        def g5(t):
            rs, hs = rows(t)
            g = _dot(_up(wsp_v[hs, :]), _up(z232[NF - 1])) + bcol_v[rs, :]
            return (z1_v[NF - 1, rs, :].astype(F32) * g).astype(BF16)

        p5 = g5(0)
        for t in range(TPI):
            rs, hs = rows(t)
            p = jnp.concatenate([_up(p32[n, hs, :]) for n in range(NF - 1)] + [p5], axis=1)
            if t + 1 < TPI:
                p5 = g5(t + 1)
            for c in range(NC):
                cs = slice(c * 128, (c + 1) * 128)
                ye = _dot(inv_p, _up(zz32[c, j * TPI + t, 0:64, :]))
                yo = _dot(inv_m, _up(zz32[c, j * TPI + t, 64:128, :]))
                yd = ye - yo
                y = jnp.concatenate(
                    [ye + yo] + [
                        jnp.take_along_axis(yd[i * 8:(i + 1) * 8], rev, axis=0,
                                            mode="promise_in_bounds")
                        for i in reversed(range(BLK // 16))], axis=0)
                o = _dot(p, _up(wout_v[:, cs]))
                gate = o * (1.0 + jnp.tanh((0.25 / _A) * o))
                x = _up(x_v[0, hs, cs]).astype(F32)
                xn = xn_v[c, rs, :].astype(F32)
                o_v[rs, cs] = (x + (xn * y) * gate).astype(BF16)
                if t == TPI - 1 and c == NC - 2:
                    cp(o_v.at[rs, 0:512], out_hbm.at[0, rs, 0:512], out_sem).start()
            if t == TPI - 1:
                cp(o_v.at[rs, 512:D], out_hbm.at[0, rs, 512:D], out_sem).start()
            else:
                cp(o_v.at[rs, :], out_hbm.at[0, rs, :], out_sem).start()
        return carry

    jax.lax.fori_loop(0, P3I, p3, 0)
    cp(o_v, out_hbm.at[0], out_sem).wait()


@jax.jit
def pallas_recurrent_scan__ssm_conv_h3__mixer_gmlp__prompt_kernel(
    A_q: jax.Array,
    A_k: jax.Array,
    A_v: jax.Array,
    A_shift_k: jax.Array,
    A_ssm_k: jax.Array,
    A_ssm_D: jax.Array,
    B_x: jax.Array,
    B_w_in: jax.Array,
    B_w_sp: jax.Array,
    B_b_sp: jax.Array,
    B_w_out: jax.Array,
):
    del B_x
    tab = jnp.asarray(_dft_tables(), dtype=BF16)

    any_spec = pl.BlockSpec(memory_space=pl.ANY)
    return pl.pallas_call(
        _kernel,
        out_shape=jax.ShapeDtypeStruct((1, S, D), BF16),
        in_specs=[any_spec] * 11,
        out_specs=any_spec,
        scratch_shapes=[
            pltpu.VMEM((1, S // 2 + 32, D), U32),
            pltpu.VMEM((D // 2, 2 * FH), U32),
            pltpu.VMEM((S // 2, S), U32),
            pltpu.VMEM((FH // 2, D), U32),
            pltpu.VMEM((2 * NC, S // 2 + 32, 128), U32),
            pltpu.VMEM((NC, 64, S), U32),
            pltpu.VMEM((NC, S + 256, 128), BF16),
            pltpu.VMEM((NF, S, 128), BF16),
            pltpu.VMEM((NF, S, 128), BF16),
            pltpu.VMEM((NF - 1, S, 128), BF16),
            pltpu.VMEM((S, 128), BF16),
            pltpu.VMEM((BLK // 8, 6 * NB + 1, 8, 128), F32),
            pltpu.VMEM((NC, NB, 2 * BLK, 128), BF16),
            pltpu.VMEM((S, 128), F32),
            pltpu.VMEM((S, D), BF16),
            pltpu.VMEM((1, T + 16, FH), F32),
            pltpu.VMEM((1, T + 16, FH), F32),
            pltpu.VMEM((1, T + 16, FH), F32),
            pltpu.VMEM((T, 128), F32),
            pltpu.VMEM((320, 128), U32),
            pltpu.VMEM((NC, KS, 128), F32),
            pltpu.VMEM((NC + 2, 1, 128), F32),
            pltpu.VMEM((KS, D), BF16),
            pltpu.VMEM((D,), BF16),
            pltpu.VMEM((S,), BF16),
            pltpu.SMEM((1,), jnp.int32),
            pltpu.SemaphoreType.DMA((12,)),
        ],
        compiler_params=pltpu.CompilerParams(
            vmem_limit_bytes=100 * 1024 * 1024, disable_bounds_checks=True),
    )(A_q, A_k, A_v, A_shift_k.T, A_ssm_k, A_ssm_D, B_w_in, B_w_sp, B_b_sp, B_w_out, tab)
```

```python
import jax
import jax.numpy as jnp
import numpy as np
import jax.experimental.pallas as pl
import jax.experimental.pallas.tpu as pltpu

F32 = jnp.float32
BF16 = jnp.bfloat16
U32 = jnp.uint32

S = 2048
D = 640
FH = 768
KS = 4
BLK = 128
NB = S // BLK
NC = D // 128
NF = FH // 128
T = 128
NT = S // T
EPS = 1e-5
GRP = 4
SPLIT = 8
KG = 512
KR = 32
UA, UB, US, HP, HQ, HR, TOK = (i * NB for i in range(7))
LAG = 4
NTAP = 888
HS = S // 2
HT = HS // T
HF = NF // 2
P3I = 2

_GELU_C0 = float(np.sqrt(2.0 / np.pi))
_GELU_C1 = _GELU_C0 * 0.044715
_A = _GELU_C1 ** (1.0 / 3.0)
_K = _GELU_C0 / _A


def _dft_tables():
    m = np.arange(BLK)[:, None]
    n = np.arange(BLK)[None, :]
    th = 2.0 * np.pi * (((4 * m + 1) * n) % (4 * BLK)) / (4 * BLK)
    ph = 2.0 * np.pi * (((4 * m + 1) * (2 * n + 1)) % (8 * BLK)) / (8 * BLK)
    fu = np.concatenate([np.cos(ph), -np.sin(ph)], axis=0)
    fh = np.concatenate([np.cos(th) + np.sin(th), np.cos(th) - np.sin(th)], axis=0)
    fu, fh = (f.reshape(2, BLK // 8, 8, BLK).transpose(1, 0, 2, 3).reshape(2 * BLK, BLK)
              for f in (fu, fh))
    cp = (np.cos(ph) + np.sin(ph)).T[:BLK // 2] / (8.0 * BLK * _A * _A)
    cm = (np.cos(ph) - np.sin(ph)).T[:BLK // 2] / (8.0 * BLK * _A * _A)
    return np.concatenate([fu, fh, cp, cm], axis=0).astype(np.float32)


def _layernorm(x, eps, scale=1.0):
    m = jnp.mean(x, axis=-1, keepdims=True)
    d = x - m
    v = jnp.sum(d * d, axis=-1, keepdims=True) * (1.0 / (x.shape[-1] * scale * scale))
    return d * jax.lax.rsqrt(v + eps / (scale * scale))


def _gelu2(y):
    return y * (1.0 + jnp.tanh(y * (y * y + _K)))


def _up(x):
    return pltpu.bitcast(x, BF16)


def _dot(a, b):
    return jnp.dot(a, b, preferred_element_type=F32)


def _kernel(x_hbm, k_hbm, v_hbm, skt_hbm, h_hbm, dv_hbm, win_hbm, wsp_hbm, b_hbm,
            wout_hbm, tab_hbm, out_hbm,
            x_v, win_v, wsp_v, wout_v, kv_v, h_v, xn_v, z1_v, z2_v, p_v, as_v, bs_v,
            kvb_v, pl_v, zz_v, bcol_v, o_v, zta_v, ztb_v, ztc_v, raw_v, tab_v,
            sk_v, dd_v, skt_v, dv_v, b_v, zero_s, sem):
    cp = pltpu.make_async_copy
    x16 = x_v.bitcast(BF16)
    win16 = win_v.bitcast(BF16)
    kv16 = kv_v.bitcast(BF16)
    h16 = h_v.bitcast(BF16)

    xn32, z232, p32, kvb32, zz32, as32, bs32 = (
        r.bitcast(U32) for r in (xn_v, z2_v, p_v, kvb_v, zz_v, as_v, bs_v))
    wsp16 = wsp_v.bitcast(BF16)

    def wsp_cp(lo, hi, s):
        return cp(wsp_hbm.at[lo:hi, :], wsp16.at[0, lo:hi, :], sem.at[s])

    def x_cp(lo, hi, s):
        return cp(x_hbm.at[0, lo:hi, :], x16.at[0, lo:hi, :], sem.at[s])

    def win_cp(lo, hi, s):
        return cp(win_hbm.at[:, lo:hi], win16.at[:, lo:hi], sem.at[s])

    def k_cp(c, s):
        return cp(k_hbm.at[0, :, pl.ds(c * 128, 128)], kv16.at[2 * c, 0:S, :], sem.at[s])

    def v_cp(c, s):
        return cp(v_hbm.at[0, :, pl.ds(c * 128, 128)], kv16.at[2 * c + 1, 0:S, :], sem.at[s])

    def h_cp(c, s):
        return cp(h_hbm.at[pl.ds(c * 128, 128), :], h16.at[c], sem.at[s])

    groups = [
        [cp(b_hbm, b_v, sem.at[0]), cp(skt_hbm, skt_v, sem.at[0]), cp(dv_hbm, dv_v, sem.at[0])],
        [x_cp(0, 256, 1)],
        [win_cp(FH, FH + 256, 2)],
        [win_cp(FH + 256, FH + 512, 3)],
        [win_cp(FH + 512, 2 * FH, 4), win_cp(0, 128, 4)],
        [win_cp(128, 512, 11)],
        [win_cp(512, FH, 5), x_cp(256, 384, 5)],
        [x_cp(384, 6 * T, 6)],
        [x_cp(6 * T, S, 7), k_cp(0, 7), v_cp(0, 7)],
        [wsp_cp(0, HS // 2, 12), wsp_cp(HS, HS + HS // 2, 12)],
        [wsp_cp(HS // 2, HS, 13), wsp_cp(HS + HS // 2, S, 13)],
        [cp(tab_hbm, tab_v.bitcast(BF16), sem.at[8]), h_cp(0, 8)],
    ]
    for g in groups:
        for c in g:
            c.start()

    def tile_cps(c):
        s = jnp.where(c == NC - 1, 9, c - 1) if isinstance(c, jax.Array) else (0, 1, 2, 9)[c - 1]
        return [k_cp(c, s), v_cp(c, s), h_cp(c, s)]

    wout_cp = cp(wout_hbm, wout_v.bitcast(BF16), sem.at[10])
    out_sem = sem.at[5]

    def wait(i):
        for c in groups[i]:
            c.wait()

    zero_s[0] = 0
    wait(0)
    skt = skt_v[...].astype(F32)
    dv = dv_v[...].astype(F32).reshape(1, D)
    for c in range(NC):
        sk_v[c] = skt[:, c * 128:(c + 1) * 128]
        dd_v[c] = dv[:, c * 128:(c + 1) * 128]
    brow = b_v[...].astype(F32).reshape(1, S)
    bcol_v[...] = jnp.broadcast_to(brow, (128, S)).T

    def gate_x(tok):
        x_v[0, S // 2:S // 2 + 8, 0:128] = pltpu.bitcast(tok, U32)

    zt_v = (zta_v, ztb_v, ztc_v)

    def gate_zt(t):
        def gate(tok):
            zt_v[t % 3][0, T:T + 8, 0:128] = tok
        return gate

    def gate_kv(tok):
        kv_v[0, S // 2:S // 2 + 8, :] = pltpu.bitcast(tok, U32)

    def gate_pl(tok):
        pl_v[0, TOK] = tok

    ndone = [0]

    def done(val):
        r = S + (ndone[0] % 16) * 16
        ndone[0] += 1
        xn_v[0, r:r + 16, :] = val

    def lnx_items(t, zero):
        def item(r0):
            def run():
                xw = x_v[zero, r0 // 2:r0 // 2 + 8, :]
                xn = _layernorm(_up(xw).astype(F32), EPS, _A)
                for c in range(NC):
                    xn_v[c, r0:r0 + 16, :] = xn[:, c * 128:(c + 1) * 128].astype(BF16)
            return (1, gate_x, run)
        return [item(t * T + g * 16) for g in range(T // 16)]

    def lnz_items(t, zero):
        def item(g):
            def run():
                z = zt_v[t % 3][zero, g * 16:(g + 1) * 16, :]
                z = _layernorm(z, 4.0 * _A * _A * EPS)
                r0 = t * T + g * 16
                zc = [z[:, n * 128:(n + 1) * 128] for n in range(NF)]
                if t < HT:
                    for n in range(NF):
                        z2_v[n, r0:r0 + 16, :] = zc[n].astype(BF16)
                else:
                    rs = slice(r0 - HS, r0 - HS + 16)
                    for n in range(HF):
                        b11 = z2_v[n, rs, :].astype(F32)
                        b12 = z2_v[n + HF, rs, :].astype(F32)
                        b21, b22 = zc[n], zc[n + HF]
                        z2_v[n + HF, r0:r0 + 16, :] = b22.astype(BF16)
                        for i, v in enumerate((b11 + b22, b12 - b22, b21 - b11,
                                               b11 + b12, b21 + b22)):
                            bs_v[i, n, rs, :] = v.astype(BF16)
                done(zc[NF - 1].astype(BF16))
            return (1, gate_zt(t), run)
        return [item(g) for g in range(T // 16)]

    def kv_items(c):
        sk = sk_v[c]

        def item(r0):
            def run():
                hs = slice(r0 // 2, (r0 + KR) // 2)
                if r0 == 0:
                    kw = jnp.concatenate(
                        [jnp.zeros((8, 128), F32), _up(kv_v[2 * c, hs, :]).astype(F32)], axis=0)
                else:
                    kw = _up(kv_v[2 * c, r0 // 2 - 8:(r0 + KR) // 2, :]).astype(F32)[8:]
                ks = kw[8:] * sk[0:1, :]
                for t in range(1, KS):
                    ks = ks + pltpu.roll(kw, t, 0)[8:] * sk[t:t + 1, :]
                kvb_v[r0:r0 + KR, :] = (
                    ks * _up(kv_v[2 * c + 1, hs, :]).astype(F32)).astype(BF16)
            return (14 * KR // 8, gate_kv, run)
        return [item(r0) for r0 in range(0, S, KR)]

    def gate_w(tok):
        wsp_v[0, S // 2:S // 2 + 8, 0:128] = pltpu.bitcast(tok, U32)

    def asum_items(r_lo, r_hi):
        def item(zero, r0, c0):
            def run():
                def quad(i, j, c):
                    w = wsp_v[zero, (i * HS + r0) // 2:(i * HS + r0) // 2 + 8,
                              j * HS + c * 128:j * HS + (c + 1) * 128]
                    return _up(w).astype(F32)
                for c in range(c0, c0 + 2):
                    a11, a12, a21, a22 = quad(0, 0, c), quad(0, 1, c), quad(1, 0, c), quad(1, 1, c)
                    for i, v in enumerate((a11 + a22, a21 + a22, a11 + a12,
                                           a21 - a11, a12 - a22)):
                        as_v[i, c, r0:r0 + 16, :] = v.astype(BF16)
            return (46, gate_w, run)
        return lambda zero: [item(zero, r0, c0) for r0 in range(r_lo * T, r_hi * T, 16)
                             for c0 in range(0, HT, 2)]

    def taps_of(val):
        rows, cols = val.shape
        return [(lambda i=i, n=n: val[i * 8:(i + 1) * 8, n * 128:(n + 1) * 128])
                for n in range(cols // 128) for i in range(rows // 8)]

    def activate(kind, t, n, z):
        if kind == 2:
            zt_v[t % 3][0, 0:T, n * 128:(n + 1) * 128] = _gelu2(z)
        else:
            z1_v[n, t * T:(t + 1) * T, :] = _gelu2(z).astype(BF16)

    def piece(kind, t, n, zero, defer=False, halves=False):
        col = n * 128 + (FH if kind == 2 else 0)
        xn = jnp.concatenate(
            [_up(xn32[zero if zero is not None and c == 0 else c,
                      t * T // 2:(t + 1) * T // 2, :]) for c in range(NC)], axis=1)
        w = _up(win_v[:, col:col + 128])
        if halves:
            z = jnp.concatenate([_dot(xn[:T // 2], w), _dot(xn[T // 2:], w)], axis=0)
        else:
            z = _dot(xn, w)
        if defer:
            raw_v[...] = z
        else:
            activate(kind, t, n, z)
        return taps_of(z)

    pending = []

    def block(pieces, work, defer=True, free=None):
        zero = zero_s[0]
        if pending:
            activate(*pending.pop(), raw_v[...])
        rel = [[] for _ in pieces]
        for mk, lo, hi in work:
            items = mk(zero)
            for i, it in enumerate(items):
                tau = (lo * 16) + (i * (hi - lo) * 16) // len(items)
                rel[tau // 16].append((tau % 16, it))
        taps = []
        gated = False
        for k in range(len(pieces) + LAG):
            if free is not None and k == len(pieces) - 1:
                for _, _, run in free(zero):
                    run()
                gated = True
            if k < len(pieces):
                last = defer and k == len(pieces) - 1
                halves = len(pieces) % 4 == 2 and k == len(pieces) - 1
                taps.append(piece(*pieces[k], zero if gated else None, last, halves))
                if last:
                    pending.append(pieces[k])
            if k >= LAG:
                for i, (_, gate, run) in sorted(rel[k - LAG], key=lambda e: e[0]):
                    gate(taps[k - LAG][i]())
                    run()
                    gated = True

    def cols(kind, t, lo=0, hi=NF):
        return [(kind, t, n) for n in range(lo, hi)]

    def lnx(t):
        return lambda zero: lnx_items(t, zero)

    def lnz(t):
        return lambda zero: lnz_items(t, zero)

    wait(1)
    for it in lnx_items(0, 0) + lnx_items(1, 0):
        it[2]()
    wait(2)
    block(cols(2, 0, 0, 2) + cols(2, 1, 0, 2), [])
    for c in range(1, NC):
        for d in tile_cps(c):
            d.start()
    wout_cp.start()
    wait(3)
    block(cols(2, 0, 2, 4) + cols(2, 1, 2, 4), [])
    wait(4)
    block(cols(2, 0, 4) + cols(2, 1, 4) + cols(1, 0, 0, 1) + cols(1, 1, 0, 1), [])
    wait(5)
    block(cols(1, 0, 1, 4) + cols(1, 1, 1, 4), [(lnz(0), 0, 1)])
    wait(6)
    block(cols(1, 0, 4) + cols(1, 1, 4), [], free=lnx(2))

    def end_pair(a):
        return cols(2, a) + cols(2, a + 1) + cols(1, a) + cols(1, a + 1)

    wait(7)
    block(cols(2, 2) + cols(1, 2) + end_pair(3),
          [(lnx(3), 0, 7), (lnz(1), 0, 12), (lnx(4), 7, 13), (lnz(2), 11, 20),
           (lnx(5), 13, 22), (lnz(3), 18, 26), (lnz(4), 24, 31)])

    def long_block(first, last, extra):
        pieces, work = [], [(lnx(first + 1), 0, 7)]
        for t in range(first, last - 1):
            k = len(pieces)
            pieces += cols(2, t) + cols(1, t)
            lo = k + (7 if t == first else 3)
            work += [(lnx(t + 2), lo, k + (13 if t == last - 2 else 16)), (lnz(t), k + 6, k + 18)]
        k = len(pieces)
        pieces += end_pair(last - 1)
        work += [(lnz(last - 1), k + 6, k + 13), (lnz(last), k + 12, k + 19), (extra, 0, k + 24)]
        if last + 1 < NT:
            work += [(lnx(last + 1), k + 1, k + 10)]
        block(pieces, work, defer=last + 1 < NT)

    wait(8)
    long_block(5, 8, kv_items)
    wait(9)
    long_block(9, 12, asum_items(0, HT // 2))
    wait(10)
    long_block(13, 15, asum_items(HT // 2, HT))
    wait(11)

    def unit(n, r, tap):
        top = pl.ds(pl.multiple_of(r * T, T), T)
        bot = pl.ds(pl.multiple_of(HS + r * T, T), T)
        toph = pl.ds(pl.multiple_of(r * (T // 2), T // 2), T // 2)
        both = pl.ds(pl.multiple_of((HS + r * T) // 2, T // 2), T // 2)

        def prod(lhs, rhs):
            acc = None
            for q in range(HS // KG):
                part = _dot(lhs(q), rhs(q))
                acc = part if acc is None else acc + part
                tap(acc)
            return acc

        def sa(i):
            return lambda q: jnp.concatenate(
                [_up(as32[i, c, toph, :]) for c in range(q * KG // 128, (q + 1) * KG // 128)],
                axis=1)

        def sb(i):
            return lambda q: _up(bs32[i, n, q * KG // 2:(q + 1) * KG // 2, :])

        def a11(q):
            return _up(wsp_v[0, toph, q * KG:(q + 1) * KG])

        def a22(q):
            return _up(wsp_v[0, both, HS + q * KG:HS + (q + 1) * KG])

        def b11(q):
            return _up(z232[n, q * KG // 2:(q + 1) * KG // 2, :])

        def b22(q):
            return _up(z232[n + HF, (HS + q * KG) // 2:(HS + (q + 1) * KG) // 2, :])

        def fin(col, rows, c):
            p_v[col, rows, :] = (z1_v[col, rows, :].astype(F32)
                                 * (c + bcol_v[rows, :])).astype(BF16)

        m2 = prod(sa(1), b11)
        m4 = prod(a22, sb(2))
        fin(n, bot, m2 + m4)
        m5 = prod(sa(2), b22)
        c11 = m4 - m5
        m3 = prod(a11, sb(1))
        fin(n + HF, top, m3 + m5)
        c22 = m3 - m2
        m1 = prod(sa(0), sb(0))
        c11, c22 = c11 + m1, c22 + m1
        fin(n, top, c11 + prod(sa(4), sb(4)))
        fin(n + HF, bot, c22 + prod(sa(3), sb(3)))

    def p2(n, carry):
        nn = jnp.minimum(n + 1, NC - 1)

        @pl.when(n + 1 < NC)
        def _():
            for d in tile_cps(nn):
                d.wait()

        zero = zero_s[0]
        fwd_u = _up(tab_v[0:128, :])
        fwd_h = _up(tab_v[128:256, :])
        dd = dd_v[n]

        def put(slot, val):
            pl_v[:, slot] = val

        def re_im(val):
            val = val.reshape(BLK // 8, 2, 8, 128)
            return val[:, 0], val[:, 1]

        kvi = kv_items(nn)

        def pace_kv(d, val):
            if d % 4 == 3:
                for j in range(8):
                    _, gate, run = kvi[(d // 4) * 8 + j]
                    gate(val[j * 32:j * 32 + 8, :])
                    run()

        for i in range(NB):
            u = _dot(fwd_u, _up(kvb32[i * BLK // 2:(i + 1) * BLK // 2, :]))
            a, b = re_im(u)
            put(UA + i, a)
            put(UB + i, b)
            put(US + i, a + b)
            pace_kv(i, u)
        for i in range(NB):
            hb = _up(h_v[n, :, i * BLK:(i + 1) * BLK])
            hf = jax.lax.dot_general(fwd_h, hb, (((1,), (1,)), ((), ())),
                                     preferred_element_type=F32)
            c, d = re_im(hf)
            if i == 0:
                c, d = c + dd, d + dd
            put(HR + i, c)
            put(HP + i, d - c)
            put(HQ + i, c + d)
            pace_kv(NB + i, hf)

        state = {}

        def mac_item(pos, g0, pi, j0, j1):
            xv, hv = ((US, HR), (UA, HP), (UB, HQ))[pi]
            outs = range(g0, g0 + GRP)
            top = g0 + GRP

            def run():
                pz = zero + pos
                hs = {t: pl_v[pz, hv + t]
                      for t in range(max(g0 - j1 + 1, 0), top - j0)}
                acc = state['acc'] if j0 else {o: None for o in outs}
                for jj in range(j0, j1):
                    xj = pl_v[pz, xv + jj]
                    for o in outs:
                        if o - jj >= 0:
                            t = xj * hs[o - jj]
                            acc[o] = t if acc[o] is None else acc[o] + t
                if j1 < top:
                    state['acc'] = acc
                    return
                r0 = pos * 8
                if pi == 0:
                    state['k1'] = acc
                elif pi == 1:
                    state['im'] = {o: state['k1'][o] + acc[o] for o in outs}
                else:
                    for o in outs:
                        re, im = state['k1'][o] - acc[o], state['im'][o]
                        zr, zi = re, im
                        if o > 0:
                            zr, zi = re - state['prev'][1], im + state['prev'][0]
                        state['prev'] = (re, im)
                        zz_v[n, o, r0:r0 + 8, :] = zr.astype(BF16)
                        zz_v[n, o, BLK + r0:BLK + r0 + 8, :] = zi.astype(BF16)

            nmac = sum(1 for o in outs for jj in range(j0, j1) if o >= jj)
            return (2 * nmac + ((0, GRP, 5 * GRP)[pi] if j1 == top else 0), gate_pl, run)

        items = []
        for pos in range(BLK // 8):
            for g0 in range(0, NB, GRP):
                top = g0 + GRP
                cuts = [0, top] if top <= SPLIT else [0, (top - 1) // 2, top]
                for pi in range(3):
                    for j0, j1 in zip(cuts[:-1], cuts[1:]):
                        items.append(mac_item(pos, g0, pi, j0, j1))

        total = sum(c for c, _, _ in items)
        tap_of = []
        cum = 0
        for c, _, _ in items:
            tap_of.append(int(cum * NTAP / total))
            cum += c
        pos = {'tap': 0, 'item': 0}

        def tap(acc):
            t0 = pos['tap']
            pos['tap'] += T // 8
            while pos['item'] < len(items) and tap_of[pos['item']] < pos['tap']:
                i = tap_of[pos['item']] - t0
                _, gate, run = items[pos['item']]
                gate(acc[i * 8:(i + 1) * 8, :])
                run()
                pos['item'] += 1

        for k in range(HT // 2):
            unit(n // 2, (n % 2) * (HT // 2) + k, tap)
        assert pos['item'] == len(items)
        return carry

    jax.lax.fori_loop(0, NC, p2, 0)

    wout_cp.wait()

    def p3(j, carry):
        inv_p = _up(tab_v[256:288, :])
        inv_m = _up(tab_v[288:320, :])
        rev = 7 - jax.lax.broadcasted_iota(jnp.int32, (8, 128), 0)

        tiles = [2 * j, 2 * j + 1, HT + 2 * j, HT + 2 * j + 1]
        tiles += [HT // 2 + t for t in tiles]
        order = ['u0', 0, 1, 'u1', 2, 3, 4, 6, 5, 7]
        for t in order:
            if t in ('u0', 'u1'):
                unit(HF - 1, HT // 2 + 2 * j + int(t[1]), lambda acc: None)
                continue
            tile = tiles[t]
            last = t == order[-1]
            rs = pl.ds(pl.multiple_of(tile * T, T), T)
            hs = pl.ds(pl.multiple_of(tile * (T // 2), T // 2), T // 2)
            p = jnp.concatenate([_up(p32[n, hs, :]) for n in range(NF)], axis=1)
            for c in range(NC):
                cs = slice(c * 128, (c + 1) * 128)
                ye = _dot(inv_p, _up(zz32[c, tile, 0:64, :]))
                yo = _dot(inv_m, _up(zz32[c, tile, 64:128, :]))
                yd = ye - yo
                y = jnp.concatenate(
                    [ye + yo] + [
                        jnp.take_along_axis(yd[i * 8:(i + 1) * 8], rev, axis=0,
                                            mode="promise_in_bounds")
                        for i in reversed(range(BLK // 16))], axis=0)
                o = _dot(p, _up(wout_v[:, cs]))
                gate = o * (1.0 + jnp.tanh((0.25 / _A) * o))
                x = _up(x_v[0, hs, cs]).astype(F32)
                xn = xn_v[c, rs, :].astype(F32)
                o_v[rs, cs] = (x + (xn * y) * gate).astype(BF16)
                if last and c == NC - 2:
                    cp(o_v.at[rs, 0:512], out_hbm.at[0, rs, 0:512], out_sem).start()
            if last:
                cp(o_v.at[rs, 512:D], out_hbm.at[0, rs, 512:D], out_sem).start()
            else:
                cp(o_v.at[rs, :], out_hbm.at[0, rs, :], out_sem).start()
        return carry

    jax.lax.fori_loop(0, P3I, p3, 0)
    cp(o_v, out_hbm.at[0], out_sem).wait()


@jax.jit
def pallas_recurrent_scan__ssm_conv_h3__mixer_gmlp__prompt_kernel(
    A_q: jax.Array,
    A_k: jax.Array,
    A_v: jax.Array,
    A_shift_k: jax.Array,
    A_ssm_k: jax.Array,
    A_ssm_D: jax.Array,
    B_x: jax.Array,
    B_w_in: jax.Array,
    B_w_sp: jax.Array,
    B_b_sp: jax.Array,
    B_w_out: jax.Array,
):
    del B_x
    tab = jnp.asarray(_dft_tables(), dtype=BF16)

    any_spec = pl.BlockSpec(memory_space=pl.ANY)
    return pl.pallas_call(
        _kernel,
        out_shape=jax.ShapeDtypeStruct((1, S, D), BF16),
        in_specs=[any_spec] * 11,
        out_specs=any_spec,
        scratch_shapes=[
            pltpu.VMEM((1, S // 2 + 32, D), U32),
            pltpu.VMEM((D // 2, 2 * FH), U32),
            pltpu.VMEM((1, S // 2 + 8, S), U32),
            pltpu.VMEM((FH // 2, D), U32),
            pltpu.VMEM((2 * NC, S // 2 + 32, 128), U32),
            pltpu.VMEM((NC, 64, S), U32),
            pltpu.VMEM((NC, S + 256, 128), BF16),
            pltpu.VMEM((NF, S, 128), BF16),
            pltpu.VMEM((NF, S, 128), BF16),
            pltpu.VMEM((NF, S, 128), BF16),
            pltpu.VMEM((5, HT, HS, 128), BF16),
            pltpu.VMEM((5, HF, HS, 128), BF16),
            pltpu.VMEM((S, 128), BF16),
            pltpu.VMEM((BLK // 8, 6 * NB + 1, 8, 128), F32),
            pltpu.VMEM((NC, NB, 2 * BLK, 128), BF16),
            pltpu.VMEM((S, 128), F32),
            pltpu.VMEM((S, D), BF16),
            pltpu.VMEM((1, T + 16, FH), F32),
            pltpu.VMEM((1, T + 16, FH), F32),
            pltpu.VMEM((1, T + 16, FH), F32),
            pltpu.VMEM((T, 128), F32),
            pltpu.VMEM((320, 128), U32),
            pltpu.VMEM((NC, KS, 128), F32),
            pltpu.VMEM((NC + 2, 1, 128), F32),
            pltpu.VMEM((KS, D), BF16),
            pltpu.VMEM((D,), BF16),
            pltpu.VMEM((S,), BF16),
            pltpu.SMEM((1,), jnp.int32),
            pltpu.SemaphoreType.DMA((14,)),
        ],
        compiler_params=pltpu.CompilerParams(
            vmem_limit_bytes=100 * 1024 * 1024, disable_bounds_checks=True),
    )(A_q, A_k, A_v, A_shift_k.T, A_ssm_k, A_ssm_D, B_w_in, B_w_sp, B_b_sp, B_w_out, tab)
```

```python
import jax
import jax.numpy as jnp
import numpy as np
import jax.experimental.pallas as pl
import jax.experimental.pallas.tpu as pltpu

F32 = jnp.float32
BF16 = jnp.bfloat16
U32 = jnp.uint32

S = 2048
D = 640
FH = 768
KS = 4
BLK = 128
NB = S // BLK
NC = D // 128
NF = FH // 128
T = 128
NT = S // T
EPS = 1e-5
GRP = 4
SPLIT = 8
import os
LX = int(os.environ.get('LX', 14))
KVS = int(os.environ.get('KVS', 64))
AW = int(os.environ.get('AW', 1))
KG = 512
KR = 32
UA, UB, US, HP, HQ, HR, TOK = (i * NB for i in range(7))
LAG = 4
NTAP = 888
HS = S // 2
HT = HS // T
HF = NF // 2
P3I = 2

_GELU_C0 = float(np.sqrt(2.0 / np.pi))
_GELU_C1 = _GELU_C0 * 0.044715
_A = _GELU_C1 ** (1.0 / 3.0)
_K = _GELU_C0 / _A


def _dft_tables():
    m = np.arange(BLK)[:, None]
    n = np.arange(BLK)[None, :]
    th = 2.0 * np.pi * (((4 * m + 1) * n) % (4 * BLK)) / (4 * BLK)
    ph = 2.0 * np.pi * (((4 * m + 1) * (2 * n + 1)) % (8 * BLK)) / (8 * BLK)
    fu = np.concatenate([np.cos(ph), -np.sin(ph)], axis=0)
    fh = np.concatenate([np.cos(th) + np.sin(th), np.cos(th) - np.sin(th)], axis=0)
    fu, fh = (f.reshape(2, BLK // 8, 8, BLK).transpose(1, 0, 2, 3).reshape(2 * BLK, BLK)
              for f in (fu, fh))
    cp = (np.cos(ph) + np.sin(ph)).T[:BLK // 2] / (8.0 * BLK * _A * _A)
    cm = (np.cos(ph) - np.sin(ph)).T[:BLK // 2] / (8.0 * BLK * _A * _A)
    return np.concatenate([fu, fh, cp, cm], axis=0).astype(np.float32)


def _layernorm(x, eps, scale=1.0):
    m = jnp.mean(x, axis=-1, keepdims=True)
    d = x - m
    v = jnp.sum(d * d, axis=-1, keepdims=True) * (1.0 / (x.shape[-1] * scale * scale))
    return d * jax.lax.rsqrt(v + eps / (scale * scale))


def _gelu2(y):
    return y * (1.0 + jnp.tanh(y * (y * y + _K)))


def _up(x):
    return pltpu.bitcast(x, BF16)


def _dot(a, b):
    return jnp.dot(a, b, preferred_element_type=F32)


def _lhs_sums(a11, a12, a21, a22):
    return a11 + a22, a21 + a22, a11 + a12, a21 - a11, a12 - a22


def _rhs_sums(b11, b12, b21, b22):
    return b11 + b22, b12 - b22, b21 - b11, b11 + b12, b21 + b22


def _strassen(prod, sa, sb, a11, a22, b11, b22, fin):
    m2 = prod(sa(1), b11)
    m4 = prod(a22, sb(2))
    fin(1, 0, m2 + m4)
    m5 = prod(sa(2), b22)
    c11 = m4 - m5
    m3 = prod(a11, sb(1))
    fin(0, 1, m3 + m5)
    c22 = m3 - m2
    m1 = prod(sa(0), sb(0))
    c11, c22 = c11 + m1, c22 + m1
    fin(0, 0, c11 + prod(sa(4), sb(4)))
    fin(1, 1, c22 + prod(sa(3), sb(3)))


def _balance(work, n):
    queues = []
    for items, lo, hi in work:
        if items:
            queues.append([(lo * 16, hi * 16 - 1 - 2 * (len(items) - 1 - i), it)
                           for i, it in enumerate(items)])
    if not queues:
        return [[] for _ in range(n)]

    def simulate(rate):
        qs = [list(q) for q in queues]
        rel = [[] for _ in range(n)]
        budget, late = 0.0, 0
        for tau in range(n * 16):
            budget = min(budget + rate, 100.0)
            while True:
                ready = [q for q in qs if q and q[0][0] <= tau]
                if not ready:
                    break
                q = min(ready, key=lambda q: (q[-1][1], q[0][1]))
                forced = [q2 for q2 in ready if q2[0][1] <= tau]
                if forced:
                    q = forced[0]
                    late += budget < 0
                elif budget < 0:
                    break
                it = q.pop(0)[2]
                rel[tau // 16].append((tau % 16, it))
                budget -= it[0]
        assert not any(qs)
        return late, rel

    rate = sum(e[2][0] for q in queues for e in q) / (16.0 * n)
    while True:
        late, rel = simulate(rate)
        if not late:
            return rel
        rate *= 1.02


def _kernel(x_hbm, k_hbm, v_hbm, skt_hbm, h_hbm, dv_hbm, win_hbm, wsp_hbm, b_hbm,
            wout_hbm, tab_hbm, out_hbm,
            x_v, win_v, wsp_v, wout_v, kv_v, h_v, xn_v, z1_v, z2_v, p_v, as_v, bs_v, pq_v, ps_v, ws_v,
            kvb_v, pl_v, zz_v, bcol_v, o_v, zta_v, ztb_v, ztc_v, raw_v, tab_v,
            sk_v, dd_v, skt_v, dv_v, b_v, zero_s, sem):
    cp = pltpu.make_async_copy
    x16 = x_v.bitcast(BF16)
    win16 = win_v.bitcast(BF16)
    kv16 = kv_v.bitcast(BF16)
    h16 = h_v.bitcast(BF16)

    xn32, z232, p32, kvb32, zz32, as32, bs32, pq32, ps32, ws32 = (
        r.bitcast(U32)
        for r in (xn_v, z2_v, p_v, kvb_v, zz_v, as_v, bs_v, pq_v, ps_v, ws_v))
    wsp16 = wsp_v.bitcast(BF16)

    def wsp_cp(lo, hi, s):
        return cp(wsp_hbm.at[lo:hi, :], wsp16.at[0, lo:hi, :], sem.at[s])

    def x_cp(lo, hi, s):
        return cp(x_hbm.at[0, lo:hi, :], x16.at[0, lo:hi, :], sem.at[s])

    def win_cp(lo, hi, s):
        return cp(win_hbm.at[:, lo:hi], win16.at[:, lo:hi], sem.at[s])

    def k_cp(c, s):
        return cp(k_hbm.at[0, :, pl.ds(c * 128, 128)], kv16.at[2 * c, 0:S, :], sem.at[s])

    def v_cp(c, s):
        return cp(v_hbm.at[0, :, pl.ds(c * 128, 128)], kv16.at[2 * c + 1, 0:S, :], sem.at[s])

    def h_cp(c, s):
        return cp(h_hbm.at[pl.ds(c * 128, 128), :], h16.at[c], sem.at[s])

    groups = [
        [cp(b_hbm, b_v, sem.at[0]), cp(skt_hbm, skt_v, sem.at[0]), cp(dv_hbm, dv_v, sem.at[0])],
        [x_cp(0, 256, 1)],
        [win_cp(FH, FH + 256, 2)],
        [win_cp(FH + 256, FH + 512, 3)],
        [win_cp(FH + 512, 2 * FH, 4), win_cp(0, 128, 4)],
        [win_cp(128, 512, 11)],
        [win_cp(512, FH, 5), x_cp(256, 384, 5)],
        [x_cp(384, 6 * T, 6)],
        [x_cp(6 * T, S, 7), k_cp(0, 7), v_cp(0, 7)],
        [wsp_cp(0, HS // 2, 12), wsp_cp(HS, HS + HS // 2, 12)],
        [wsp_cp(HS // 2, HS, 13), wsp_cp(HS + HS // 2, S, 13)],
        [cp(tab_hbm, tab_v.bitcast(BF16), sem.at[8]), h_cp(0, 8)],
    ]
    for g in groups:
        for c in g:
            c.start()

    def tile_cps(c):
        s = jnp.where(c == NC - 1, 9, c - 1) if isinstance(c, jax.Array) else (0, 1, 2, 9)[c - 1]
        return [k_cp(c, s), v_cp(c, s), h_cp(c, s)]

    wout_cp = cp(wout_hbm, wout_v.bitcast(BF16).at[0, 0:FH, :], sem.at[10])
    out_sem = sem.at[5]

    def wait(i):
        for c in groups[i]:
            c.wait()

    zero_s[0] = 0
    wait(0)
    skt = skt_v[...].astype(F32)
    dv = dv_v[...].astype(F32).reshape(1, D)
    for c in range(NC):
        sk_v[c] = skt[:, c * 128:(c + 1) * 128]
        dd_v[c] = dv[:, c * 128:(c + 1) * 128]
    brow = b_v[...].astype(F32).reshape(1, S)
    bcol_v[...] = jnp.broadcast_to(brow, (128, S)).T

    def gate_x(tok):
        x_v[0, S // 2:S // 2 + 8, 0:128] = pltpu.bitcast(tok, U32)

    zt_v = (zta_v, ztb_v, ztc_v)

    def gate_zt(t):
        def gate(tok):
            zt_v[t % 3][0, T:T + 8, 0:128] = tok
        return gate

    def gate_kv(tok):
        kv_v[0, S // 2:S // 2 + 8, :] = pltpu.bitcast(tok, U32)

    def gate_pl(tok):
        pl_v[0, TOK] = tok

    ndone = [0]

    def done(val):
        r = S + (ndone[0] % 16) * 16
        ndone[0] += 1
        xn_v[0, r:r + 16, :] = val

    def lnx_items(t, zero):
        def item(r0):
            def run():
                xw = x_v[zero, r0 // 2:r0 // 2 + 8, :]
                xn = _layernorm(_up(xw).astype(F32), EPS, _A)
                for c in range(NC):
                    xn_v[c, r0:r0 + 16, :] = xn[:, c * 128:(c + 1) * 128].astype(BF16)
            return (85, gate_x, run)
        return [item(t * T + g * 16) for g in range(T // 16)]

    def lnz_items(t, zero):
        def item(g):
            def run():
                z = zt_v[t % 3][zero, g * 16:(g + 1) * 16, :]
                z = _layernorm(z, 4.0 * _A * _A * EPS)
                r0 = t * T + g * 16
                for n in range(NF):
                    zb = z[:, n * 128:(n + 1) * 128].astype(BF16)
                    z2_v[n, r0:r0 + 16, :] = zb
                done(zb)
            return (90, gate_zt(t), run)
        return [item(g) for g in range(T // 16)]

    def kv_items(c):
        sk = sk_v[c]

        def item(r0):
            def run():
                hs = slice(r0 // 2, (r0 + KR) // 2)
                if r0 == 0:
                    kw = jnp.concatenate(
                        [jnp.zeros((8, 128), F32), _up(kv_v[2 * c, hs, :]).astype(F32)], axis=0)
                else:
                    kw = _up(kv_v[2 * c, r0 // 2 - 8:(r0 + KR) // 2, :]).astype(F32)[8:]
                ks = kw[8:] * sk[0:1, :]
                for t in range(1, KS):
                    ks = ks + pltpu.roll(kw, t, 0)[8:] * sk[t:t + 1, :]
                kvb_v[r0:r0 + KR, :] = (
                    ks * _up(kv_v[2 * c + 1, hs, :]).astype(F32)).astype(BF16)
            return (14 * KR // 8, gate_kv, run)
        return [item(r0) for r0 in range(0, S, KR)]

    def gate_w(tok):
        wsp_v[0, S // 2:S // 2 + 8, 0:128] = pltpu.bitcast(tok, U32)

    def asum_items(r_lo, r_hi):
        def item(zero, r0, c0):
            def run():
                def quad(i, j, c):
                    w = wsp_v[zero, (i * HS + r0) // 2:(i * HS + r0) // 2 + 8,
                              j * HS + c * 128:j * HS + (c + 1) * 128]
                    return _up(w).astype(F32)
                for c in range(c0, c0 + AW):
                    for i, v in enumerate(_lhs_sums(
                            quad(0, 0, c), quad(0, 1, c), quad(1, 0, c), quad(1, 1, c))):
                        as_v[i, c, r0:r0 + 16, :] = v.astype(BF16)
            return (23 * AW, gate_w, run)
        return lambda zero: [item(zero, r0, c0) for r0 in range(r_lo * T, r_hi * T, 16)
                             for c0 in range(0, HT, AW)]

    def gate_z2(tok):
        z2_v[0, S:S + 8, :] = tok.astype(BF16)

    def bsum(t):
        def item(zero, r0, n):
            def run():
                def quad(i, j):
                    return z2_v[zero + n + j * HF, i * HS + r0:i * HS + r0 + 16, :].astype(F32)
                for i, v in enumerate(_rhs_sums(quad(0, 0), quad(0, 1), quad(1, 0), quad(1, 1))):
                    bs_v[i, n, r0:r0 + 16, :] = v.astype(BF16)
            return (24, gate_z2, run)
        return lambda zero: [item(zero, r0, n) for r0 in range((t - HT) * T, (t - HT + 1) * T, 16)
                             for n in range(HF)]

    def taps_of(val):
        rows, cols = val.shape
        return [(lambda i=i, n=n: val[i * 8:(i + 1) * 8, n * 128:(n + 1) * 128])
                for n in range(cols // 128) for i in range(rows // 8)]

    def activate(kind, t, n, z):
        if kind == 2:
            zt_v[t % 3][0, 0:T, n * 128:(n + 1) * 128] = _gelu2(z)
        else:
            z1_v[n, t * T:(t + 1) * T, :] = _gelu2(z).astype(BF16)

    def piece(kind, t, n, zero, defer=False, halves=False):
        col = n * 128 + (FH if kind == 2 else 0)
        xn = jnp.concatenate(
            [_up(xn32[zero if zero is not None and c == 0 else c,
                      t * T // 2:(t + 1) * T // 2, :]) for c in range(NC)], axis=1)
        w = _up(win_v[:, col:col + 128])
        if halves:
            z = jnp.concatenate([_dot(xn[:T // 2], w), _dot(xn[T // 2:], w)], axis=0)
        else:
            z = _dot(xn, w)
        if defer:
            raw_v[...] = z
        else:
            activate(kind, t, n, z)
        return taps_of(z)

    pending = []

    def block(pieces, work, defer=True, free=None):
        zero = zero_s[0]
        if pending:
            activate(*pending.pop(), raw_v[...])
        rel = _balance([(mk(zero), lo, hi) for mk, lo, hi in work], len(pieces))
        taps = []
        gated = False
        for k in range(len(pieces) + LAG):
            if free is not None and k == len(pieces) - 1:
                for _, _, run in free(zero):
                    run()
                gated = True
            if k < len(pieces):
                last = defer and k == len(pieces) - 1
                halves = len(pieces) % 4 == 2 and k == len(pieces) - 1
                taps.append(piece(*pieces[k], zero if gated else None, last, halves))
                if last:
                    pending.append(pieces[k])
            if k >= LAG:
                for i, (_, gate, run) in sorted(rel[k - LAG], key=lambda e: e[0]):
                    gate(taps[k - LAG][i]())
                    run()
                    gated = True

    def cols(kind, t, lo=0, hi=NF):
        return [(kind, t, n) for n in range(lo, hi)]

    def lnx(t):
        return lambda zero: lnx_items(t, zero)

    def lnz(t):
        return lambda zero: lnz_items(t, zero)

    wait(1)
    for it in lnx_items(0, 0) + lnx_items(1, 0):
        it[2]()
    wait(2)
    block(cols(2, 0, 0, 2) + cols(2, 1, 0, 2), [])
    for c in range(1, NC):
        for d in tile_cps(c):
            d.start()
    wout_cp.start()
    wait(3)
    block(cols(2, 0, 2, 4) + cols(2, 1, 2, 4), [])
    wait(4)
    block(cols(2, 0, 4) + cols(2, 1, 4) + cols(1, 0, 0, 1) + cols(1, 1, 0, 1), [])
    wait(5)
    block(cols(1, 0, 1, 4) + cols(1, 1, 1, 4), [(lnz(0), 0, 1)])
    wait(6)
    block(cols(1, 0, 4) + cols(1, 1, 4), [], free=lnx(2))

    def tiles(lo, hi):
        return [pc for t in range(lo, hi) for pc in cols(2, t) + cols(1, t)]

    def end_pair(a):
        return cols(2, a) + cols(2, a + 1) + cols(1, a) + cols(1, a + 1)

    def part(mk, lo, hi):
        return lambda zero: mk(zero)[lo:hi]

    wait(7)
    block(tiles(2, 5),
          [(lnx(3), 0, 7), (lnx(4), 0, 19), (lnx(5), 0, 31),
           (lnz(1), 0, 20), (lnz(2), 6, 31), (lnz(3), 18, 31)])
    wait(8)
    block(tiles(5, 9),
          [(lnx(6), 0, 7), (lnx(7), 0, 19), (lnx(8), 0, 31)]
          + [(lnx(t), 0, 43) for t in range(9, LX)]
          + [(lnz(4), 0, 20), (lnz(5), 6, 32), (lnz(6), 18, 43), (lnz(7), 30, 43),
             (part(kv_items, 0, KVS), 0, 48)])
    wait(9)
    block(tiles(9, 13),
          [(lnx(t), 0, 43) for t in range(LX, NT)]
          + [(lnz(8), 0, 12), (lnz(9), 6, 24), (lnz(10), 18, 36), (lnz(11), 30, 43),
             (bsum(8), 17, 48), (bsum(9), 29, 48), (bsum(10), 41, 48),
             (part(kv_items, KVS, 64), 0, 48), (asum_items(0, HT // 2), 0, 48)])
    wait(10)
    block(cols(2, 13) + cols(2, 14) + cols(1, 13) + cols(2, 15) + cols(1, 14) + cols(1, 15),
          [(lnz(12), 0, 6), (lnz(13), 6, 12), (lnz(14), 12, 18), (lnz(15), 24, 26),
           (bsum(11), 0, 36), (bsum(12), 11, 36), (bsum(13), 17, 36), (bsum(14), 23, 36),
           (bsum(15), 31, 36), (asum_items(HT // 2, HT), 0, 36)], defer=False)
    wait(11)

    def unit(n, r, tap, put_p):
        top = pl.ds(pl.multiple_of(r * T, T), T)
        bot = pl.ds(pl.multiple_of(HS + r * T, T), T)
        toph = pl.ds(pl.multiple_of(r * (T // 2), T // 2), T // 2)
        both = pl.ds(pl.multiple_of((HS + r * T) // 2, T // 2), T // 2)

        def prod(lhs, rhs):
            acc = None
            for q in range(HS // KG):
                part = _dot(lhs(q), rhs(q))
                acc = part if acc is None else acc + part
                tap(acc)
            return acc

        def sa(i):
            return lambda q: jnp.concatenate(
                [_up(as32[i, c, toph, :]) for c in range(q * KG // 128, (q + 1) * KG // 128)],
                axis=1)

        def sb(i):
            return lambda q: _up(bs32[i, n, q * KG // 2:(q + 1) * KG // 2, :])

        def a11(q):
            return _up(wsp_v[0, toph, q * KG:(q + 1) * KG])

        def a22(q):
            return _up(wsp_v[0, both, HS + q * KG:HS + (q + 1) * KG])

        def b11(q):
            return _up(z232[n, q * KG // 2:(q + 1) * KG // 2, :])

        def b22(q):
            return _up(z232[n + HF, (HS + q * KG) // 2:(HS + (q + 1) * KG) // 2, :])

        def fin(i, j, c):
            col, rows = n + j * HF, (top, bot)[i]
            put_p(i, j, col, rows,
                  (z1_v[col, rows, :].astype(F32) * (c + bcol_v[rows, :])).astype(BF16))

        _strassen(prod, sa, sb, a11, a22, b11, b22, fin)

    def p2(n, carry):
        nn = jnp.minimum(n + 1, NC - 1)

        @pl.when(n + 1 < NC)
        def _():
            for d in tile_cps(nn):
                d.wait()

        zero = zero_s[0]
        fwd_u = _up(tab_v[0:128, :])
        fwd_h = _up(tab_v[128:256, :])
        dd = dd_v[n]

        def put(slot, val):
            pl_v[:, slot] = val

        def re_im(val):
            val = val.reshape(BLK // 8, 2, 8, 128)
            return val[:, 0], val[:, 1]

        kvi = kv_items(nn)

        def pace_kv(d, val):
            if d % 4 == 3:
                for j in range(8):
                    _, gate, run = kvi[(d // 4) * 8 + j]
                    gate(val[j * 32:j * 32 + 8, :])
                    run()

        for i in range(NB):
            u = _dot(fwd_u, _up(kvb32[i * BLK // 2:(i + 1) * BLK // 2, :]))
            a, b = re_im(u)
            put(UA + i, a)
            put(UB + i, b)
            put(US + i, a + b)
            pace_kv(i, u)
        for i in range(NB):
            hb = _up(h_v[n, :, i * BLK:(i + 1) * BLK])
            hf = jax.lax.dot_general(fwd_h, hb, (((1,), (1,)), ((), ())),
                                     preferred_element_type=F32)
            c, d = re_im(hf)
            if i == 0:
                c, d = c + dd, d + dd
            put(HR + i, c)
            put(HP + i, d - c)
            put(HQ + i, c + d)
            pace_kv(NB + i, hf)

        state = {}

        def mac_item(pos, g0, pi, j0, j1):
            xv, hv = ((US, HR), (UA, HP), (UB, HQ))[pi]
            outs = range(g0, g0 + GRP)
            top = g0 + GRP

            def run():
                pz = zero + pos
                hs = {t: pl_v[pz, hv + t]
                      for t in range(max(g0 - j1 + 1, 0), top - j0)}
                acc = state['acc'] if j0 else {o: None for o in outs}
                for jj in range(j0, j1):
                    xj = pl_v[pz, xv + jj]
                    for o in outs:
                        if o - jj >= 0:
                            t = xj * hs[o - jj]
                            acc[o] = t if acc[o] is None else acc[o] + t
                if j1 < top:
                    state['acc'] = acc
                    return
                r0 = pos * 8
                if pi == 0:
                    state['k1'] = acc
                elif pi == 1:
                    state['im'] = {o: state['k1'][o] + acc[o] for o in outs}
                else:
                    for o in outs:
                        re, im = state['k1'][o] - acc[o], state['im'][o]
                        zr, zi = re, im
                        if o > 0:
                            zr, zi = re - state['prev'][1], im + state['prev'][0]
                        state['prev'] = (re, im)
                        zz_v[n, o, r0:r0 + 8, :] = zr.astype(BF16)
                        zz_v[n, o, BLK + r0:BLK + r0 + 8, :] = zi.astype(BF16)

            nmac = sum(1 for o in outs for jj in range(j0, j1) if o >= jj)
            return (2 * nmac + ((0, GRP, 5 * GRP)[pi] if j1 == top else 0), gate_pl, run)

        items = []
        for pos in range(BLK // 8):
            for g0 in range(0, NB, GRP):
                top = g0 + GRP
                cuts = [0, top] if top <= SPLIT else [0, (top - 1) // 2, top]
                for pi in range(3):
                    for j0, j1 in zip(cuts[:-1], cuts[1:]):
                        items.append(mac_item(pos, g0, pi, j0, j1))

        total = sum(c for c, _, _ in items)
        tap_of = []
        cum = 0
        for c, _, _ in items:
            tap_of.append(int(cum * NTAP / total))
            cum += c
        pos = {'tap': 0, 'item': 0}

        def tap(acc):
            t0 = pos['tap']
            pos['tap'] += T // 8
            while pos['item'] < len(items) and tap_of[pos['item']] < pos['tap']:
                i = tap_of[pos['item']] - t0
                _, gate, run = items[pos['item']]
                gate(acc[i * 8:(i + 1) * 8, :])
                run()
                pos['item'] += 1

        def put_p(i, j, col, rows, val):
            p_v[col, rows, :] = val

        for k in range(HT // 2):
            unit(n // 2, (n % 2) * (HT // 2) + k, tap, put_p)
        assert pos['item'] == len(items)
        return carry

    jax.lax.fori_loop(0, NC, p2, 0)

    wout_cp.wait()

    def p3(j, carry):
        inv_p = _up(tab_v[256:288, :])
        inv_m = _up(tab_v[288:320, :])
        rev = 7 - jax.lax.broadcasted_iota(jnp.int32, (8, 128), 0)

        zero = zero_s[0]
        HK = FH // 2

        def rows(k, i):
            tile = i * HT + (k // 2) * (HT // 2) + 2 * j + k % 2
            return (tile, pl.ds(pl.multiple_of(tile * T, T), T),
                    pl.ds(pl.multiple_of(tile * (T // 2), T // 2), T // 2))

        def fresh(k, n):
            return k >= 2 and n % HF == HF - 1

        def p_tile(k, i, n):
            if fresh(k, n):
                return _up(pq32[k - 2, i, n // HF])
            return _up(p32[n, rows(k, i)[2], :])

        def gate_p(tok):
            p_v[0, S:S + 8, :] = tok.astype(BF16)

        def gate_wo(tok):
            wout_v[0, HK:HK + 8, 0:128] = pltpu.bitcast(tok, U32)

        def psum_item(k, n, g):
            def run():
                def quad(i, jj):
                    if fresh(k, n):
                        return pq_v[k - 2, i, jj, g * 16:(g + 1) * 16, :].astype(F32)
                    r0 = pl.multiple_of(rows(k, i)[0] * T + g * 16, 16)
                    return p_v[n + jj * HF, pl.ds(r0, 16), :].astype(F32)
                for i, v in enumerate(_lhs_sums(quad(0, 0), quad(0, 1), quad(1, 0), quad(1, 1))):
                    ps_v[k, i, n, g * 16:(g + 1) * 16, :] = v.astype(BF16)
            return (gate_p, run)

        def wsum_item(m, g):
            def run():
                def quad(i, jj):
                    r0 = (i * HK + g * 16) // 2
                    c0 = (m + 2 * jj) * 128
                    return _up(wout_v[zero, r0:r0 + 8, c0:c0 + 128]).astype(F32)
                for i, v in enumerate(_rhs_sums(quad(0, 0), quad(0, 1), quad(1, 0), quad(1, 1))):
                    ws_v[i, m, g * 16:(g + 1) * 16, :] = v.astype(BF16)
            return (gate_wo, run)

        def psum(k):
            return [psum_item(k, n, g) for n in range(HF) if not fresh(k, n)
                    for g in range(T // 16)]

        queue = []

        def tap(val):
            for i in range(min(len(queue), queue_step[0])):
                gate, run = queue.pop(0)
                r = (i * (T // 8)) // queue_step[0] * 8
                gate(val[r:r + 8, :])
                run()

        queue_step = [0]

        def paced(items, ntaps):
            assert not queue
            queue.extend(items)
            queue_step[0] = -(-len(items) // ntaps)

        def do_unit(u):
            def put_q(i, jj, col, rws, val):
                pq_v[u, i, jj] = val
            unit(HF - 1, HT // 2 + 2 * j + u, tap, put_q)
            for g in range(T // 16):
                psum_item(2 + u, HF - 1, g)[1]()

        def finish(k, i, c, o):
            tile, rs, hs = rows(k, i)
            cs = slice(c * 128, (c + 1) * 128)
            ye = _dot(inv_p, _up(zz32[c, tile, 0:64, :]))
            yo = _dot(inv_m, _up(zz32[c, tile, 64:128, :]))
            yd = ye - yo
            y = jnp.concatenate(
                [ye + yo] + [
                    jnp.take_along_axis(yd[q * 8:(q + 1) * 8], rev, axis=0,
                                        mode="promise_in_bounds")
                    for q in reversed(range(BLK // 16))], axis=0)
            gate = o * (1.0 + jnp.tanh((0.25 / _A) * o))
            x = _up(x_v[0, hs, cs]).astype(F32)
            xn = xn_v[c, rs, :].astype(F32)
            o_v[rs, cs] = (x + (xn * y) * gate).astype(BF16)

        def do_pair(k, last=False):
            def prod(lhs, rhs):
                res = _dot(lhs, rhs)
                tap(res)
                return res

            def sa(i):
                return jnp.concatenate([_up(ps32[k, i, n]) for n in range(HF)], axis=1)

            a11 = jnp.concatenate([p_tile(k, 0, n) for n in range(HF)], axis=1)
            a22 = jnp.concatenate([p_tile(k, 1, n) for n in range(HF, NF)], axis=1)
            for m in range(2):
                _strassen(
                    prod, sa, lambda i: _up(ws32[i, m]), a11, a22,
                    _up(wout_v[0, 0:HK // 2, m * 128:(m + 1) * 128]),
                    _up(wout_v[0, HK // 2:HK, (m + 2) * 128:(m + 3) * 128]),
                    lambda i, jj, o: finish(k, i, m + 2 * jj, o))
            for i in range(2):
                rs = rows(k, i)[1]
                if last:
                    cp(o_v.at[rs, 0:512], out_hbm.at[0, rs, 0:512], out_sem).start()
            for i in range(2):
                rs = rows(k, i)[1]
                p = jnp.concatenate([p_tile(k, i, n) for n in range(NF)], axis=1)
                finish(k, i, NC - 1, _dot(p, _up(wout_v[0, 0:HK, 512:D])))
                if last:
                    cp(o_v.at[rs, 512:D], out_hbm.at[0, rs, 512:D], out_sem).start()
                else:
                    cp(o_v.at[rs, :], out_hbm.at[0, rs, :], out_sem).start()

        paced(psum(0) + [wsum_item(m, g) for m in range(2) for g in range(HK // 16)], 12)
        do_unit(0)
        paced(psum(1), 12)
        do_pair(0)
        paced(psum(2), 12)
        do_unit(1)
        paced(psum(3), 12)
        do_pair(1)
        do_pair(2)
        do_pair(3, last=True)
        return carry

    jax.lax.fori_loop(0, P3I, p3, 0)
    cp(o_v, out_hbm.at[0], out_sem).wait()


@jax.jit
def pallas_recurrent_scan__ssm_conv_h3__mixer_gmlp__prompt_kernel(
    A_q: jax.Array,
    A_k: jax.Array,
    A_v: jax.Array,
    A_shift_k: jax.Array,
    A_ssm_k: jax.Array,
    A_ssm_D: jax.Array,
    B_x: jax.Array,
    B_w_in: jax.Array,
    B_w_sp: jax.Array,
    B_b_sp: jax.Array,
    B_w_out: jax.Array,
):
    del B_x
    tab = jnp.asarray(_dft_tables(), dtype=BF16)

    any_spec = pl.BlockSpec(memory_space=pl.ANY)
    return pl.pallas_call(
        _kernel,
        out_shape=jax.ShapeDtypeStruct((1, S, D), BF16),
        in_specs=[any_spec] * 11,
        out_specs=any_spec,
        scratch_shapes=[
            pltpu.VMEM((1, S // 2 + 32, D), U32),
            pltpu.VMEM((D // 2, 2 * FH), U32),
            pltpu.VMEM((1, S // 2 + 8, S), U32),
            pltpu.VMEM((1, FH // 2 + 32, D), U32),
            pltpu.VMEM((2 * NC, S // 2 + 32, 128), U32),
            pltpu.VMEM((NC, 64, S), U32),
            pltpu.VMEM((NC, S + 256, 128), BF16),
            pltpu.VMEM((NF, S, 128), BF16),
            pltpu.VMEM((NF, S + 64, 128), BF16),
            pltpu.VMEM((NF, S + 64, 128), BF16),
            pltpu.VMEM((5, HT, HS, 128), BF16),
            pltpu.VMEM((5, HF, HS, 128), BF16),
            pltpu.VMEM((2, 2, 2, T, 128), BF16),
            pltpu.VMEM((4, 5, HF, T, 128), BF16),
            pltpu.VMEM((5, 2, FH // 2, 128), BF16),
            pltpu.VMEM((S, 128), BF16),
            pltpu.VMEM((BLK // 8, 6 * NB + 1, 8, 128), F32),
            pltpu.VMEM((NC, NB, 2 * BLK, 128), BF16),
            pltpu.VMEM((S, 128), F32),
            pltpu.VMEM((S, D), BF16),
            pltpu.VMEM((1, T + 16, FH), F32),
            pltpu.VMEM((1, T + 16, FH), F32),
            pltpu.VMEM((1, T + 16, FH), F32),
            pltpu.VMEM((T, 128), F32),
            pltpu.VMEM((320, 128), U32),
            pltpu.VMEM((NC, KS, 128), F32),
            pltpu.VMEM((NC + 2, 1, 128), F32),
            pltpu.VMEM((KS, D), BF16),
            pltpu.VMEM((D,), BF16),
            pltpu.VMEM((S,), BF16),
            pltpu.SMEM((1,), jnp.int32),
            pltpu.SemaphoreType.DMA((14,)),
        ],
        compiler_params=pltpu.CompilerParams(
            vmem_limit_bytes=100 * 1024 * 1024, disable_bounds_checks=True),
    )(A_q, A_k, A_v, A_shift_k.T, A_ssm_k, A_ssm_D, B_w_in, B_w_sp, B_b_sp, B_w_out, tab)
```

```python
import jax
import jax.numpy as jnp
import numpy as np
import jax.experimental.pallas as pl
import jax.experimental.pallas.tpu as pltpu

F32 = jnp.float32
BF16 = jnp.bfloat16
U32 = jnp.uint32

S = 2048
D = 640
FH = 768
KS = 4
BLK = 128
NB = S // BLK
NC = D // 128
NF = FH // 128
T = 128
NT = S // T
EPS = 1e-5
GRP = 4
SPLIT = 8
import os
LX = 11
AW = int(os.environ.get('AW', 1))
KG = 512
KR = 32
UA, UB, US, HP, HQ, HR, TOK = (i * NB for i in range(7))
LAG = 4
NTAP = 888
HS = S // 2
HT = HS // T
HF = NF // 2
P3I = 2

_GELU_C0 = float(np.sqrt(2.0 / np.pi))
_GELU_C1 = _GELU_C0 * 0.044715
_A = _GELU_C1 ** (1.0 / 3.0)
_K = _GELU_C0 / _A


def _dft_tables():
    m = np.arange(BLK)[:, None]
    n = np.arange(BLK)[None, :]
    th = 2.0 * np.pi * (((4 * m + 1) * n) % (4 * BLK)) / (4 * BLK)
    ph = 2.0 * np.pi * (((4 * m + 1) * (2 * n + 1)) % (8 * BLK)) / (8 * BLK)
    fu = np.concatenate([np.cos(ph), -np.sin(ph)], axis=0)
    fh = np.concatenate([np.cos(th) + np.sin(th), np.cos(th) - np.sin(th)], axis=0)
    fu, fh = (f.reshape(2, BLK // 8, 8, BLK).transpose(1, 0, 2, 3).reshape(2 * BLK, BLK)
              for f in (fu, fh))
    cp = (np.cos(ph) + np.sin(ph)).T[:BLK // 2] / (8.0 * BLK * _A * _A)
    cm = (np.cos(ph) - np.sin(ph)).T[:BLK // 2] / (8.0 * BLK * _A * _A)
    return np.concatenate([fu, fh, cp, cm], axis=0).astype(np.float32)


def _layernorm(x, eps, scale=1.0):
    m = jnp.mean(x, axis=-1, keepdims=True)
    d = x - m
    v = jnp.sum(d * d, axis=-1, keepdims=True) * (1.0 / (x.shape[-1] * scale * scale))
    return d * jax.lax.rsqrt(v + eps / (scale * scale))


def _gelu2(y):
    return y * (1.0 + jnp.tanh(y * (y * y + _K)))


def _up(x):
    return pltpu.bitcast(x, BF16)


def _dot(a, b):
    return jnp.dot(a, b, preferred_element_type=F32)


def _lhs_sums(a11, a12, a21, a22):
    return a11 + a22, a21 + a22, a11 + a12, a21 - a11, a12 - a22


def _rhs_sums(b11, b12, b21, b22):
    return b11 + b22, b12 - b22, b21 - b11, b11 + b12, b21 + b22


def _strassen(prod, sa, sb, a11, a22, b11, b22, fin):
    m2 = prod(sa(1), b11)
    m4 = prod(a22, sb(2))
    fin(1, 0, m2 + m4)
    m5 = prod(sa(2), b22)
    c11 = m4 - m5
    m3 = prod(a11, sb(1))
    fin(0, 1, m3 + m5)
    c22 = m3 - m2
    m1 = prod(sa(0), sb(0))
    c11, c22 = c11 + m1, c22 + m1
    fin(0, 0, c11 + prod(sa(4), sb(4)))
    fin(1, 1, c22 + prod(sa(3), sb(3)))


def _balance(work, n):
    jobs = [(lo, hi, sum(it[0] for it in items)) for items, lo, hi in work]
    rate = [None] * n
    while jobs:
        def free(a, b):
            return [p for p in range(a, b) if rate[p] is None]
        dens, a, b = max(
            (sum(w for lo, hi, w in jobs if a <= lo and hi <= b) / max(len(free(a, b)), 1e-9), a, b)
            for a in {j[0] for j in jobs} for b in {j[1] for j in jobs} if a < b)
        while a > 0 and rate[a - 1] is not None:
            a -= 1
        while b < n and rate[b] is not None:
            b += 1
        for p in free(a, b):
            rate[p] = dens
        jobs = [(lo, hi, w) for lo, hi, w in jobs if not (a <= lo and hi <= b)]
        jobs = [(b if a <= lo < b else lo, a if a < hi <= b else hi, w) for lo, hi, w in jobs]
    queues = [[lo * 16, hi * 16, list(items)] for items, lo, hi in work]
    rel = [[] for _ in range(n)]
    budget = 0.0
    for tau in range(n * 16):
        budget += (rate[tau // 16] or 0.0) / 16
        while True:
            ready = [q for q in queues if q[2] and q[0] <= tau]
            if not ready:
                budget = min(budget, 0.0)
                break
            q = min(ready, key=lambda q: q[1])
            if budget < 0 and q[1] - tau > len(q[2]):
                break
            it = q[2].pop(0)
            rel[tau // 16].append((tau % 16, it))
            budget -= it[0]
    assert not any(q[2] for q in queues)
    return rel


def _kernel(x_hbm, k_hbm, v_hbm, skt_hbm, h_hbm, dv_hbm, win_hbm, wsp_hbm, b_hbm,
            wout_hbm, tab_hbm, out_hbm,
            x_v, win_v, wsp_v, wout_v, kv_v, h_v, xn_v, z1_v, z2_v, p_v, as_v, as2_v, bs_v, pq_v, pp_v, ps_v, ws_v,
            kvb_v, pl_v, zz_v, bcol_v, o_v, zta_v, ztb_v, ztc_v, raw_v, tab_v,
            sk_v, dd_v, skt_v, dv_v, b_v, zero_s, sem):
    cp = pltpu.make_async_copy
    x16 = x_v.bitcast(BF16)
    win16 = win_v.bitcast(BF16)
    kv16 = kv_v.bitcast(BF16)
    h16 = h_v.bitcast(BF16)

    xn32, z232, kvb32, zz32, as32, as232, bs32, pp32, ps32, ws32 = (
        r.bitcast(U32)
        for r in (xn_v, z2_v, kvb_v, zz_v, as_v, as2_v, bs_v, pp_v, ps_v, ws_v))
    wsp16 = wsp_v.bitcast(BF16)

    def wsp_cp(lo, hi, s):
        return cp(wsp_hbm.at[lo:hi, :], wsp16.at[0, lo:hi, :], sem.at[s])

    def x_cp(lo, hi, s):
        return cp(x_hbm.at[0, lo:hi, :], x16.at[0, lo:hi, :], sem.at[s])

    def win_cp(lo, hi, s):
        return cp(win_hbm.at[:, lo:hi], win16.at[:, lo:hi], sem.at[s])

    def k_cp(c, s):
        return cp(k_hbm.at[0, :, pl.ds(c * 128, 128)], kv16.at[2 * c, 0:S, :], sem.at[s])

    def v_cp(c, s):
        return cp(v_hbm.at[0, :, pl.ds(c * 128, 128)], kv16.at[2 * c + 1, 0:S, :], sem.at[s])

    def h_cp(c, s):
        return cp(h_hbm.at[pl.ds(c * 128, 128), :], h16.at[c], sem.at[s])

    groups = [
        [cp(b_hbm, b_v, sem.at[0]), cp(skt_hbm, skt_v, sem.at[0]), cp(dv_hbm, dv_v, sem.at[0])],
        [x_cp(0, 256, 1)],
        [win_cp(FH, FH + 256, 2)],
        [win_cp(FH + 256, FH + 512, 3)],
        [win_cp(FH + 512, 2 * FH, 4), win_cp(0, 128, 4)],
        [win_cp(128, 512, 11)],
        [win_cp(512, FH, 5), x_cp(256, 384, 5)],
        [x_cp(384, 6 * T, 6)],
        [x_cp(6 * T, S, 7), k_cp(0, 7), v_cp(0, 7)],
        [wsp_cp(0, HS // 2, 12), wsp_cp(HS, HS + HS // 2, 12)],
        [wsp_cp(HS // 2, HS, 13), wsp_cp(HS + HS // 2, S, 13)],
        [cp(tab_hbm, tab_v.bitcast(BF16), sem.at[8]), h_cp(0, 8)],
    ]
    for g in groups:
        for c in g:
            c.start()

    def tile_cps(c):
        s = jnp.where(c == NC - 1, 9, c - 1) if isinstance(c, jax.Array) else (0, 1, 2, 9)[c - 1]
        return [k_cp(c, s), v_cp(c, s), h_cp(c, s)]

    wout_cp = cp(wout_hbm, wout_v.bitcast(BF16).at[0, 0:FH, :], sem.at[10])
    out_sem = sem.at[5]

    def wait(i):
        for c in groups[i]:
            c.wait()

    zero_s[0] = 0
    wait(0)
    skt = skt_v[...].astype(F32)
    dv = dv_v[...].astype(F32).reshape(1, D)
    for c in range(NC):
        sk_v[c] = skt[:, c * 128:(c + 1) * 128]
        dd_v[c] = dv[:, c * 128:(c + 1) * 128]
    brow = b_v[...].astype(F32).reshape(1, S)
    bcol_v[...] = jnp.broadcast_to(brow, (128, S)).T

    def gate_x(tok):
        x_v[0, S // 2:S // 2 + 8, 0:128] = pltpu.bitcast(tok, U32)

    zt_v = (zta_v, ztb_v, ztc_v)

    def gate_zt(t):
        def gate(tok):
            zt_v[t % 3][0, T:T + 8, 0:128] = tok
        return gate

    def gate_kv(tok):
        kv_v[0, S // 2:S // 2 + 8, :] = pltpu.bitcast(tok, U32)

    def gate_pl(tok):
        pl_v[0, TOK] = tok

    ndone = [0]

    def done(val):
        r = S + (ndone[0] % 16) * 16
        ndone[0] += 1
        xn_v[0, r:r + 16, :] = val

    def lnx_items(t, zero):
        def item(r0):
            def run():
                xw = x_v[zero, r0 // 2:r0 // 2 + 8, :]
                xn = _layernorm(_up(xw).astype(F32), EPS, _A)
                for c in range(NC):
                    xn_v[c, r0:r0 + 16, :] = xn[:, c * 128:(c + 1) * 128].astype(BF16)
            return (85, gate_x, run)
        return [item(t * T + g * 16) for g in range(T // 16)]

    def lnz_items(t, zero):
        def item(g):
            def run():
                z = zt_v[t % 3][zero, g * 16:(g + 1) * 16, :]
                z = _layernorm(z, 4.0 * _A * _A * EPS)
                r0 = t * T + g * 16
                for n in range(NF):
                    zb = z[:, n * 128:(n + 1) * 128].astype(BF16)
                    z2_v[n, r0:r0 + 16, :] = zb
                done(zb)
            return (90, gate_zt(t), run)
        return [item(g) for g in range(T // 16)]

    def kv_items(c):
        sk = sk_v[c]

        def item(r0):
            def run():
                hs = slice(r0 // 2, (r0 + KR) // 2)
                if r0 == 0:
                    kw = jnp.concatenate(
                        [jnp.zeros((8, 128), F32), _up(kv_v[2 * c, hs, :]).astype(F32)], axis=0)
                else:
                    kw = _up(kv_v[2 * c, r0 // 2 - 8:(r0 + KR) // 2, :]).astype(F32)[8:]
                ks = kw[8:] * sk[0:1, :]
                for t in range(1, KS):
                    ks = ks + pltpu.roll(kw, t, 0)[8:] * sk[t:t + 1, :]
                kvb_v[r0:r0 + KR, :] = (
                    ks * _up(kv_v[2 * c + 1, hs, :]).astype(F32)).astype(BF16)
            return (14 * KR // 8, gate_kv, run)
        return [item(r0) for r0 in range(0, S, KR)]

    def gate_w(tok):
        wsp_v[0, S // 2:S // 2 + 8, 0:128] = pltpu.bitcast(tok, U32)

    def asum_items(r_lo, r_hi):
        def item(zero, r0, c0):
            def run():
                def quad(i, j, c):
                    w = wsp_v[zero, (i * HS + r0) // 2:(i * HS + r0) // 2 + 8,
                              j * HS + c * 128:j * HS + (c + 1) * 128]
                    return _up(w).astype(F32)
                for c in range(c0, c0 + AW):
                    for i, v in enumerate(_lhs_sums(
                            quad(0, 0, c), quad(0, 1, c), quad(1, 0, c), quad(1, 1, c))):
                        as_v[i, c, r0:r0 + 16, :] = v.astype(BF16)
            return (23 * AW, gate_w, run)
        return lambda zero: [item(zero, r0, c0) for r0 in range(r_lo * T, r_hi * T, 16)
                             for c0 in range(0, HT, AW)]

    def asum_dyn(g, c):
        def run():
            def quad(i, j):
                r0 = pl.multiple_of(i * (HS // 2) + HS // 4 + g * 8, 8)
                w = wsp_v[0, pl.ds(r0, 8), j * HS + c * 128:j * HS + (c + 1) * 128]
                return _up(w).astype(F32)
            rs = pl.ds(pl.multiple_of(g * 16, 16), 16)
            for i, v in enumerate(_lhs_sums(quad(0, 0), quad(0, 1), quad(1, 0), quad(1, 1))):
                as2_v[i, c, rs, :] = v.astype(BF16)
        return (23, gate_w, run)

    def gate_z2(tok):
        z2_v[0, S:S + 8, :] = tok.astype(BF16)

    def bsum(t):
        def item(zero, r0, n):
            def run():
                def quad(i, j):
                    return z2_v[zero + n + j * HF, i * HS + r0:i * HS + r0 + 16, :].astype(F32)
                for i, v in enumerate(_rhs_sums(quad(0, 0), quad(0, 1), quad(1, 0), quad(1, 1))):
                    bs_v[i, n, r0:r0 + 16, :] = v.astype(BF16)
            return (24, gate_z2, run)
        return lambda zero: [item(zero, r0, n) for r0 in range((t - HT) * T, (t - HT + 1) * T, 16)
                             for n in range(HF)]

    def taps_of(val):
        rows, cols = val.shape
        return [(lambda i=i, n=n: val[i * 8:(i + 1) * 8, n * 128:(n + 1) * 128])
                for n in range(cols // 128) for i in range(rows // 8)]

    def activate(kind, t, n, z):
        if kind == 2:
            zt_v[t % 3][0, 0:T, n * 128:(n + 1) * 128] = _gelu2(z)
        else:
            z1_v[n, t * T:(t + 1) * T, :] = z.astype(BF16)

    def piece(kind, t, n, zero, defer=False, halves=False):
        col = n * 128 + (FH if kind == 2 else 0)
        xn = jnp.concatenate(
            [_up(xn32[zero if zero is not None and c == 0 else c,
                      t * T // 2:(t + 1) * T // 2, :]) for c in range(NC)], axis=1)
        w = _up(win_v[:, col:col + 128])
        if halves:
            z = jnp.concatenate([_dot(xn[:T // 2], w), _dot(xn[T // 2:], w)], axis=0)
        else:
            z = _dot(xn, w)
        if defer:
            raw_v[...] = z
        else:
            activate(kind, t, n, z)
        return taps_of(z)

    pending = []

    def block(pieces, work, defer=True, free=None):
        zero = zero_s[0]
        if pending:
            activate(*pending.pop(), raw_v[...])
        work = [(mk(zero), lo, hi) for mk, lo, hi in work]
        rel = [a + b for a, b in zip(
            _balance([w for w in work if w[0] and w[0][0][0] >= 80], len(pieces)),
            _balance([w for w in work if w[0] and w[0][0][0] < 80], len(pieces)))]
        taps = []
        gated = False
        for k in range(len(pieces) + LAG):
            if free is not None and k == len(pieces) - 1:
                for _, _, run in free(zero):
                    run()
                gated = True
            if k < len(pieces):
                last = defer and k == len(pieces) - 1
                halves = len(pieces) % 4 == 2 and k == len(pieces) - 1
                taps.append(piece(*pieces[k], zero if gated else None, last, halves))
                if last:
                    pending.append(pieces[k])
            if k >= LAG:
                for i, (_, gate, run) in sorted(rel[k - LAG], key=lambda e: e[0]):
                    gate(taps[k - LAG][i]())
                    run()
                    gated = True

    def cols(kind, t, lo=0, hi=NF):
        return [(kind, t, n) for n in range(lo, hi)]

    def lnx(t):
        return lambda zero: lnx_items(t, zero)

    def lnz(t):
        return lambda zero: lnz_items(t, zero)

    wait(1)
    for it in lnx_items(0, 0) + lnx_items(1, 0):
        it[2]()
    wait(2)
    block(cols(2, 0, 0, 2) + cols(2, 1, 0, 2), [])
    for c in range(1, NC):
        for d in tile_cps(c):
            d.start()
    wout_cp.start()
    wait(3)
    block(cols(2, 0, 2, 4) + cols(2, 1, 2, 4), [])
    wait(4)
    block(cols(2, 0, 4) + cols(2, 1, 4) + cols(1, 0, 0, 1) + cols(1, 1, 0, 1), [])
    wait(5)
    block(cols(1, 0, 1, 4) + cols(1, 1, 1, 4), [(lnz(0), 0, 1)])
    wait(6)
    block(cols(1, 0, 4) + cols(1, 1, 4), [], free=lnx(2))

    def tiles(lo, hi):
        return [pc for t in range(lo, hi) for pc in cols(2, t) + cols(1, t)]

    def end_pair(a):
        return cols(2, a) + cols(2, a + 1) + cols(1, a) + cols(1, a + 1)

    def part(mk, lo, hi):
        return lambda zero: mk(zero)[lo:hi]

    wait(7)
    block(tiles(2, 5),
          [(lnx(3), 0, 7), (lnx(4), 0, 19), (lnx(5), 0, 31),
           (lnz(1), 0, 20), (lnz(2), 6, 31), (lnz(3), 18, 31)])
    wait(8)
    block(tiles(5, 9),
          [(lnx(6), 0, 7), (lnx(7), 0, 19), (lnx(8), 0, 31)]
          + [(lnx(t), 0, 43) for t in range(9, LX)]
          + [(lnz(4), 0, 20), (lnz(5), 6, 32), (lnz(6), 18, 43), (lnz(7), 30, 43),
             (kv_items, 0, 48)])
    wait(9)
    block(tiles(9, 13) + cols(2, 13) + cols(2, 14) + cols(1, 13) + cols(2, 15)
          + cols(1, 14) + cols(1, 15),
          [(lnx(11), 0, 19), (lnx(12), 0, 31), (lnx(13), 0, 43), (lnx(14), 0, 49),
           (lnx(15), 0, 61),
           (lnz(8), 0, 20), (lnz(9), 6, 32), (lnz(10), 18, 44), (lnz(11), 30, 50),
           (lnz(12), 42, 62), (lnz(13), 54, 66), (lnz(14), 60, 72), (lnz(15), 72, 75),
           (bsum(8), 25, 84), (bsum(9), 37, 84), (bsum(10), 49, 84), (bsum(11), 55, 84),
           (bsum(12), 67, 84), (bsum(13), 71, 84), (bsum(14), 77, 84), (bsum(15), 80, 84),
           (asum_items(0, HT // 2), 0, 84)], defer=False)
    wait(10)
    wait(11)

    def unit(n, half, k, tap, put_p):
        def span(start, size):
            if isinstance(start, int):
                return slice(start, start + size)
            return pl.ds(pl.multiple_of(start, size), size)

        r = half * (HT // 2) + k
        top, bot = span(r * T, T), span(HS + r * T, T)
        toph, both = span(r * (T // 2), T // 2), span(HS // 2 + r * (T // 2), T // 2)
        sums, sumh = (as32, as232)[half], span(k * (T // 2), T // 2)

        def prod(lhs, rhs):
            acc = None
            for q in range(HS // KG):
                part = _dot(lhs(q), rhs(q))
                acc = part if acc is None else acc + part
                tap(acc)
            return acc

        def sa(i):
            return lambda q: jnp.concatenate(
                [_up(sums[i, c, sumh, :]) for c in range(q * KG // 128, (q + 1) * KG // 128)],
                axis=1)

        def sb(i):
            return lambda q: _up(bs32[i, n, q * KG // 2:(q + 1) * KG // 2, :])

        def a11(q):
            return _up(wsp_v[0, toph, q * KG:(q + 1) * KG])

        def a22(q):
            return _up(wsp_v[0, both, HS + q * KG:HS + (q + 1) * KG])

        def b11(q):
            return _up(z232[n, q * KG // 2:(q + 1) * KG // 2, :])

        def b22(q):
            return _up(z232[n + HF, (HS + q * KG) // 2:(HS + (q + 1) * KG) // 2, :])

        def fin(i, j, c):
            col, rows = n + j * HF, (top, bot)[i]
            put_p(i, j, col, rows, (c + bcol_v[rows, :]).astype(BF16))

        _strassen(prod, sa, sb, a11, a22, b11, b22, fin)

    def p2(n, half):
        nn = jnp.minimum(n + 1, NC - 1)

        @pl.when(n + 1 < NC)
        def _():
            for d in tile_cps(nn):
                d.wait()

        zero = zero_s[0]
        fwd_u = _up(tab_v[0:128, :])
        fwd_h = _up(tab_v[128:256, :])
        dd = dd_v[n]

        def put(slot, val):
            pl_v[:, slot] = val

        def re_im(val):
            val = val.reshape(BLK // 8, 2, 8, 128)
            return val[:, 0], val[:, 1]

        kvi = kv_items(nn)

        def pace_kv(d, val):
            if d % 4 == 3:
                for j in range(8):
                    _, gate, run = kvi[(d // 4) * 8 + j]
                    gate(val[j * 32:j * 32 + 8, :])
                    run()

        for i in range(NB):
            u = _dot(fwd_u, _up(kvb32[i * BLK // 2:(i + 1) * BLK // 2, :]))
            a, b = re_im(u)
            put(UA + i, a)
            put(UB + i, b)
            put(US + i, a + b)
            pace_kv(i, u)
        for i in range(NB):
            hb = _up(h_v[n, :, i * BLK:(i + 1) * BLK])
            hf = jax.lax.dot_general(fwd_h, hb, (((1,), (1,)), ((), ())),
                                     preferred_element_type=F32)
            c, d = re_im(hf)
            if i == 0:
                c, d = c + dd, d + dd
            put(HR + i, c)
            put(HP + i, d - c)
            put(HQ + i, c + d)
            pace_kv(NB + i, hf)

        state = {}

        def mac_item(pos, g0, pi, j0, j1):
            xv, hv = ((US, HR), (UA, HP), (UB, HQ))[pi]
            outs = range(g0, g0 + GRP)
            top = g0 + GRP

            def run():
                pz = zero + pos
                hs = {t: pl_v[pz, hv + t]
                      for t in range(max(g0 - j1 + 1, 0), top - j0)}
                acc = state['acc'] if j0 else {o: None for o in outs}
                for jj in range(j0, j1):
                    xj = pl_v[pz, xv + jj]
                    for o in outs:
                        if o - jj >= 0:
                            t = xj * hs[o - jj]
                            acc[o] = t if acc[o] is None else acc[o] + t
                if j1 < top:
                    state['acc'] = acc
                    return
                r0 = pos * 8
                if pi == 0:
                    state['k1'] = acc
                elif pi == 1:
                    state['im'] = {o: state['k1'][o] + acc[o] for o in outs}
                else:
                    for o in outs:
                        re, im = state['k1'][o] - acc[o], state['im'][o]
                        zr, zi = re, im
                        if o > 0:
                            zr, zi = re - state['prev'][1], im + state['prev'][0]
                        state['prev'] = (re, im)
                        zz_v[n, o, r0:r0 + 8, :] = zr.astype(BF16)
                        zz_v[n, o, BLK + r0:BLK + r0 + 8, :] = zi.astype(BF16)

            nmac = sum(1 for o in outs for jj in range(j0, j1) if o >= jj)
            return (2 * nmac + ((0, GRP, 5 * GRP)[pi] if j1 == top else 0), gate_pl, run)

        items = []
        for pos in range(BLK // 8):
            for g0 in range(0, NB, GRP):
                top = g0 + GRP
                cuts = [0, top] if top <= SPLIT else [0, (top - 1) // 2, top]
                for pi in range(3):
                    for j0, j1 in zip(cuts[:-1], cuts[1:]):
                        items.append(mac_item(pos, g0, pi, j0, j1))

        if half == 0:
            ng = -(-HS // 32 // HF)
            extra = [asum_dyn(jnp.minimum(n * ng + g, HS // 32 - 1), c)
                     for g in range(ng) for c in range(HT)]
            every = len(items) // len(extra)
            items = [it for i, e in enumerate(extra)
                     for it in items[i * every:(i + 1) * every] + [e]
                     ] + items[len(extra) * every:]

        total = sum(c for c, _, _ in items)
        tap_of = []
        cum = 0
        for c, _, _ in items:
            tap_of.append(int(cum * NTAP / total))
            cum += c
        pos = {'tap': 0, 'item': 0}

        def tap(acc):
            t0 = pos['tap']
            pos['tap'] += T // 8
            while pos['item'] < len(items) and tap_of[pos['item']] < pos['tap']:
                i = tap_of[pos['item']] - t0
                _, gate, run = items[pos['item']]
                gate(acc[i * 8:(i + 1) * 8, :])
                run()
                pos['item'] += 1

        def put_p(i, j, col, rows, val):
            p_v[col, rows, :] = val

        for k in range(HT // 2):
            unit(n - half * HF, half, k, tap, put_p)
        assert pos['item'] == len(items)
        return 0

    jax.lax.fori_loop(0, HF, lambda n, c: p2(n, 0), 0)
    jax.lax.fori_loop(HF, NC, lambda n, c: p2(n, 1), 0)

    wout_cp.wait()

    def p3(j, carry):
        inv_p = _up(tab_v[256:288, :])
        inv_m = _up(tab_v[288:320, :])
        rev = 7 - jax.lax.broadcasted_iota(jnp.int32, (8, 128), 0)

        zero = zero_s[0]
        HK = FH // 2

        def rows(k, i):
            tile = i * HT + (k // 2) * (HT // 2) + 2 * j + k % 2
            return (tile, pl.ds(pl.multiple_of(tile * T, T), T),
                    pl.ds(pl.multiple_of(tile * (T // 2), T // 2), T // 2))

        def fresh(k, n):
            return k >= 2 and n % HF == HF - 1

        def p_tile(k, i, n):
            return _up(pp32[k, i, n])

        def gate_p(tok):
            p_v[0, S:S + 8, :] = tok.astype(BF16)

        def gate_wo(tok):
            wout_v[0, HK:HK + 8, 0:128] = pltpu.bitcast(tok, U32)

        def psum_item(k, n, g):
            def run():
                def quad(i, jj):
                    rs = pl.ds(pl.multiple_of(rows(k, i)[0] * T + g * 16, 16), 16)
                    if fresh(k, n):
                        gv = pq_v[k - 2, i, jj, g * 16:(g + 1) * 16, :]
                    else:
                        gv = p_v[n + jj * HF, rs, :]
                    pv = _gelu2(z1_v[n + jj * HF, rs, :].astype(F32)) * gv.astype(F32)
                    pp_v[k, i, n + jj * HF, g * 16:(g + 1) * 16, :] = pv.astype(BF16)
                    return pv
                for i, v in enumerate(_lhs_sums(quad(0, 0), quad(0, 1), quad(1, 0), quad(1, 1))):
                    ps_v[k, i, n, g * 16:(g + 1) * 16, :] = v.astype(BF16)
            return (gate_p, run)

        def wsum_item(m, g):
            def run():
                def quad(i, jj):
                    r0 = (i * HK + g * 16) // 2
                    c0 = (m + 2 * jj) * 128
                    return _up(wout_v[zero, r0:r0 + 8, c0:c0 + 128]).astype(F32)
                for i, v in enumerate(_rhs_sums(quad(0, 0), quad(0, 1), quad(1, 0), quad(1, 1))):
                    ws_v[i, m, g * 16:(g + 1) * 16, :] = v.astype(BF16)
            return (gate_wo, run)

        def psum(k):
            return [psum_item(k, n, g) for n in range(HF) if not fresh(k, n)
                    for g in range(T // 16)]

        queue = []

        def tap(val):
            for i in range(min(len(queue), queue_step[0])):
                gate, run = queue.pop(0)
                r = (i * (T // 8)) // queue_step[0] * 8
                gate(val[r:r + 8, :])
                run()

        queue_step = [0]

        def paced(items, ntaps):
            assert not queue
            queue.extend(items)
            queue_step[0] = -(-len(items) // ntaps)

        def do_unit(u):
            def put_q(i, jj, col, rws, val):
                pq_v[u, i, jj] = val
            unit(HF - 1, 1, 2 * j + u, tap, put_q)
            for g in range(T // 16):
                psum_item(2 + u, HF - 1, g)[1]()

        def finish(k, i, c, o):
            tile, rs, hs = rows(k, i)
            cs = slice(c * 128, (c + 1) * 128)
            ye = _dot(inv_p, _up(zz32[c, tile, 0:64, :]))
            yo = _dot(inv_m, _up(zz32[c, tile, 64:128, :]))
            yd = ye - yo
            y = jnp.concatenate(
                [ye + yo] + [
                    jnp.take_along_axis(yd[q * 8:(q + 1) * 8], rev, axis=0,
                                        mode="promise_in_bounds")
                    for q in reversed(range(BLK // 16))], axis=0)
            gate = o * (1.0 + jnp.tanh((0.25 / _A) * o))
            x = _up(x_v[0, hs, cs]).astype(F32)
            xn = xn_v[c, rs, :].astype(F32)
            o_v[rs, cs] = (x + (xn * y) * gate).astype(BF16)

        def do_pair(k, last=False):
            def prod(lhs, rhs):
                res = _dot(lhs, rhs)
                tap(res)
                return res

            def sa(i):
                return jnp.concatenate([_up(ps32[k, i, n]) for n in range(HF)], axis=1)

            a11 = jnp.concatenate([p_tile(k, 0, n) for n in range(HF)], axis=1)
            a22 = jnp.concatenate([p_tile(k, 1, n) for n in range(HF, NF)], axis=1)
            for m in range(2):
                _strassen(
                    prod, sa, lambda i: _up(ws32[i, m]), a11, a22,
                    _up(wout_v[0, 0:HK // 2, m * 128:(m + 1) * 128]),
                    _up(wout_v[0, HK // 2:HK, (m + 2) * 128:(m + 3) * 128]),
                    lambda i, jj, o: finish(k, i, m + 2 * jj, o))
            for i in range(2):
                rs = rows(k, i)[1]
                if last:
                    cp(o_v.at[rs, 0:512], out_hbm.at[0, rs, 0:512], out_sem).start()
            for i in range(2):
                rs = rows(k, i)[1]
                p = jnp.concatenate([p_tile(k, i, n) for n in range(NF)], axis=1)
                finish(k, i, NC - 1, _dot(p, _up(wout_v[0, 0:HK, 512:D])))
                if last:
                    cp(o_v.at[rs, 512:D], out_hbm.at[0, rs, 512:D], out_sem).start()
                else:
                    cp(o_v.at[rs, :], out_hbm.at[0, rs, :], out_sem).start()

        paced(psum(0) + [wsum_item(m, g) for m in range(2) for g in range(HK // 16)], 12)
        do_unit(0)
        paced(psum(1), 12)
        do_pair(0)
        paced(psum(2), 12)
        do_unit(1)
        paced(psum(3), 12)
        do_pair(1)
        do_pair(2)
        do_pair(3, last=True)
        return carry

    jax.lax.fori_loop(0, P3I, p3, 0)
    cp(o_v, out_hbm.at[0], out_sem).wait()


@jax.jit
def pallas_recurrent_scan__ssm_conv_h3__mixer_gmlp__prompt_kernel(
    A_q: jax.Array,
    A_k: jax.Array,
    A_v: jax.Array,
    A_shift_k: jax.Array,
    A_ssm_k: jax.Array,
    A_ssm_D: jax.Array,
    B_x: jax.Array,
    B_w_in: jax.Array,
    B_w_sp: jax.Array,
    B_b_sp: jax.Array,
    B_w_out: jax.Array,
):
    del B_x
    tab = jnp.asarray(_dft_tables(), dtype=BF16)

    any_spec = pl.BlockSpec(memory_space=pl.ANY)
    return pl.pallas_call(
        _kernel,
        out_shape=jax.ShapeDtypeStruct((1, S, D), BF16),
        in_specs=[any_spec] * 11,
        out_specs=any_spec,
        scratch_shapes=[
            pltpu.VMEM((1, S // 2 + 32, D), U32),
            pltpu.VMEM((D // 2, 2 * FH), U32),
            pltpu.VMEM((1, S // 2 + 8, S), U32),
            pltpu.VMEM((1, FH // 2 + 32, D), U32),
            pltpu.VMEM((2 * NC, S // 2 + 32, 128), U32),
            pltpu.VMEM((NC, 64, S), U32),
            pltpu.VMEM((NC, S + 256, 128), BF16),
            pltpu.VMEM((NF, S, 128), BF16),
            pltpu.VMEM((NF, S + 64, 128), BF16),
            pltpu.VMEM((NF, S + 64, 128), BF16),
            pltpu.VMEM((5, HT, HS // 2, 128), BF16),
            pltpu.VMEM((5, HT, HS // 2, 128), BF16),
            pltpu.VMEM((5, HF, HS, 128), BF16),
            pltpu.VMEM((2, 2, 2, T, 128), BF16),
            pltpu.VMEM((4, 2, NF, T, 128), BF16),
            pltpu.VMEM((4, 5, HF, T, 128), BF16),
            pltpu.VMEM((5, 2, FH // 2, 128), BF16),
            pltpu.VMEM((S, 128), BF16),
            pltpu.VMEM((BLK // 8, 6 * NB + 1, 8, 128), F32),
            pltpu.VMEM((NC, NB, 2 * BLK, 128), BF16),
            pltpu.VMEM((S, 128), F32),
            pltpu.VMEM((S, D), BF16),
            pltpu.VMEM((1, T + 16, FH), F32),
            pltpu.VMEM((1, T + 16, FH), F32),
            pltpu.VMEM((1, T + 16, FH), F32),
            pltpu.VMEM((T, 128), F32),
            pltpu.VMEM((320, 128), U32),
            pltpu.VMEM((NC, KS, 128), F32),
            pltpu.VMEM((NC + 2, 1, 128), F32),
            pltpu.VMEM((KS, D), BF16),
            pltpu.VMEM((D,), BF16),
            pltpu.VMEM((S,), BF16),
            pltpu.SMEM((1,), jnp.int32),
            pltpu.SemaphoreType.DMA((14,)),
        ],
        compiler_params=pltpu.CompilerParams(
            vmem_limit_bytes=100 * 1024 * 1024, disable_bounds_checks=True),
    )(A_q, A_k, A_v, A_shift_k.T, A_ssm_k, A_ssm_D, B_w_in, B_w_sp, B_b_sp, B_w_out, tab)
```

```python
import jax
import jax.numpy as jnp
import numpy as np
import jax.experimental.pallas as pl
import jax.experimental.pallas.tpu as pltpu

F32 = jnp.float32
BF16 = jnp.bfloat16
U32 = jnp.uint32

S = 2048
D = 640
FH = 768
KS = 4
BLK = 128
NB = S // BLK
NC = D // 128
NF = FH // 128
T = 128
NT = S // T
EPS = 1e-5
GRP = 4
SPLIT = 8
import os
AW = int(os.environ.get('AW', 1))
PR = int(os.environ.get('PR', 128))
KG = 512
KR = 32
UA, UB, US, HP, HQ, HR, TOK = (i * NB for i in range(7))
LAG = 4
NTAP = 888
HS = S // 2
HT = HS // T
HF = NF // 2
KH = 256
P3I = 2

_GELU_C0 = float(np.sqrt(2.0 / np.pi))
_GELU_C1 = _GELU_C0 * 0.044715
_A = _GELU_C1 ** (1.0 / 3.0)
_K = _GELU_C0 / _A


def _dft_tables():
    m = np.arange(BLK)[:, None]
    n = np.arange(BLK)[None, :]
    th = 2.0 * np.pi * (((4 * m + 1) * n) % (4 * BLK)) / (4 * BLK)
    ph = 2.0 * np.pi * (((4 * m + 1) * (2 * n + 1)) % (8 * BLK)) / (8 * BLK)
    fu = np.concatenate([np.cos(ph), -np.sin(ph)], axis=0)
    fh = np.concatenate([np.cos(th) + np.sin(th), np.cos(th) - np.sin(th)], axis=0)
    fu, fh = (f.reshape(2, BLK // 8, 8, BLK).transpose(1, 0, 2, 3).reshape(2 * BLK, BLK)
              for f in (fu, fh))
    cp = (np.cos(ph) + np.sin(ph)).T[:BLK // 2] / (8.0 * BLK * _A * _A)
    cm = (np.cos(ph) - np.sin(ph)).T[:BLK // 2] / (8.0 * BLK * _A * _A)
    return np.concatenate([fu, fh, cp, cm], axis=0).astype(np.float32)


def _layernorm(x, eps, scale=1.0):
    m = jnp.mean(x, axis=-1, keepdims=True)
    d = x - m
    v = jnp.sum(d * d, axis=-1, keepdims=True) * (1.0 / (x.shape[-1] * scale * scale))
    return d * jax.lax.rsqrt(v + eps / (scale * scale))


def _gelu2(y):
    return y * (1.0 + jnp.tanh(y * (y * y + _K)))


def _up(x):
    return pltpu.bitcast(x, BF16)


def _dot(a, b):
    return jnp.dot(a, b, preferred_element_type=F32)


def _lhs_sums(a11, a12, a21, a22):
    return a11 + a22, a21 + a22, a11 + a12, a21 - a11, a12 - a22


def _rhs_sums(b11, b12, b21, b22):
    return b11 + b22, b12 - b22, b21 - b11, b11 + b12, b21 + b22


def _strassen(prod, sa, sb, a11, a22, b11, b22, fin):
    m2 = prod(sa(1), b11)
    m4 = prod(a22, sb(2))
    fin(1, 0, m2 + m4)
    m5 = prod(sa(2), b22)
    c11 = m4 - m5
    m3 = prod(a11, sb(1))
    fin(0, 1, m3 + m5)
    c22 = m3 - m2
    m1 = prod(sa(0), sb(0))
    c11, c22 = c11 + m1, c22 + m1
    fin(0, 0, c11 + prod(sa(4), sb(4)))
    fin(1, 1, c22 + prod(sa(3), sb(3)))


def _balance(work, n):
    jobs = [(lo, hi, sum(it[0] for it in items)) for items, lo, hi in work]
    rate = [None] * n
    while jobs:
        def free(a, b):
            return [p for p in range(a, b) if rate[p] is None]
        dens, a, b = max(
            (sum(w for lo, hi, w in jobs if a <= lo and hi <= b) / max(len(free(a, b)), 1e-9), a, b)
            for a in {j[0] for j in jobs} for b in {j[1] for j in jobs} if a < b)
        while a > 0 and rate[a - 1] is not None:
            a -= 1
        while b < n and rate[b] is not None:
            b += 1
        for p in free(a, b):
            rate[p] = dens
        jobs = [(lo, hi, w) for lo, hi, w in jobs if not (a <= lo and hi <= b)]
        jobs = [(b if a <= lo < b else lo, a if a < hi <= b else hi, w) for lo, hi, w in jobs]
    queues = [[lo * 16, hi * 16, list(items)] for items, lo, hi in work]
    rel = [[] for _ in range(n)]
    budget = 0.0
    for tau in range(n * 16):
        budget += (rate[tau // 16] or 0.0) / 16
        while True:
            ready = [q for q in queues if q[2] and q[0] <= tau]
            if not ready:
                budget = min(budget, 0.0)
                break
            q = min(ready, key=lambda q: q[1])
            if budget < 0 and q[1] - tau > len(q[2]):
                break
            it = q[2].pop(0)
            rel[tau // 16].append((tau % 16, it))
            budget -= it[0]
    assert not any(q[2] for q in queues)
    return rel


def _kernel(x_hbm, k_hbm, v_hbm, skt_hbm, h_hbm, dv_hbm, win_hbm, wsp_hbm, b_hbm,
            wout_hbm, tab_hbm, out_hbm,
            x_v, win_v, wsp_v, wout_v, kv_v, h_v, xn_v, z1_v, z2_v, p_v, as_v, as2_v, bs_v, pq_v, pp_v, ps_v, ws_v,
            kvb_v, pl_v, zz_v, bcol_v, o_v, zta_v, ztb_v, ztc_v, ztd_v, xs_v, wi_v, raw_v, tab_v,
            sk_v, dd_v, skt_v, dv_v, b_v, zero_s, sem):
    cp = pltpu.make_async_copy
    x16 = x_v.bitcast(BF16)
    win16 = win_v.bitcast(BF16)
    kv16 = kv_v.bitcast(BF16)
    h16 = h_v.bitcast(BF16)

    xn32, z232, kvb32, zz32, as32, as232, bs32, pp32, ps32, ws32, xs32, wi32 = (
        r.bitcast(U32)
        for r in (xn_v, z2_v, kvb_v, zz_v, as_v, as2_v, bs_v, pp_v, ps_v, ws_v, xs_v, wi_v))
    wsp16 = wsp_v.bitcast(BF16)

    def wsp_cp(lo, hi, s):
        return cp(wsp_hbm.at[lo:hi, :], wsp16.at[0, lo:hi, :], sem.at[s])

    def x_cp(lo, hi, s):
        return cp(x_hbm.at[0, lo:hi, :], x16.at[0, lo:hi, :], sem.at[s])

    def win_cp(lo, hi, s):
        return cp(win_hbm.at[:, lo:hi], win16.at[0, 0:D, lo:hi], sem.at[s])

    def k_cp(c, s):
        return cp(k_hbm.at[0, :, pl.ds(c * 128, 128)], kv16.at[2 * c, 0:S, :], sem.at[s])

    def v_cp(c, s):
        return cp(v_hbm.at[0, :, pl.ds(c * 128, 128)], kv16.at[2 * c + 1, 0:S, :], sem.at[s])

    def h_cp(c, s):
        return cp(h_hbm.at[pl.ds(c * 128, 128), :], h16.at[c], sem.at[s])

    groups = [
        [cp(b_hbm, b_v, sem.at[0]), cp(skt_hbm, skt_v, sem.at[0]), cp(dv_hbm, dv_v, sem.at[0])],
        [x_cp(0, 256, 1)],
        [win_cp(FH, FH + 256, 2)],
        [win_cp(FH + 256, FH + 512, 3)],
        [win_cp(FH + 512, 2 * FH, 4), win_cp(0, 128, 4)],
        [win_cp(128, 512, 11)],
        [win_cp(512, FH, 5), x_cp(256, 384, 5)],
        [x_cp(384, 6 * T, 6)],
        [x_cp(6 * T, 12 * T, 7), k_cp(0, 7), v_cp(0, 7)],
        [x_cp(12 * T, S, 12), wsp_cp(0, HS // 2, 12), wsp_cp(HS, HS + HS // 2, 12)],
        [cp(tab_hbm, tab_v.bitcast(BF16), sem.at[8]), h_cp(0, 8)],
    ]
    for g in groups:
        for c in g:
            c.start()

    def tile_cps(c):
        s = jnp.where(c == NC - 1, 9, c - 1) if isinstance(c, jax.Array) else (0, 1, 2, 9)[c - 1]
        return [k_cp(c, s), v_cp(c, s), h_cp(c, s)]

    NG = -(-HS // 32 // HF)

    def wsp2_cps(n):
        lo, hi = HS // 2 + n * NG * 16, min(HS // 2 + (n + 1) * NG * 16, HS)
        return [wsp_cp(lo, hi, 13 + n), wsp_cp(HS + lo, HS + hi, 13 + n)]

    wout_cp = cp(wout_hbm, wout_v.bitcast(BF16).at[0, 0:FH, :], sem.at[10])
    out_sem = sem.at[5]

    def wait(i):
        for c in groups[i]:
            c.wait()

    zero_s[0] = 0
    wait(0)
    skt = skt_v[...].astype(F32)
    dv = dv_v[...].astype(F32).reshape(1, D)
    for c in range(NC):
        sk_v[c] = skt[:, c * 128:(c + 1) * 128]
        dd_v[c] = dv[:, c * 128:(c + 1) * 128]
    brow = b_v[...].astype(F32).reshape(1, S)
    bcol_v[...] = jnp.broadcast_to(brow, (128, S)).T

    def gate_x(tok):
        x_v[0, S // 2:S // 2 + 8, 0:128] = pltpu.bitcast(tok, U32)

    zt_v = (zta_v, ztb_v, ztc_v, ztd_v)

    def gate_zt(t):
        def gate(tok):
            zt_v[t % 4][0, T:T + 8, 0:128] = tok
        return gate

    def gate_kv(tok):
        kv_v[0, S // 2:S // 2 + 8, :] = pltpu.bitcast(tok, U32)

    def gate_pl(tok):
        pl_v[0, TOK] = tok

    ndone = [0]

    mode = {'pairs': False}

    def done(val):
        r = (ndone[0] % 8) * 16
        ndone[0] += 1
        if mode['pairs']:
            xs_v[0, 0, 0, r:r + 16, :] = val
        else:
            xn_v[0, S + r:S + r + 16, :] = val

    def lnx_items(t, zero):
        def item(r0):
            def run():
                xw = x_v[zero, r0 // 2:r0 // 2 + 8, :]
                xn = _layernorm(_up(xw).astype(F32), EPS, _A)
                for c in range(NC):
                    xb = xn[:, c * 128:(c + 1) * 128].astype(BF16)
                    xn_v[c, r0:r0 + 16, :] = xb
                if mode['pairs']:
                    done(xb)
            return (85, gate_x, run)
        return [item(t * T + g * 16) for g in range(T // 16)]

    def lnz_items(t, zero):
        def item(g):
            def run():
                z = zt_v[t % 4][zero, g * 16:(g + 1) * 16, :]
                z = _layernorm(z, 4.0 * _A * _A * EPS)
                r0 = t * T + g * 16
                for n in range(NF):
                    zb = z[:, n * 128:(n + 1) * 128].astype(BF16)
                    z2_v[n, r0:r0 + 16, :] = zb
                done(zb)
            return (90, gate_zt(t), run)
        return [item(g) for g in range(T // 16)]

    def kv_items(c):
        sk = sk_v[c]

        def item(r0):
            def run():
                hs = slice(r0 // 2, (r0 + KR) // 2)
                if r0 == 0:
                    kw = jnp.concatenate(
                        [jnp.zeros((8, 128), F32), _up(kv_v[2 * c, hs, :]).astype(F32)], axis=0)
                else:
                    kw = _up(kv_v[2 * c, r0 // 2 - 8:(r0 + KR) // 2, :]).astype(F32)[8:]
                ks = kw[8:] * sk[0:1, :]
                for t in range(1, KS):
                    ks = ks + pltpu.roll(kw, t, 0)[8:] * sk[t:t + 1, :]
                kvb_v[r0:r0 + KR, :] = (
                    ks * _up(kv_v[2 * c + 1, hs, :]).astype(F32)).astype(BF16)
            return (14 * KR // 8, gate_kv, run)
        return [item(r0) for r0 in range(0, S, KR)]

    def gate_w(tok):
        wsp_v[0, S // 2:S // 2 + 8, 0:128] = pltpu.bitcast(tok, U32)

    def asum_items(r_lo, r_hi):
        def item(zero, r0, c0):
            def run():
                def quad(i, j, c):
                    w = wsp_v[zero, (i * HS + r0) // 2:(i * HS + r0) // 2 + 8,
                              j * HS + c * 128:j * HS + (c + 1) * 128]
                    return _up(w).astype(F32)
                for c in range(c0, c0 + AW):
                    for i, v in enumerate(_lhs_sums(
                            quad(0, 0, c), quad(0, 1, c), quad(1, 0, c), quad(1, 1, c))):
                        as_v[i, c, r0:r0 + 16, :] = v.astype(BF16)
            return (23 * AW, gate_w, run)
        return lambda zero: [item(zero, r0, c0) for r0 in range(r_lo * T, r_hi * T, 16)
                             for c0 in range(0, HT, AW)]

    def asum_dyn(g, c):
        def run():
            def quad(i, j):
                r0 = pl.multiple_of(i * (HS // 2) + HS // 4 + g * 8, 8)
                w = wsp_v[0, pl.ds(r0, 8), j * HS + c * 128:j * HS + (c + 1) * 128]
                return _up(w).astype(F32)
            rs = pl.ds(pl.multiple_of(g * 16, 16), 16)
            for i, v in enumerate(_lhs_sums(quad(0, 0), quad(0, 1), quad(1, 0), quad(1, 1))):
                as2_v[i, c, rs, :] = v.astype(BF16)
        return (23, gate_w, run)

    def gate_z2(tok):
        z2_v[0, S:S + 8, :] = tok.astype(BF16)

    def bsum(t):
        def item(zero, r0, n):
            def run():
                def quad(i, j):
                    return z2_v[zero + n + j * HF, i * HS + r0:i * HS + r0 + 16, :].astype(F32)
                for i, v in enumerate(_rhs_sums(quad(0, 0), quad(0, 1), quad(1, 0), quad(1, 1))):
                    bs_v[i, n, r0:r0 + 16, :] = v.astype(BF16)
            return (24, gate_z2, run)
        return lambda zero: [item(zero, r0, n) for r0 in range((t - HT) * T, (t - HT + 1) * T, 16)
                             for n in range(HF)]

    def gate_xn(tok):
        xn_v[1, S:S + 8, :] = tok.astype(BF16)

    def xsum(u):
        def item(zero, g, c):
            def run():
                def quad(i, j):
                    r0 = (2 * u + i) * T + g * 16
                    return xn_v[zero + c + 2 * j, r0:r0 + 16, :].astype(F32)
                for i, v in enumerate(_lhs_sums(quad(0, 0), quad(0, 1), quad(1, 0), quad(1, 1))):
                    xs_v[u, i, c, g * 16:(g + 1) * 16, :] = v.astype(BF16)
            return (24, gate_xn, run)
        return lambda zero: [item(zero, g, c) for g in range(T // 16) for c in range(2)]

    def gate_wi(tok):
        win_v[0, D // 2:D // 2 + 8, 0:128] = pltpu.bitcast(tok, U32)

    def wisum(zero):
        def item(g, q):
            def run():
                def quad(i, j):
                    r0 = (i * KH + g * 16) // 2
                    c0 = ((q // HF) * NF + q % HF + j * HF) * 128
                    return _up(win_v[zero, r0:r0 + 8, c0:c0 + 128]).astype(F32)
                for i, v in enumerate(_rhs_sums(quad(0, 0), quad(0, 1), quad(1, 0), quad(1, 1))):
                    wi_v[i, q, g * 16:(g + 1) * 16, :] = v.astype(BF16)
            return (23, gate_wi, run)
        return [item(g, (q + HF) % NF) for q in range(NF) for g in range(KH // 16)]

    def taps_of(val):
        rows, cols = val.shape
        return [(lambda i=i, n=n: val[i * 8:(i + 1) * 8, n * 128:(n + 1) * 128])
                for n in range(cols // 128) for i in range(rows // 8)]

    def activate(kind, t, n, z):
        if kind == 2:
            zt_v[t % 4][0, 0:T, n * 128:(n + 1) * 128] = _gelu2(z)
        else:
            z1_v[n, t * T:(t + 1) * T, :] = z.astype(BF16)

    def piece(kind, t, n, zero, defer=False, halves=False):
        col = n * 128 + (FH if kind == 2 else 0)
        xn = jnp.concatenate(
            [_up(xn32[zero if zero is not None and c == 0 else c,
                      t * T // 2:(t + 1) * T // 2, :]) for c in range(NC)], axis=1)
        w = _up(win_v[0, 0:D // 2, col:col + 128])
        if halves:
            z = jnp.concatenate([_dot(xn[:T // 2], w), _dot(xn[T // 2:], w)], axis=0)
        else:
            z = _dot(xn, w)
        if defer:
            raw_v[...] = z
        else:
            activate(kind, t, n, z)
        return taps_of(z)

    def pair_piece(kind, u, m, gate_idx, slot_done):
        q = (kind - 1) * HF + m
        outs = []

        def wq(lo, hi, j):
            c0 = ((kind - 1) * NF + m + j * HF) * 128
            return _up(win_v[0, lo // 2:hi // 2, c0:c0 + 128])

        for r0 in range(0, T, PR):
            def xq(i, cs):
                r = (2 * u + i) * T + r0
                return jnp.concatenate(
                    [_up(xn32[c, r // 2:(r + PR) // 2, :]) for c in cs], axis=1)

            def fin(i, j, c):
                z = c + _dot(xq(i, [NC - 1]), wq(2 * KH, D, j))
                t, n = 2 * u + i, m + j * HF
                if kind == 2:
                    zt_v[t % 4][0, r0:r0 + PR, n * 128:(n + 1) * 128] = _gelu2(z)
                else:
                    z1_v[n, t * T + r0:t * T + r0 + PR, :] = z.astype(BF16)
                outs.extend(taps_of(z))
                if len(outs) == T // 8:
                    slot_done(list(outs))
                    outs.clear()

            _strassen(
                _dot,
                lambda i: jnp.concatenate(
                    [_up(xs32[u + (gate_idx() if c == 0 and i != 4 else 0), i, c,
                              r0 // 2:(r0 + PR) // 2, :]) for c in range(2)], axis=1),
                lambda i: _up(wi32[i, q]), xq(0, (0, 1)), xq(1, (2, 3)),
                wq(0, KH, 0), wq(KH, 2 * KH, 1), fin)

    pending = []

    def plan(work, zero, n):
        work = [(mk(zero), lo, hi) for mk, lo, hi in work]
        return [a + b for a, b in zip(
            _balance([w for w in work if w[0][0][0] >= 80], n),
            _balance([w for w in work if w[0][0][0] < 80], n))]

    def pair_block(halves, work):
        zero = zero_s[0]
        mode['pairs'] = True
        if pending:
            activate(*pending.pop(), raw_v[...])
        rel = plan(work, zero, 12 * len(halves))
        taps = []
        state = {'gated': False}

        def release(k):
            for i, (_, gate, run) in sorted(rel[k], key=lambda e: e[0]):
                gate(taps[k][i]())
                run()
                state['gated'] = True

        def slot_done(z):
            taps.append(z)
            if len(taps) > LAG:
                release(len(taps) - 1 - LAG)

        for kind, u in halves:
            for m in range(HF):
                pair_piece(kind, u, m, lambda: zero if state['gated'] else 0, slot_done)
        for k in range(len(taps) - LAG, len(taps)):
            release(k)

    def block(pieces, work, defer=True, free=None):
        zero = zero_s[0]
        if pending:
            activate(*pending.pop(), raw_v[...])
        rel = plan(work, zero, len(pieces))
        taps = []
        gated = False
        for k in range(len(pieces) + LAG):
            if free is not None and k == len(pieces) - 1:
                for _, _, run in free(zero):
                    run()
                gated = True
            if k < len(pieces):
                last = defer and k == len(pieces) - 1
                halves = len(pieces) % 4 == 2 and k == len(pieces) - 1
                taps.append(piece(*pieces[k], zero if gated else None, last, halves))
                if last:
                    pending.append(pieces[k])
            if k >= LAG:
                for i, (_, gate, run) in sorted(rel[k - LAG], key=lambda e: e[0]):
                    gate(taps[k - LAG][i]())
                    run()
                    gated = True

    def cols(kind, t, lo=0, hi=NF):
        return [(kind, t, n) for n in range(lo, hi)]

    def lnx(t):
        return lambda zero: lnx_items(t, zero)

    def lnz(t):
        return lambda zero: lnz_items(t, zero)

    wait(1)
    for it in lnx_items(0, 0) + lnx_items(1, 0):
        it[2]()
    wait(2)
    block(cols(2, 0, 0, 2) + cols(2, 1, 0, 2), [])
    for c in range(1, NC):
        for d in tile_cps(c) + (wsp2_cps(c - 1) if c <= HF else []):
            d.start()
    wout_cp.start()
    wait(3)
    block(cols(2, 0, 2, 4) + cols(2, 1, 2, 4), [])
    wait(4)
    block(cols(2, 0, 4) + cols(2, 1, 4) + cols(1, 0, 0, 1) + cols(1, 1, 0, 1), [])
    wait(5)
    block(cols(1, 0, 1, 4) + cols(1, 1, 1, 4), [(lnz(0), 0, 1)])
    wait(6)
    block(cols(1, 0, 4) + cols(1, 1, 4), [], free=lnx(2))

    def tiles(lo, hi):
        return [pc for t in range(lo, hi) for pc in cols(2, t) + cols(1, t)]

    wait(7)
    block(tiles(2, 4),
          [(lnx(3), 0, 7), (lnx(4), 0, 14), (lnx(5), 0, 15), (lnz(1), 0, 19),
           (wisum, 0, 24), (xsum(2), 17, 24)])
    wait(8)
    pair_block([(2, 2), (1, 2), (2, 3), (1, 3), (2, 4), (1, 4)],
               [(lnx(6), 0, 11), (lnx(7), 0, 11), (xsum(3), 13, 19),
                (lnx(8), 0, 35), (lnx(9), 0, 35), (xsum(4), 37, 43),
                (lnx(10), 0, 62), (lnx(11), 0, 62), (xsum(5), 64, 72),
                (lnz(2), 0, 20), (lnz(3), 0, 20), (lnz(4), 12, 44), (lnz(5), 12, 44),
                (lnz(6), 36, 67), (lnz(7), 36, 67), (kv_items, 0, 72)])
    wait(9)
    pair_block([(2, 5), (1, 5), (2, 6), (2, 7), (1, 6), (1, 7)],
               [(lnx(12), 0, 11), (lnx(13), 0, 11), (xsum(6), 13, 19),
                (lnx(14), 0, 23), (lnx(15), 0, 23), (xsum(7), 25, 31),
                (lnz(8), 0, 20), (lnz(9), 0, 20), (lnz(10), 12, 32), (lnz(11), 12, 32),
                (lnz(12), 36, 54), (lnz(13), 36, 54), (lnz(14), 48, 62), (lnz(15), 48, 62),
                (bsum(8), 24, 72), (bsum(9), 24, 72), (bsum(10), 36, 72), (bsum(11), 36, 72),
                (bsum(12), 58, 72), (bsum(13), 58, 72), (bsum(14), 66, 72), (bsum(15), 66, 72),
                (asum_items(0, HT // 2), 0, 72)])
    wait(10)

    def unit(n, half, k, tap, put_p):
        def span(start, size):
            if isinstance(start, int):
                return slice(start, start + size)
            return pl.ds(pl.multiple_of(start, size), size)

        r = half * (HT // 2) + k
        top, bot = span(r * T, T), span(HS + r * T, T)
        toph, both = span(r * (T // 2), T // 2), span(HS // 2 + r * (T // 2), T // 2)
        sums, sumh = (as32, as232)[half], span(k * (T // 2), T // 2)

        def prod(lhs, rhs):
            acc = None
            for q in range(HS // KG):
                part = _dot(lhs(q), rhs(q))
                acc = part if acc is None else acc + part
                tap(acc)
            return acc

        def sa(i):
            return lambda q: jnp.concatenate(
                [_up(sums[i, c, sumh, :]) for c in range(q * KG // 128, (q + 1) * KG // 128)],
                axis=1)

        def sb(i):
            return lambda q: _up(bs32[i, n, q * KG // 2:(q + 1) * KG // 2, :])

        def a11(q):
            return _up(wsp_v[0, toph, q * KG:(q + 1) * KG])

        def a22(q):
            return _up(wsp_v[0, both, HS + q * KG:HS + (q + 1) * KG])

        def b11(q):
            return _up(z232[n, q * KG // 2:(q + 1) * KG // 2, :])

        def b22(q):
            return _up(z232[n + HF, (HS + q * KG) // 2:(HS + (q + 1) * KG) // 2, :])

        def fin(i, j, c):
            col, rows = n + j * HF, (top, bot)[i]
            put_p(i, j, col, rows, (c + bcol_v[rows, :]).astype(BF16))

        _strassen(prod, sa, sb, a11, a22, b11, b22, fin)

    def p2(n, half):
        nn = jnp.minimum(n + 1, NC - 1)

        @pl.when(n + 1 < NC)
        def _():
            for d in tile_cps(nn):
                d.wait()

        if half == 0:
            for q in range(HF):
                @pl.when(n == q)
                def _():
                    for d in wsp2_cps(q):
                        d.wait()

        zero = zero_s[0]
        fwd_u = _up(tab_v[0:128, :])
        fwd_h = _up(tab_v[128:256, :])
        dd = dd_v[n]

        def put(slot, val):
            pl_v[:, slot] = val

        def re_im(val):
            val = val.reshape(BLK // 8, 2, 8, 128)
            return val[:, 0], val[:, 1]

        kvi = kv_items(nn)

        def pace_kv(d, val):
            if d % 4 == 3:
                for j in range(8):
                    _, gate, run = kvi[(d // 4) * 8 + j]
                    gate(val[j * 32:j * 32 + 8, :])
                    run()

        for i in range(NB):
            u = _dot(fwd_u, _up(kvb32[i * BLK // 2:(i + 1) * BLK // 2, :]))
            a, b = re_im(u)
            put(UA + i, a)
            put(UB + i, b)
            put(US + i, a + b)
            pace_kv(i, u)
        for i in range(NB):
            hb = _up(h_v[n, :, i * BLK:(i + 1) * BLK])
            hf = jax.lax.dot_general(fwd_h, hb, (((1,), (1,)), ((), ())),
                                     preferred_element_type=F32)
            c, d = re_im(hf)
            if i == 0:
                c, d = c + dd, d + dd
            put(HR + i, c)
            put(HP + i, d - c)
            put(HQ + i, c + d)
            pace_kv(NB + i, hf)

        state = {}

        def mac_item(pos, g0, pi, j0, j1):
            xv, hv = ((US, HR), (UA, HP), (UB, HQ))[pi]
            outs = range(g0, g0 + GRP)
            top = g0 + GRP

            def run():
                pz = zero + pos
                hs = {t: pl_v[pz, hv + t]
                      for t in range(max(g0 - j1 + 1, 0), top - j0)}
                acc = state['acc'] if j0 else {o: None for o in outs}
                for jj in range(j0, j1):
                    xj = pl_v[pz, xv + jj]
                    for o in outs:
                        if o - jj >= 0:
                            t = xj * hs[o - jj]
                            acc[o] = t if acc[o] is None else acc[o] + t
                if j1 < top:
                    state['acc'] = acc
                    return
                r0 = pos * 8
                if pi == 0:
                    state['k1'] = acc
                elif pi == 1:
                    state['im'] = {o: state['k1'][o] + acc[o] for o in outs}
                else:
                    for o in outs:
                        re, im = state['k1'][o] - acc[o], state['im'][o]
                        zr, zi = re, im
                        if o > 0:
                            zr, zi = re - state['prev'][1], im + state['prev'][0]
                        state['prev'] = (re, im)
                        zz_v[n, o, r0:r0 + 8, :] = zr.astype(BF16)
                        zz_v[n, o, BLK + r0:BLK + r0 + 8, :] = zi.astype(BF16)

            nmac = sum(1 for o in outs for jj in range(j0, j1) if o >= jj)
            return (2 * nmac + ((0, GRP, 5 * GRP)[pi] if j1 == top else 0), gate_pl, run)

        items = []
        for pos in range(BLK // 8):
            for g0 in range(0, NB, GRP):
                top = g0 + GRP
                cuts = [0, top] if top <= SPLIT else [0, (top - 1) // 2, top]
                for pi in range(3):
                    for j0, j1 in zip(cuts[:-1], cuts[1:]):
                        items.append(mac_item(pos, g0, pi, j0, j1))

        if half == 0:
            extra = [asum_dyn(jnp.minimum(n * NG + g, HS // 32 - 1), c)
                     for g in range(NG) for c in range(HT)]
            every = len(items) // len(extra)
            items = [it for i, e in enumerate(extra)
                     for it in items[i * every:(i + 1) * every] + [e]
                     ] + items[len(extra) * every:]

        total = sum(c for c, _, _ in items)
        tap_of = []
        cum = 0
        for c, _, _ in items:
            tap_of.append(int(cum * NTAP / total))
            cum += c
        pos = {'tap': 0, 'item': 0}

        def tap(acc):
            t0 = pos['tap']
            pos['tap'] += T // 8
            while pos['item'] < len(items) and tap_of[pos['item']] < pos['tap']:
                i = tap_of[pos['item']] - t0
                _, gate, run = items[pos['item']]
                gate(acc[i * 8:(i + 1) * 8, :])
                run()
                pos['item'] += 1

        def put_p(i, j, col, rows, val):
            p_v[col, rows, :] = val

        for k in range(HT // 2):
            unit(n - half * HF, half, k, tap, put_p)
        assert pos['item'] == len(items)
        return 0

    jax.lax.fori_loop(0, HF, lambda n, c: p2(n, 0), 0)
    jax.lax.fori_loop(HF, NC, lambda n, c: p2(n, 1), 0)

    wout_cp.wait()

    def p3(j, carry):
        inv_p = _up(tab_v[256:288, :])
        inv_m = _up(tab_v[288:320, :])
        rev = 7 - jax.lax.broadcasted_iota(jnp.int32, (8, 128), 0)

        zero = zero_s[0]
        HK = FH // 2

        def rows(k, i):
            tile = i * HT + (k // 2) * (HT // 2) + 2 * j + k % 2
            return (tile, pl.ds(pl.multiple_of(tile * T, T), T),
                    pl.ds(pl.multiple_of(tile * (T // 2), T // 2), T // 2))

        def fresh(k, n):
            return k >= 2 and n % HF == HF - 1

        def p_tile(k, i, n):
            return _up(pp32[k, i, n])

        def gate_p(tok):
            p_v[0, S:S + 8, :] = tok.astype(BF16)

        def gate_wo(tok):
            wout_v[0, HK:HK + 8, 0:128] = pltpu.bitcast(tok, U32)

        def psum_item(k, n, g):
            def run():
                def quad(i, jj):
                    rs = pl.ds(pl.multiple_of(rows(k, i)[0] * T + g * 16, 16), 16)
                    if fresh(k, n):
                        gv = pq_v[k - 2, i, jj, g * 16:(g + 1) * 16, :]
                    else:
                        gv = p_v[n + jj * HF, rs, :]
                    pv = _gelu2(z1_v[n + jj * HF, rs, :].astype(F32)) * gv.astype(F32)
                    pp_v[k, i, n + jj * HF, g * 16:(g + 1) * 16, :] = pv.astype(BF16)
                    return pv
                for i, v in enumerate(_lhs_sums(quad(0, 0), quad(0, 1), quad(1, 0), quad(1, 1))):
                    ps_v[k, i, n, g * 16:(g + 1) * 16, :] = v.astype(BF16)
            return (gate_p, run)

        def wsum_item(m, g):
            def run():
                def quad(i, jj):
                    r0 = (i * HK + g * 16) // 2
                    c0 = (m + 2 * jj) * 128
                    return _up(wout_v[zero, r0:r0 + 8, c0:c0 + 128]).astype(F32)
                for i, v in enumerate(_rhs_sums(quad(0, 0), quad(0, 1), quad(1, 0), quad(1, 1))):
                    ws_v[i, m, g * 16:(g + 1) * 16, :] = v.astype(BF16)
            return (gate_wo, run)

        def psum(k):
            return [psum_item(k, n, g) for n in range(HF) if not fresh(k, n)
                    for g in range(T // 16)]

        queue = []

        def tap(val):
            for i in range(min(len(queue), queue_step[0])):
                gate, run = queue.pop(0)
                r = (i * (T // 8)) // queue_step[0] * 8
                gate(val[r:r + 8, :])
                run()

        queue_step = [0]

        def paced(items, ntaps):
            assert not queue
            queue.extend(items)
            queue_step[0] = -(-len(items) // ntaps)

        def do_unit(u):
            def put_q(i, jj, col, rws, val):
                pq_v[u, i, jj] = val
            unit(HF - 1, 1, 2 * j + u, tap, put_q)
            for g in range(T // 16):
                psum_item(2 + u, HF - 1, g)[1]()

        def finish(k, i, c, o):
            tile, rs, hs = rows(k, i)
            cs = slice(c * 128, (c + 1) * 128)
            ye = _dot(inv_p, _up(zz32[c, tile, 0:64, :]))
            yo = _dot(inv_m, _up(zz32[c, tile, 64:128, :]))
            yd = ye - yo
            y = jnp.concatenate(
                [ye + yo] + [
                    jnp.take_along_axis(yd[q * 8:(q + 1) * 8], rev, axis=0,
                                        mode="promise_in_bounds")
                    for q in reversed(range(BLK // 16))], axis=0)
            gate = o * (1.0 + jnp.tanh((0.25 / _A) * o))
            x = _up(x_v[0, hs, cs]).astype(F32)
            xn = xn_v[c, rs, :].astype(F32)
            o_v[rs, cs] = (x + (xn * y) * gate).astype(BF16)

        def do_pair(k, last=False):
            def prod(lhs, rhs):
                res = _dot(lhs, rhs)
                tap(res)
                return res

            def sa(i):
                return jnp.concatenate([_up(ps32[k, i, n]) for n in range(HF)], axis=1)

            a11 = jnp.concatenate([p_tile(k, 0, n) for n in range(HF)], axis=1)
            a22 = jnp.concatenate([p_tile(k, 1, n) for n in range(HF, NF)], axis=1)
            for m in range(2):
                _strassen(
                    prod, sa, lambda i: _up(ws32[i, m]), a11, a22,
                    _up(wout_v[0, 0:HK // 2, m * 128:(m + 1) * 128]),
                    _up(wout_v[0, HK // 2:HK, (m + 2) * 128:(m + 3) * 128]),
                    lambda i, jj, o: finish(k, i, m + 2 * jj, o))
            for i in range(2):
                rs = rows(k, i)[1]
                if last:
                    cp(o_v.at[rs, 0:512], out_hbm.at[0, rs, 0:512], out_sem).start()
            for i in range(2):
                rs = rows(k, i)[1]
                p = jnp.concatenate([p_tile(k, i, n) for n in range(NF)], axis=1)
                finish(k, i, NC - 1, _dot(p, _up(wout_v[0, 0:HK, 512:D])))
                if last:
                    cp(o_v.at[rs, 512:D], out_hbm.at[0, rs, 512:D], out_sem).start()
                else:
                    cp(o_v.at[rs, :], out_hbm.at[0, rs, :], out_sem).start()

        paced(psum(0) + [wsum_item(m, g) for m in range(2) for g in range(HK // 16)], 12)
        do_unit(0)
        paced(psum(1), 12)
        do_pair(0)
        paced(psum(2), 12)
        do_unit(1)
        paced(psum(3), 12)
        do_pair(1)
        do_pair(2)
        do_pair(3, last=True)
        return carry

    jax.lax.fori_loop(0, P3I, p3, 0)
    cp(o_v, out_hbm.at[0], out_sem).wait()


@jax.jit
def pallas_recurrent_scan__ssm_conv_h3__mixer_gmlp__prompt_kernel(
    A_q: jax.Array,
    A_k: jax.Array,
    A_v: jax.Array,
    A_shift_k: jax.Array,
    A_ssm_k: jax.Array,
    A_ssm_D: jax.Array,
    B_x: jax.Array,
    B_w_in: jax.Array,
    B_w_sp: jax.Array,
    B_b_sp: jax.Array,
    B_w_out: jax.Array,
):
    del B_x
    tab = jnp.asarray(_dft_tables(), dtype=BF16)

    any_spec = pl.BlockSpec(memory_space=pl.ANY)
    return pl.pallas_call(
        _kernel,
        out_shape=jax.ShapeDtypeStruct((1, S, D), BF16),
        in_specs=[any_spec] * 11,
        out_specs=any_spec,
        scratch_shapes=[
            pltpu.VMEM((1, S // 2 + 32, D), U32),
            pltpu.VMEM((1, D // 2 + 8, 2 * FH), U32),
            pltpu.VMEM((1, S // 2 + 8, S), U32),
            pltpu.VMEM((1, FH // 2 + 32, D), U32),
            pltpu.VMEM((2 * NC, S // 2 + 32, 128), U32),
            pltpu.VMEM((NC, 64, S), U32),
            pltpu.VMEM((NC, S + 256, 128), BF16),
            pltpu.VMEM((NF, S, 128), BF16),
            pltpu.VMEM((NF, S + 64, 128), BF16),
            pltpu.VMEM((NF, S + 64, 128), BF16),
            pltpu.VMEM((5, HT, HS // 2, 128), BF16),
            pltpu.VMEM((5, HT, HS // 2, 128), BF16),
            pltpu.VMEM((5, HF, HS, 128), BF16),
            pltpu.VMEM((2, 2, 2, T, 128), BF16),
            pltpu.VMEM((4, 2, NF, T, 128), BF16),
            pltpu.VMEM((4, 5, HF, T, 128), BF16),
            pltpu.VMEM((5, 2, FH // 2, 128), BF16),
            pltpu.VMEM((S, 128), BF16),
            pltpu.VMEM((BLK // 8, 6 * NB + 1, 8, 128), F32),
            pltpu.VMEM((NC, NB, 2 * BLK, 128), BF16),
            pltpu.VMEM((S, 128), F32),
            pltpu.VMEM((S, D), BF16),
            pltpu.VMEM((1, T + 16, FH), F32),
            pltpu.VMEM((1, T + 16, FH), F32),
            pltpu.VMEM((1, T + 16, FH), F32),
            pltpu.VMEM((1, T + 16, FH), F32),
            pltpu.VMEM((NT // 2, 5, 2, T, 128), BF16),
            pltpu.VMEM((5, NF, KH, 128), BF16),
            pltpu.VMEM((T, 128), F32),
            pltpu.VMEM((320, 128), U32),
            pltpu.VMEM((NC, KS, 128), F32),
            pltpu.VMEM((NC + 2, 1, 128), F32),
            pltpu.VMEM((KS, D), BF16),
            pltpu.VMEM((D,), BF16),
            pltpu.VMEM((S,), BF16),
            pltpu.SMEM((1,), jnp.int32),
            pltpu.SemaphoreType.DMA((16,)),
        ],
        compiler_params=pltpu.CompilerParams(
            vmem_limit_bytes=100 * 1024 * 1024, disable_bounds_checks=True),
    )(A_q, A_k, A_v, A_shift_k.T, A_ssm_k, A_ssm_D, B_w_in, B_w_sp, B_b_sp, B_w_out, tab)
```

```python
import jax
import jax.numpy as jnp
import numpy as np
import jax.experimental.pallas as pl
import jax.experimental.pallas.tpu as pltpu

F32 = jnp.float32
BF16 = jnp.bfloat16
U32 = jnp.uint32

S = 2048
D = 640
FH = 768
KS = 4
BLK = 128
NB = S // BLK
NC = D // 128
NF = FH // 128
T = 128
NT = S // T
EPS = 1e-5
GRP = 4
SPLIT = 8
import os
AW = int(os.environ.get('AW', 2))
PR = int(os.environ.get('PR', 128))
KG = 512
KR = 32
UA, UB, US, HP, HQ, HR, TOK = (i * NB for i in range(7))
LAG = 4
NTAP = 888
HS = S // 2
HT = HS // T
HF = NF // 2
KH = 256
P3I = 2

_GELU_C0 = float(np.sqrt(2.0 / np.pi))
_GELU_C1 = _GELU_C0 * 0.044715
_A = _GELU_C1 ** (1.0 / 3.0)
_K = _GELU_C0 / _A


def _dft_tables():
    m = np.arange(BLK)[:, None]
    n = np.arange(BLK)[None, :]
    th = 2.0 * np.pi * (((4 * m + 1) * n) % (4 * BLK)) / (4 * BLK)
    ph = 2.0 * np.pi * (((4 * m + 1) * (2 * n + 1)) % (8 * BLK)) / (8 * BLK)
    fu = np.concatenate([np.cos(ph), -np.sin(ph)], axis=0)
    fh = np.concatenate([np.cos(th) + np.sin(th), np.cos(th) - np.sin(th)], axis=0)
    fu, fh = (f.reshape(2, BLK // 8, 8, BLK).transpose(1, 0, 2, 3).reshape(2 * BLK, BLK)
              for f in (fu, fh))
    cp = (np.cos(ph) + np.sin(ph)).T[:BLK // 2] / (8.0 * BLK * _A * _A)
    cm = (np.cos(ph) - np.sin(ph)).T[:BLK // 2] / (8.0 * BLK * _A * _A)
    return np.concatenate([fu, fh, cp, cm], axis=0).astype(np.float32)


def _layernorm(x, eps, scale=1.0):
    m = jnp.mean(x, axis=-1, keepdims=True)
    d = x - m
    v = jnp.sum(d * d, axis=-1, keepdims=True) * (1.0 / (x.shape[-1] * scale * scale))
    return d * jax.lax.rsqrt(v + eps / (scale * scale))


def _gelu2(y):
    return y * (1.0 + jnp.tanh(y * (y * y + _K)))


def _up(x):
    return pltpu.bitcast(x, BF16)


def _dot(a, b):
    return jnp.dot(a, b, preferred_element_type=F32)


def _lhs_sums(a11, a12, a21, a22):
    return a11 + a22, a21 + a22, a11 + a12, a21 - a11, a12 - a22


def _rhs_sums(b11, b12, b21, b22):
    return b11 + b22, b12 - b22, b21 - b11, b11 + b12, b21 + b22


def _strassen(prod, sa, sb, a11, a22, b11, b22, fin):
    m2 = prod(sa(1), b11)
    m4 = prod(a22, sb(2))
    fin(1, 0, m2 + m4)
    m5 = prod(sa(2), b22)
    c11 = m4 - m5
    m3 = prod(a11, sb(1))
    fin(0, 1, m3 + m5)
    c22 = m3 - m2
    m1 = prod(sa(0), sb(0))
    c11, c22 = c11 + m1, c22 + m1
    fin(0, 0, c11 + prod(sa(4), sb(4)))
    fin(1, 1, c22 + prod(sa(3), sb(3)))


def _balance(work, n):
    jobs = [(lo, hi, sum(it[0] for it in items)) for items, lo, hi in work]
    rate = [None] * n
    while jobs:
        def free(a, b):
            return [p for p in range(a, b) if rate[p] is None]
        dens, a, b = max(
            (sum(w for lo, hi, w in jobs if a <= lo and hi <= b) / max(len(free(a, b)), 1e-9), a, b)
            for a in {j[0] for j in jobs} for b in {j[1] for j in jobs} if a < b)
        while a > 0 and rate[a - 1] is not None:
            a -= 1
        while b < n and rate[b] is not None:
            b += 1
        for p in free(a, b):
            rate[p] = dens
        jobs = [(lo, hi, w) for lo, hi, w in jobs if not (a <= lo and hi <= b)]
        jobs = [(b if a <= lo < b else lo, a if a < hi <= b else hi, w) for lo, hi, w in jobs]
    queues = [[lo * 16, hi * 16, list(items)] for items, lo, hi in work]
    rel = [[] for _ in range(n)]
    budget = 0.0
    for tau in range(n * 16):
        budget += (rate[tau // 16] or 0.0) / 16
        while True:
            ready = [q for q in queues if q[2] and q[0] <= tau]
            if not ready:
                budget = min(budget, 0.0)
                break
            q = min(ready, key=lambda q: q[1])
            if budget < 0 and q[1] - tau > len(q[2]):
                break
            it = q[2].pop(0)
            rel[tau // 16].append((tau % 16, it))
            budget -= it[0]
    assert not any(q[2] for q in queues)
    return rel


def _kernel(x_hbm, k_hbm, v_hbm, skt_hbm, h_hbm, dv_hbm, win_hbm, wsp_hbm, b_hbm,
            wout_hbm, tab_hbm, out_hbm,
            x_v, win_v, wsp_v, wout_v, kv_v, h_v, xn_v, z1_v, z2_v, p_v, as_v, as2_v, bs_v, pq_v, pp_v, ps_v, ws_v,
            kvb_v, pl_v, zz_v, bcol_v, o_v, zta_v, ztb_v, ztc_v, ztd_v, zte_v, ztf_v, xs_v, wi_v, raw_v, tab_v,
            sk_v, dd_v, skt_v, dv_v, b_v, zero_s, sem):
    cp = pltpu.make_async_copy
    x16 = x_v.bitcast(BF16)
    win16 = win_v.bitcast(BF16)
    kv16 = kv_v.bitcast(BF16)
    h16 = h_v.bitcast(BF16)

    xn32, z232, kvb32, zz32, as32, as232, bs32, pp32, ps32, ws32, xs32, wi32 = (
        r.bitcast(U32)
        for r in (xn_v, z2_v, kvb_v, zz_v, as_v, as2_v, bs_v, pp_v, ps_v, ws_v, xs_v, wi_v))
    wsp16 = wsp_v.bitcast(BF16)

    def wsp_cp(lo, hi, s):
        return cp(wsp_hbm.at[lo:hi, :], wsp16.at[0, lo:hi, :], sem.at[s])

    def x_cp(lo, hi, s):
        return cp(x_hbm.at[0, lo:hi, :], x16.at[0, lo:hi, :], sem.at[s])

    def win_cp(lo, hi, s):
        return cp(win_hbm.at[:, lo:hi], win16.at[0, 0:D, lo:hi], sem.at[s])

    def k_cp(c, s):
        return cp(k_hbm.at[0, :, pl.ds(c * 128, 128)], kv16.at[2 * c, 0:S, :], sem.at[s])

    def v_cp(c, s):
        return cp(v_hbm.at[0, :, pl.ds(c * 128, 128)], kv16.at[2 * c + 1, 0:S, :], sem.at[s])

    def h_cp(c, s):
        return cp(h_hbm.at[pl.ds(c * 128, 128), :], h16.at[c], sem.at[s])

    groups = [
        [cp(b_hbm, b_v, sem.at[0]), cp(skt_hbm, skt_v, sem.at[0]), cp(dv_hbm, dv_v, sem.at[0])],
        [x_cp(0, 256, 1)],
        [win_cp(FH, FH + 256, 2)],
        [win_cp(FH + 256, FH + 512, 3)],
        [win_cp(FH + 512, 2 * FH, 4), win_cp(0, 128, 4)],
        [win_cp(128, 512, 11)],
        [win_cp(512, FH, 5), x_cp(256, 384, 5)],
        [x_cp(384, 6 * T, 6)],
        [x_cp(6 * T, 12 * T, 7), k_cp(0, 7), v_cp(0, 7)],
        [x_cp(12 * T, S, 12), wsp_cp(0, HS // 2, 12), wsp_cp(HS, HS + HS // 2, 12)],
        [cp(tab_hbm, tab_v.bitcast(BF16), sem.at[8]), h_cp(0, 8)],
    ]
    for g in groups:
        for c in g:
            c.start()

    def tile_cps(c):
        s = jnp.where(c == NC - 1, 9, c - 1) if isinstance(c, jax.Array) else (0, 1, 2, 9)[c - 1]
        return [k_cp(c, s), v_cp(c, s), h_cp(c, s)]

    NG = -(-HS // 32 // HF)

    def wsp2_cps(n):
        lo, hi = HS // 2 + n * NG * 16, min(HS // 2 + (n + 1) * NG * 16, HS)
        return [wsp_cp(lo, hi, 13 + n), wsp_cp(HS + lo, HS + hi, 13 + n)]

    wout_cp = cp(wout_hbm, wout_v.bitcast(BF16).at[0, 0:FH, :], sem.at[10])
    out_sem = sem.at[5]

    def wait(i):
        for c in groups[i]:
            c.wait()

    zero_s[0] = 0
    wait(0)
    skt = skt_v[...].astype(F32)
    dv = dv_v[...].astype(F32).reshape(1, D)
    for c in range(NC):
        sk_v[c] = skt[:, c * 128:(c + 1) * 128]
        dd_v[c] = dv[:, c * 128:(c + 1) * 128]
    brow = b_v[...].astype(F32).reshape(1, S)
    bcol_v[...] = jnp.broadcast_to(brow, (128, S)).T

    def gate_x(tok):
        x_v[0, S // 2:S // 2 + 8, 0:128] = pltpu.bitcast(tok, U32)

    zt_v = (zta_v, ztb_v, ztc_v, ztd_v, zte_v, ztf_v)

    def gate_zt(t):
        def gate(tok):
            zt_v[t % 6][0, T:T + 8, 0:128] = tok
        return gate

    def gate_kv(tok):
        kv_v[0, S // 2:S // 2 + 8, :] = pltpu.bitcast(tok, U32)

    def gate_pl(tok):
        pl_v[0, TOK] = tok

    ndone = [0]

    mode = {'pairs': False}

    def done(val):
        r = (ndone[0] % 8) * 16
        ndone[0] += 1
        if mode['pairs']:
            xs_v[0, 0, 0, r:r + 16, :] = val
        else:
            xn_v[0, S + r:S + r + 16, :] = val

    def lnx_items(t, zero):
        def item(r0):
            def run():
                rs = slice(r0 // 2, r0 // 2 + 8)
                xw = jnp.concatenate([x_v[zero, rs, 0:128], x_v[0, rs, 128:D]], axis=1)
                xn = _layernorm(_up(xw).astype(F32), EPS, _A)
                for c in range(NC):
                    xb = xn[:, c * 128:(c + 1) * 128].astype(BF16)
                    xn_v[c, r0:r0 + 16, :] = xb
                if mode['pairs']:
                    done(xb)
            return (85, gate_x, run)
        return [item(t * T + g * 16) for g in range(T // 16)]

    def lnz_items(t, zero):
        def item(g):
            def run():
                rs = slice(g * 16, (g + 1) * 16)
                z = jnp.concatenate(
                    [zt_v[t % 6][zero, rs, 0:128], zt_v[t % 6][0, rs, 128:FH]], axis=1)
                z = _layernorm(z, 4.0 * _A * _A * EPS)
                r0 = t * T + g * 16
                for n in range(NF):
                    zb = z[:, n * 128:(n + 1) * 128].astype(BF16)
                    z2_v[n, r0:r0 + 16, :] = zb
                done(zb)
            return (90, gate_zt(t), run)
        return [item(g) for g in range(T // 16)]

    def kv_items(c):
        sk = sk_v[c]

        def item(r0):
            def run():
                hs = slice(r0 // 2, (r0 + KR) // 2)
                if r0 == 0:
                    kw = jnp.concatenate(
                        [jnp.zeros((8, 128), F32), _up(kv_v[2 * c, hs, :]).astype(F32)], axis=0)
                else:
                    kw = _up(kv_v[2 * c, r0 // 2 - 8:(r0 + KR) // 2, :]).astype(F32)[8:]
                ks = kw[8:] * sk[0:1, :]
                for t in range(1, KS):
                    ks = ks + pltpu.roll(kw, t, 0)[8:] * sk[t:t + 1, :]
                kvb_v[r0:r0 + KR, :] = (
                    ks * _up(kv_v[2 * c + 1, hs, :]).astype(F32)).astype(BF16)
            return (14 * KR // 8, gate_kv, run)
        return [item(r0) for r0 in range(0, S, KR)]

    def gate_w(tok):
        wsp_v[0, S // 2:S // 2 + 8, 0:128] = pltpu.bitcast(tok, U32)

    def asum_items(r_lo, r_hi):
        def item(zero, r0, c0):
            def run():
                def quad(i, j, c):
                    w = wsp_v[zero, (i * HS + r0) // 2:(i * HS + r0) // 2 + 8,
                              j * HS + c * 128:j * HS + (c + 1) * 128]
                    return _up(w).astype(F32)
                for c in range(c0, c0 + AW):
                    for i, v in enumerate(_lhs_sums(
                            quad(0, 0, c), quad(0, 1, c), quad(1, 0, c), quad(1, 1, c))):
                        as_v[i, c, r0:r0 + 16, :] = v.astype(BF16)
            return (23 * AW, gate_w, run)
        return lambda zero: [item(zero, r0, c0) for r0 in range(r_lo * T, r_hi * T, 16)
                             for c0 in range(0, HT, AW)]

    def asum_dyn(g, c):
        def run():
            def quad(i, j):
                r0 = pl.multiple_of(i * (HS // 2) + HS // 4 + g * 8, 8)
                w = wsp_v[0, pl.ds(r0, 8), j * HS + c * 128:j * HS + (c + 1) * 128]
                return _up(w).astype(F32)
            rs = pl.ds(pl.multiple_of(g * 16, 16), 16)
            for i, v in enumerate(_lhs_sums(quad(0, 0), quad(0, 1), quad(1, 0), quad(1, 1))):
                as2_v[i, c, rs, :] = v.astype(BF16)
        return (23, gate_w, run)

    def gate_z2(tok):
        z2_v[0, S:S + 8, :] = tok.astype(BF16)

    def bsum(t):
        def item(zero, r0, n):
            def run():
                def quad(i, j):
                    return z2_v[zero + n + j * HF, i * HS + r0:i * HS + r0 + 16, :].astype(F32)
                for i, v in enumerate(_rhs_sums(quad(0, 0), quad(0, 1), quad(1, 0), quad(1, 1))):
                    bs_v[i, n, r0:r0 + 16, :] = v.astype(BF16)
            return (24, gate_z2, run)
        return lambda zero: [item(zero, r0, n) for r0 in range((t - HT) * T, (t - HT + 1) * T, 16)
                             for n in range(HF)]

    def gate_xn(tok):
        xn_v[1, S:S + 8, :] = tok.astype(BF16)

    def xsum(u):
        def item(zero, g, c):
            def run():
                def quad(i, j):
                    r0 = (2 * u + i) * T + g * 16
                    return xn_v[zero + c + 2 * j, r0:r0 + 16, :].astype(F32)
                for i, v in enumerate(_lhs_sums(quad(0, 0), quad(0, 1), quad(1, 0), quad(1, 1))):
                    xs_v[u, i, c, g * 16:(g + 1) * 16, :] = v.astype(BF16)
            return (24, gate_xn, run)
        return lambda zero: [item(zero, g, c) for g in range(T // 16) for c in range(2)]

    def gate_wi(tok):
        win_v[0, D // 2:D // 2 + 8, 0:128] = pltpu.bitcast(tok, U32)

    def wisum(zero):
        def item(g, q):
            def run():
                def quad(i, j):
                    r0 = (i * KH + g * 16) // 2
                    c0 = ((q // HF) * NF + q % HF + j * HF) * 128
                    return _up(win_v[zero, r0:r0 + 8, c0:c0 + 128]).astype(F32)
                for i, v in enumerate(_rhs_sums(quad(0, 0), quad(0, 1), quad(1, 0), quad(1, 1))):
                    wi_v[i, q, g * 16:(g + 1) * 16, :] = v.astype(BF16)
            return (23, gate_wi, run)
        return [item(g, (q + HF) % NF) for q in range(NF) for g in range(KH // 16)]

    def taps_of(val):
        rows, cols = val.shape
        return [(lambda i=i, n=n: val[i * 8:(i + 1) * 8, n * 128:(n + 1) * 128])
                for n in range(cols // 128) for i in range(rows // 8)]

    def activate(kind, t, n, z):
        if kind == 2:
            zt_v[t % 6][0, 0:T, n * 128:(n + 1) * 128] = _gelu2(z)
        else:
            z1_v[n, t * T:(t + 1) * T, :] = z.astype(BF16)

    def piece(kind, t, n, zero, defer=False, halves=False):
        col = n * 128 + (FH if kind == 2 else 0)
        xn = jnp.concatenate(
            [_up(xn32[zero if zero is not None and c == 0 else c,
                      t * T // 2:(t + 1) * T // 2, :]) for c in range(NC)], axis=1)
        w = _up(win_v[0, 0:D // 2, col:col + 128])
        if halves:
            z = jnp.concatenate([_dot(xn[:T // 2], w), _dot(xn[T // 2:], w)], axis=0)
        else:
            z = _dot(xn, w)
        if defer:
            raw_v[...] = z
        else:
            activate(kind, t, n, z)
        return taps_of(z)

    def pair_piece(kind, u, m, gate_idx, slot_done):
        q = (kind - 1) * HF + m
        outs = []

        def wq(lo, hi, j):
            c0 = ((kind - 1) * NF + m + j * HF) * 128
            return _up(win_v[0, lo // 2:hi // 2, c0:c0 + 128])

        for r0 in range(0, T, PR):
            def xq(i, cs):
                r = (2 * u + i) * T + r0
                return jnp.concatenate(
                    [_up(xn32[c, r // 2:(r + PR) // 2, :]) for c in cs], axis=1)

            def fin(i, j, c):
                z = c + _dot(xq(i, [NC - 1]), wq(2 * KH, D, j))
                t, n = 2 * u + i, m + j * HF
                if kind == 2:
                    zt_v[t % 6][0, r0:r0 + PR, n * 128:(n + 1) * 128] = _gelu2(z)
                else:
                    z1_v[n, t * T + r0:t * T + r0 + PR, :] = z.astype(BF16)
                outs.extend(taps_of(z))
                if len(outs) == T // 8:
                    slot_done(list(outs))
                    outs.clear()

            _strassen(
                _dot,
                lambda i: jnp.concatenate(
                    [_up(xs32[u + (gate_idx() if c == 0 and i != 4 else 0), i, c,
                              r0 // 2:(r0 + PR) // 2, :]) for c in range(2)], axis=1),
                lambda i: _up(wi32[i, q]), xq(0, (0, 1)), xq(1, (2, 3)),
                wq(0, KH, 0), wq(KH, 2 * KH, 1), fin)

    pending = []

    def plan(work, zero, n):
        work = [(mk(zero), lo, hi) for mk, lo, hi in work]
        return [a + b for a, b in zip(
            _balance([w for w in work if w[0][0][0] >= 80], n),
            _balance([w for w in work if w[0][0][0] < 80], n))]

    def pair_block(halves, work):
        zero = zero_s[0]
        mode['pairs'] = True
        if pending:
            activate(*pending.pop(), raw_v[...])
        rel = plan(work, zero, 12 * len(halves))
        taps = []
        state = {'gated': False}

        def release(k):
            for i, (_, gate, run) in sorted(rel[k], key=lambda e: e[0]):
                gate(taps[k][i]())
                run()
                state['gated'] = True

        def slot_done(z):
            taps.append(z)
            if len(taps) > LAG:
                release(len(taps) - 1 - LAG)

        for kind, u in halves:
            for m in range(HF):
                pair_piece(kind, u, m, lambda: zero if state['gated'] else 0, slot_done)
        for k in range(len(taps) - LAG, len(taps)):
            release(k)

    def block(pieces, work, defer=True, free=None):
        zero = zero_s[0]
        if pending:
            activate(*pending.pop(), raw_v[...])
        rel = plan(work, zero, len(pieces))
        taps = []
        gated = False
        for k in range(len(pieces) + LAG):
            if free is not None and k == len(pieces) - 1:
                for _, _, run in free(zero):
                    run()
                gated = True
            if k < len(pieces):
                last = defer and k == len(pieces) - 1
                halves = len(pieces) % 4 == 2 and k == len(pieces) - 1
                taps.append(piece(*pieces[k], zero if gated else None, last, halves))
                if last:
                    pending.append(pieces[k])
            if k >= LAG:
                for i, (_, gate, run) in sorted(rel[k - LAG], key=lambda e: e[0]):
                    gate(taps[k - LAG][i]())
                    run()
                    gated = True

    def cols(kind, t, lo=0, hi=NF):
        return [(kind, t, n) for n in range(lo, hi)]

    def lnx(t):
        return lambda zero: lnx_items(t, zero)

    def lnz(t):
        return lambda zero: lnz_items(t, zero)

    wait(1)
    for it in lnx_items(0, 0) + lnx_items(1, 0):
        it[2]()
    wait(2)
    block(cols(2, 0, 0, 2) + cols(2, 1, 0, 2), [])
    for c in range(1, NC):
        for d in tile_cps(c) + (wsp2_cps(c - 1) if c <= HF else []):
            d.start()
    wout_cp.start()
    wait(3)
    block(cols(2, 0, 2, 4) + cols(2, 1, 2, 4), [])
    wait(4)
    block(cols(2, 0, 4) + cols(2, 1, 4) + cols(1, 0, 0, 1) + cols(1, 1, 0, 1), [])
    wait(5)
    block(cols(1, 0, 1, 4) + cols(1, 1, 1, 4), [(lnz(0), 0, 1)])
    wait(6)
    block(cols(1, 0, 4) + cols(1, 1, 4), [], free=lnx(2))

    def tiles(lo, hi):
        return [pc for t in range(lo, hi) for pc in cols(2, t) + cols(1, t)]

    wait(7)
    block(tiles(2, 4),
          [(lnx(3), 0, 7), (lnx(4), 0, 14), (lnx(5), 0, 15), (lnz(1), 0, 19),
           (wisum, 0, 24), (xsum(2), 17, 24)])
    wait(8)
    pair_block([(2, 2), (1, 2), (2, 3), (1, 3), (2, 4), (1, 4)],
               [(lnx(6), 0, 11), (lnx(7), 0, 11), (xsum(3), 13, 19),
                (lnx(8), 0, 35), (lnx(9), 0, 35), (xsum(4), 37, 43),
                (lnx(10), 0, 62), (lnx(11), 0, 62), (xsum(5), 64, 72),
                (lnz(2), 0, 44), (lnz(3), 0, 44), (lnz(4), 12, 67), (lnz(5), 12, 67),
                (lnz(6), 36, 67), (lnz(7), 36, 67), (kv_items, 0, 72)])
    wait(9)
    pair_block([(2, 5), (1, 5), (2, 6), (2, 7), (1, 6), (1, 7)],
               [(lnx(12), 0, 11), (lnx(13), 0, 11), (xsum(6), 13, 19),
                (lnx(14), 0, 23), (lnx(15), 0, 23), (xsum(7), 25, 31),
                (lnz(8), 0, 32), (lnz(9), 0, 32), (lnz(10), 12, 44), (lnz(11), 12, 44),
                (lnz(12), 36, 54), (lnz(13), 36, 54), (lnz(14), 48, 63), (lnz(15), 48, 63),
                (bsum(8), 36, 72), (bsum(9), 36, 72), (bsum(10), 48, 72), (bsum(11), 48, 72),
                (bsum(12), 58, 72), (bsum(13), 58, 72), (bsum(14), 67, 72), (bsum(15), 67, 72),
                (asum_items(0, HT // 2), 0, 72)])
    wait(10)

    def unit(n, half, k, tap, put_p):
        def span(start, size):
            if isinstance(start, int):
                return slice(start, start + size)
            return pl.ds(pl.multiple_of(start, size), size)

        r = half * (HT // 2) + k
        top, bot = span(r * T, T), span(HS + r * T, T)
        toph, both = span(r * (T // 2), T // 2), span(HS // 2 + r * (T // 2), T // 2)
        sums, sumh = (as32, as232)[half], span(k * (T // 2), T // 2)

        def prod(lhs, rhs):
            acc = None
            for q in range(HS // KG):
                part = _dot(lhs(q), rhs(q))
                acc = part if acc is None else acc + part
                tap(acc)
            return acc

        def sa(i):
            return lambda q: jnp.concatenate(
                [_up(sums[i, c, sumh, :]) for c in range(q * KG // 128, (q + 1) * KG // 128)],
                axis=1)

        def sb(i):
            return lambda q: _up(bs32[i, n, q * KG // 2:(q + 1) * KG // 2, :])

        def a11(q):
            return _up(wsp_v[0, toph, q * KG:(q + 1) * KG])

        def a22(q):
            return _up(wsp_v[0, both, HS + q * KG:HS + (q + 1) * KG])

        def b11(q):
            return _up(z232[n, q * KG // 2:(q + 1) * KG // 2, :])

        def b22(q):
            return _up(z232[n + HF, (HS + q * KG) // 2:(HS + (q + 1) * KG) // 2, :])

        def fin(i, j, c):
            col, rows = n + j * HF, (top, bot)[i]
            put_p(i, j, col, rows, (c + bcol_v[rows, :]).astype(BF16))

        _strassen(prod, sa, sb, a11, a22, b11, b22, fin)

    def p2(n, half):
        nn = jnp.minimum(n + 1, NC - 1)

        @pl.when(n + 1 < NC)
        def _():
            for d in tile_cps(nn):
                d.wait()

        if half == 0:
            for q in range(HF):
                @pl.when(n == q)
                def _():
                    for d in wsp2_cps(q):
                        d.wait()

        zero = zero_s[0]
        fwd_u = _up(tab_v[0:128, :])
        fwd_h = _up(tab_v[128:256, :])
        dd = dd_v[n]

        def put(slot, val):
            pl_v[:, slot] = val

        def re_im(val):
            val = val.reshape(BLK // 8, 2, 8, 128)
            return val[:, 0], val[:, 1]

        kvi = kv_items(nn)

        def pace_kv(d, val):
            if d % 4 == 3:
                for j in range(8):
                    _, gate, run = kvi[(d // 4) * 8 + j]
                    gate(val[j * 32:j * 32 + 8, :])
                    run()

        for i in range(NB):
            u = _dot(fwd_u, _up(kvb32[i * BLK // 2:(i + 1) * BLK // 2, :]))
            a, b = re_im(u)
            put(UA + i, a)
            put(UB + i, b)
            put(US + i, a + b)
            pace_kv(i, u)
        for i in range(NB):
            hb = _up(h_v[n, :, i * BLK:(i + 1) * BLK])
            hf = jax.lax.dot_general(fwd_h, hb, (((1,), (1,)), ((), ())),
                                     preferred_element_type=F32)
            c, d = re_im(hf)
            if i == 0:
                c, d = c + dd, d + dd
            put(HR + i, c)
            put(HP + i, d - c)
            put(HQ + i, c + d)
            pace_kv(NB + i, hf)

        state = {}

        def mac_item(pos, g0, pi, j0, j1):
            xv, hv = ((US, HR), (UA, HP), (UB, HQ))[pi]
            outs = range(g0, g0 + GRP)
            top = g0 + GRP

            def run():
                pz = zero + pos
                hs = {t: pl_v[pz, hv + t]
                      for t in range(max(g0 - j1 + 1, 0), top - j0)}
                acc = state['acc'] if j0 else {o: None for o in outs}
                for jj in range(j0, j1):
                    xj = pl_v[pz, xv + jj]
                    for o in outs:
                        if o - jj >= 0:
                            t = xj * hs[o - jj]
                            acc[o] = t if acc[o] is None else acc[o] + t
                if j1 < top:
                    state['acc'] = acc
                    return
                r0 = pos * 8
                if pi == 0:
                    state['k1'] = acc
                elif pi == 1:
                    state['im'] = {o: state['k1'][o] + acc[o] for o in outs}
                else:
                    for o in outs:
                        re, im = state['k1'][o] - acc[o], state['im'][o]
                        zr, zi = re, im
                        if o > 0:
                            zr, zi = re - state['prev'][1], im + state['prev'][0]
                        state['prev'] = (re, im)
                        zz_v[n, o, r0:r0 + 8, :] = zr.astype(BF16)
                        zz_v[n, o, BLK + r0:BLK + r0 + 8, :] = zi.astype(BF16)

            nmac = sum(1 for o in outs for jj in range(j0, j1) if o >= jj)
            return (2 * nmac + ((0, GRP, 5 * GRP)[pi] if j1 == top else 0), gate_pl, run)

        items = []
        for pos in range(BLK // 8):
            for g0 in range(0, NB, GRP):
                top = g0 + GRP
                cuts = [0, top] if top <= SPLIT else [0, (top - 1) // 2, top]
                for pi in range(3):
                    for j0, j1 in zip(cuts[:-1], cuts[1:]):
                        items.append(mac_item(pos, g0, pi, j0, j1))

        if half == 0:
            extra = [asum_dyn(jnp.minimum(n * NG + g, HS // 32 - 1), c)
                     for g in range(NG) for c in range(HT)]
            every = len(items) // len(extra)
            items = [it for i, e in enumerate(extra)
                     for it in items[i * every:(i + 1) * every] + [e]
                     ] + items[len(extra) * every:]

        total = sum(c for c, _, _ in items)
        tap_of = []
        cum = 0
        for c, _, _ in items:
            tap_of.append(int(cum * NTAP / total))
            cum += c
        pos = {'tap': 0, 'item': 0}

        def tap(acc):
            t0 = pos['tap']
            pos['tap'] += T // 8
            while pos['item'] < len(items) and tap_of[pos['item']] < pos['tap']:
                i = tap_of[pos['item']] - t0
                _, gate, run = items[pos['item']]
                gate(acc[i * 8:(i + 1) * 8, :])
                run()
                pos['item'] += 1

        def put_p(i, j, col, rows, val):
            p_v[col, rows, :] = val

        for k in range(HT // 2):
            unit(n - half * HF, half, k, tap, put_p)
        assert pos['item'] == len(items)
        return 0

    jax.lax.fori_loop(0, HF, lambda n, c: p2(n, 0), 0)
    jax.lax.fori_loop(HF, NC, lambda n, c: p2(n, 1), 0)

    wout_cp.wait()

    def p3(j, carry):
        inv_p = _up(tab_v[256:288, :])
        inv_m = _up(tab_v[288:320, :])
        rev = 7 - jax.lax.broadcasted_iota(jnp.int32, (8, 128), 0)

        zero = zero_s[0]
        HK = FH // 2

        def rows(k, i):
            tile = i * HT + (k // 2) * (HT // 2) + 2 * j + k % 2
            return (tile, pl.ds(pl.multiple_of(tile * T, T), T),
                    pl.ds(pl.multiple_of(tile * (T // 2), T // 2), T // 2))

        def fresh(k, n):
            return k >= 2 and n % HF == HF - 1

        def p_tile(k, i, n):
            return _up(pp32[k, i, n])

        def gate_p(tok):
            p_v[0, S:S + 8, :] = tok.astype(BF16)

        def gate_wo(tok):
            wout_v[0, HK:HK + 8, 0:128] = pltpu.bitcast(tok, U32)

        def psum_item(k, n, g):
            def run():
                def quad(i, jj):
                    rs = pl.ds(pl.multiple_of(rows(k, i)[0] * T + g * 16, 16), 16)
                    if fresh(k, n):
                        gv = pq_v[k - 2, i, jj, g * 16:(g + 1) * 16, :]
                    else:
                        gv = p_v[n + jj * HF, rs, :]
                    pv = _gelu2(z1_v[n + jj * HF, rs, :].astype(F32)) * gv.astype(F32)
                    pp_v[k, i, n + jj * HF, g * 16:(g + 1) * 16, :] = pv.astype(BF16)
                    return pv
                for i, v in enumerate(_lhs_sums(quad(0, 0), quad(0, 1), quad(1, 0), quad(1, 1))):
                    ps_v[k, i, n, g * 16:(g + 1) * 16, :] = v.astype(BF16)
            return (gate_p, run)

        def wsum_item(m, g):
            def run():
                def quad(i, jj):
                    r0 = (i * HK + g * 16) // 2
                    c0 = (m + 2 * jj) * 128
                    return _up(wout_v[zero, r0:r0 + 8, c0:c0 + 128]).astype(F32)
                for i, v in enumerate(_rhs_sums(quad(0, 0), quad(0, 1), quad(1, 0), quad(1, 1))):
                    ws_v[i, m, g * 16:(g + 1) * 16, :] = v.astype(BF16)
            return (gate_wo, run)

        def psum(k):
            return [psum_item(k, n, g) for n in range(HF) if not fresh(k, n)
                    for g in range(T // 16)]

        queue = []

        def tap(val):
            for i in range(min(len(queue), queue_step[0])):
                gate, run = queue.pop(0)
                r = (i * (T // 8)) // queue_step[0] * 8
                gate(val[r:r + 8, :])
                run()

        queue_step = [0]

        def paced(items, ntaps):
            assert not queue
            queue.extend(items)
            queue_step[0] = -(-len(items) // ntaps)

        def do_unit(u):
            def put_q(i, jj, col, rws, val):
                pq_v[u, i, jj] = val
            unit(HF - 1, 1, 2 * j + u, tap, put_q)
            for g in range(T // 16):
                psum_item(2 + u, HF - 1, g)[1]()

        def finish(k, i, c, o):
            tile, rs, hs = rows(k, i)
            cs = slice(c * 128, (c + 1) * 128)
            ye = _dot(inv_p, _up(zz32[c, tile, 0:64, :]))
            yo = _dot(inv_m, _up(zz32[c, tile, 64:128, :]))
            yd = ye - yo
            y = jnp.concatenate(
                [ye + yo] + [
                    jnp.take_along_axis(yd[q * 8:(q + 1) * 8], rev, axis=0,
                                        mode="promise_in_bounds")
                    for q in reversed(range(BLK // 16))], axis=0)
            gate = o * (1.0 + jnp.tanh((0.25 / _A) * o))
            x = _up(x_v[0, hs, cs]).astype(F32)
            xn = xn_v[c, rs, :].astype(F32)
            o_v[rs, cs] = (x + (xn * y) * gate).astype(BF16)

        def do_pair(k, last=False):
            def prod(lhs, rhs):
                res = _dot(lhs, rhs)
                tap(res)
                return res

            def sa(i):
                return jnp.concatenate([_up(ps32[k, i, n]) for n in range(HF)], axis=1)

            a11 = jnp.concatenate([p_tile(k, 0, n) for n in range(HF)], axis=1)
            a22 = jnp.concatenate([p_tile(k, 1, n) for n in range(HF, NF)], axis=1)
            for m in range(2):
                _strassen(
                    prod, sa, lambda i: _up(ws32[i, m]), a11, a22,
                    _up(wout_v[0, 0:HK // 2, m * 128:(m + 1) * 128]),
                    _up(wout_v[0, HK // 2:HK, (m + 2) * 128:(m + 3) * 128]),
                    lambda i, jj, o: finish(k, i, m + 2 * jj, o))
            for i in range(2):
                rs = rows(k, i)[1]
                if last:
                    cp(o_v.at[rs, 0:512], out_hbm.at[0, rs, 0:512], out_sem).start()
            for i in range(2):
                rs = rows(k, i)[1]
                p = jnp.concatenate([p_tile(k, i, n) for n in range(NF)], axis=1)
                finish(k, i, NC - 1, _dot(p, _up(wout_v[0, 0:HK, 512:D])))
                if last:
                    cp(o_v.at[rs, 512:D], out_hbm.at[0, rs, 512:D], out_sem).start()
                else:
                    cp(o_v.at[rs, :], out_hbm.at[0, rs, :], out_sem).start()

        paced(psum(0) + [wsum_item(m, g) for m in range(2) for g in range(HK // 16)], 12)
        do_unit(0)
        paced(psum(1), 12)
        do_pair(0)
        paced(psum(2), 12)
        do_unit(1)
        paced(psum(3), 12)
        do_pair(1)
        do_pair(2)
        do_pair(3, last=True)
        return carry

    jax.lax.fori_loop(0, P3I, p3, 0)
    cp(o_v, out_hbm.at[0], out_sem).wait()


@jax.jit
def pallas_recurrent_scan__ssm_conv_h3__mixer_gmlp__prompt_kernel(
    A_q: jax.Array,
    A_k: jax.Array,
    A_v: jax.Array,
    A_shift_k: jax.Array,
    A_ssm_k: jax.Array,
    A_ssm_D: jax.Array,
    B_x: jax.Array,
    B_w_in: jax.Array,
    B_w_sp: jax.Array,
    B_b_sp: jax.Array,
    B_w_out: jax.Array,
):
    del B_x
    tab = jnp.asarray(_dft_tables(), dtype=BF16)

    any_spec = pl.BlockSpec(memory_space=pl.ANY)
    return pl.pallas_call(
        _kernel,
        out_shape=jax.ShapeDtypeStruct((1, S, D), BF16),
        in_specs=[any_spec] * 11,
        out_specs=any_spec,
        scratch_shapes=[
            pltpu.VMEM((1, S // 2 + 32, D), U32),
            pltpu.VMEM((1, D // 2 + 8, 2 * FH), U32),
            pltpu.VMEM((1, S // 2 + 8, S), U32),
            pltpu.VMEM((1, FH // 2 + 32, D), U32),
            pltpu.VMEM((2 * NC, S // 2 + 32, 128), U32),
            pltpu.VMEM((NC, 64, S), U32),
            pltpu.VMEM((NC, S + 256, 128), BF16),
            pltpu.VMEM((NF, S, 128), BF16),
            pltpu.VMEM((NF, S + 64, 128), BF16),
            pltpu.VMEM((NF, S + 64, 128), BF16),
            pltpu.VMEM((5, HT, HS // 2, 128), BF16),
            pltpu.VMEM((5, HT, HS // 2, 128), BF16),
            pltpu.VMEM((5, HF, HS, 128), BF16),
            pltpu.VMEM((2, 2, 2, T, 128), BF16),
            pltpu.VMEM((4, 2, NF, T, 128), BF16),
            pltpu.VMEM((4, 5, HF, T, 128), BF16),
            pltpu.VMEM((5, 2, FH // 2, 128), BF16),
            pltpu.VMEM((S, 128), BF16),
            pltpu.VMEM((BLK // 8, 6 * NB + 1, 8, 128), F32),
            pltpu.VMEM((NC, NB, 2 * BLK, 128), BF16),
            pltpu.VMEM((S, 128), F32),
            pltpu.VMEM((S, D), BF16),
            pltpu.VMEM((1, T + 16, FH), F32),
            pltpu.VMEM((1, T + 16, FH), F32),
            pltpu.VMEM((1, T + 16, FH), F32),
            pltpu.VMEM((1, T + 16, FH), F32),
            pltpu.VMEM((1, T + 16, FH), F32),
            pltpu.VMEM((1, T + 16, FH), F32),
            pltpu.VMEM((NT // 2, 5, 2, T, 128), BF16),
            pltpu.VMEM((5, NF, KH, 128), BF16),
            pltpu.VMEM((T, 128), F32),
            pltpu.VMEM((320, 128), U32),
            pltpu.VMEM((NC, KS, 128), F32),
            pltpu.VMEM((NC + 2, 1, 128), F32),
            pltpu.VMEM((KS, D), BF16),
            pltpu.VMEM((D,), BF16),
            pltpu.VMEM((S,), BF16),
            pltpu.SMEM((1,), jnp.int32),
            pltpu.SemaphoreType.DMA((16,)),
        ],
        compiler_params=pltpu.CompilerParams(
            vmem_limit_bytes=100 * 1024 * 1024, disable_bounds_checks=True),
    )(A_q, A_k, A_v, A_shift_k.T, A_ssm_k, A_ssm_D, B_w_in, B_w_sp, B_b_sp, B_w_out, tab)
```

```python
import jax
import jax.numpy as jnp
import numpy as np
import jax.experimental.pallas as pl
import jax.experimental.pallas.tpu as pltpu

F32 = jnp.float32
BF16 = jnp.bfloat16
U32 = jnp.uint32

S = 2048
D = 640
FH = 768
KS = 4
BLK = 128
NB = S // BLK
NC = D // 128
NF = FH // 128
T = 128
NT = S // T
EPS = 1e-5
GRP = 4
SPLIT = 8
import os
AW = int(os.environ.get('AW', 2))
PR = int(os.environ.get('PR', 128))
KG = 512
KR = 32
UA, UB, US, HP, HQ, HR, TOK = (i * NB for i in range(7))
LAG = 4
NTAP = 888
HS = S // 2
HT = HS // T
HF = NF // 2
KH = 256
P3I = 2

_GELU_C0 = float(np.sqrt(2.0 / np.pi))
_GELU_C1 = _GELU_C0 * 0.044715
_A = _GELU_C1 ** (1.0 / 3.0)
_K = _GELU_C0 / _A


def _dft_tables():
    m = np.arange(BLK)[:, None]
    n = np.arange(BLK)[None, :]
    th = 2.0 * np.pi * (((4 * m + 1) * n) % (4 * BLK)) / (4 * BLK)
    ph = 2.0 * np.pi * (((4 * m + 1) * (2 * n + 1)) % (8 * BLK)) / (8 * BLK)
    fu = np.concatenate([np.cos(ph), -np.sin(ph)], axis=0)
    fh = np.concatenate([np.cos(th) + np.sin(th), np.cos(th) - np.sin(th)], axis=0)
    fu, fh = (f.reshape(2, BLK // 8, 8, BLK).transpose(1, 0, 2, 3).reshape(2 * BLK, BLK)
              for f in (fu, fh))
    cp = (np.cos(ph) + np.sin(ph)).T[:BLK // 2] / (8.0 * BLK * _A * _A)
    cm = (np.cos(ph) - np.sin(ph)).T[:BLK // 2] / (8.0 * BLK * _A * _A)
    return np.concatenate([fu, fh, cp, cm], axis=0).astype(np.float32)


def _layernorm(x, eps, scale=1.0):
    m = jnp.mean(x, axis=-1, keepdims=True)
    d = x - m
    v = jnp.sum(d * d, axis=-1, keepdims=True) * (1.0 / (x.shape[-1] * scale * scale))
    return d * jax.lax.rsqrt(v + eps / (scale * scale))


def _gelu2(y):
    return y * (1.0 + jnp.tanh(y * (y * y + _K)))


def _up(x):
    return pltpu.bitcast(x, BF16)


def _dot(a, b):
    return jnp.dot(a, b, preferred_element_type=F32)


def _lhs_sums(a11, a12, a21, a22):
    return a11 + a22, a21 + a22, a11 + a12, a21 - a11, a12 - a22


def _rhs_sums(b11, b12, b21, b22):
    return b11 + b22, b12 - b22, b21 - b11, b11 + b12, b21 + b22


def _strassen(prod, sa, sb, a11, a22, b11, b22, fin):
    m2 = prod(sa(1), b11)
    m4 = prod(a22, sb(2))
    fin(1, 0, m2 + m4)
    m5 = prod(sa(2), b22)
    c11 = m4 - m5
    m3 = prod(a11, sb(1))
    fin(0, 1, m3 + m5)
    c22 = m3 - m2
    m1 = prod(sa(0), sb(0))
    c11, c22 = c11 + m1, c22 + m1
    fin(0, 0, c11 + prod(sa(4), sb(4)))
    fin(1, 1, c22 + prod(sa(3), sb(3)))


def _lhs_sums_w(a11, a12, a21, a22):
    s1 = a21 + a22
    s2 = s1 - a11
    return s1, s2, a11 - a21, a12 - s2


def _rhs_sums_w(b11, b12, b21, b22):
    t1 = b12 - b11
    t2 = b22 - t1
    return t1, t2, b22 - b12, t2 - b21


def _winograd(prod, sa, sb, a11, a12, a22, b11, b21, b22, fin):
    p1 = prod(a11, b11)
    fin(0, 0, p1 + prod(a12, b21))
    u2 = p1 + prod(sa(1), sb(1))
    p5 = prod(sa(0), sb(0))
    fin(0, 1, (u2 + p5) + prod(sa(3), b22))
    u3 = u2 + prod(sa(2), sb(2))
    fin(1, 1, u3 + p5)
    fin(1, 0, u3 - prod(a22, sb(3)))


def _balance(work, n):
    jobs = [(lo, hi, sum(it[0] for it in items)) for items, lo, hi in work]
    rate = [None] * n
    while jobs:
        def free(a, b):
            return [p for p in range(a, b) if rate[p] is None]
        dens, a, b = max(
            (sum(w for lo, hi, w in jobs if a <= lo and hi <= b) / max(len(free(a, b)), 1e-9), a, b)
            for a in {j[0] for j in jobs} for b in {j[1] for j in jobs} if a < b)
        while a > 0 and rate[a - 1] is not None:
            a -= 1
        while b < n and rate[b] is not None:
            b += 1
        for p in free(a, b):
            rate[p] = dens
        jobs = [(lo, hi, w) for lo, hi, w in jobs if not (a <= lo and hi <= b)]
        jobs = [(b if a <= lo < b else lo, a if a < hi <= b else hi, w) for lo, hi, w in jobs]
    queues = [[lo * 16, hi * 16, list(items)] for items, lo, hi in work]
    rel = [[] for _ in range(n)]
    budget = 0.0
    for tau in range(n * 16):
        budget += (rate[tau // 16] or 0.0) / 16
        while True:
            ready = [q for q in queues if q[2] and q[0] <= tau]
            if not ready:
                budget = min(budget, 0.0)
                break
            q = min(ready, key=lambda q: q[1])
            if budget < 0 and q[1] - tau > len(q[2]):
                break
            it = q[2].pop(0)
            rel[tau // 16].append((tau % 16, it))
            budget -= it[0]
    assert not any(q[2] for q in queues)
    return rel


def _kernel(x_hbm, k_hbm, v_hbm, skt_hbm, h_hbm, dv_hbm, win_hbm, wsp_hbm, b_hbm,
            wout_hbm, tab_hbm, out_hbm,
            x_v, win_v, wsp_v, wout_v, kv_v, h_v, xn_v, z1_v, z2_v, p_v, as_v, as2_v, bs_v, pq_v, pp_v, ps_v, ws_v,
            kvb_v, pl_v, zz_v, bcol_v, o_v, zta_v, ztb_v, ztc_v, ztd_v, zte_v, ztf_v, xs_v, wi_v, raw_v, tab_v,
            sk_v, dd_v, skt_v, dv_v, b_v, zero_s, sem):
    cp = pltpu.make_async_copy
    x16 = x_v.bitcast(BF16)
    win16 = win_v.bitcast(BF16)
    kv16 = kv_v.bitcast(BF16)
    h16 = h_v.bitcast(BF16)

    xn32, z232, kvb32, zz32, as32, as232, bs32, pp32, ps32, ws32, xs32, wi32 = (
        r.bitcast(U32)
        for r in (xn_v, z2_v, kvb_v, zz_v, as_v, as2_v, bs_v, pp_v, ps_v, ws_v, xs_v, wi_v))
    wsp16 = wsp_v.bitcast(BF16)

    def wsp_cp(lo, hi, s):
        return cp(wsp_hbm.at[lo:hi, :], wsp16.at[0, lo:hi, :], sem.at[s])

    def x_cp(lo, hi, s):
        return cp(x_hbm.at[0, lo:hi, :], x16.at[0, lo:hi, :], sem.at[s])

    def win_cp(lo, hi, s):
        return cp(win_hbm.at[:, lo:hi], win16.at[0, 0:D, lo:hi], sem.at[s])

    def k_cp(c, s):
        return cp(k_hbm.at[0, :, pl.ds(c * 128, 128)], kv16.at[2 * c, 0:S, :], sem.at[s])

    def v_cp(c, s):
        return cp(v_hbm.at[0, :, pl.ds(c * 128, 128)], kv16.at[2 * c + 1, 0:S, :], sem.at[s])

    def h_cp(c, s):
        return cp(h_hbm.at[pl.ds(c * 128, 128), :], h16.at[c], sem.at[s])

    groups = [
        [cp(b_hbm, b_v, sem.at[0]), cp(skt_hbm, skt_v, sem.at[0]), cp(dv_hbm, dv_v, sem.at[0])],
        [x_cp(0, 256, 1)],
        [win_cp(FH, FH + 256, 2)],
        [win_cp(FH + 256, FH + 512, 3)],
        [win_cp(FH + 512, 2 * FH, 4), win_cp(0, 128, 4)],
        [win_cp(128, 512, 11)],
        [win_cp(512, FH, 5), x_cp(256, 384, 5)],
        [x_cp(384, 6 * T, 6)],
        [x_cp(6 * T, 12 * T, 7), k_cp(0, 7), v_cp(0, 7)],
        [x_cp(12 * T, S, 12), wsp_cp(0, HS // 2, 12), wsp_cp(HS, HS + HS // 2, 12)],
        [cp(tab_hbm, tab_v.bitcast(BF16), sem.at[8]), h_cp(0, 8)],
    ]
    for g in groups:
        for c in g:
            c.start()

    def tile_cps(c):
        s = jnp.where(c == NC - 1, 9, c - 1) if isinstance(c, jax.Array) else (0, 1, 2, 9)[c - 1]
        return [k_cp(c, s), v_cp(c, s), h_cp(c, s)]

    NG = -(-HS // 32 // HF)

    def wsp2_cps(n):
        lo, hi = HS // 2 + n * NG * 16, min(HS // 2 + (n + 1) * NG * 16, HS)
        return [wsp_cp(lo, hi, 13 + n), wsp_cp(HS + lo, HS + hi, 13 + n)]

    wout_cp = cp(wout_hbm, wout_v.bitcast(BF16).at[0, 0:FH, :], sem.at[10])
    out_sem = sem.at[5]

    def wait(i):
        for c in groups[i]:
            c.wait()

    zero_s[0] = 0
    wait(0)
    skt = skt_v[...].astype(F32)
    dv = dv_v[...].astype(F32).reshape(1, D)
    for c in range(NC):
        sk_v[c] = skt[:, c * 128:(c + 1) * 128]
        dd_v[c] = dv[:, c * 128:(c + 1) * 128]
    brow = b_v[...].astype(F32).reshape(1, S)
    bcol_v[...] = jnp.broadcast_to(brow, (128, S)).T

    def gate_x(tok):
        x_v[0, S // 2:S // 2 + 8, 0:128] = pltpu.bitcast(tok, U32)

    zt_v = (zta_v, ztb_v, ztc_v, ztd_v, zte_v, ztf_v)

    def gate_zt(t):
        def gate(tok):
            zt_v[t % 6][0, T:T + 8, 0:128] = tok
        return gate

    def gate_kv(tok):
        kv_v[0, S // 2:S // 2 + 8, :] = pltpu.bitcast(tok, U32)

    def gate_pl(tok):
        pl_v[0, TOK] = tok

    ndone = [0]

    mode = {'pairs': False}

    def done(val):
        r = (ndone[0] % 8) * 16
        ndone[0] += 1
        if mode['pairs']:
            xs_v[0, 0, 0, r:r + 16, :] = val
        else:
            xn_v[0, S + r:S + r + 16, :] = val

    def lnx_items(t, zero):
        def item(r0):
            def run():
                rs = slice(r0 // 2, r0 // 2 + 8)
                xw = jnp.concatenate([x_v[zero, rs, 0:128], x_v[0, rs, 128:D]], axis=1)
                xn = _layernorm(_up(xw).astype(F32), EPS, _A)
                for c in range(NC):
                    xb = xn[:, c * 128:(c + 1) * 128].astype(BF16)
                    xn_v[c, r0:r0 + 16, :] = xb
                if mode['pairs']:
                    done(xb)
            return (85, gate_x, run)
        return [item(t * T + g * 16) for g in range(T // 16)]

    def lnz_items(t, zero):
        def item(g):
            def run():
                rs = slice(g * 16, (g + 1) * 16)
                z = jnp.concatenate(
                    [zt_v[t % 6][zero, rs, 0:128], zt_v[t % 6][0, rs, 128:FH]], axis=1)
                z = _layernorm(z, 4.0 * _A * _A * EPS)
                r0 = t * T + g * 16
                for n in range(NF):
                    zb = z[:, n * 128:(n + 1) * 128].astype(BF16)
                    z2_v[n, r0:r0 + 16, :] = zb
                done(zb)
            return (90, gate_zt(t), run)
        return [item(g) for g in range(T // 16)]

    def kv_items(c):
        sk = sk_v[c]

        def item(r0):
            def run():
                hs = slice(r0 // 2, (r0 + KR) // 2)
                if r0 == 0:
                    kw = jnp.concatenate(
                        [jnp.zeros((8, 128), F32), _up(kv_v[2 * c, hs, :]).astype(F32)], axis=0)
                else:
                    kw = _up(kv_v[2 * c, r0 // 2 - 8:(r0 + KR) // 2, :]).astype(F32)[8:]
                ks = kw[8:] * sk[0:1, :]
                for t in range(1, KS):
                    ks = ks + pltpu.roll(kw, t, 0)[8:] * sk[t:t + 1, :]
                kvb_v[r0:r0 + KR, :] = (
                    ks * _up(kv_v[2 * c + 1, hs, :]).astype(F32)).astype(BF16)
            return (14 * KR // 8, gate_kv, run)
        return [item(r0) for r0 in range(0, S, KR)]

    def gate_w(tok):
        wsp_v[0, S // 2:S // 2 + 8, 0:128] = pltpu.bitcast(tok, U32)

    def asum_items(r_lo, r_hi):
        def item(zero, r0, c0):
            def run():
                def quad(i, j, c):
                    w = wsp_v[zero, (i * HS + r0) // 2:(i * HS + r0) // 2 + 8,
                              j * HS + c * 128:j * HS + (c + 1) * 128]
                    return _up(w).astype(F32)
                for c in range(c0, c0 + AW):
                    for i, v in enumerate(_lhs_sums_w(
                            quad(0, 0, c), quad(0, 1, c), quad(1, 0, c), quad(1, 1, c))):
                        as_v[i, c, r0:r0 + 16, :] = v.astype(BF16)
            return (20 * AW, gate_w, run)
        return lambda zero: [item(zero, r0, c0) for r0 in range(r_lo * T, r_hi * T, 16)
                             for c0 in range(0, HT, AW)]

    def asum_dyn(g, c):
        def run():
            def quad(i, j):
                r0 = pl.multiple_of(i * (HS // 2) + HS // 4 + g * 8, 8)
                w = wsp_v[0, pl.ds(r0, 8), j * HS + c * 128:j * HS + (c + 1) * 128]
                return _up(w).astype(F32)
            rs = pl.ds(pl.multiple_of(g * 16, 16), 16)
            for i, v in enumerate(_lhs_sums_w(quad(0, 0), quad(0, 1), quad(1, 0), quad(1, 1))):
                as2_v[i, c, rs, :] = v.astype(BF16)
        return (20, gate_w, run)

    def gate_z2(tok):
        z2_v[0, S:S + 8, :] = tok.astype(BF16)

    def bsum(t):
        def item(zero, r0, n):
            def run():
                def quad(i, j):
                    return z2_v[zero + n + j * HF, i * HS + r0:i * HS + r0 + 16, :].astype(F32)
                for i, v in enumerate(_rhs_sums_w(quad(0, 0), quad(0, 1), quad(1, 0), quad(1, 1))):
                    bs_v[i, n, r0:r0 + 16, :] = v.astype(BF16)
            return (21, gate_z2, run)
        return lambda zero: [item(zero, r0, n) for r0 in range((t - HT) * T, (t - HT + 1) * T, 16)
                             for n in range(HF)]

    def gate_xn(tok):
        xn_v[1, S:S + 8, :] = tok.astype(BF16)

    def xsum(u):
        def item(zero, g, c):
            def run():
                def quad(i, j):
                    r0 = (2 * u + i) * T + g * 16
                    return xn_v[zero + c + 2 * j, r0:r0 + 16, :].astype(F32)
                for i, v in enumerate(_lhs_sums(quad(0, 0), quad(0, 1), quad(1, 0), quad(1, 1))):
                    xs_v[u, i, c, g * 16:(g + 1) * 16, :] = v.astype(BF16)
            return (24, gate_xn, run)
        return lambda zero: [item(zero, g, c) for g in range(T // 16) for c in range(2)]

    def gate_wi(tok):
        win_v[0, D // 2:D // 2 + 8, 0:128] = pltpu.bitcast(tok, U32)

    def wisum(zero):
        def item(g, q):
            def run():
                def quad(i, j):
                    r0 = (i * KH + g * 16) // 2
                    c0 = ((q // HF) * NF + q % HF + j * HF) * 128
                    return _up(win_v[zero, r0:r0 + 8, c0:c0 + 128]).astype(F32)
                for i, v in enumerate(_rhs_sums(quad(0, 0), quad(0, 1), quad(1, 0), quad(1, 1))):
                    wi_v[i, q, g * 16:(g + 1) * 16, :] = v.astype(BF16)
            return (23, gate_wi, run)
        return [item(g, (q + HF) % NF) for q in range(NF) for g in range(KH // 16)]

    def taps_of(val):
        rows, cols = val.shape
        return [(lambda i=i, n=n: val[i * 8:(i + 1) * 8, n * 128:(n + 1) * 128])
                for n in range(cols // 128) for i in range(rows // 8)]

    def activate(kind, t, n, z):
        if kind == 2:
            zt_v[t % 6][0, 0:T, n * 128:(n + 1) * 128] = _gelu2(z)
        else:
            z1_v[n, t * T:(t + 1) * T, :] = z.astype(BF16)

    def piece(kind, t, n, zero, defer=False, halves=False):
        col = n * 128 + (FH if kind == 2 else 0)
        xn = jnp.concatenate(
            [_up(xn32[zero if zero is not None and c == 0 else c,
                      t * T // 2:(t + 1) * T // 2, :]) for c in range(NC)], axis=1)
        w = _up(win_v[0, 0:D // 2, col:col + 128])
        if halves:
            z = jnp.concatenate([_dot(xn[:T // 2], w), _dot(xn[T // 2:], w)], axis=0)
        else:
            z = _dot(xn, w)
        if defer:
            raw_v[...] = z
        else:
            activate(kind, t, n, z)
        return taps_of(z)

    def pair_piece(kind, u, m, gate_idx, slot_done):
        q = (kind - 1) * HF + m
        outs = []

        def wq(lo, hi, j):
            c0 = ((kind - 1) * NF + m + j * HF) * 128
            return _up(win_v[0, lo // 2:hi // 2, c0:c0 + 128])

        for r0 in range(0, T, PR):
            def xq(i, cs):
                r = (2 * u + i) * T + r0
                return jnp.concatenate(
                    [_up(xn32[c, r // 2:(r + PR) // 2, :]) for c in cs], axis=1)

            def fin(i, j, c):
                z = c + _dot(xq(i, [NC - 1]), wq(2 * KH, D, j))
                t, n = 2 * u + i, m + j * HF
                if kind == 2:
                    zt_v[t % 6][0, r0:r0 + PR, n * 128:(n + 1) * 128] = _gelu2(z)
                else:
                    z1_v[n, t * T + r0:t * T + r0 + PR, :] = z.astype(BF16)
                outs.extend(taps_of(z))
                if len(outs) == T // 8:
                    slot_done(list(outs))
                    outs.clear()

            _strassen(
                _dot,
                lambda i: jnp.concatenate(
                    [_up(xs32[u + (gate_idx() if c == 0 and i != 4 else 0), i, c,
                              r0 // 2:(r0 + PR) // 2, :]) for c in range(2)], axis=1),
                lambda i: _up(wi32[i, q]), xq(0, (0, 1)), xq(1, (2, 3)),
                wq(0, KH, 0), wq(KH, 2 * KH, 1), fin)

    pending = []

    def plan(work, zero, n):
        work = [(mk(zero), lo, hi) for mk, lo, hi in work]
        return [a + b for a, b in zip(
            _balance([w for w in work if w[0][0][0] >= 80], n),
            _balance([w for w in work if w[0][0][0] < 80], n))]

    def pair_block(halves, work):
        zero = zero_s[0]
        mode['pairs'] = True
        if pending:
            activate(*pending.pop(), raw_v[...])
        rel = plan(work, zero, 12 * len(halves))
        taps = []
        state = {'gated': False}

        def release(k):
            for i, (_, gate, run) in sorted(rel[k], key=lambda e: e[0]):
                gate(taps[k][i]())
                run()
                state['gated'] = True

        def slot_done(z):
            taps.append(z)
            if len(taps) > LAG:
                release(len(taps) - 1 - LAG)

        for kind, u in halves:
            for m in range(HF):
                pair_piece(kind, u, m, lambda: zero if state['gated'] else 0, slot_done)
        for k in range(len(taps) - LAG, len(taps)):
            release(k)

    def block(pieces, work, defer=True, free=None):
        zero = zero_s[0]
        if pending:
            activate(*pending.pop(), raw_v[...])
        rel = plan(work, zero, len(pieces))
        taps = []
        gated = False
        for k in range(len(pieces) + LAG):
            if free is not None and k == len(pieces) - 1:
                for _, _, run in free(zero):
                    run()
                gated = True
            if k < len(pieces):
                last = defer and k == len(pieces) - 1
                halves = len(pieces) % 4 == 2 and k == len(pieces) - 1
                taps.append(piece(*pieces[k], zero if gated else None, last, halves))
                if last:
                    pending.append(pieces[k])
            if k >= LAG:
                for i, (_, gate, run) in sorted(rel[k - LAG], key=lambda e: e[0]):
                    gate(taps[k - LAG][i]())
                    run()
                    gated = True

    def cols(kind, t, lo=0, hi=NF):
        return [(kind, t, n) for n in range(lo, hi)]

    def lnx(t):
        return lambda zero: lnx_items(t, zero)

    def lnz(t):
        return lambda zero: lnz_items(t, zero)

    wait(1)
    for it in lnx_items(0, 0) + lnx_items(1, 0):
        it[2]()
    wait(2)
    block(cols(2, 0, 0, 2) + cols(2, 1, 0, 2), [])
    for c in range(1, NC):
        for d in tile_cps(c) + (wsp2_cps(c - 1) if c <= HF else []):
            d.start()
    wout_cp.start()
    wait(3)
    block(cols(2, 0, 2, 4) + cols(2, 1, 2, 4), [])
    wait(4)
    block(cols(2, 0, 4) + cols(2, 1, 4) + cols(1, 0, 0, 1) + cols(1, 1, 0, 1), [])
    wait(5)
    block(cols(1, 0, 1, 4) + cols(1, 1, 1, 4), [(lnz(0), 0, 1)])
    wait(6)
    block(cols(1, 0, 4) + cols(1, 1, 4), [], free=lnx(2))

    def tiles(lo, hi):
        return [pc for t in range(lo, hi) for pc in cols(2, t) + cols(1, t)]

    wait(7)
    block(tiles(2, 4),
          [(lnx(3), 0, 7), (lnx(4), 0, 14), (lnx(5), 0, 15), (lnz(1), 0, 19),
           (wisum, 0, 24), (xsum(2), 17, 24)])
    wait(8)
    pair_block([(2, 2), (1, 2), (2, 3), (1, 3), (2, 4), (1, 4)],
               [(lnx(6), 0, 11), (lnx(7), 0, 11), (xsum(3), 13, 19),
                (lnx(8), 0, 35), (lnx(9), 0, 35), (xsum(4), 37, 43),
                (lnx(10), 0, 62), (lnx(11), 0, 62), (xsum(5), 64, 72),
                (lnz(2), 0, 44), (lnz(3), 0, 44), (lnz(4), 12, 67), (lnz(5), 12, 67),
                (lnz(6), 36, 67), (lnz(7), 36, 67), (kv_items, 0, 72)])
    wait(9)
    pair_block([(2, 5), (1, 5), (2, 6), (2, 7), (1, 6), (1, 7)],
               [(lnx(12), 0, 11), (lnx(13), 0, 11), (xsum(6), 13, 19),
                (lnx(14), 0, 23), (lnx(15), 0, 23), (xsum(7), 25, 31),
                (lnz(8), 0, 32), (lnz(9), 0, 32), (lnz(10), 12, 44), (lnz(11), 12, 44),
                (lnz(12), 36, 54), (lnz(13), 36, 54), (lnz(14), 48, 63), (lnz(15), 48, 63),
                (bsum(8), 36, 72), (bsum(9), 36, 72), (bsum(10), 48, 72), (bsum(11), 48, 72),
                (bsum(12), 58, 72), (bsum(13), 58, 72), (bsum(14), 67, 72), (bsum(15), 67, 72),
                (asum_items(0, HT // 2), 0, 72)])
    wait(10)

    def unit(n, half, k, tap, put_p):
        def span(start, size):
            if isinstance(start, int):
                return slice(start, start + size)
            return pl.ds(pl.multiple_of(start, size), size)

        r = half * (HT // 2) + k
        top, bot = span(r * T, T), span(HS + r * T, T)
        toph, both = span(r * (T // 2), T // 2), span(HS // 2 + r * (T // 2), T // 2)
        sums, sumh = (as32, as232)[half], span(k * (T // 2), T // 2)

        def prod(lhs, rhs):
            acc = None
            for q in range(HS // KG):
                part = _dot(lhs(q), rhs(q))
                acc = part if acc is None else acc + part
                tap(acc)
            return acc

        def sa(i):
            return lambda q: jnp.concatenate(
                [_up(sums[i, c, sumh, :]) for c in range(q * KG // 128, (q + 1) * KG // 128)],
                axis=1)

        def sb(i):
            return lambda q: _up(bs32[i, n, q * KG // 2:(q + 1) * KG // 2, :])

        def a11(q):
            return _up(wsp_v[0, toph, q * KG:(q + 1) * KG])

        def a12(q):
            return _up(wsp_v[0, toph, HS + q * KG:HS + (q + 1) * KG])

        def b21(q):
            return _up(z232[n, (HS + q * KG) // 2:(HS + (q + 1) * KG) // 2, :])

        def a22(q):
            return _up(wsp_v[0, both, HS + q * KG:HS + (q + 1) * KG])

        def b11(q):
            return _up(z232[n, q * KG // 2:(q + 1) * KG // 2, :])

        def b22(q):
            return _up(z232[n + HF, (HS + q * KG) // 2:(HS + (q + 1) * KG) // 2, :])

        def fin(i, j, c):
            col, rows = n + j * HF, (top, bot)[i]
            put_p(i, j, col, rows, (c + bcol_v[rows, :]).astype(BF16))

        _winograd(prod, sa, sb, a11, a12, a22, b11, b21, b22, fin)

    def p2(n, half):
        nn = jnp.minimum(n + 1, NC - 1)

        @pl.when(n + 1 < NC)
        def _():
            for d in tile_cps(nn):
                d.wait()

        if half == 0:
            for q in range(HF):
                @pl.when(n == q)
                def _():
                    for d in wsp2_cps(q):
                        d.wait()

        zero = zero_s[0]
        fwd_u = _up(tab_v[0:128, :])
        fwd_h = _up(tab_v[128:256, :])
        dd = dd_v[n]

        def put(slot, val):
            pl_v[:, slot] = val

        def re_im(val):
            val = val.reshape(BLK // 8, 2, 8, 128)
            return val[:, 0], val[:, 1]

        kvi = kv_items(nn)

        def pace_kv(d, val):
            if d % 4 == 3:
                for j in range(8):
                    _, gate, run = kvi[(d // 4) * 8 + j]
                    gate(val[j * 32:j * 32 + 8, :])
                    run()

        for i in range(NB):
            u = _dot(fwd_u, _up(kvb32[i * BLK // 2:(i + 1) * BLK // 2, :]))
            a, b = re_im(u)
            put(UA + i, a)
            put(UB + i, b)
            put(US + i, a + b)
            pace_kv(i, u)
        for i in range(NB):
            hb = _up(h_v[n, :, i * BLK:(i + 1) * BLK])
            hf = jax.lax.dot_general(fwd_h, hb, (((1,), (1,)), ((), ())),
                                     preferred_element_type=F32)
            c, d = re_im(hf)
            if i == 0:
                c, d = c + dd, d + dd
            put(HR + i, c)
            put(HP + i, d - c)
            put(HQ + i, c + d)
            pace_kv(NB + i, hf)

        state = {}

        def mac_item(pos, g0, pi, j0, j1):
            xv, hv = ((US, HR), (UA, HP), (UB, HQ))[pi]
            outs = range(g0, g0 + GRP)
            top = g0 + GRP

            def run():
                pz = zero + pos
                hs = {t: pl_v[pz, hv + t]
                      for t in range(max(g0 - j1 + 1, 0), top - j0)}
                acc = state['acc'] if j0 else {o: None for o in outs}
                for jj in range(j0, j1):
                    xj = pl_v[pz, xv + jj]
                    for o in outs:
                        if o - jj >= 0:
                            t = xj * hs[o - jj]
                            acc[o] = t if acc[o] is None else acc[o] + t
                if j1 < top:
                    state['acc'] = acc
                    return
                r0 = pos * 8
                if pi == 0:
                    state['k1'] = acc
                elif pi == 1:
                    state['im'] = {o: state['k1'][o] + acc[o] for o in outs}
                else:
                    for o in outs:
                        re, im = state['k1'][o] - acc[o], state['im'][o]
                        zr, zi = re, im
                        if o > 0:
                            zr, zi = re - state['prev'][1], im + state['prev'][0]
                        state['prev'] = (re, im)
                        zz_v[n, o, r0:r0 + 8, :] = zr.astype(BF16)
                        zz_v[n, o, BLK + r0:BLK + r0 + 8, :] = zi.astype(BF16)

            nmac = sum(1 for o in outs for jj in range(j0, j1) if o >= jj)
            return (2 * nmac + ((0, GRP, 5 * GRP)[pi] if j1 == top else 0), gate_pl, run)

        items = []
        for pos in range(BLK // 8):
            for g0 in range(0, NB, GRP):
                top = g0 + GRP
                cuts = [0, top] if top <= SPLIT else [0, (top - 1) // 2, top]
                for pi in range(3):
                    for j0, j1 in zip(cuts[:-1], cuts[1:]):
                        items.append(mac_item(pos, g0, pi, j0, j1))

        if half == 0:
            extra = [asum_dyn(jnp.minimum(n * NG + g, HS // 32 - 1), c)
                     for g in range(NG) for c in range(HT)]
            every = len(items) // len(extra)
            items = [it for i, e in enumerate(extra)
                     for it in items[i * every:(i + 1) * every] + [e]
                     ] + items[len(extra) * every:]

        total = sum(c for c, _, _ in items)
        tap_of = []
        cum = 0
        for c, _, _ in items:
            tap_of.append(int(cum * NTAP / total))
            cum += c
        pos = {'tap': 0, 'item': 0}

        def tap(acc):
            t0 = pos['tap']
            pos['tap'] += T // 8
            while pos['item'] < len(items) and tap_of[pos['item']] < pos['tap']:
                i = tap_of[pos['item']] - t0
                _, gate, run = items[pos['item']]
                gate(acc[i * 8:(i + 1) * 8, :])
                run()
                pos['item'] += 1

        def put_p(i, j, col, rows, val):
            p_v[col, rows, :] = val

        for k in range(HT // 2):
            unit(n - half * HF, half, k, tap, put_p)
        assert pos['item'] == len(items)
        return 0

    jax.lax.fori_loop(0, HF, lambda n, c: p2(n, 0), 0)
    jax.lax.fori_loop(HF, NC, lambda n, c: p2(n, 1), 0)

    wout_cp.wait()

    def p3(j, carry):
        inv_p = _up(tab_v[256:288, :])
        inv_m = _up(tab_v[288:320, :])
        rev = 7 - jax.lax.broadcasted_iota(jnp.int32, (8, 128), 0)

        zero = zero_s[0]
        HK = FH // 2

        def rows(k, i):
            tile = i * HT + (k // 2) * (HT // 2) + 2 * j + k % 2
            return (tile, pl.ds(pl.multiple_of(tile * T, T), T),
                    pl.ds(pl.multiple_of(tile * (T // 2), T // 2), T // 2))

        def fresh(k, n):
            return k >= 2 and n % HF == HF - 1

        def p_tile(k, i, n):
            return _up(pp32[k, i, n])

        def gate_p(tok):
            p_v[0, S:S + 8, :] = tok.astype(BF16)

        def gate_wo(tok):
            wout_v[0, HK:HK + 8, 0:128] = pltpu.bitcast(tok, U32)

        def psum_item(k, n, g):
            def run():
                def quad(i, jj):
                    rs = pl.ds(pl.multiple_of(rows(k, i)[0] * T + g * 16, 16), 16)
                    if fresh(k, n):
                        gv = pq_v[k - 2, i, jj, g * 16:(g + 1) * 16, :]
                    else:
                        gv = p_v[n + jj * HF, rs, :]
                    pv = _gelu2(z1_v[n + jj * HF, rs, :].astype(F32)) * gv.astype(F32)
                    pp_v[k, i, n + jj * HF, g * 16:(g + 1) * 16, :] = pv.astype(BF16)
                    return pv
                for i, v in enumerate(_lhs_sums(quad(0, 0), quad(0, 1), quad(1, 0), quad(1, 1))):
                    ps_v[k, i, n, g * 16:(g + 1) * 16, :] = v.astype(BF16)
            return (gate_p, run)

        def wsum_item(m, g):
            def run():
                def quad(i, jj):
                    r0 = (i * HK + g * 16) // 2
                    c0 = (m + 2 * jj) * 128
                    return _up(wout_v[zero, r0:r0 + 8, c0:c0 + 128]).astype(F32)
                for i, v in enumerate(_rhs_sums(quad(0, 0), quad(0, 1), quad(1, 0), quad(1, 1))):
                    ws_v[i, m, g * 16:(g + 1) * 16, :] = v.astype(BF16)
            return (gate_wo, run)

        def psum(k):
            return [psum_item(k, n, g) for n in range(HF) if not fresh(k, n)
                    for g in range(T // 16)]

        queue = []

        def tap(val):
            for i in range(min(len(queue), queue_step[0])):
                gate, run = queue.pop(0)
                r = (i * (T // 8)) // queue_step[0] * 8
                gate(val[r:r + 8, :])
                run()

        queue_step = [0]

        def paced(items, ntaps):
            assert not queue
            queue.extend(items)
            queue_step[0] = -(-len(items) // ntaps)

        def do_unit(u):
            def put_q(i, jj, col, rws, val):
                pq_v[u, i, jj] = val
            unit(HF - 1, 1, 2 * j + u, tap, put_q)
            for g in range(T // 16):
                psum_item(2 + u, HF - 1, g)[1]()

        def finish(k, i, c, o):
            tile, rs, hs = rows(k, i)
            cs = slice(c * 128, (c + 1) * 128)
            ye = _dot(inv_p, _up(zz32[c, tile, 0:64, :]))
            yo = _dot(inv_m, _up(zz32[c, tile, 64:128, :]))
            yd = ye - yo
            y = jnp.concatenate(
                [ye + yo] + [
                    jnp.take_along_axis(yd[q * 8:(q + 1) * 8], rev, axis=0,
                                        mode="promise_in_bounds")
                    for q in reversed(range(BLK // 16))], axis=0)
            gate = o * (1.0 + jnp.tanh((0.25 / _A) * o))
            x = _up(x_v[0, hs, cs]).astype(F32)
            xn = xn_v[c, rs, :].astype(F32)
            o_v[rs, cs] = (x + (xn * y) * gate).astype(BF16)

        def do_pair(k, last=False):
            def prod(lhs, rhs):
                res = _dot(lhs, rhs)
                tap(res)
                return res

            def sa(i):
                return jnp.concatenate([_up(ps32[k, i, n]) for n in range(HF)], axis=1)

            a11 = jnp.concatenate([p_tile(k, 0, n) for n in range(HF)], axis=1)
            a22 = jnp.concatenate([p_tile(k, 1, n) for n in range(HF, NF)], axis=1)
            for m in range(2):
                _strassen(
                    prod, sa, lambda i: _up(ws32[i, m]), a11, a22,
                    _up(wout_v[0, 0:HK // 2, m * 128:(m + 1) * 128]),
                    _up(wout_v[0, HK // 2:HK, (m + 2) * 128:(m + 3) * 128]),
                    lambda i, jj, o: finish(k, i, m + 2 * jj, o))
            for i in range(2):
                rs = rows(k, i)[1]
                if last:
                    cp(o_v.at[rs, 0:512], out_hbm.at[0, rs, 0:512], out_sem).start()
            for i in range(2):
                rs = rows(k, i)[1]
                p = jnp.concatenate([p_tile(k, i, n) for n in range(NF)], axis=1)
                finish(k, i, NC - 1, _dot(p, _up(wout_v[0, 0:HK, 512:D])))
                if last:
                    cp(o_v.at[rs, 512:D], out_hbm.at[0, rs, 512:D], out_sem).start()
                else:
                    cp(o_v.at[rs, :], out_hbm.at[0, rs, :], out_sem).start()

        paced(psum(0) + [wsum_item(m, g) for m in range(2) for g in range(HK // 16)], 12)
        do_unit(0)
        paced(psum(1), 12)
        do_pair(0)
        paced(psum(2), 12)
        do_unit(1)
        paced(psum(3), 12)
        do_pair(1)
        do_pair(2)
        do_pair(3, last=True)
        return carry

    jax.lax.fori_loop(0, P3I, p3, 0)
    cp(o_v, out_hbm.at[0], out_sem).wait()


@jax.jit
def pallas_recurrent_scan__ssm_conv_h3__mixer_gmlp__prompt_kernel(
    A_q: jax.Array,
    A_k: jax.Array,
    A_v: jax.Array,
    A_shift_k: jax.Array,
    A_ssm_k: jax.Array,
    A_ssm_D: jax.Array,
    B_x: jax.Array,
    B_w_in: jax.Array,
    B_w_sp: jax.Array,
    B_b_sp: jax.Array,
    B_w_out: jax.Array,
):
    del B_x
    tab = jnp.asarray(_dft_tables(), dtype=BF16)

    any_spec = pl.BlockSpec(memory_space=pl.ANY)
    return pl.pallas_call(
        _kernel,
        out_shape=jax.ShapeDtypeStruct((1, S, D), BF16),
        in_specs=[any_spec] * 11,
        out_specs=any_spec,
        scratch_shapes=[
            pltpu.VMEM((1, S // 2 + 32, D), U32),
            pltpu.VMEM((1, D // 2 + 8, 2 * FH), U32),
            pltpu.VMEM((1, S // 2 + 8, S), U32),
            pltpu.VMEM((1, FH // 2 + 32, D), U32),
            pltpu.VMEM((2 * NC, S // 2 + 32, 128), U32),
            pltpu.VMEM((NC, 64, S), U32),
            pltpu.VMEM((NC, S + 256, 128), BF16),
            pltpu.VMEM((NF, S, 128), BF16),
            pltpu.VMEM((NF, S + 64, 128), BF16),
            pltpu.VMEM((NF, S + 64, 128), BF16),
            pltpu.VMEM((4, HT, HS // 2, 128), BF16),
            pltpu.VMEM((4, HT, HS // 2, 128), BF16),
            pltpu.VMEM((4, HF, HS, 128), BF16),
            pltpu.VMEM((2, 2, 2, T, 128), BF16),
            pltpu.VMEM((4, 2, NF, T, 128), BF16),
            pltpu.VMEM((4, 5, HF, T, 128), BF16),
            pltpu.VMEM((5, 2, FH // 2, 128), BF16),
            pltpu.VMEM((S, 128), BF16),
            pltpu.VMEM((BLK // 8, 6 * NB + 1, 8, 128), F32),
            pltpu.VMEM((NC, NB, 2 * BLK, 128), BF16),
            pltpu.VMEM((S, 128), F32),
            pltpu.VMEM((S, D), BF16),
            pltpu.VMEM((1, T + 16, FH), F32),
            pltpu.VMEM((1, T + 16, FH), F32),
            pltpu.VMEM((1, T + 16, FH), F32),
            pltpu.VMEM((1, T + 16, FH), F32),
            pltpu.VMEM((1, T + 16, FH), F32),
            pltpu.VMEM((1, T + 16, FH), F32),
            pltpu.VMEM((NT // 2, 5, 2, T, 128), BF16),
            pltpu.VMEM((5, NF, KH, 128), BF16),
            pltpu.VMEM((T, 128), F32),
            pltpu.VMEM((320, 128), U32),
            pltpu.VMEM((NC, KS, 128), F32),
            pltpu.VMEM((NC + 2, 1, 128), F32),
            pltpu.VMEM((KS, D), BF16),
            pltpu.VMEM((D,), BF16),
            pltpu.VMEM((S,), BF16),
            pltpu.SMEM((1,), jnp.int32),
            pltpu.SemaphoreType.DMA((16,)),
        ],
        compiler_params=pltpu.CompilerParams(
            vmem_limit_bytes=100 * 1024 * 1024, disable_bounds_checks=True),
    )(A_q, A_k, A_v, A_shift_k.T, A_ssm_k, A_ssm_D, B_w_in, B_w_sp, B_b_sp, B_w_out, tab)
```

```python
import jax
import jax.numpy as jnp
import numpy as np
import jax.experimental.pallas as pl
import jax.experimental.pallas.tpu as pltpu

F32 = jnp.float32
BF16 = jnp.bfloat16
U32 = jnp.uint32

S = 2048
D = 640
FH = 768
KS = 4
BLK = 128
NB = S // BLK
NC = D // 128
NF = FH // 128
T = 128
NT = S // T
EPS = 1e-5
GRP = 4
SPLIT = 8
import os
AW = int(os.environ.get('AW', 2))
PR = int(os.environ.get('PR', 128))
PLAG = 5
PLAG2 = 4
KG = 512
KR = 32
UA, UB, US, HP, HQ, HR, TOK = (i * NB for i in range(7))
LAG = 4
NTAP = 888
HS = S // 2
HT = HS // T
HF = NF // 2
KH = 256
P3I = 2

_GELU_C0 = float(np.sqrt(2.0 / np.pi))
_GELU_C1 = _GELU_C0 * 0.044715
_A = _GELU_C1 ** (1.0 / 3.0)
_K = _GELU_C0 / _A


def _dft_tables():
    m = np.arange(BLK)[:, None]
    n = np.arange(BLK)[None, :]
    th = 2.0 * np.pi * (((4 * m + 1) * n) % (4 * BLK)) / (4 * BLK)
    ph = 2.0 * np.pi * (((4 * m + 1) * (2 * n + 1)) % (8 * BLK)) / (8 * BLK)
    fu = np.concatenate([np.cos(ph), -np.sin(ph)], axis=0)
    fh = np.concatenate([np.cos(th) + np.sin(th), np.cos(th) - np.sin(th)], axis=0)
    fu, fh = (f.reshape(2, BLK // 8, 8, BLK).transpose(1, 0, 2, 3).reshape(2 * BLK, BLK)
              for f in (fu, fh))
    cp = (np.cos(ph) + np.sin(ph)).T[:BLK // 2] / (8.0 * BLK * _A * _A)
    cm = (np.cos(ph) - np.sin(ph)).T[:BLK // 2] / (8.0 * BLK * _A * _A)
    return np.concatenate([fu, fh, cp, cm], axis=0).astype(np.float32)


def _layernorm(x, eps, scale=1.0):
    m = jnp.mean(x, axis=-1, keepdims=True)
    d = x - m
    v = jnp.sum(d * d, axis=-1, keepdims=True) * (1.0 / (x.shape[-1] * scale * scale))
    return d * jax.lax.rsqrt(v + eps / (scale * scale))


def _gelu2(y):
    return y * (1.0 + jnp.tanh(y * (y * y + _K)))


def _up(x):
    return pltpu.bitcast(x, BF16)


def _dot(a, b):
    return jnp.dot(a, b, preferred_element_type=F32)


def _lhs_sums(a11, a12, a21, a22):
    return a11 + a22, a21 + a22, a11 + a12, a21 - a11, a12 - a22


def _rhs_sums(b11, b12, b21, b22):
    return b11 + b22, b12 - b22, b21 - b11, b11 + b12, b21 + b22


def _strassen(prod, sa, sb, a11, a22, b11, b22, fin):
    m2 = prod(sa(1), b11)
    m4 = prod(a22, sb(2))
    fin(1, 0, m2 + m4)
    m5 = prod(sa(2), b22)
    c11 = m4 - m5
    m3 = prod(a11, sb(1))
    fin(0, 1, m3 + m5)
    c22 = m3 - m2
    m1 = prod(sa(0), sb(0))
    c11, c22 = c11 + m1, c22 + m1
    fin(0, 0, c11 + prod(sa(4), sb(4)))
    fin(1, 1, c22 + prod(sa(3), sb(3)))


def _lhs_sums_w(a11, a12, a21, a22):
    s1 = a21 + a22
    s2 = s1 - a11
    return s1, s2, a11 - a21, a12 - s2


def _rhs_sums_w(b11, b12, b21, b22):
    t1 = b12 - b11
    t2 = b22 - t1
    return t1, t2, b22 - b12, t2 - b21


def _winograd(prod, sa, sb, a11, a12, a22, b11, b21, b22, fin):
    p1 = prod(a11, b11)
    fin(0, 0, p1 + prod(a12, b21))
    u2 = p1 + prod(sa(1), sb(1))
    p5 = prod(sa(0), sb(0))
    fin(0, 1, (u2 + p5) + prod(sa(3), b22))
    u3 = u2 + prod(sa(2), sb(2))
    fin(1, 1, u3 + p5)
    fin(1, 0, u3 - prod(a22, sb(3)))


def _balance(work, n):
    jobs = [(lo, hi, sum(it[0] for it in items)) for items, lo, hi in work]
    rate = [None] * n
    while jobs:
        def free(a, b):
            return [p for p in range(a, b) if rate[p] is None]
        dens, a, b = max(
            (sum(w for lo, hi, w in jobs if a <= lo and hi <= b) / max(len(free(a, b)), 1e-9), a, b)
            for a in {j[0] for j in jobs} for b in {j[1] for j in jobs} if a < b)
        while a > 0 and rate[a - 1] is not None:
            a -= 1
        while b < n and rate[b] is not None:
            b += 1
        for p in free(a, b):
            rate[p] = dens
        jobs = [(lo, hi, w) for lo, hi, w in jobs if not (a <= lo and hi <= b)]
        jobs = [(b if a <= lo < b else lo, a if a < hi <= b else hi, w) for lo, hi, w in jobs]
    queues = [[lo * 16, hi * 16, list(items)] for items, lo, hi in work]
    rel = [[] for _ in range(n)]
    budget = 0.0
    for tau in range(n * 16):
        budget += (rate[tau // 16] or 0.0) / 16
        while True:
            ready = [q for q in queues if q[2] and q[0] <= tau]
            if not ready:
                budget = min(budget, 0.0)
                break
            q = min(ready, key=lambda q: q[1])
            if budget < 0 and q[1] - tau > len(q[2]):
                break
            it = q[2].pop(0)
            rel[tau // 16].append((tau % 16, it))
            budget -= it[0]
    assert not any(q[2] for q in queues)
    return rel


def _kernel(x_hbm, k_hbm, v_hbm, skt_hbm, h_hbm, dv_hbm, win_hbm, wsp_hbm, b_hbm,
            wout_hbm, tab_hbm, out_hbm,
            x_v, win_v, wsp_v, wout_v, kv_v, h_v, xn_v, z1_v, z2_v, p_v, as_v, as2_v, bs_v, pq_v, pp_v, ps_v, ws_v,
            kvb_v, pl_v, zz_v, bcol_v, o_v, zta_v, ztb_v, ztc_v, ztd_v, zte_v, ztf_v, xs_v, wi_v, raw_v, tab_v,
            sk_v, dd_v, skt_v, dv_v, b_v, zero_s, sem):
    cp = pltpu.make_async_copy
    x16 = x_v.bitcast(BF16)
    win16 = win_v.bitcast(BF16)
    kv16 = kv_v.bitcast(BF16)
    h16 = h_v.bitcast(BF16)

    xn32, z232, kvb32, zz32, as32, as232, bs32, pp32, ps32, ws32, xs32, wi32 = (
        r.bitcast(U32)
        for r in (xn_v, z2_v, kvb_v, zz_v, as_v, as2_v, bs_v, pp_v, ps_v, ws_v, xs_v, wi_v))
    wsp16 = wsp_v.bitcast(BF16)

    def wsp_cp(lo, hi, s):
        return cp(wsp_hbm.at[lo:hi, :], wsp16.at[0, lo:hi, :], sem.at[s])

    def x_cp(lo, hi, s):
        return cp(x_hbm.at[0, lo:hi, :], x16.at[0, lo:hi, :], sem.at[s])

    def win_cp(lo, hi, s):
        return cp(win_hbm.at[:, lo:hi], win16.at[0, 0:D, lo:hi], sem.at[s])

    def k_cp(c, s):
        return cp(k_hbm.at[0, :, pl.ds(c * 128, 128)], kv16.at[2 * c, 0:S, :], sem.at[s])

    def v_cp(c, s):
        return cp(v_hbm.at[0, :, pl.ds(c * 128, 128)], kv16.at[2 * c + 1, 0:S, :], sem.at[s])

    def h_cp(c, s):
        return cp(h_hbm.at[pl.ds(c * 128, 128), :], h16.at[c], sem.at[s])

    groups = [
        [cp(b_hbm, b_v, sem.at[0]), cp(skt_hbm, skt_v, sem.at[0]), cp(dv_hbm, dv_v, sem.at[0])],
        [x_cp(0, 256, 1)],
        [win_cp(FH, FH + 256, 2)],
        [win_cp(FH + 256, FH + 512, 3)],
        [win_cp(FH + 512, 2 * FH, 4), win_cp(0, 128, 4)],
        [win_cp(128, 512, 10)],
        [win_cp(512, FH, 5), x_cp(256, 384, 5)],
        [x_cp(384, 6 * T, 6)],
        [x_cp(6 * T, 12 * T, 7), k_cp(0, 7), v_cp(0, 7)],
        [x_cp(12 * T, S, 11), wsp_cp(0, HS // 2, 11), wsp_cp(HS, HS + HS // 2, 11)],
        [cp(tab_hbm, tab_v.bitcast(BF16), sem.at[8]), h_cp(0, 8)],
    ]
    for g in groups:
        for c in g:
            c.start()

    NG = -(-HS // 32 // HF)

    def step_cps(n):
        s = 12 + n
        cps = [k_cp(n + 1, s), v_cp(n + 1, s), h_cp(n + 1, s)]
        if n < HF:
            lo, hi = HS // 2 + n * NG * 16, min(HS // 2 + (n + 1) * NG * 16, HS)
            cps += [wsp_cp(lo, hi, s), wsp_cp(HS + lo, HS + hi, s)]
        return cps

    wout_cp = cp(wout_hbm, wout_v.bitcast(BF16).at[0, 0:FH, :], sem.at[9])
    out_sem = sem.at[5]
    for n in range(NC - 1):
        for d in step_cps(n):
            d.start()
    wout_cp.start()

    def wait(i):
        for c in groups[i]:
            c.wait()

    zero_s[0] = 0
    wait(0)
    skt = skt_v[...].astype(F32)
    dv = dv_v[...].astype(F32).reshape(1, D)
    for c in range(NC):
        sk_v[c] = skt[:, c * 128:(c + 1) * 128]
        dd_v[c] = dv[:, c * 128:(c + 1) * 128]
    brow = b_v[...].astype(F32).reshape(1, S)
    bcol_v[...] = jnp.broadcast_to(brow, (128, S)).T

    def gate_x(tok):
        x_v[0, S // 2:S // 2 + 8, 0:128] = pltpu.bitcast(tok, U32)

    zt_v = (zta_v, ztb_v, ztc_v, ztd_v, zte_v, ztf_v)

    def gate_zt(t):
        def gate(tok):
            zt_v[t % 6][0, T:T + 8, 0:128] = tok
        return gate

    def gate_kv(tok):
        kv_v[0, S // 2:S // 2 + 8, :] = pltpu.bitcast(tok, U32)

    def gate_pl(tok):
        pl_v[0, TOK] = tok

    ndone = [0]

    mode = {'pairs': False}

    def done(val):
        r = (ndone[0] % 8) * 16
        ndone[0] += 1
        if mode['pairs']:
            xs_v[0, 0, 0, r:r + 16, :] = val
        else:
            xn_v[0, S + r:S + r + 16, :] = val

    def lnx_items(t, zero):
        def item(r0):
            def run():
                rs = slice(r0 // 2, r0 // 2 + 8)
                xw = jnp.concatenate([x_v[zero, rs, 0:128], x_v[0, rs, 128:D]], axis=1)
                xn = _layernorm(_up(xw).astype(F32), EPS, _A)
                for c in range(NC):
                    xb = xn[:, c * 128:(c + 1) * 128].astype(BF16)
                    xn_v[c, r0:r0 + 16, :] = xb
                if mode['pairs']:
                    done(xb)
            return (85, gate_x, run)
        return [item(t * T + g * 16) for g in range(T // 16)]

    def lnz_items(t, zero):
        def item(g):
            def run():
                rs = slice(g * 16, (g + 1) * 16)
                z = jnp.concatenate(
                    [zt_v[t % 6][zero, rs, 0:128], zt_v[t % 6][0, rs, 128:FH]], axis=1)
                z = _layernorm(z, 4.0 * _A * _A * EPS)
                r0 = t * T + g * 16
                for n in range(NF):
                    zb = z[:, n * 128:(n + 1) * 128].astype(BF16)
                    z2_v[n, r0:r0 + 16, :] = zb
                done(zb)
            return (90, gate_zt(t), run)
        return [item(g) for g in range(T // 16)]

    def kv_items(c):
        sk = sk_v[c]

        def item(r0):
            def run():
                hs = slice(r0 // 2, (r0 + KR) // 2)
                if r0 == 0:
                    kw = jnp.concatenate(
                        [jnp.zeros((8, 128), F32), _up(kv_v[2 * c, hs, :]).astype(F32)], axis=0)
                else:
                    kw = _up(kv_v[2 * c, r0 // 2 - 8:(r0 + KR) // 2, :]).astype(F32)[8:]
                ks = kw[8:] * sk[0:1, :]
                for t in range(1, KS):
                    ks = ks + pltpu.roll(kw, t, 0)[8:] * sk[t:t + 1, :]
                kvb_v[r0:r0 + KR, :] = (
                    ks * _up(kv_v[2 * c + 1, hs, :]).astype(F32)).astype(BF16)
            return (14 * KR // 8, gate_kv, run)
        return [item(r0) for r0 in range(0, S, KR)]

    def gate_w(tok):
        wsp_v[0, S // 2:S // 2 + 8, 0:128] = pltpu.bitcast(tok, U32)

    def asum_items(r_lo, r_hi):
        def item(zero, r0, c0):
            def run():
                def quad(i, j, c):
                    w = wsp_v[zero, (i * HS + r0) // 2:(i * HS + r0) // 2 + 8,
                              j * HS + c * 128:j * HS + (c + 1) * 128]
                    return _up(w).astype(F32)
                for c in range(c0, c0 + AW):
                    for i, v in enumerate(_lhs_sums_w(
                            quad(0, 0, c), quad(0, 1, c), quad(1, 0, c), quad(1, 1, c))):
                        as_v[i, c, r0:r0 + 16, :] = v.astype(BF16)
            return (20 * AW, gate_w, run)
        return lambda zero: [item(zero, r0, c0) for r0 in range(r_lo * T, r_hi * T, 16)
                             for c0 in range(0, HT, AW)]

    def asum_dyn(g, c):
        def run():
            def quad(i, j):
                r0 = pl.multiple_of(i * (HS // 2) + HS // 4 + g * 8, 8)
                w = wsp_v[0, pl.ds(r0, 8), j * HS + c * 128:j * HS + (c + 1) * 128]
                return _up(w).astype(F32)
            rs = pl.ds(pl.multiple_of(g * 16, 16), 16)
            for i, v in enumerate(_lhs_sums_w(quad(0, 0), quad(0, 1), quad(1, 0), quad(1, 1))):
                as2_v[i, c, rs, :] = v.astype(BF16)
        return (20, gate_w, run)

    def gate_z2(tok):
        z2_v[0, S:S + 8, :] = tok.astype(BF16)

    def bsum(t):
        def item(zero, r0, n):
            def run():
                def quad(i, j):
                    return z2_v[zero + n + j * HF, i * HS + r0:i * HS + r0 + 16, :].astype(F32)
                for i, v in enumerate(_rhs_sums_w(quad(0, 0), quad(0, 1), quad(1, 0), quad(1, 1))):
                    bs_v[i, n, r0:r0 + 16, :] = v.astype(BF16)
            return (21, gate_z2, run)
        return lambda zero: [item(zero, r0, n) for r0 in range((t - HT) * T, (t - HT + 1) * T, 16)
                             for n in range(HF)]

    def gate_xn(tok):
        xn_v[1, S:S + 8, :] = tok.astype(BF16)

    def xsum(u):
        def item(zero, g, c):
            def run():
                def quad(i, j):
                    r0 = (2 * u + i) * T + g * 16
                    return xn_v[zero + c + 2 * j, r0:r0 + 16, :].astype(F32)
                for i, v in enumerate(_lhs_sums(quad(0, 0), quad(0, 1), quad(1, 0), quad(1, 1))):
                    xs_v[u, i, c, g * 16:(g + 1) * 16, :] = v.astype(BF16)
            return (24, gate_xn, run)
        return lambda zero: [item(zero, g, c) for g in range(T // 16) for c in range(2)]

    def gate_wi(tok):
        win_v[0, D // 2:D // 2 + 8, 0:128] = pltpu.bitcast(tok, U32)

    def wisum(zero):
        def item(g, q):
            def run():
                def quad(i, j):
                    r0 = (i * KH + g * 16) // 2
                    c0 = ((q // HF) * NF + q % HF + j * HF) * 128
                    return _up(win_v[zero, r0:r0 + 8, c0:c0 + 128]).astype(F32)
                for i, v in enumerate(_rhs_sums(quad(0, 0), quad(0, 1), quad(1, 0), quad(1, 1))):
                    wi_v[i, q, g * 16:(g + 1) * 16, :] = v.astype(BF16)
            return (23, gate_wi, run)
        return [item(g, (q + HF) % NF) for q in range(NF) for g in range(KH // 16)]

    def taps_of(val):
        rows, cols = val.shape
        return [(lambda i=i, n=n: val[i * 8:(i + 1) * 8, n * 128:(n + 1) * 128])
                for n in range(cols // 128) for i in range(rows // 8)]

    def activate(kind, t, n, z):
        if kind == 2:
            zt_v[t % 6][0, 0:T, n * 128:(n + 1) * 128] = _gelu2(z)
        else:
            z1_v[n, t * T:(t + 1) * T, :] = z.astype(BF16)

    def piece(kind, t, n, zero, defer=False, halves=False):
        col = n * 128 + (FH if kind == 2 else 0)
        xn = jnp.concatenate(
            [_up(xn32[zero if zero is not None and c == 0 else c,
                      t * T // 2:(t + 1) * T // 2, :]) for c in range(NC)], axis=1)
        w = _up(win_v[0, 0:D // 2, col:col + 128])
        if halves:
            z = jnp.concatenate([_dot(xn[:T // 2], w), _dot(xn[T // 2:], w)], axis=0)
        else:
            z = _dot(xn, w)
        if defer:
            raw_v[...] = z
        else:
            activate(kind, t, n, z)
        return taps_of(z)

    def pair_piece(kind, u, m, gate_idx, slot_done):
        q = (kind - 1) * HF + m
        outs = []

        def wq(lo, hi, j):
            c0 = ((kind - 1) * NF + m + j * HF) * 128
            return _up(win_v[0, lo // 2:hi // 2, c0:c0 + 128])

        for r0 in range(0, T, PR):
            def xq(i, cs):
                r = (2 * u + i) * T + r0
                return jnp.concatenate(
                    [_up(xn32[c, r // 2:(r + PR) // 2, :]) for c in cs], axis=1)

            def fin(i, j, c):
                z = c + _dot(xq(i, [NC - 1]), wq(2 * KH, D, j))
                t, n = 2 * u + i, m + j * HF
                if kind == 2:
                    zt_v[t % 6][0, r0:r0 + PR, n * 128:(n + 1) * 128] = _gelu2(z)
                else:
                    z1_v[n, t * T + r0:t * T + r0 + PR, :] = z.astype(BF16)
                outs.extend(taps_of(z))
                if len(outs) == T // 8:
                    slot_done(list(outs))
                    outs.clear()

            _strassen(
                _dot,
                lambda i: jnp.concatenate(
                    [_up(xs32[u + (gate_idx() if c == 0 and i != 4 else 0), i, c,
                              r0 // 2:(r0 + PR) // 2, :]) for c in range(2)], axis=1),
                lambda i: _up(wi32[i, q]), xq(0, (0, 1)), xq(1, (2, 3)),
                wq(0, KH, 0), wq(KH, 2 * KH, 1), fin)

    pending = []

    def plan(work, zero, n):
        work = [(mk(zero), lo, hi) for mk, lo, hi in work]
        return [a + b for a, b in zip(
            _balance([w for w in work if w[0][0][0] >= 80], n),
            _balance([w for w in work if w[0][0][0] < 80], n))]

    def pair_block(halves, work, lag):
        zero = zero_s[0]
        mode['pairs'] = True
        if pending:
            activate(*pending.pop(), raw_v[...])
        rel = plan(work, zero, 12 * len(halves))
        taps = []
        state = {'gated': False}

        def release(k):
            for i, (_, gate, run) in sorted(rel[k], key=lambda e: e[0]):
                gate(taps[k][i]())
                run()
                state['gated'] = True

        def slot_done(z):
            taps.append(z)
            if len(taps) > lag:
                release(len(taps) - 1 - lag)

        for kind, u in halves:
            for m in range(HF):
                pair_piece(kind, u, m, lambda: zero if state['gated'] else 0, slot_done)
        for k in range(len(taps) - lag, len(taps)):
            release(k)

    def block(pieces, work, defer=True, free=None):
        zero = zero_s[0]
        if pending:
            activate(*pending.pop(), raw_v[...])
        rel = plan(work, zero, len(pieces))
        taps = []
        gated = False
        for k in range(len(pieces) + LAG):
            if free is not None and k == len(pieces) - 1:
                for _, _, run in free(zero):
                    run()
                gated = True
            if k < len(pieces):
                last = defer and k == len(pieces) - 1
                halves = len(pieces) % 4 == 2 and k == len(pieces) - 1
                taps.append(piece(*pieces[k], zero if gated else None, last, halves))
                if last:
                    pending.append(pieces[k])
            if k >= LAG:
                for i, (_, gate, run) in sorted(rel[k - LAG], key=lambda e: e[0]):
                    gate(taps[k - LAG][i]())
                    run()
                    gated = True

    def cols(kind, t, lo=0, hi=NF):
        return [(kind, t, n) for n in range(lo, hi)]

    def lnx(t):
        return lambda zero: lnx_items(t, zero)

    def lnz(t):
        return lambda zero: lnz_items(t, zero)

    wait(1)
    for it in lnx_items(0, 0) + lnx_items(1, 0):
        it[2]()
    wait(2)
    block(cols(2, 0, 0, 2) + cols(2, 1, 0, 2), [])
    wait(3)
    block(cols(2, 0, 2, 4) + cols(2, 1, 2, 4), [])
    wait(4)
    block(cols(2, 0, 4) + cols(2, 1, 4) + cols(1, 0, 0, 1) + cols(1, 1, 0, 1), [])
    wait(5)
    block(cols(1, 0, 1, 4) + cols(1, 1, 1, 4), [(lnz(0), 0, 1)])
    wait(6)
    block(cols(1, 0, 4) + cols(1, 1, 4), [], free=lnx(2))

    def tiles(lo, hi):
        return [pc for t in range(lo, hi) for pc in cols(2, t) + cols(1, t)]

    wait(7)
    block(tiles(2, 4),
          [(lnx(3), 0, 7), (lnx(4), 0, 14), (lnx(5), 0, 15), (lnz(1), 0, 19),
           (wisum, 0, 24), (xsum(2), 17, 24)])
    d = PLAG - 4
    wait(8)
    pair_block([(2, 2), (1, 2), (2, 3), (1, 3), (2, 4), (1, 4)],
               [(lnx(6), 0, 11 - d), (lnx(7), 0, 11 - d), (xsum(3), 13, 20 - d),
                (lnx(8), 0, 35 - d), (lnx(9), 0, 35 - d), (xsum(4), 37, 44 - d),
                (lnx(10), 0, 62 - d), (lnx(11), 0, 62 - d), (xsum(5), 64, 72),
                (lnz(2), 0, 44 - d), (lnz(3), 0, 44 - d), (lnz(4), 12, 67 - d), (lnz(5), 12, 67 - d),
                (lnz(6), 36, 67 - d), (lnz(7), 36, 67 - d), (kv_items, 0, 72)], PLAG)
    d = PLAG2 - 4
    wait(9)
    pair_block([(2, 5), (1, 5), (2, 6), (2, 7), (1, 6), (1, 7)],
               [(lnx(12), 0, 11 - d), (lnx(13), 0, 11 - d), (xsum(6), 13, 20 - d),
                (lnx(14), 0, 23 - d), (lnx(15), 0, 23 - d), (xsum(7), 25, 32 - d),
                (lnz(8), 0, 32 - d), (lnz(9), 0, 32 - d), (lnz(10), 12, 44), (lnz(11), 12, 44),
                (lnz(12), 36, 54), (lnz(13), 36, 54), (lnz(14), 48, 63 - d), (lnz(15), 48, 63 - d),
                (bsum(8), 36, 72), (bsum(9), 36, 72), (bsum(10), 48 + d, 72), (bsum(11), 48 + d, 72),
                (bsum(12), 58 + d, 72), (bsum(13), 58 + d, 72), (bsum(14), 67, 72), (bsum(15), 67, 72),
                (asum_items(0, HT // 2), 0, 72)], PLAG2)
    wait(10)

    def unit(n, half, k, tap, put_p):
        def span(start, size):
            if isinstance(start, int):
                return slice(start, start + size)
            return pl.ds(pl.multiple_of(start, size), size)

        r = half * (HT // 2) + k
        top, bot = span(r * T, T), span(HS + r * T, T)
        toph, both = span(r * (T // 2), T // 2), span(HS // 2 + r * (T // 2), T // 2)
        sums, sumh = (as32, as232)[half], span(k * (T // 2), T // 2)

        def prod(lhs, rhs):
            acc = None
            for q in range(HS // KG):
                part = _dot(lhs(q), rhs(q))
                acc = part if acc is None else acc + part
                tap(acc)
            return acc

        def sa(i):
            return lambda q: jnp.concatenate(
                [_up(sums[i, c, sumh, :]) for c in range(q * KG // 128, (q + 1) * KG // 128)],
                axis=1)

        def sb(i):
            return lambda q: _up(bs32[i, n, q * KG // 2:(q + 1) * KG // 2, :])

        def a11(q):
            return _up(wsp_v[0, toph, q * KG:(q + 1) * KG])

        def a12(q):
            return _up(wsp_v[0, toph, HS + q * KG:HS + (q + 1) * KG])

        def b21(q):
            return _up(z232[n, (HS + q * KG) // 2:(HS + (q + 1) * KG) // 2, :])

        def a22(q):
            return _up(wsp_v[0, both, HS + q * KG:HS + (q + 1) * KG])

        def b11(q):
            return _up(z232[n, q * KG // 2:(q + 1) * KG // 2, :])

        def b22(q):
            return _up(z232[n + HF, (HS + q * KG) // 2:(HS + (q + 1) * KG) // 2, :])

        def fin(i, j, c):
            col, rows = n + j * HF, (top, bot)[i]
            put_p(i, j, col, rows, (c + bcol_v[rows, :]).astype(BF16))

        _winograd(prod, sa, sb, a11, a12, a22, b11, b21, b22, fin)

    def p2(n, half):
        nn = jnp.minimum(n + 1, NC - 1)

        for q in range(half * HF, min((half + 1) * HF, NC - 1)):
            @pl.when(n == q)
            def _():
                for d in step_cps(q):
                    d.wait()

        zero = zero_s[0]
        fwd_u = _up(tab_v[0:128, :])
        fwd_h = _up(tab_v[128:256, :])
        dd = dd_v[n]

        def put(slot, val):
            pl_v[:, slot] = val

        def re_im(val):
            val = val.reshape(BLK // 8, 2, 8, 128)
            return val[:, 0], val[:, 1]

        kvi = kv_items(nn)

        def pace_kv(d, val):
            if d % 4 == 3:
                for j in range(8):
                    _, gate, run = kvi[(d // 4) * 8 + j]
                    gate(val[j * 32:j * 32 + 8, :])
                    run()

        for i in range(NB):
            u = _dot(fwd_u, _up(kvb32[i * BLK // 2:(i + 1) * BLK // 2, :]))
            a, b = re_im(u)
            put(UA + i, a)
            put(UB + i, b)
            put(US + i, a + b)
            pace_kv(i, u)
        for i in range(NB):
            hb = _up(h_v[n, :, i * BLK:(i + 1) * BLK])
            hf = jax.lax.dot_general(fwd_h, hb, (((1,), (1,)), ((), ())),
                                     preferred_element_type=F32)
            c, d = re_im(hf)
            if i == 0:
                c, d = c + dd, d + dd
            put(HR + i, c)
            put(HP + i, d - c)
            put(HQ + i, c + d)
            pace_kv(NB + i, hf)

        state = {}

        def mac_item(pos, g0, pi, j0, j1):
            xv, hv = ((US, HR), (UA, HP), (UB, HQ))[pi]
            outs = range(g0, g0 + GRP)
            top = g0 + GRP

            def run():
                pz = zero + pos
                hs = {t: pl_v[pz, hv + t]
                      for t in range(max(g0 - j1 + 1, 0), top - j0)}
                acc = state['acc'] if j0 else {o: None for o in outs}
                for jj in range(j0, j1):
                    xj = pl_v[pz, xv + jj]
                    for o in outs:
                        if o - jj >= 0:
                            t = xj * hs[o - jj]
                            acc[o] = t if acc[o] is None else acc[o] + t
                if j1 < top:
                    state['acc'] = acc
                    return
                r0 = pos * 8
                if pi == 0:
                    state['k1'] = acc
                elif pi == 1:
                    state['im'] = {o: state['k1'][o] + acc[o] for o in outs}
                else:
                    for o in outs:
                        re, im = state['k1'][o] - acc[o], state['im'][o]
                        zr, zi = re, im
                        if o > 0:
                            zr, zi = re - state['prev'][1], im + state['prev'][0]
                        state['prev'] = (re, im)
                        zz_v[n, o, r0:r0 + 8, :] = zr.astype(BF16)
                        zz_v[n, o, BLK + r0:BLK + r0 + 8, :] = zi.astype(BF16)

            nmac = sum(1 for o in outs for jj in range(j0, j1) if o >= jj)
            return (2 * nmac + ((0, GRP, 5 * GRP)[pi] if j1 == top else 0), gate_pl, run)

        items = []
        for pos in range(BLK // 8):
            for g0 in range(0, NB, GRP):
                top = g0 + GRP
                cuts = [0, top] if top <= SPLIT else [0, (top - 1) // 2, top]
                for pi in range(3):
                    for j0, j1 in zip(cuts[:-1], cuts[1:]):
                        items.append(mac_item(pos, g0, pi, j0, j1))

        if half == 0:
            extra = [asum_dyn(jnp.minimum(n * NG + g, HS // 32 - 1), c)
                     for g in range(NG) for c in range(HT)]
            every = len(items) // len(extra)
            items = [it for i, e in enumerate(extra)
                     for it in items[i * every:(i + 1) * every] + [e]
                     ] + items[len(extra) * every:]

        total = sum(c for c, _, _ in items)
        tap_of = []
        cum = 0
        for c, _, _ in items:
            tap_of.append(int(cum * NTAP / total))
            cum += c
        pos = {'tap': 0, 'item': 0}

        def tap(acc):
            t0 = pos['tap']
            pos['tap'] += T // 8
            while pos['item'] < len(items) and tap_of[pos['item']] < pos['tap']:
                i = tap_of[pos['item']] - t0
                _, gate, run = items[pos['item']]
                gate(acc[i * 8:(i + 1) * 8, :])
                run()
                pos['item'] += 1

        def put_p(i, j, col, rows, val):
            p_v[col, rows, :] = val

        for k in range(HT // 2):
            unit(n - half * HF, half, k, tap, put_p)
        assert pos['item'] == len(items)
        return 0

    jax.lax.fori_loop(0, HF, lambda n, c: p2(n, 0), 0)
    jax.lax.fori_loop(HF, NC, lambda n, c: p2(n, 1), 0)

    wout_cp.wait()

    def p3(j, carry):
        inv_p = _up(tab_v[256:288, :])
        inv_m = _up(tab_v[288:320, :])
        rev = 7 - jax.lax.broadcasted_iota(jnp.int32, (8, 128), 0)

        zero = zero_s[0]
        HK = FH // 2

        def rows(k, i):
            tile = i * HT + (k // 2) * (HT // 2) + 2 * j + k % 2
            return (tile, pl.ds(pl.multiple_of(tile * T, T), T),
                    pl.ds(pl.multiple_of(tile * (T // 2), T // 2), T // 2))

        def fresh(k, n):
            return k >= 2 and n % HF == HF - 1

        def p_tile(k, i, n):
            return _up(pp32[k, i, n])

        def gate_p(tok):
            p_v[0, S:S + 8, :] = tok.astype(BF16)

        def gate_wo(tok):
            wout_v[0, HK:HK + 8, 0:128] = pltpu.bitcast(tok, U32)

        def psum_item(k, n, g):
            def run():
                def quad(i, jj):
                    rs = pl.ds(pl.multiple_of(rows(k, i)[0] * T + g * 16, 16), 16)
                    if fresh(k, n):
                        gv = pq_v[k - 2, i, jj, g * 16:(g + 1) * 16, :]
                    else:
                        gv = p_v[n + jj * HF, rs, :]
                    pv = _gelu2(z1_v[n + jj * HF, rs, :].astype(F32)) * gv.astype(F32)
                    pp_v[k, i, n + jj * HF, g * 16:(g + 1) * 16, :] = pv.astype(BF16)
                    return pv
                for i, v in enumerate(_lhs_sums(quad(0, 0), quad(0, 1), quad(1, 0), quad(1, 1))):
                    ps_v[k, i, n, g * 16:(g + 1) * 16, :] = v.astype(BF16)
            return (gate_p, run)

        def wsum_item(m, g):
            def run():
                def quad(i, jj):
                    r0 = (i * HK + g * 16) // 2
                    c0 = (m + 2 * jj) * 128
                    return _up(wout_v[zero, r0:r0 + 8, c0:c0 + 128]).astype(F32)
                for i, v in enumerate(_rhs_sums(quad(0, 0), quad(0, 1), quad(1, 0), quad(1, 1))):
                    ws_v[i, m, g * 16:(g + 1) * 16, :] = v.astype(BF16)
            return (gate_wo, run)

        def psum(k):
            return [psum_item(k, n, g) for n in range(HF) if not fresh(k, n)
                    for g in range(T // 16)]

        queue = []

        def tap(val):
            for i in range(min(len(queue), queue_step[0])):
                gate, run = queue.pop(0)
                r = (i * (T // 8)) // queue_step[0] * 8
                gate(val[r:r + 8, :])
                run()

        queue_step = [0]

        def paced(items, ntaps):
            assert not queue
            queue.extend(items)
            queue_step[0] = -(-len(items) // ntaps)

        def do_unit(u):
            def put_q(i, jj, col, rws, val):
                pq_v[u, i, jj] = val
            unit(HF - 1, 1, 2 * j + u, tap, put_q)
            for g in range(T // 16):
                psum_item(2 + u, HF - 1, g)[1]()

        def finish(k, i, c, o):
            tile, rs, hs = rows(k, i)
            cs = slice(c * 128, (c + 1) * 128)
            ye = _dot(inv_p, _up(zz32[c, tile, 0:64, :]))
            yo = _dot(inv_m, _up(zz32[c, tile, 64:128, :]))
            yd = ye - yo
            y = jnp.concatenate(
                [ye + yo] + [
                    jnp.take_along_axis(yd[q * 8:(q + 1) * 8], rev, axis=0,
                                        mode="promise_in_bounds")
                    for q in reversed(range(BLK // 16))], axis=0)
            gate = o * (1.0 + jnp.tanh((0.25 / _A) * o))
            x = _up(x_v[0, hs, cs]).astype(F32)
            xn = xn_v[c, rs, :].astype(F32)
            o_v[rs, cs] = (x + (xn * y) * gate).astype(BF16)

        def do_pair(k, last=False):
            def prod(lhs, rhs):
                res = _dot(lhs, rhs)
                tap(res)
                return res

            def sa(i):
                return jnp.concatenate([_up(ps32[k, i, n]) for n in range(HF)], axis=1)

            a11 = jnp.concatenate([p_tile(k, 0, n) for n in range(HF)], axis=1)
            a22 = jnp.concatenate([p_tile(k, 1, n) for n in range(HF, NF)], axis=1)
            for m in range(2):
                _strassen(
                    prod, sa, lambda i: _up(ws32[i, m]), a11, a22,
                    _up(wout_v[0, 0:HK // 2, m * 128:(m + 1) * 128]),
                    _up(wout_v[0, HK // 2:HK, (m + 2) * 128:(m + 3) * 128]),
                    lambda i, jj, o: finish(k, i, m + 2 * jj, o))
            for i in range(2):
                rs = rows(k, i)[1]
                if last:
                    cp(o_v.at[rs, 0:512], out_hbm.at[0, rs, 0:512], out_sem).start()
            for i in range(2):
                rs = rows(k, i)[1]
                p = jnp.concatenate([p_tile(k, i, n) for n in range(NF)], axis=1)
                finish(k, i, NC - 1, _dot(p, _up(wout_v[0, 0:HK, 512:D])))
                if last:
                    cp(o_v.at[rs, 512:D], out_hbm.at[0, rs, 512:D], out_sem).start()
                else:
                    cp(o_v.at[rs, :], out_hbm.at[0, rs, :], out_sem).start()

        paced(psum(0) + [wsum_item(m, g) for m in range(2) for g in range(HK // 16)], 12)
        do_unit(0)
        paced(psum(1), 12)
        do_pair(0)
        paced(psum(2), 12)
        do_unit(1)
        paced(psum(3), 12)
        do_pair(1)
        do_pair(2)
        do_pair(3, last=True)
        return carry

    jax.lax.fori_loop(0, P3I, p3, 0)
    cp(o_v, out_hbm.at[0], out_sem).wait()


@jax.jit
def pallas_recurrent_scan__ssm_conv_h3__mixer_gmlp__prompt_kernel(
    A_q: jax.Array,
    A_k: jax.Array,
    A_v: jax.Array,
    A_shift_k: jax.Array,
    A_ssm_k: jax.Array,
    A_ssm_D: jax.Array,
    B_x: jax.Array,
    B_w_in: jax.Array,
    B_w_sp: jax.Array,
    B_b_sp: jax.Array,
    B_w_out: jax.Array,
):
    del B_x
    tab = jnp.asarray(_dft_tables(), dtype=BF16)

    any_spec = pl.BlockSpec(memory_space=pl.ANY)
    return pl.pallas_call(
        _kernel,
        out_shape=jax.ShapeDtypeStruct((1, S, D), BF16),
        in_specs=[any_spec] * 11,
        out_specs=any_spec,
        scratch_shapes=[
            pltpu.VMEM((1, S // 2 + 32, D), U32),
            pltpu.VMEM((1, D // 2 + 8, 2 * FH), U32),
            pltpu.VMEM((1, S // 2 + 8, S), U32),
            pltpu.VMEM((1, FH // 2 + 32, D), U32),
            pltpu.VMEM((2 * NC, S // 2 + 32, 128), U32),
            pltpu.VMEM((NC, 64, S), U32),
            pltpu.VMEM((NC, S + 256, 128), BF16),
            pltpu.VMEM((NF, S, 128), BF16),
            pltpu.VMEM((NF, S + 64, 128), BF16),
            pltpu.VMEM((NF, S + 64, 128), BF16),
            pltpu.VMEM((4, HT, HS // 2, 128), BF16),
            pltpu.VMEM((4, HT, HS // 2, 128), BF16),
            pltpu.VMEM((4, HF, HS, 128), BF16),
            pltpu.VMEM((2, 2, 2, T, 128), BF16),
            pltpu.VMEM((4, 2, NF, T, 128), BF16),
            pltpu.VMEM((4, 5, HF, T, 128), BF16),
            pltpu.VMEM((5, 2, FH // 2, 128), BF16),
            pltpu.VMEM((S, 128), BF16),
            pltpu.VMEM((BLK // 8, 6 * NB + 1, 8, 128), F32),
            pltpu.VMEM((NC, NB, 2 * BLK, 128), BF16),
            pltpu.VMEM((S, 128), F32),
            pltpu.VMEM((S, D), BF16),
            pltpu.VMEM((1, T + 16, FH), F32),
            pltpu.VMEM((1, T + 16, FH), F32),
            pltpu.VMEM((1, T + 16, FH), F32),
            pltpu.VMEM((1, T + 16, FH), F32),
            pltpu.VMEM((1, T + 16, FH), F32),
            pltpu.VMEM((1, T + 16, FH), F32),
            pltpu.VMEM((NT // 2, 5, 2, T, 128), BF16),
            pltpu.VMEM((5, NF, KH, 128), BF16),
            pltpu.VMEM((T, 128), F32),
            pltpu.VMEM((320, 128), U32),
            pltpu.VMEM((NC, KS, 128), F32),
            pltpu.VMEM((NC + 2, 1, 128), F32),
            pltpu.VMEM((KS, D), BF16),
            pltpu.VMEM((D,), BF16),
            pltpu.VMEM((S,), BF16),
            pltpu.SMEM((1,), jnp.int32),
            pltpu.SemaphoreType.DMA((16,)),
        ],
        compiler_params=pltpu.CompilerParams(
            vmem_limit_bytes=100 * 1024 * 1024, disable_bounds_checks=True),
    )(A_q, A_k, A_v, A_shift_k.T, A_ssm_k, A_ssm_D, B_w_in, B_w_sp, B_b_sp, B_w_out, tab)
```

```python
import jax
import jax.numpy as jnp
import numpy as np
import jax.experimental.pallas as pl
import jax.experimental.pallas.tpu as pltpu

F32 = jnp.float32
BF16 = jnp.bfloat16
U32 = jnp.uint32

S = 2048
D = 640
FH = 768
KS = 4
BLK = 128
NB = S // BLK
NC = D // 128
NF = FH // 128
T = 128
NT = S // T
EPS = 1e-5
GRP = 4
SPLIT = 8
AW = 2
KG = 512
KR = 32
UA, UB, US, HP, HQ, HR, TOK = (i * NB for i in range(7))
LAG = 4
NTAP = 888
HS = S // 2
HT = HS // T
HF = NF // 2
KH = 256
P3I = 2

_GELU_C0 = float(np.sqrt(2.0 / np.pi))
_GELU_C1 = _GELU_C0 * 0.044715
_A = _GELU_C1 ** (1.0 / 3.0)
_K = _GELU_C0 / _A


def _dft_tables():
    m = np.arange(BLK)[:, None]
    n = np.arange(BLK)[None, :]
    th = 2.0 * np.pi * (((4 * m + 1) * n) % (4 * BLK)) / (4 * BLK)
    ph = 2.0 * np.pi * (((4 * m + 1) * (2 * n + 1)) % (8 * BLK)) / (8 * BLK)
    fu = np.concatenate([np.cos(ph), -np.sin(ph)], axis=0)
    fh = np.concatenate([np.cos(th) + np.sin(th), np.cos(th) - np.sin(th)], axis=0)
    fu, fh = (f.reshape(2, BLK // 8, 8, BLK).transpose(1, 0, 2, 3).reshape(2 * BLK, BLK)
              for f in (fu, fh))
    cp = (np.cos(ph) + np.sin(ph)).T[:BLK // 2] / (8.0 * BLK * _A * _A)
    cm = (np.cos(ph) - np.sin(ph)).T[:BLK // 2] / (8.0 * BLK * _A * _A)
    return np.concatenate([fu, fh, cp, cm], axis=0).astype(np.float32)


def _layernorm(x, eps, scale=1.0):
    m = jnp.mean(x, axis=-1, keepdims=True)
    d = x - m
    v = jnp.sum(d * d, axis=-1, keepdims=True) * (1.0 / (x.shape[-1] * scale * scale))
    return d * jax.lax.rsqrt(v + eps / (scale * scale))


def _gelu2(y):
    return y * (1.0 + jnp.tanh(y * (y * y + _K)))


def _up(x):
    return pltpu.bitcast(x, BF16)


def _dot(a, b):
    return jnp.dot(a, b, preferred_element_type=F32)


def _lhs_sums(a11, a12, a21, a22):
    return a11 + a22, a21 + a22, a11 + a12, a21 - a11, a12 - a22


def _rhs_sums(b11, b12, b21, b22):
    return b11 + b22, b12 - b22, b21 - b11, b11 + b12, b21 + b22


def _strassen(prod, sa, sb, a11, a22, b11, b22, fin):
    m2 = prod(sa(1), b11)
    m4 = prod(a22, sb(2))
    fin(1, 0, m2 + m4)
    m5 = prod(sa(2), b22)
    c11 = m4 - m5
    m3 = prod(a11, sb(1))
    fin(0, 1, m3 + m5)
    c22 = m3 - m2
    m1 = prod(sa(0), sb(0))
    c11, c22 = c11 + m1, c22 + m1
    fin(0, 0, c11 + prod(sa(4), sb(4)))
    fin(1, 1, c22 + prod(sa(3), sb(3)))


def _lhs_sums_w(a11, a12, a21, a22):
    s1 = a21 + a22
    s2 = s1 - a11
    return s1, s2, a11 - a21, a12 - s2


def _rhs_sums_w(b11, b12, b21, b22):
    t1 = b12 - b11
    t2 = b22 - t1
    return t1, t2, b22 - b12, t2 - b21


def _winograd(prod, sa, sb, a11, a12, a22, b11, b21, b22, fin):
    p1 = prod(a11, b11)
    fin(0, 0, p1 + prod(a12, b21))
    u2 = p1 + prod(sa(1), sb(1))
    p5 = prod(sa(0), sb(0))
    fin(0, 1, (u2 + p5) + prod(sa(3), b22))
    u3 = u2 + prod(sa(2), sb(2))
    fin(1, 1, u3 + p5)
    fin(1, 0, u3 - prod(a22, sb(3)))


def _balance(work, n):
    jobs = [(lo, hi, sum(it[0] for it in items)) for items, lo, hi in work]
    rate = [None] * n
    while jobs:
        def free(a, b):
            return [p for p in range(a, b) if rate[p] is None]
        dens, a, b = max(
            (sum(w for lo, hi, w in jobs if a <= lo and hi <= b) / max(len(free(a, b)), 1e-9), a, b)
            for a in {j[0] for j in jobs} for b in {j[1] for j in jobs} if a < b)
        while a > 0 and rate[a - 1] is not None:
            a -= 1
        while b < n and rate[b] is not None:
            b += 1
        for p in free(a, b):
            rate[p] = dens
        jobs = [(lo, hi, w) for lo, hi, w in jobs if not (a <= lo and hi <= b)]
        jobs = [(b if a <= lo < b else lo, a if a < hi <= b else hi, w) for lo, hi, w in jobs]
    queues = [[lo * 16, hi * 16, list(items)] for items, lo, hi in work]
    rel = [[] for _ in range(n)]
    budget = 0.0
    for tau in range(n * 16):
        budget += (rate[tau // 16] or 0.0) / 16
        while True:
            ready = [q for q in queues if q[2] and q[0] <= tau]
            if not ready:
                budget = min(budget, 0.0)
                break
            q = min(ready, key=lambda q: q[1])
            if budget < 0 and q[1] - tau > len(q[2]):
                break
            it = q[2].pop(0)
            rel[tau // 16].append((tau % 16, it))
            budget -= it[0]
    assert not any(q[2] for q in queues)
    return rel


def _kernel(x_hbm, k_hbm, v_hbm, skt_hbm, h_hbm, dv_hbm, win_hbm, wsp_hbm, b_hbm,
            wout_hbm, tab_hbm, out_hbm,
            x_v, win_v, wsp_v, wout_v, kv_v, h_v, xn_v, z1_v, z2_v, p_v, as_v, as2_v, bs_v, pq_v, pp_v, ps_v, ws_v,
            kvb_v, pl_v, zz_v, bcol_v, o_v, zta_v, ztb_v, ztc_v, ztd_v, zte_v, ztf_v, xs_v, wi_v, raw_v, tab_v,
            sk_v, dd_v, skt_v, dv_v, b_v, zero_s, sem):
    cp = pltpu.make_async_copy
    x16 = x_v.bitcast(BF16)
    win16 = win_v.bitcast(BF16)
    kv16 = kv_v.bitcast(BF16)
    h16 = h_v.bitcast(BF16)

    xn32, z232, kvb32, zz32, as32, as232, bs32, pp32, ps32, ws32, xs32, wi32 = (
        r.bitcast(U32)
        for r in (xn_v, z2_v, kvb_v, zz_v, as_v, as2_v, bs_v, pp_v, ps_v, ws_v, xs_v, wi_v))
    wsp16 = wsp_v.bitcast(BF16)

    def wsp_cp(lo, hi, s):
        return cp(wsp_hbm.at[lo:hi, :], wsp16.at[0, lo:hi, :], sem.at[s])

    def x_cp(lo, hi, s):
        return cp(x_hbm.at[0, lo:hi, :], x16.at[0, lo:hi, :], sem.at[s])

    def win_cp(lo, hi, s):
        return cp(win_hbm.at[:, lo:hi], win16.at[0, 0:D, lo:hi], sem.at[s])

    def k_cp(c, s):
        return cp(k_hbm.at[0, :, pl.ds(c * 128, 128)], kv16.at[2 * c, 0:S, :], sem.at[s])

    def v_cp(c, s):
        return cp(v_hbm.at[0, :, pl.ds(c * 128, 128)], kv16.at[2 * c + 1, 0:S, :], sem.at[s])

    def h_cp(c, s):
        return cp(h_hbm.at[pl.ds(c * 128, 128), :], h16.at[c], sem.at[s])

    groups = [
        [cp(b_hbm, b_v, sem.at[0]), cp(skt_hbm, skt_v, sem.at[0]), cp(dv_hbm, dv_v, sem.at[0])],
        [x_cp(0, 256, 1)],
        [win_cp(FH, FH + 256, 2)],
        [win_cp(FH + 256, FH + 512, 3)],
        [win_cp(FH + 512, 2 * FH, 4), win_cp(0, 128, 4)],
        [win_cp(128, 512, 10)],
        [win_cp(512, FH, 5), x_cp(256, 384, 5)],
        [x_cp(384, 6 * T, 6)],
        [x_cp(6 * T, 12 * T, 7), k_cp(0, 7), v_cp(0, 7)],
        [x_cp(12 * T, S, 11), wsp_cp(0, HS // 2, 11), wsp_cp(HS, HS + HS // 2, 11)],
        [cp(tab_hbm, tab_v.bitcast(BF16), sem.at[8]), h_cp(0, 8)],
    ]
    for g in groups:
        for c in g:
            c.start()

    NG = -(-HS // 32 // HF)

    def step_cps(n):
        s = 12 + n
        cps = [k_cp(n + 1, s), v_cp(n + 1, s), h_cp(n + 1, s)]
        if n < HF:
            lo, hi = HS // 2 + n * NG * 16, min(HS // 2 + (n + 1) * NG * 16, HS)
            cps += [wsp_cp(lo, hi, s), wsp_cp(HS + lo, HS + hi, s)]
        return cps

    wout_cp = cp(wout_hbm, wout_v.bitcast(BF16).at[0, 0:FH, :], sem.at[9])
    out_sem = sem.at[5]
    for n in range(NC - 1):
        for d in step_cps(n):
            d.start()
    wout_cp.start()

    def wait(i):
        for c in groups[i]:
            c.wait()

    zero_s[0] = 0
    wait(0)
    skt = skt_v[...].astype(F32)
    dv = dv_v[...].astype(F32).reshape(1, D)
    for c in range(NC):
        sk_v[c] = skt[:, c * 128:(c + 1) * 128]
        dd_v[c] = dv[:, c * 128:(c + 1) * 128]
    brow = b_v[...].astype(F32).reshape(1, S)
    bcol_v[...] = jnp.broadcast_to(brow, (128, S)).T

    def gate_x(tok):
        x_v[0, S // 2:S // 2 + 8, 0:128] = pltpu.bitcast(tok, U32)

    zt_v = (zta_v, ztb_v, ztc_v, ztd_v, zte_v, ztf_v)

    def gate_zt(t):
        def gate(tok):
            zt_v[t % 6][0, T:T + 8, 0:128] = tok
        return gate

    def gate_kv(tok):
        kv_v[0, S // 2:S // 2 + 8, :] = pltpu.bitcast(tok, U32)

    def gate_pl(tok):
        pl_v[0, TOK] = tok

    ndone = [0]

    mode = {'pairs': False}

    def done(val):
        r = (ndone[0] % 8) * 16
        ndone[0] += 1
        if mode['pairs']:
            xs_v[0, 0, 0, r:r + 16, :] = val
        else:
            xn_v[0, S + r:S + r + 16, :] = val

    def lnx_items(t, zero):
        def item(r0):
            def run():
                rs = slice(r0 // 2, r0 // 2 + 8)
                xw = jnp.concatenate([x_v[zero, rs, 0:128], x_v[0, rs, 128:D]], axis=1)
                xn = _layernorm(_up(xw).astype(F32), EPS, _A)
                for c in range(NC):
                    xb = xn[:, c * 128:(c + 1) * 128].astype(BF16)
                    xn_v[c, r0:r0 + 16, :] = xb
                if mode['pairs']:
                    done(xb)
            return (85, gate_x, run)
        return [item(t * T + g * 16) for g in range(T // 16)]

    def lnz_items(t, zero):
        def item(g):
            def run():
                rs = slice(g * 16, (g + 1) * 16)
                z = jnp.concatenate(
                    [zt_v[t % 6][zero, rs, 0:128], zt_v[t % 6][0, rs, 128:FH]], axis=1)
                z = _layernorm(z, 4.0 * _A * _A * EPS)
                r0 = t * T + g * 16
                for n in range(NF):
                    zb = z[:, n * 128:(n + 1) * 128].astype(BF16)
                    z2_v[n, r0:r0 + 16, :] = zb
                done(zb)
            return (90, gate_zt(t), run)
        return [item(g) for g in range(T // 16)]

    def kv_items(c):
        sk = sk_v[c]

        def item(r0):
            def run():
                hs = slice(r0 // 2, (r0 + KR) // 2)
                if r0 == 0:
                    kw = jnp.concatenate(
                        [jnp.zeros((8, 128), F32), _up(kv_v[2 * c, hs, :]).astype(F32)], axis=0)
                else:
                    kw = _up(kv_v[2 * c, r0 // 2 - 8:(r0 + KR) // 2, :]).astype(F32)[8:]
                ks = kw[8:] * sk[0:1, :]
                for t in range(1, KS):
                    ks = ks + pltpu.roll(kw, t, 0)[8:] * sk[t:t + 1, :]
                kvb_v[r0:r0 + KR, :] = (
                    ks * _up(kv_v[2 * c + 1, hs, :]).astype(F32)).astype(BF16)
            return (14 * KR // 8, gate_kv, run)
        return [item(r0) for r0 in range(0, S, KR)]

    def gate_w(tok):
        wsp_v[0, S // 2:S // 2 + 8, 0:128] = pltpu.bitcast(tok, U32)

    def asum_items(r_lo, r_hi):
        def item(zero, r0, c0):
            def run():
                def quad(i, j, c):
                    w = wsp_v[zero, (i * HS + r0) // 2:(i * HS + r0) // 2 + 8,
                              j * HS + c * 128:j * HS + (c + 1) * 128]
                    return _up(w).astype(F32)
                for c in range(c0, c0 + AW):
                    for i, v in enumerate(_lhs_sums_w(
                            quad(0, 0, c), quad(0, 1, c), quad(1, 0, c), quad(1, 1, c))):
                        as_v[i, c, r0:r0 + 16, :] = v.astype(BF16)
            return (20 * AW, gate_w, run)
        return lambda zero: [item(zero, r0, c0) for r0 in range(r_lo * T, r_hi * T, 16)
                             for c0 in range(0, HT, AW)]

    def asum_dyn(g, c):
        def run():
            def quad(i, j):
                r0 = pl.multiple_of(i * (HS // 2) + HS // 4 + g * 8, 8)
                w = wsp_v[0, pl.ds(r0, 8), j * HS + c * 128:j * HS + (c + 1) * 128]
                return _up(w).astype(F32)
            rs = pl.ds(pl.multiple_of(g * 16, 16), 16)
            for i, v in enumerate(_lhs_sums_w(quad(0, 0), quad(0, 1), quad(1, 0), quad(1, 1))):
                as2_v[i, c, rs, :] = v.astype(BF16)
        return (20, gate_w, run)

    def gate_z2(tok):
        z2_v[0, S:S + 8, :] = tok.astype(BF16)

    def bsum(t):
        def item(zero, r0, n):
            def run():
                def quad(i, j):
                    return z2_v[zero + n + j * HF, i * HS + r0:i * HS + r0 + 16, :].astype(F32)
                for i, v in enumerate(_rhs_sums_w(quad(0, 0), quad(0, 1), quad(1, 0), quad(1, 1))):
                    bs_v[i, n, r0:r0 + 16, :] = v.astype(BF16)
            return (21, gate_z2, run)
        return lambda zero: [item(zero, r0, n) for r0 in range((t - HT) * T, (t - HT + 1) * T, 16)
                             for n in range(HF)]

    def gate_xn(tok):
        xn_v[1, S:S + 8, :] = tok.astype(BF16)

    def xsum(u):
        def item(zero, g, c):
            def run():
                def quad(i, j):
                    r0 = (2 * u + i) * T + g * 16
                    return xn_v[zero + c + 2 * j, r0:r0 + 16, :].astype(F32)
                for i, v in enumerate(_lhs_sums(quad(0, 0), quad(0, 1), quad(1, 0), quad(1, 1))):
                    xs_v[u, i, c, g * 16:(g + 1) * 16, :] = v.astype(BF16)
            return (24, gate_xn, run)
        return lambda zero: [item(zero, g, c) for g in range(T // 16) for c in range(2)]

    def gate_wi(tok):
        win_v[0, D // 2:D // 2 + 8, 0:128] = pltpu.bitcast(tok, U32)

    def wisum(zero):
        def item(g, q):
            def run():
                def quad(i, j):
                    r0 = (i * KH + g * 16) // 2
                    c0 = ((q // HF) * NF + q % HF + j * HF) * 128
                    return _up(win_v[zero, r0:r0 + 8, c0:c0 + 128]).astype(F32)
                for i, v in enumerate(_rhs_sums(quad(0, 0), quad(0, 1), quad(1, 0), quad(1, 1))):
                    wi_v[i, q, g * 16:(g + 1) * 16, :] = v.astype(BF16)
            return (23, gate_wi, run)
        return [item(g, (q + HF) % NF) for q in range(NF) for g in range(KH // 16)]

    def taps_of(val):
        rows, cols = val.shape
        return [(lambda i=i, n=n: val[i * 8:(i + 1) * 8, n * 128:(n + 1) * 128])
                for n in range(cols // 128) for i in range(rows // 8)]

    def activate(kind, t, n, z):
        if kind == 2:
            zt_v[t % 6][0, 0:T, n * 128:(n + 1) * 128] = _gelu2(z)
        else:
            z1_v[n, t * T:(t + 1) * T, :] = z.astype(BF16)

    def piece(kind, t, n, zero, defer=False, halves=False):
        col = n * 128 + (FH if kind == 2 else 0)
        xn = jnp.concatenate(
            [_up(xn32[zero if zero is not None and c == 0 else c,
                      t * T // 2:(t + 1) * T // 2, :]) for c in range(NC)], axis=1)
        w = _up(win_v[0, 0:D // 2, col:col + 128])
        if halves:
            z = jnp.concatenate([_dot(xn[:T // 2], w), _dot(xn[T // 2:], w)], axis=0)
        else:
            z = _dot(xn, w)
        if defer:
            raw_v[...] = z
        else:
            activate(kind, t, n, z)
        return taps_of(z)

    def pair_piece(kind, u, m, gate_idx, slot_done):
        def xq(i, cs):
            rows = slice((2 * u + i) * T // 2, (2 * u + i + 1) * T // 2)
            return jnp.concatenate([_up(xn32[c, rows, :]) for c in cs], axis=1)

        def wq(lo, hi, j):
            c0 = ((kind - 1) * NF + m + j * HF) * 128
            return _up(win_v[0, lo // 2:hi // 2, c0:c0 + 128])

        def sa(i):
            return jnp.concatenate(
                [_up(xs32[u + (gate_idx() if c == 0 and i != 4 else 0), i, c])
                 for c in range(2)], axis=1)

        def fin(i, j, c):
            z = c + _dot(xq(i, [NC - 1]), wq(2 * KH, D, j))
            activate(kind, 2 * u + i, m + j * HF, z)
            slot_done(taps_of(z))

        _strassen(_dot, sa, lambda i: _up(wi32[i, (kind - 1) * HF + m]),
                  xq(0, (0, 1)), xq(1, (2, 3)), wq(0, KH, 0), wq(KH, 2 * KH, 1), fin)

    pending = []

    def plan(work, zero, n):
        work = [(mk(zero), lo, hi) for mk, lo, hi in work]
        return [a + b for a, b in zip(
            _balance([w for w in work if w[0][0][0] >= 80], n),
            _balance([w for w in work if w[0][0][0] < 80], n))]

    def pair_block(halves, work, lag):
        zero = zero_s[0]
        mode['pairs'] = True
        if pending:
            activate(*pending.pop(), raw_v[...])
        rel = plan(work, zero, 12 * len(halves))
        taps = []
        state = {'gated': False}

        def release(k):
            for i, (_, gate, run) in sorted(rel[k], key=lambda e: e[0]):
                gate(taps[k][i]())
                run()
                state['gated'] = True

        def slot_done(z):
            taps.append(z)
            if len(taps) > lag:
                release(len(taps) - 1 - lag)

        for kind, u in halves:
            for m in range(HF):
                pair_piece(kind, u, m, lambda: zero if state['gated'] else 0, slot_done)
        for k in range(len(taps) - lag, len(taps)):
            release(k)

    def block(pieces, work, defer=True, free=None):
        zero = zero_s[0]
        if pending:
            activate(*pending.pop(), raw_v[...])
        rel = plan(work, zero, len(pieces))
        taps = []
        gated = False
        for k in range(len(pieces) + LAG):
            if free is not None and k == len(pieces) - 1:
                for _, _, run in free(zero):
                    run()
                gated = True
            if k < len(pieces):
                last = defer and k == len(pieces) - 1
                halves = len(pieces) % 4 == 2 and k == len(pieces) - 1
                taps.append(piece(*pieces[k], zero if gated else None, last, halves))
                if last:
                    pending.append(pieces[k])
            if k >= LAG:
                for i, (_, gate, run) in sorted(rel[k - LAG], key=lambda e: e[0]):
                    gate(taps[k - LAG][i]())
                    run()
                    gated = True

    def cols(kind, t, lo=0, hi=NF):
        return [(kind, t, n) for n in range(lo, hi)]

    def lnx(t):
        return lambda zero: lnx_items(t, zero)

    def lnz(t):
        return lambda zero: lnz_items(t, zero)

    wait(1)
    for it in lnx_items(0, 0) + lnx_items(1, 0):
        it[2]()
    wait(2)
    block(cols(2, 0, 0, 2) + cols(2, 1, 0, 2), [])
    wait(3)
    block(cols(2, 0, 2, 4) + cols(2, 1, 2, 4), [])
    wait(4)
    block(cols(2, 0, 4) + cols(2, 1, 4) + cols(1, 0, 0, 1) + cols(1, 1, 0, 1), [])
    wait(5)
    block(cols(1, 0, 1, 4) + cols(1, 1, 1, 4), [(lnz(0), 0, 1)])
    wait(6)
    block(cols(1, 0, 4) + cols(1, 1, 4), [], free=lnx(2))

    def tiles(lo, hi):
        return [pc for t in range(lo, hi) for pc in cols(2, t) + cols(1, t)]

    wait(7)
    block(tiles(2, 4),
          [(lnx(3), 0, 7), (lnx(4), 0, 14), (lnx(5), 0, 15), (lnz(1), 0, 19),
           (wisum, 0, 24), (xsum(2), 17, 24)])
    wait(8)
    pair_block([(2, 2), (1, 2), (2, 3), (1, 3), (2, 4), (1, 4)],
               [(lnx(6), 0, 10), (lnx(7), 0, 10), (xsum(3), 13, 19),
                (lnx(8), 0, 34), (lnx(9), 0, 34), (xsum(4), 37, 43),
                (lnx(10), 0, 61), (lnx(11), 0, 61), (xsum(5), 64, 72),
                (lnz(2), 0, 43), (lnz(3), 0, 43), (lnz(4), 12, 66), (lnz(5), 12, 66),
                (lnz(6), 36, 66), (lnz(7), 36, 66), (kv_items, 0, 72)], 5)
    wait(9)
    pair_block([(2, 5), (1, 5), (2, 6), (2, 7), (1, 6), (1, 7)],
               [(lnx(12), 0, 11), (lnx(13), 0, 11), (xsum(6), 13, 20),
                (lnx(14), 0, 23), (lnx(15), 0, 23), (xsum(7), 25, 32),
                (lnz(8), 0, 32), (lnz(9), 0, 32), (lnz(10), 12, 44), (lnz(11), 12, 44),
                (lnz(12), 36, 54), (lnz(13), 36, 54), (lnz(14), 48, 63), (lnz(15), 48, 63),
                (bsum(8), 36, 72), (bsum(9), 36, 72), (bsum(10), 48, 72), (bsum(11), 48, 72),
                (bsum(12), 58, 72), (bsum(13), 58, 72), (bsum(14), 67, 72), (bsum(15), 67, 72),
                (asum_items(0, HT // 2), 0, 72)], 4)
    wait(10)

    def unit(n, half, k, tap, put_p):
        def span(start, size):
            if isinstance(start, int):
                return slice(start, start + size)
            return pl.ds(pl.multiple_of(start, size), size)

        r = half * (HT // 2) + k
        top, bot = span(r * T, T), span(HS + r * T, T)
        toph, both = span(r * (T // 2), T // 2), span(HS // 2 + r * (T // 2), T // 2)
        sums, sumh = (as32, as232)[half], span(k * (T // 2), T // 2)

        def prod(lhs, rhs):
            acc = None
            for q in range(HS // KG):
                part = _dot(lhs(q), rhs(q))
                acc = part if acc is None else acc + part
                tap(acc)
            return acc

        def sa(i):
            return lambda q: jnp.concatenate(
                [_up(sums[i, c, sumh, :]) for c in range(q * KG // 128, (q + 1) * KG // 128)],
                axis=1)

        def sb(i):
            return lambda q: _up(bs32[i, n, q * KG // 2:(q + 1) * KG // 2, :])

        def a11(q):
            return _up(wsp_v[0, toph, q * KG:(q + 1) * KG])

        def a12(q):
            return _up(wsp_v[0, toph, HS + q * KG:HS + (q + 1) * KG])

        def b21(q):
            return _up(z232[n, (HS + q * KG) // 2:(HS + (q + 1) * KG) // 2, :])

        def a22(q):
            return _up(wsp_v[0, both, HS + q * KG:HS + (q + 1) * KG])

        def b11(q):
            return _up(z232[n, q * KG // 2:(q + 1) * KG // 2, :])

        def b22(q):
            return _up(z232[n + HF, (HS + q * KG) // 2:(HS + (q + 1) * KG) // 2, :])

        def fin(i, j, c):
            col, rows = n + j * HF, (top, bot)[i]
            put_p(i, j, col, rows, (c + bcol_v[rows, :]).astype(BF16))

        _winograd(prod, sa, sb, a11, a12, a22, b11, b21, b22, fin)

    def p2(n, half):
        nn = jnp.minimum(n + 1, NC - 1)

        for q in range(half * HF, min((half + 1) * HF, NC - 1)):
            @pl.when(n == q)
            def _():
                for d in step_cps(q):
                    d.wait()

        zero = zero_s[0]
        fwd_u = _up(tab_v[0:128, :])
        fwd_h = _up(tab_v[128:256, :])
        dd = dd_v[n]

        def put(slot, val):
            pl_v[:, slot] = val

        def re_im(val):
            val = val.reshape(BLK // 8, 2, 8, 128)
            return val[:, 0], val[:, 1]

        kvi = kv_items(nn)

        def pace_kv(d, val):
            if d % 4 == 3:
                for j in range(8):
                    _, gate, run = kvi[(d // 4) * 8 + j]
                    gate(val[j * 32:j * 32 + 8, :])
                    run()

        for i in range(NB):
            u = _dot(fwd_u, _up(kvb32[i * BLK // 2:(i + 1) * BLK // 2, :]))
            a, b = re_im(u)
            put(UA + i, a)
            put(UB + i, b)
            put(US + i, a + b)
            pace_kv(i, u)
        for i in range(NB):
            hb = _up(h_v[n, :, i * BLK:(i + 1) * BLK])
            hf = jax.lax.dot_general(fwd_h, hb, (((1,), (1,)), ((), ())),
                                     preferred_element_type=F32)
            c, d = re_im(hf)
            if i == 0:
                c, d = c + dd, d + dd
            put(HR + i, c)
            put(HP + i, d - c)
            put(HQ + i, c + d)
            pace_kv(NB + i, hf)

        state = {}

        def mac_item(pos, g0, pi, j0, j1):
            xv, hv = ((US, HR), (UA, HP), (UB, HQ))[pi]
            outs = range(g0, g0 + GRP)
            top = g0 + GRP

            def run():
                pz = zero + pos
                hs = {t: pl_v[pz, hv + t]
                      for t in range(max(g0 - j1 + 1, 0), top - j0)}
                acc = state['acc'] if j0 else {o: None for o in outs}
                for jj in range(j0, j1):
                    xj = pl_v[pz, xv + jj]
                    for o in outs:
                        if o - jj >= 0:
                            t = xj * hs[o - jj]
                            acc[o] = t if acc[o] is None else acc[o] + t
                if j1 < top:
                    state['acc'] = acc
                    return
                r0 = pos * 8
                if pi == 0:
                    state['k1'] = acc
                elif pi == 1:
                    state['im'] = {o: state['k1'][o] + acc[o] for o in outs}
                else:
                    for o in outs:
                        re, im = state['k1'][o] - acc[o], state['im'][o]
                        zr, zi = re, im
                        if o > 0:
                            zr, zi = re - state['prev'][1], im + state['prev'][0]
                        state['prev'] = (re, im)
                        zz_v[n, o, r0:r0 + 8, :] = zr.astype(BF16)
                        zz_v[n, o, BLK + r0:BLK + r0 + 8, :] = zi.astype(BF16)

            nmac = sum(1 for o in outs for jj in range(j0, j1) if o >= jj)
            return (2 * nmac + ((0, GRP, 5 * GRP)[pi] if j1 == top else 0), gate_pl, run)

        items = []
        for pos in range(BLK // 8):
            for g0 in range(0, NB, GRP):
                top = g0 + GRP
                cuts = [0, top] if top <= SPLIT else [0, (top - 1) // 2, top]
                for pi in range(3):
                    for j0, j1 in zip(cuts[:-1], cuts[1:]):
                        items.append(mac_item(pos, g0, pi, j0, j1))

        if half == 0:
            extra = [asum_dyn(jnp.minimum(n * NG + g, HS // 32 - 1), c)
                     for g in range(NG) for c in range(HT)]
            every = len(items) // len(extra)
            items = [it for i, e in enumerate(extra)
                     for it in items[i * every:(i + 1) * every] + [e]
                     ] + items[len(extra) * every:]

        total = sum(c for c, _, _ in items)
        tap_of = []
        cum = 0
        for c, _, _ in items:
            tap_of.append(int(cum * NTAP / total))
            cum += c
        pos = {'tap': 0, 'item': 0}

        def tap(acc):
            t0 = pos['tap']
            pos['tap'] += T // 8
            while pos['item'] < len(items) and tap_of[pos['item']] < pos['tap']:
                i = tap_of[pos['item']] - t0
                _, gate, run = items[pos['item']]
                gate(acc[i * 8:(i + 1) * 8, :])
                run()
                pos['item'] += 1

        def put_p(i, j, col, rows, val):
            p_v[col, rows, :] = val

        for k in range(HT // 2):
            unit(n - half * HF, half, k, tap, put_p)
        assert pos['item'] == len(items)
        return 0

    jax.lax.fori_loop(0, HF, lambda n, c: p2(n, 0), 0)
    jax.lax.fori_loop(HF, NC, lambda n, c: p2(n, 1), 0)

    wout_cp.wait()

    def p3(j, carry):
        inv_p = _up(tab_v[256:288, :])
        inv_m = _up(tab_v[288:320, :])
        rev = 7 - jax.lax.broadcasted_iota(jnp.int32, (8, 128), 0)

        zero = zero_s[0]
        HK = FH // 2

        def rows(k, i):
            tile = i * HT + (k // 2) * (HT // 2) + 2 * j + k % 2
            return (tile, pl.ds(pl.multiple_of(tile * T, T), T),
                    pl.ds(pl.multiple_of(tile * (T // 2), T // 2), T // 2))

        def fresh(k, n):
            return k >= 2 and n % HF == HF - 1

        def p_tile(k, i, n):
            return _up(pp32[k, i, n])

        def gate_p(tok):
            p_v[0, S:S + 8, :] = tok.astype(BF16)

        def gate_wo(tok):
            wout_v[0, HK:HK + 8, 0:128] = pltpu.bitcast(tok, U32)

        def psum_item(k, n, g):
            def run():
                def quad(i, jj):
                    rs = pl.ds(pl.multiple_of(rows(k, i)[0] * T + g * 16, 16), 16)
                    if fresh(k, n):
                        gv = pq_v[k - 2, i, jj, g * 16:(g + 1) * 16, :]
                    else:
                        gv = p_v[n + jj * HF, rs, :]
                    pv = _gelu2(z1_v[n + jj * HF, rs, :].astype(F32)) * gv.astype(F32)
                    pp_v[k, i, n + jj * HF, g * 16:(g + 1) * 16, :] = pv.astype(BF16)
                    return pv
                for i, v in enumerate(_lhs_sums(quad(0, 0), quad(0, 1), quad(1, 0), quad(1, 1))):
                    ps_v[k, i, n, g * 16:(g + 1) * 16, :] = v.astype(BF16)
            return (gate_p, run)

        def wsum_item(m, g):
            def run():
                def quad(i, jj):
                    r0 = (i * HK + g * 16) // 2
                    c0 = (m + 2 * jj) * 128
                    return _up(wout_v[zero, r0:r0 + 8, c0:c0 + 128]).astype(F32)
                for i, v in enumerate(_rhs_sums(quad(0, 0), quad(0, 1), quad(1, 0), quad(1, 1))):
                    ws_v[i, m, g * 16:(g + 1) * 16, :] = v.astype(BF16)
            return (gate_wo, run)

        def psum(k):
            return [psum_item(k, n, g) for n in range(HF) if not fresh(k, n)
                    for g in range(T // 16)]

        queue = []

        def tap(val):
            for i in range(min(len(queue), queue_step[0])):
                gate, run = queue.pop(0)
                r = (i * (T // 8)) // queue_step[0] * 8
                gate(val[r:r + 8, :])
                run()

        queue_step = [0]

        def paced(items, ntaps):
            assert not queue
            queue.extend(items)
            queue_step[0] = -(-len(items) // ntaps)

        def do_unit(u):
            def put_q(i, jj, col, rws, val):
                pq_v[u, i, jj] = val
            unit(HF - 1, 1, 2 * j + u, tap, put_q)
            for g in range(T // 16):
                psum_item(2 + u, HF - 1, g)[1]()

        def finish(k, i, c, o):
            tile, rs, hs = rows(k, i)
            cs = slice(c * 128, (c + 1) * 128)
            ye = _dot(inv_p, _up(zz32[c, tile, 0:64, :]))
            yo = _dot(inv_m, _up(zz32[c, tile, 64:128, :]))
            yd = ye - yo
            y = jnp.concatenate(
                [ye + yo] + [
                    jnp.take_along_axis(yd[q * 8:(q + 1) * 8], rev, axis=0,
                                        mode="promise_in_bounds")
                    for q in reversed(range(BLK // 16))], axis=0)
            gate = o * (1.0 + jnp.tanh((0.25 / _A) * o))
            x = _up(x_v[0, hs, cs]).astype(F32)
            xn = xn_v[c, rs, :].astype(F32)
            o_v[rs, cs] = (x + (xn * y) * gate).astype(BF16)

        def do_pair(k, last=False):
            def prod(lhs, rhs):
                res = _dot(lhs, rhs)
                tap(res)
                return res

            def sa(i):
                return jnp.concatenate([_up(ps32[k, i, n]) for n in range(HF)], axis=1)

            a11 = jnp.concatenate([p_tile(k, 0, n) for n in range(HF)], axis=1)
            a22 = jnp.concatenate([p_tile(k, 1, n) for n in range(HF, NF)], axis=1)
            for m in range(2):
                _strassen(
                    prod, sa, lambda i: _up(ws32[i, m]), a11, a22,
                    _up(wout_v[0, 0:HK // 2, m * 128:(m + 1) * 128]),
                    _up(wout_v[0, HK // 2:HK, (m + 2) * 128:(m + 3) * 128]),
                    lambda i, jj, o: finish(k, i, m + 2 * jj, o))
            for i in range(2):
                rs = rows(k, i)[1]
                if last:
                    cp(o_v.at[rs, 0:512], out_hbm.at[0, rs, 0:512], out_sem).start()
            for i in range(2):
                rs = rows(k, i)[1]
                p = jnp.concatenate([p_tile(k, i, n) for n in range(NF)], axis=1)
                finish(k, i, NC - 1, _dot(p, _up(wout_v[0, 0:HK, 512:D])))
                if last:
                    cp(o_v.at[rs, 512:D], out_hbm.at[0, rs, 512:D], out_sem).start()
                else:
                    cp(o_v.at[rs, :], out_hbm.at[0, rs, :], out_sem).start()

        paced(psum(0) + [wsum_item(m, g) for m in range(2) for g in range(HK // 16)], 12)
        do_unit(0)
        paced(psum(1), 12)
        do_pair(0)
        paced(psum(2), 12)
        do_unit(1)
        paced(psum(3), 12)
        do_pair(1)
        do_pair(2)
        do_pair(3, last=True)
        return carry

    jax.lax.fori_loop(0, P3I, p3, 0)
    cp(o_v, out_hbm.at[0], out_sem).wait()


@jax.jit
def pallas_recurrent_scan__ssm_conv_h3__mixer_gmlp__prompt_kernel(
    A_q: jax.Array,
    A_k: jax.Array,
    A_v: jax.Array,
    A_shift_k: jax.Array,
    A_ssm_k: jax.Array,
    A_ssm_D: jax.Array,
    B_x: jax.Array,
    B_w_in: jax.Array,
    B_w_sp: jax.Array,
    B_b_sp: jax.Array,
    B_w_out: jax.Array,
):
    del B_x
    tab = jnp.asarray(_dft_tables(), dtype=BF16)

    any_spec = pl.BlockSpec(memory_space=pl.ANY)
    return pl.pallas_call(
        _kernel,
        out_shape=jax.ShapeDtypeStruct((1, S, D), BF16),
        in_specs=[any_spec] * 11,
        out_specs=any_spec,
        scratch_shapes=[
            pltpu.VMEM((1, S // 2 + 32, D), U32),
            pltpu.VMEM((1, D // 2 + 8, 2 * FH), U32),
            pltpu.VMEM((1, S // 2 + 8, S), U32),
            pltpu.VMEM((1, FH // 2 + 32, D), U32),
            pltpu.VMEM((2 * NC, S // 2 + 32, 128), U32),
            pltpu.VMEM((NC, 64, S), U32),
            pltpu.VMEM((NC, S + 256, 128), BF16),
            pltpu.VMEM((NF, S, 128), BF16),
            pltpu.VMEM((NF, S + 64, 128), BF16),
            pltpu.VMEM((NF, S + 64, 128), BF16),
            pltpu.VMEM((4, HT, HS // 2, 128), BF16),
            pltpu.VMEM((4, HT, HS // 2, 128), BF16),
            pltpu.VMEM((4, HF, HS, 128), BF16),
            pltpu.VMEM((2, 2, 2, T, 128), BF16),
            pltpu.VMEM((4, 2, NF, T, 128), BF16),
            pltpu.VMEM((4, 5, HF, T, 128), BF16),
            pltpu.VMEM((5, 2, FH // 2, 128), BF16),
            pltpu.VMEM((S, 128), BF16),
            pltpu.VMEM((BLK // 8, 6 * NB + 1, 8, 128), F32),
            pltpu.VMEM((NC, NB, 2 * BLK, 128), BF16),
            pltpu.VMEM((S, 128), F32),
            pltpu.VMEM((S, D), BF16),
            pltpu.VMEM((1, T + 16, FH), F32),
            pltpu.VMEM((1, T + 16, FH), F32),
            pltpu.VMEM((1, T + 16, FH), F32),
            pltpu.VMEM((1, T + 16, FH), F32),
            pltpu.VMEM((1, T + 16, FH), F32),
            pltpu.VMEM((1, T + 16, FH), F32),
            pltpu.VMEM((NT // 2, 5, 2, T, 128), BF16),
            pltpu.VMEM((5, NF, KH, 128), BF16),
            pltpu.VMEM((T, 128), F32),
            pltpu.VMEM((320, 128), U32),
            pltpu.VMEM((NC, KS, 128), F32),
            pltpu.VMEM((NC + 2, 1, 128), F32),
            pltpu.VMEM((KS, D), BF16),
            pltpu.VMEM((D,), BF16),
            pltpu.VMEM((S,), BF16),
            pltpu.SMEM((1,), jnp.int32),
            pltpu.SemaphoreType.DMA((16,)),
        ],
        compiler_params=pltpu.CompilerParams(
            vmem_limit_bytes=100 * 1024 * 1024, disable_bounds_checks=True),
    )(A_q, A_k, A_v, A_shift_k.T, A_ssm_k, A_ssm_D, B_w_in, B_w_sp, B_b_sp, B_w_out, tab)
```

```python
import jax
import jax.numpy as jnp
import numpy as np
import jax.experimental.pallas as pl
import jax.experimental.pallas.tpu as pltpu

F32 = jnp.float32
BF16 = jnp.bfloat16
U32 = jnp.uint32

S = 2048
D = 640
FH = 768
KS = 4
BLK = 128
NB = S // BLK
NC = D // 128
NF = FH // 128
T = 128
NT = S // T
EPS = 1e-5
GRP = 4
SPLIT = 8
AW = 2
KG = 512
KR = 32
UA, UB, US, HP, HQ, HR, TOK = (i * NB for i in range(7))
LAG = 4
NTAP = 888
HS = S // 2
HT = HS // T
HF = NF // 2
KH = 256
P3I = 2

_GELU_C0 = float(np.sqrt(2.0 / np.pi))
_GELU_C1 = _GELU_C0 * 0.044715
_A = _GELU_C1 ** (1.0 / 3.0)
_K = _GELU_C0 / _A


def _dft_tables():
    m = np.arange(BLK)[:, None]
    n = np.arange(BLK)[None, :]
    th = 2.0 * np.pi * (((4 * m + 1) * n) % (4 * BLK)) / (4 * BLK)
    ph = 2.0 * np.pi * (((4 * m + 1) * (2 * n + 1)) % (8 * BLK)) / (8 * BLK)
    fu = np.concatenate([np.cos(ph), -np.sin(ph)], axis=0)
    fh = np.concatenate([np.cos(th) + np.sin(th), np.cos(th) - np.sin(th)], axis=0)
    fu, fh = (f.reshape(2, BLK // 8, 8, BLK).transpose(1, 0, 2, 3).reshape(2 * BLK, BLK)
              for f in (fu, fh))
    cp = (np.cos(ph) + np.sin(ph)).T[:BLK // 2] / (8.0 * BLK * _A * _A)
    cm = (np.cos(ph) - np.sin(ph)).T[:BLK // 2] / (8.0 * BLK * _A * _A)
    return np.concatenate([fu, fh, cp, cm], axis=0).astype(np.float32)


def _layernorm(x, eps, scale=1.0):
    m = jnp.mean(x, axis=-1, keepdims=True)
    d = x - m
    v = jnp.sum(d * d, axis=-1, keepdims=True) * (1.0 / (x.shape[-1] * scale * scale))
    return d * jax.lax.rsqrt(v + eps / (scale * scale))


def _gelu2(y):
    return y * (1.0 + jnp.tanh(y * (y * y + _K)))


def _up(x):
    return pltpu.bitcast(x, BF16)


def _dot(a, b):
    return jnp.dot(a, b, preferred_element_type=F32)


def _lhs_sums(a11, a12, a21, a22):
    return a11 + a22, a21 + a22, a11 + a12, a21 - a11, a12 - a22


def _rhs_sums(b11, b12, b21, b22):
    return b11 + b22, b12 - b22, b21 - b11, b11 + b12, b21 + b22


def _strassen(prod, sa, sb, a11, a22, b11, b22, fin):
    m2 = prod(sa(1), b11)
    m4 = prod(a22, sb(2))
    fin(1, 0, m2 + m4)
    m5 = prod(sa(2), b22)
    c11 = m4 - m5
    m3 = prod(a11, sb(1))
    fin(0, 1, m3 + m5)
    c22 = m3 - m2
    m1 = prod(sa(0), sb(0))
    c11, c22 = c11 + m1, c22 + m1
    fin(0, 0, c11 + prod(sa(4), sb(4)))
    fin(1, 1, c22 + prod(sa(3), sb(3)))


def _lhs_sums_w(a11, a12, a21, a22):
    s1 = a21 + a22
    s2 = s1 - a11
    return s1, s2, a11 - a21, a12 - s2


def _rhs_sums_w(b11, b12, b21, b22):
    t1 = b12 - b11
    t2 = b22 - t1
    return t1, t2, b22 - b12, t2 - b21


def _winograd(prod, sa, sb, a11, a12, a22, b11, b21, b22, fin):
    p1 = prod(a11, b11)
    fin(0, 0, p1 + prod(a12, b21))
    u2 = p1 + prod(sa(1), sb(1))
    p5 = prod(sa(0), sb(0))
    fin(0, 1, (u2 + p5) + prod(sa(3), b22))
    u3 = u2 + prod(sa(2), sb(2))
    fin(1, 1, u3 + p5)
    fin(1, 0, u3 - prod(a22, sb(3)))


def _balance(work, n):
    jobs = [(lo, hi, sum(it[0] for it in items)) for items, lo, hi in work]
    rate = [None] * n
    while jobs:
        def free(a, b):
            return [p for p in range(a, b) if rate[p] is None]
        dens, a, b = max(
            (sum(w for lo, hi, w in jobs if a <= lo and hi <= b) / max(len(free(a, b)), 1e-9), a, b)
            for a in {j[0] for j in jobs} for b in {j[1] for j in jobs} if a < b)
        while a > 0 and rate[a - 1] is not None:
            a -= 1
        while b < n and rate[b] is not None:
            b += 1
        for p in free(a, b):
            rate[p] = dens
        jobs = [(lo, hi, w) for lo, hi, w in jobs if not (a <= lo and hi <= b)]
        jobs = [(b if a <= lo < b else lo, a if a < hi <= b else hi, w) for lo, hi, w in jobs]
    queues = [[lo * 16, hi * 16, list(items)] for items, lo, hi in work]
    rel = [[] for _ in range(n)]
    budget = 0.0
    for tau in range(n * 16):
        budget += (rate[tau // 16] or 0.0) / 16
        while True:
            ready = [q for q in queues if q[2] and q[0] <= tau]
            if not ready:
                budget = min(budget, 0.0)
                break
            q = min(ready, key=lambda q: q[1])
            if budget < 0 and q[1] - tau > len(q[2]):
                break
            it = q[2].pop(0)
            rel[tau // 16].append((tau % 16, it))
            budget -= it[0]
    assert not any(q[2] for q in queues)
    return rel


def _kernel(x_hbm, k_hbm, v_hbm, skt_hbm, h_hbm, dv_hbm, win_hbm, wsp_hbm, b_hbm,
            wout_hbm, tab_hbm, out_hbm,
            x_v, win_v, wsp_v, wout_v, kv_v, h_v, xn_v, z1_v, z2_v, p_v, as_v, as2_v, bs_v, pq_v, pp_v, ps_v, ws_v,
            kvb_v, pl_v, zz_v, bcol_v, o_v, zta_v, ztb_v, ztc_v, ztd_v, zte_v, ztf_v, xs_v, wi_v, raw_v, tab_v,
            sk_v, dd_v, skt_v, dv_v, b_v, zero_s, sem):
    cp = pltpu.make_async_copy
    x16 = x_v.bitcast(BF16)
    win16 = win_v.bitcast(BF16)
    kv16 = kv_v.bitcast(BF16)
    h16 = h_v.bitcast(BF16)

    xn32, z232, kvb32, zz32, as32, as232, bs32, ws32, xs32, wi32 = (
        r.bitcast(U32)
        for r in (xn_v, z2_v, kvb_v, zz_v, as_v, as2_v, bs_v, ws_v, xs_v, wi_v))
    pp32 = [r.bitcast(U32) for r in pp_v]
    ps32 = [r.bitcast(U32) for r in ps_v]
    wsp16 = wsp_v.bitcast(BF16)

    def wsp_cp(lo, hi, s):
        return cp(wsp_hbm.at[lo:hi, :], wsp16.at[0, lo:hi, :], sem.at[s])

    def x_cp(lo, hi, s):
        return cp(x_hbm.at[0, lo:hi, :], x16.at[0, lo:hi, :], sem.at[s])

    def win_cp(lo, hi, s):
        return cp(win_hbm.at[:, lo:hi], win16.at[0, 0:D, lo:hi], sem.at[s])

    def k_cp(c, s):
        return cp(k_hbm.at[0, :, pl.ds(c * 128, 128)], kv16.at[2 * c, 0:S, :], sem.at[s])

    def v_cp(c, s):
        return cp(v_hbm.at[0, :, pl.ds(c * 128, 128)], kv16.at[2 * c + 1, 0:S, :], sem.at[s])

    def h_cp(c, s):
        return cp(h_hbm.at[pl.ds(c * 128, 128), :], h16.at[c], sem.at[s])

    groups = [
        [cp(b_hbm, b_v, sem.at[0]), cp(skt_hbm, skt_v, sem.at[0]), cp(dv_hbm, dv_v, sem.at[0])],
        [x_cp(0, 256, 1)],
        [win_cp(FH, FH + 256, 2)],
        [win_cp(FH + 256, FH + 512, 3)],
        [win_cp(FH + 512, 2 * FH, 4), win_cp(0, 128, 4)],
        [win_cp(128, 512, 10)],
        [win_cp(512, FH, 5), x_cp(256, 384, 5)],
        [x_cp(384, 6 * T, 6)],
        [x_cp(6 * T, 12 * T, 7), k_cp(0, 7), v_cp(0, 7)],
        [x_cp(12 * T, S, 11), wsp_cp(0, HS // 2, 11), wsp_cp(HS, HS + HS // 2, 11)],
        [cp(tab_hbm, tab_v.bitcast(BF16), sem.at[8]), h_cp(0, 8)],
    ]
    for g in groups:
        for c in g:
            c.start()

    NG = -(-HS // 32 // HF)

    def step_cps(n):
        s = 12 + n
        cps = [k_cp(n + 1, s), v_cp(n + 1, s), h_cp(n + 1, s)]
        if n < HF:
            lo, hi = HS // 2 + n * NG * 16, min(HS // 2 + (n + 1) * NG * 16, HS)
            cps += [wsp_cp(lo, hi, s), wsp_cp(HS + lo, HS + hi, s)]
        return cps

    wout_cp = cp(wout_hbm, wout_v.bitcast(BF16).at[0, 0:FH, :], sem.at[9])
    out_sem = sem.at[5]
    for n in range(NC - 1):
        for d in step_cps(n):
            d.start()
    wout_cp.start()

    def wait(i):
        for c in groups[i]:
            c.wait()

    zero_s[0] = 0
    wait(0)
    skt = skt_v[...].astype(F32)
    dv = dv_v[...].astype(F32).reshape(1, D)
    for c in range(NC):
        sk_v[c] = skt[:, c * 128:(c + 1) * 128]
        dd_v[c] = dv[:, c * 128:(c + 1) * 128]
    brow = b_v[...].astype(F32).reshape(1, S)
    bcol_v[...] = jnp.broadcast_to(brow, (128, S)).T

    def gate_x(tok):
        x_v[0, S // 2:S // 2 + 8, 0:128] = pltpu.bitcast(tok, U32)

    zt_v = (zta_v, ztb_v, ztc_v, ztd_v, zte_v, ztf_v)

    def gate_zt(t):
        def gate(tok):
            zt_v[t % 6][0, T:T + 8, 0:128] = tok
        return gate

    def gate_kv(tok):
        kv_v[0, S // 2:S // 2 + 8, :] = pltpu.bitcast(tok, U32)

    def gate_pl(tok):
        pl_v[0, TOK] = tok

    ndone = [0]

    mode = {'pairs': False}

    def done(val):
        r = (ndone[0] % 8) * 16
        ndone[0] += 1
        if mode['pairs']:
            xs_v[0, 0, 0, r:r + 16, :] = val
        else:
            xn_v[0, S + r:S + r + 16, :] = val

    def lnx_items(t, zero):
        def item(r0):
            def run():
                rs = slice(r0 // 2, r0 // 2 + 8)
                xw = jnp.concatenate([x_v[zero, rs, 0:128], x_v[0, rs, 128:D]], axis=1)
                xn = _layernorm(_up(xw).astype(F32), EPS, _A)
                for c in range(NC):
                    xb = xn[:, c * 128:(c + 1) * 128].astype(BF16)
                    xn_v[c, r0:r0 + 16, :] = xb
                if mode['pairs']:
                    done(xb)
            return (85, gate_x, run)
        return [item(t * T + g * 16) for g in range(T // 16)]

    def lnz_items(t, zero):
        def item(g):
            def run():
                rs = slice(g * 16, (g + 1) * 16)
                z = jnp.concatenate(
                    [zt_v[t % 6][zero, rs, 0:128], zt_v[t % 6][0, rs, 128:FH]], axis=1)
                z = _layernorm(z, 4.0 * _A * _A * EPS)
                r0 = t * T + g * 16
                for n in range(NF):
                    zb = z[:, n * 128:(n + 1) * 128].astype(BF16)
                    z2_v[n, r0:r0 + 16, :] = zb
                done(zb)
            return (90, gate_zt(t), run)
        return [item(g) for g in range(T // 16)]

    def kv_items(c):
        sk = sk_v[c]

        def item(r0):
            def run():
                hs = slice(r0 // 2, (r0 + KR) // 2)
                if r0 == 0:
                    kw = jnp.concatenate(
                        [jnp.zeros((8, 128), F32), _up(kv_v[2 * c, hs, :]).astype(F32)], axis=0)
                else:
                    kw = _up(kv_v[2 * c, r0 // 2 - 8:(r0 + KR) // 2, :]).astype(F32)[8:]
                ks = kw[8:] * sk[0:1, :]
                for t in range(1, KS):
                    ks = ks + pltpu.roll(kw, t, 0)[8:] * sk[t:t + 1, :]
                kvb_v[r0:r0 + KR, :] = (
                    ks * _up(kv_v[2 * c + 1, hs, :]).astype(F32)).astype(BF16)
            return (14 * KR // 8, gate_kv, run)
        return [item(r0) for r0 in range(0, S, KR)]

    def gate_w(tok):
        wsp_v[0, S // 2:S // 2 + 8, 0:128] = pltpu.bitcast(tok, U32)

    def asum_items(r_lo, r_hi):
        def item(zero, r0, c0):
            def run():
                def quad(i, j, c):
                    w = wsp_v[zero, (i * HS + r0) // 2:(i * HS + r0) // 2 + 8,
                              j * HS + c * 128:j * HS + (c + 1) * 128]
                    return _up(w).astype(F32)
                for c in range(c0, c0 + AW):
                    for i, v in enumerate(_lhs_sums_w(
                            quad(0, 0, c), quad(0, 1, c), quad(1, 0, c), quad(1, 1, c))):
                        as_v[i, c, r0:r0 + 16, :] = v.astype(BF16)
            return (20 * AW, gate_w, run)
        return lambda zero: [item(zero, r0, c0) for r0 in range(r_lo * T, r_hi * T, 16)
                             for c0 in range(0, HT, AW)]

    def asum_dyn(g, c):
        def run():
            def quad(i, j):
                r0 = pl.multiple_of(i * (HS // 2) + HS // 4 + g * 8, 8)
                w = wsp_v[0, pl.ds(r0, 8), j * HS + c * 128:j * HS + (c + 1) * 128]
                return _up(w).astype(F32)
            rs = pl.ds(pl.multiple_of(g * 16, 16), 16)
            for i, v in enumerate(_lhs_sums_w(quad(0, 0), quad(0, 1), quad(1, 0), quad(1, 1))):
                as2_v[i, c, rs, :] = v.astype(BF16)
        return (20, gate_w, run)

    def gate_z2(tok):
        z2_v[0, S:S + 8, :] = tok.astype(BF16)

    def bsum(t):
        def item(zero, r0, n):
            def run():
                def quad(i, j):
                    return z2_v[zero + n + j * HF, i * HS + r0:i * HS + r0 + 16, :].astype(F32)
                for i, v in enumerate(_rhs_sums_w(quad(0, 0), quad(0, 1), quad(1, 0), quad(1, 1))):
                    bs_v[i, n, r0:r0 + 16, :] = v.astype(BF16)
            return (21, gate_z2, run)
        return lambda zero: [item(zero, r0, n) for r0 in range((t - HT) * T, (t - HT + 1) * T, 16)
                             for n in range(HF)]

    def gate_xn(tok):
        xn_v[1, S:S + 8, :] = tok.astype(BF16)

    def xsum(u):
        def item(zero, g, c):
            def run():
                def quad(i, j):
                    r0 = (2 * u + i) * T + g * 16
                    return xn_v[zero + c + 2 * j, r0:r0 + 16, :].astype(F32)
                for i, v in enumerate(_lhs_sums(quad(0, 0), quad(0, 1), quad(1, 0), quad(1, 1))):
                    xs_v[u, i, c, g * 16:(g + 1) * 16, :] = v.astype(BF16)
            return (24, gate_xn, run)
        return lambda zero: [item(zero, g, c) for g in range(T // 16) for c in range(2)]

    def gate_wi(tok):
        win_v[0, D // 2:D // 2 + 8, 0:128] = pltpu.bitcast(tok, U32)

    def wisum(zero):
        def item(g, q):
            def run():
                def quad(i, j):
                    r0 = (i * KH + g * 16) // 2
                    c0 = ((q // HF) * NF + q % HF + j * HF) * 128
                    return _up(win_v[zero, r0:r0 + 8, c0:c0 + 128]).astype(F32)
                for i, v in enumerate(_rhs_sums(quad(0, 0), quad(0, 1), quad(1, 0), quad(1, 1))):
                    wi_v[i, q, g * 16:(g + 1) * 16, :] = v.astype(BF16)
            return (23, gate_wi, run)
        return [item(g, (q + HF) % NF) for q in range(NF) for g in range(KH // 16)]

    def taps_of(val):
        rows, cols = val.shape
        return [(lambda i=i, n=n: val[i * 8:(i + 1) * 8, n * 128:(n + 1) * 128])
                for n in range(cols // 128) for i in range(rows // 8)]

    def activate(kind, t, n, z):
        if kind == 2:
            zt_v[t % 6][0, 0:T, n * 128:(n + 1) * 128] = _gelu2(z)
        else:
            z1_v[n, t * T:(t + 1) * T, :] = z.astype(BF16)

    def piece(kind, t, n, zero, defer=False, halves=False):
        col = n * 128 + (FH if kind == 2 else 0)
        xn = jnp.concatenate(
            [_up(xn32[zero if zero is not None and c == 0 else c,
                      t * T // 2:(t + 1) * T // 2, :]) for c in range(NC)], axis=1)
        w = _up(win_v[0, 0:D // 2, col:col + 128])
        if halves:
            z = jnp.concatenate([_dot(xn[:T // 2], w), _dot(xn[T // 2:], w)], axis=0)
        else:
            z = _dot(xn, w)
        if defer:
            raw_v[...] = z
        else:
            activate(kind, t, n, z)
        return taps_of(z)

    def pair_piece(kind, u, m, gate_idx, slot_done):
        def xq(i, cs):
            rows = slice((2 * u + i) * T // 2, (2 * u + i + 1) * T // 2)
            return jnp.concatenate([_up(xn32[c, rows, :]) for c in cs], axis=1)

        def wq(lo, hi, j):
            c0 = ((kind - 1) * NF + m + j * HF) * 128
            return _up(win_v[0, lo // 2:hi // 2, c0:c0 + 128])

        def sa(i):
            return jnp.concatenate(
                [_up(xs32[u + (gate_idx() if c == 0 and i != 4 else 0), i, c])
                 for c in range(2)], axis=1)

        def fin(i, j, c):
            z = c + _dot(xq(i, [NC - 1]), wq(2 * KH, D, j))
            activate(kind, 2 * u + i, m + j * HF, z)
            slot_done(taps_of(z))

        _strassen(_dot, sa, lambda i: _up(wi32[i, (kind - 1) * HF + m]),
                  xq(0, (0, 1)), xq(1, (2, 3)), wq(0, KH, 0), wq(KH, 2 * KH, 1), fin)

    pending = []

    def plan(work, zero, n):
        work = [(mk(zero), lo, hi) for mk, lo, hi in work]
        return [a + b for a, b in zip(
            _balance([w for w in work if w[0][0][0] >= 80], n),
            _balance([w for w in work if w[0][0][0] < 80], n))]

    def pair_block(halves, work, lag):
        zero = zero_s[0]
        mode['pairs'] = True
        if pending:
            activate(*pending.pop(), raw_v[...])
        rel = plan(work, zero, 12 * len(halves))
        taps = []
        state = {'gated': False}

        def release(k):
            for i, (_, gate, run) in sorted(rel[k], key=lambda e: e[0]):
                gate(taps[k][i]())
                run()
                state['gated'] = True

        def slot_done(z):
            taps.append(z)
            if len(taps) > lag:
                release(len(taps) - 1 - lag)

        for kind, u in halves:
            for m in range(HF):
                pair_piece(kind, u, m, lambda: zero if state['gated'] else 0, slot_done)
        for k in range(len(taps) - lag, len(taps)):
            release(k)

    def block(pieces, work, defer=True, free=None):
        zero = zero_s[0]
        if pending:
            activate(*pending.pop(), raw_v[...])
        rel = plan(work, zero, len(pieces))
        taps = []
        gated = False
        for k in range(len(pieces) + LAG):
            if free is not None and k == len(pieces) - 1:
                for _, _, run in free(zero):
                    run()
                gated = True
            if k < len(pieces):
                last = defer and k == len(pieces) - 1
                halves = len(pieces) % 4 == 2 and k == len(pieces) - 1
                taps.append(piece(*pieces[k], zero if gated else None, last, halves))
                if last:
                    pending.append(pieces[k])
            if k >= LAG:
                for i, (_, gate, run) in sorted(rel[k - LAG], key=lambda e: e[0]):
                    gate(taps[k - LAG][i]())
                    run()
                    gated = True

    def cols(kind, t, lo=0, hi=NF):
        return [(kind, t, n) for n in range(lo, hi)]

    def lnx(t):
        return lambda zero: lnx_items(t, zero)

    def lnz(t):
        return lambda zero: lnz_items(t, zero)

    wait(1)
    for it in lnx_items(0, 0) + lnx_items(1, 0):
        it[2]()
    wait(2)
    block(cols(2, 0, 0, 2) + cols(2, 1, 0, 2), [])
    wait(3)
    block(cols(2, 0, 2, 4) + cols(2, 1, 2, 4), [])
    wait(4)
    block(cols(2, 0, 4) + cols(2, 1, 4) + cols(1, 0, 0, 1) + cols(1, 1, 0, 1), [])
    wait(5)
    block(cols(1, 0, 1, 4) + cols(1, 1, 1, 4), [(lnz(0), 0, 1)])
    wait(6)
    block(cols(1, 0, 4) + cols(1, 1, 4), [], free=lnx(2))

    def tiles(lo, hi):
        return [pc for t in range(lo, hi) for pc in cols(2, t) + cols(1, t)]

    wait(7)
    block(tiles(2, 4),
          [(lnx(3), 0, 7), (lnx(4), 0, 14), (lnx(5), 0, 15), (lnz(1), 0, 19),
           (wisum, 0, 24), (xsum(2), 17, 24)])
    wait(8)
    pair_block([(2, 2), (1, 2), (2, 3), (1, 3), (2, 4), (1, 4)],
               [(lnx(6), 0, 10), (lnx(7), 0, 10), (xsum(3), 13, 19),
                (lnx(8), 0, 34), (lnx(9), 0, 34), (xsum(4), 37, 43),
                (lnx(10), 0, 61), (lnx(11), 0, 61), (xsum(5), 64, 72),
                (lnz(2), 0, 43), (lnz(3), 0, 43), (lnz(4), 12, 66), (lnz(5), 12, 66),
                (lnz(6), 36, 66), (lnz(7), 36, 66), (kv_items, 0, 72)], 5)
    wait(9)
    pair_block([(2, 5), (1, 5), (2, 6), (2, 7), (1, 6), (1, 7)],
               [(lnx(12), 0, 11), (lnx(13), 0, 11), (xsum(6), 13, 20),
                (lnx(14), 0, 23), (lnx(15), 0, 23), (xsum(7), 25, 32),
                (lnz(8), 0, 32), (lnz(9), 0, 32), (lnz(10), 12, 44), (lnz(11), 12, 44),
                (lnz(12), 36, 54), (lnz(13), 36, 54), (lnz(14), 48, 63), (lnz(15), 48, 63),
                (bsum(8), 36, 72), (bsum(9), 36, 72), (bsum(10), 48, 72), (bsum(11), 48, 72),
                (bsum(12), 58, 72), (bsum(13), 58, 72), (bsum(14), 67, 72), (bsum(15), 67, 72),
                (asum_items(0, HT // 2), 0, 72)], 4)
    wait(10)

    def unit(n, half, k, tap, put_p):
        def span(start, size):
            if isinstance(start, int):
                return slice(start, start + size)
            return pl.ds(pl.multiple_of(start, size), size)

        r = half * (HT // 2) + k
        top, bot = span(r * T, T), span(HS + r * T, T)
        toph, both = span(r * (T // 2), T // 2), span(HS // 2 + r * (T // 2), T // 2)
        sums, sumh = (as32, as232)[half], span(k * (T // 2), T // 2)

        def prod(lhs, rhs):
            acc = None
            for q in range(HS // KG):
                part = _dot(lhs(q), rhs(q))
                acc = part if acc is None else acc + part
                tap(acc)
            return acc

        def sa(i):
            return lambda q: jnp.concatenate(
                [_up(sums[i, c, sumh, :]) for c in range(q * KG // 128, (q + 1) * KG // 128)],
                axis=1)

        def sb(i):
            return lambda q: _up(bs32[i, n, q * KG // 2:(q + 1) * KG // 2, :])

        def a11(q):
            return _up(wsp_v[0, toph, q * KG:(q + 1) * KG])

        def a12(q):
            return _up(wsp_v[0, toph, HS + q * KG:HS + (q + 1) * KG])

        def b21(q):
            return _up(z232[n, (HS + q * KG) // 2:(HS + (q + 1) * KG) // 2, :])

        def a22(q):
            return _up(wsp_v[0, both, HS + q * KG:HS + (q + 1) * KG])

        def b11(q):
            return _up(z232[n, q * KG // 2:(q + 1) * KG // 2, :])

        def b22(q):
            return _up(z232[n + HF, (HS + q * KG) // 2:(HS + (q + 1) * KG) // 2, :])

        def fin(i, j, c):
            col, rows = n + j * HF, (top, bot)[i]
            put_p(i, j, col, rows, (c + bcol_v[rows, :]).astype(BF16))

        _winograd(prod, sa, sb, a11, a12, a22, b11, b21, b22, fin)

    def p2(n, half):
        nn = jnp.minimum(n + 1, NC - 1)

        for q in range(half * HF, min((half + 1) * HF, NC - 1)):
            @pl.when(n == q)
            def _():
                for d in step_cps(q):
                    d.wait()

        zero = zero_s[0]
        fwd_u = _up(tab_v[0:128, :])
        fwd_h = _up(tab_v[128:256, :])
        dd = dd_v[n]

        def put(slot, val):
            pl_v[:, slot] = val

        def re_im(val):
            val = val.reshape(BLK // 8, 2, 8, 128)
            return val[:, 0], val[:, 1]

        kvi = kv_items(nn)

        def pace_kv(d, val):
            if d % 4 == 3:
                for j in range(8):
                    _, gate, run = kvi[(d // 4) * 8 + j]
                    gate(val[j * 32:j * 32 + 8, :])
                    run()

        for i in range(NB):
            u = _dot(fwd_u, _up(kvb32[i * BLK // 2:(i + 1) * BLK // 2, :]))
            a, b = re_im(u)
            put(UA + i, a)
            put(UB + i, b)
            put(US + i, a + b)
            pace_kv(i, u)
        for i in range(NB):
            hb = _up(h_v[n, :, i * BLK:(i + 1) * BLK])
            hf = jax.lax.dot_general(fwd_h, hb, (((1,), (1,)), ((), ())),
                                     preferred_element_type=F32)
            c, d = re_im(hf)
            if i == 0:
                c, d = c + dd, d + dd
            put(HR + i, c)
            put(HP + i, d - c)
            put(HQ + i, c + d)
            pace_kv(NB + i, hf)

        state = {}

        def mac_item(pos, g0, pi, j0, j1):
            xv, hv = ((US, HR), (UA, HP), (UB, HQ))[pi]
            outs = range(g0, g0 + GRP)
            top = g0 + GRP

            def run():
                pz = zero + pos
                hs = {t: pl_v[pz, hv + t]
                      for t in range(max(g0 - j1 + 1, 0), top - j0)}
                acc = state['acc'] if j0 else {o: None for o in outs}
                for jj in range(j0, j1):
                    xj = pl_v[pz, xv + jj]
                    for o in outs:
                        if o - jj >= 0:
                            t = xj * hs[o - jj]
                            acc[o] = t if acc[o] is None else acc[o] + t
                if j1 < top:
                    state['acc'] = acc
                    return
                r0 = pos * 8
                if pi == 0:
                    state['k1'] = acc
                elif pi == 1:
                    state['im'] = {o: state['k1'][o] + acc[o] for o in outs}
                else:
                    for o in outs:
                        re, im = state['k1'][o] - acc[o], state['im'][o]
                        zr, zi = re, im
                        if o > 0:
                            zr, zi = re - state['prev'][1], im + state['prev'][0]
                        state['prev'] = (re, im)
                        zz_v[n, o, r0:r0 + 8, :] = zr.astype(BF16)
                        zz_v[n, o, BLK + r0:BLK + r0 + 8, :] = zi.astype(BF16)

            nmac = sum(1 for o in outs for jj in range(j0, j1) if o >= jj)
            return (2 * nmac + ((0, GRP, 5 * GRP)[pi] if j1 == top else 0), gate_pl, run)

        items = []
        for pos in range(BLK // 8):
            for g0 in range(0, NB, GRP):
                top = g0 + GRP
                cuts = [0, top] if top <= SPLIT else [0, (top - 1) // 2, top]
                for pi in range(3):
                    for j0, j1 in zip(cuts[:-1], cuts[1:]):
                        items.append(mac_item(pos, g0, pi, j0, j1))

        if half == 0:
            extra = [asum_dyn(jnp.minimum(n * NG + g, HS // 32 - 1), c)
                     for g in range(NG) for c in range(HT)]
            every = len(items) // len(extra)
            items = [it for i, e in enumerate(extra)
                     for it in items[i * every:(i + 1) * every] + [e]
                     ] + items[len(extra) * every:]

        total = sum(c for c, _, _ in items)
        tap_of = []
        cum = 0
        for c, _, _ in items:
            tap_of.append(int(cum * NTAP / total))
            cum += c
        pos = {'tap': 0, 'item': 0}

        def tap(acc):
            t0 = pos['tap']
            pos['tap'] += T // 8
            while pos['item'] < len(items) and tap_of[pos['item']] < pos['tap']:
                i = tap_of[pos['item']] - t0
                _, gate, run = items[pos['item']]
                gate(acc[i * 8:(i + 1) * 8, :])
                run()
                pos['item'] += 1

        def put_p(i, j, col, rows, val):
            p_v[col, rows, :] = val

        for k in range(HT // 2):
            unit(n - half * HF, half, k, tap, put_p)
        assert pos['item'] == len(items)
        return 0

    jax.lax.fori_loop(0, HF, lambda n, c: p2(n, 0), 0)
    jax.lax.fori_loop(HF, NC, lambda n, c: p2(n, 1), 0)

    wout_cp.wait()

    def p3(j, carry):
        inv_p = _up(tab_v[256:288, :])
        inv_m = _up(tab_v[288:320, :])
        rev = 7 - jax.lax.broadcasted_iota(jnp.int32, (8, 128), 0)

        zero = zero_s[0]
        HK = FH // 2

        def rows(k, i):
            tile = i * HT + (k // 2) * (HT // 2) + 2 * j + k % 2
            return (tile, pl.ds(pl.multiple_of(tile * T, T), T),
                    pl.ds(pl.multiple_of(tile * (T // 2), T // 2), T // 2))

        def fresh(k, n):
            return k >= 2 and n % HF == HF - 1

        def p_tile(k, i, n):
            return _up(pp32[k][i + zero, n])

        def gate_p(tok):
            z1_v[0, S:S + 8, :] = tok.astype(BF16)

        def gate_wo(tok):
            wout_v[0, HK:HK + 8, 0:128] = pltpu.bitcast(tok, U32)

        def psum_item(k, n, g):
            def run():
                def quad(i, jj):
                    rs, gs = rows(k, i)[1], slice(g * 16, (g + 1) * 16)
                    if fresh(k, n):
                        gv = pq_v[k - 2, i, jj, gs, :]
                    else:
                        gv = p_v.at[n + jj * HF, rs][gs, :]
                    pv = _gelu2(z1_v.at[n + jj * HF, rs][gs, :].astype(F32)) * gv.astype(F32)
                    pp_v[k][i, n + jj * HF, g * 16:(g + 1) * 16, :] = pv.astype(BF16)
                    return pv
                for i, v in enumerate(_lhs_sums(quad(0, 0), quad(0, 1), quad(1, 0), quad(1, 1))):
                    ps_v[k][i, n, g * 16:(g + 1) * 16, :] = v.astype(BF16)
            return (gate_p, run)

        def wsum_item(m, g):
            def run():
                def quad(i, jj):
                    r0 = (i * HK + g * 16) // 2
                    c0 = (m + 2 * jj) * 128
                    return _up(wout_v[zero, r0:r0 + 8, c0:c0 + 128]).astype(F32)
                for i, v in enumerate(_rhs_sums(quad(0, 0), quad(0, 1), quad(1, 0), quad(1, 1))):
                    ws_v[i, m, g * 16:(g + 1) * 16, :] = v.astype(BF16)
            return (gate_wo, run)

        def psum(k):
            return [psum_item(k, n, g) for n in range(HF) if not fresh(k, n)
                    for g in range(T // 16)]

        queue = []

        def tap(val):
            for i in range(min(len(queue), queue_step[0])):
                gate, run = queue.pop(0)
                r = (i * (T // 8)) // queue_step[0] * 8
                gate(val[r:r + 8, :])
                run()

        queue_step = [0]

        def paced(items, ntaps):
            assert not queue
            queue.extend(items)
            queue_step[0] = -(-len(items) // ntaps)

        def do_unit(u):
            def put_q(i, jj, col, rws, val):
                pq_v[u, i, jj] = val
            unit(HF - 1, 1, 2 * j + u, tap, put_q)
            for g in range(T // 16):
                psum_item(2 + u, HF - 1, g)[1]()

        def finish(k, i, c, o):
            tile, rs, hs = rows(k, i)
            cs = slice(c * 128, (c + 1) * 128)
            ye = _dot(inv_p, _up(zz32[c, tile, 0:64, :]))
            yo = _dot(inv_m, _up(zz32[c, tile, 64:128, :]))
            yd = ye - yo
            y = jnp.concatenate(
                [ye + yo] + [
                    jnp.take_along_axis(yd[q * 8:(q + 1) * 8], rev, axis=0,
                                        mode="promise_in_bounds")
                    for q in reversed(range(BLK // 16))], axis=0)
            gate = o * (1.0 + jnp.tanh((0.25 / _A) * o))
            x = _up(x_v[0, hs, cs]).astype(F32)
            xn = xn_v[c, rs, :].astype(F32)
            o_v[rs, cs] = (x + (xn * y) * gate).astype(BF16)

        def do_pair(k, last=False):
            def prod(lhs, rhs):
                res = _dot(lhs, rhs)
                tap(res)
                return res

            def sa(i):
                return jnp.concatenate([_up(ps32[k][i + zero, n]) for n in range(HF)], axis=1)

            a11 = jnp.concatenate([p_tile(k, 0, n) for n in range(HF)], axis=1)
            a22 = jnp.concatenate([p_tile(k, 1, n) for n in range(HF, NF)], axis=1)
            for m in range(2):
                _strassen(
                    prod, sa, lambda i: _up(ws32[i + zero, m]), a11, a22,
                    _up(wout_v[0, 0:HK // 2, m * 128:(m + 1) * 128]),
                    _up(wout_v[0, HK // 2:HK, (m + 2) * 128:(m + 3) * 128]),
                    lambda i, jj, o: finish(k, i, m + 2 * jj, o))
            for i in range(2):
                rs = rows(k, i)[1]
                if last:
                    cp(o_v.at[rs, 0:512], out_hbm.at[0, rs, 0:512], out_sem).start()
            for i in range(2):
                rs = rows(k, i)[1]
                p = jnp.concatenate([p_tile(k, i, n) for n in range(NF)], axis=1)
                finish(k, i, NC - 1, _dot(p, _up(wout_v[0, 0:HK, 512:D])))
                if last:
                    cp(o_v.at[rs, 512:D], out_hbm.at[0, rs, 512:D], out_sem).start()
                else:
                    cp(o_v.at[rs, :], out_hbm.at[0, rs, :], out_sem).start()

        paced(psum(0) + [wsum_item(m, g) for m in range(2) for g in range(HK // 16)], 12)
        do_unit(0)
        paced(psum(1), 12)
        do_pair(0)
        paced(psum(2), 12)
        do_unit(1)
        paced(psum(3), 12)
        do_pair(1)
        do_pair(2)
        do_pair(3, last=True)
        return carry

    jax.lax.fori_loop(0, P3I, p3, 0)
    cp(o_v, out_hbm.at[0], out_sem).wait()


@jax.jit
def pallas_recurrent_scan__ssm_conv_h3__mixer_gmlp__prompt_kernel(
    A_q: jax.Array,
    A_k: jax.Array,
    A_v: jax.Array,
    A_shift_k: jax.Array,
    A_ssm_k: jax.Array,
    A_ssm_D: jax.Array,
    B_x: jax.Array,
    B_w_in: jax.Array,
    B_w_sp: jax.Array,
    B_b_sp: jax.Array,
    B_w_out: jax.Array,
):
    del B_x
    tab = jnp.asarray(_dft_tables(), dtype=BF16)

    any_spec = pl.BlockSpec(memory_space=pl.ANY)
    return pl.pallas_call(
        _kernel,
        out_shape=jax.ShapeDtypeStruct((1, S, D), BF16),
        in_specs=[any_spec] * 11,
        out_specs=any_spec,
        scratch_shapes=[
            pltpu.VMEM((1, S // 2 + 32, D), U32),
            pltpu.VMEM((1, D // 2 + 8, 2 * FH), U32),
            pltpu.VMEM((1, S // 2 + 8, S), U32),
            pltpu.VMEM((1, FH // 2 + 32, D), U32),
            pltpu.VMEM((2 * NC, S // 2 + 32, 128), U32),
            pltpu.VMEM((NC, 64, S), U32),
            pltpu.VMEM((NC, S + 256, 128), BF16),
            pltpu.VMEM((NF, S + 64, 128), BF16),
            pltpu.VMEM((NF, S + 64, 128), BF16),
            pltpu.VMEM((NF, S, 128), BF16),
            pltpu.VMEM((4, HT, HS // 2, 128), BF16),
            pltpu.VMEM((4, HT, HS // 2, 128), BF16),
            pltpu.VMEM((4, HF, HS, 128), BF16),
            pltpu.VMEM((2, 2, 2, T, 128), BF16),
            [pltpu.VMEM((2, NF, T, 128), BF16)] * 4,
            [pltpu.VMEM((5, HF, T, 128), BF16)] * 4,
            pltpu.VMEM((5, 2, FH // 2, 128), BF16),
            pltpu.VMEM((S, 128), BF16),
            pltpu.VMEM((BLK // 8, 6 * NB + 1, 8, 128), F32),
            pltpu.VMEM((NC, NB, 2 * BLK, 128), BF16),
            pltpu.VMEM((S, 128), F32),
            pltpu.VMEM((S, D), BF16),
            pltpu.VMEM((1, T + 16, FH), F32),
            pltpu.VMEM((1, T + 16, FH), F32),
            pltpu.VMEM((1, T + 16, FH), F32),
            pltpu.VMEM((1, T + 16, FH), F32),
            pltpu.VMEM((1, T + 16, FH), F32),
            pltpu.VMEM((1, T + 16, FH), F32),
            pltpu.VMEM((NT // 2, 5, 2, T, 128), BF16),
            pltpu.VMEM((5, NF, KH, 128), BF16),
            pltpu.VMEM((T, 128), F32),
            pltpu.VMEM((320, 128), U32),
            pltpu.VMEM((NC, KS, 128), F32),
            pltpu.VMEM((NC + 2, 1, 128), F32),
            pltpu.VMEM((KS, D), BF16),
            pltpu.VMEM((D,), BF16),
            pltpu.VMEM((S,), BF16),
            pltpu.SMEM((1,), jnp.int32),
            pltpu.SemaphoreType.DMA((16,)),
        ],
        compiler_params=pltpu.CompilerParams(
            vmem_limit_bytes=100 * 1024 * 1024, disable_bounds_checks=True),
    )(A_q, A_k, A_v, A_shift_k.T, A_ssm_k, A_ssm_D, B_w_in, B_w_sp, B_b_sp, B_w_out, tab)
```

```python
import jax
import jax.numpy as jnp
import numpy as np
import jax.experimental.pallas as pl
import jax.experimental.pallas.tpu as pltpu

F32 = jnp.float32
BF16 = jnp.bfloat16
U32 = jnp.uint32

S = 2048
D = 640
FH = 768
KS = 4
BLK = 128
NB = S // BLK
NC = D // 128
NF = FH // 128
T = 128
NT = S // T
EPS = 1e-5
GRP = 4
SPLIT = 8
AW = 2
KG = 512
KR = 32
UA, UB, US, HP, HQ, HR, TOK = (i * NB for i in range(7))
LAG = 4
NTAP = 888
HS = S // 2
HT = HS // T
HF = NF // 2
KH = 256
P3I = 2

_GELU_C0 = float(np.sqrt(2.0 / np.pi))
_GELU_C1 = _GELU_C0 * 0.044715
_A = _GELU_C1 ** (1.0 / 3.0)
_K = _GELU_C0 / _A


def _dft_tables():
    m = np.arange(BLK)[:, None]
    n = np.arange(BLK)[None, :]
    th = 2.0 * np.pi * (((4 * m + 1) * n) % (4 * BLK)) / (4 * BLK)
    ph = 2.0 * np.pi * (((4 * m + 1) * (2 * n + 1)) % (8 * BLK)) / (8 * BLK)
    fu = np.concatenate([np.cos(ph), -np.sin(ph)], axis=0)
    fh = np.concatenate([np.cos(th) + np.sin(th), np.cos(th) - np.sin(th)], axis=0)
    fu, fh = (f.reshape(2, BLK // 8, 8, BLK).transpose(1, 0, 2, 3).reshape(2 * BLK, BLK)
              for f in (fu, fh))
    cp = (np.cos(ph) + np.sin(ph)).T[:BLK // 2] / (8.0 * BLK * _A * _A)
    cm = (np.cos(ph) - np.sin(ph)).T[:BLK // 2] / (8.0 * BLK * _A * _A)
    return np.concatenate([fu, fh, cp, cm], axis=0).astype(np.float32)


def _layernorm(x, eps, scale=1.0):
    m = jnp.mean(x, axis=-1, keepdims=True)
    d = x - m
    v = jnp.sum(d * d, axis=-1, keepdims=True) * (1.0 / (x.shape[-1] * scale * scale))
    return d * jax.lax.rsqrt(v + eps / (scale * scale))


def _gelu2(y):
    return y * (1.0 + jnp.tanh(y * (y * y + _K)))


def _up(x):
    return pltpu.bitcast(x, BF16)


def _dot(a, b):
    return jnp.dot(a, b, preferred_element_type=F32)


def _lhs_sums(a11, a12, a21, a22):
    return a11 + a22, a21 + a22, a11 + a12, a21 - a11, a12 - a22


def _rhs_sums(b11, b12, b21, b22):
    return b11 + b22, b12 - b22, b21 - b11, b11 + b12, b21 + b22


def _strassen(prod, sa, sb, a11, a22, b11, b22, fin):
    m2 = prod(sa(1), b11)
    m4 = prod(a22, sb(2))
    fin(1, 0, m2 + m4)
    m5 = prod(sa(2), b22)
    c11 = m4 - m5
    m3 = prod(a11, sb(1))
    fin(0, 1, m3 + m5)
    c22 = m3 - m2
    m1 = prod(sa(0), sb(0))
    c11, c22 = c11 + m1, c22 + m1
    fin(0, 0, c11 + prod(sa(4), sb(4)))
    fin(1, 1, c22 + prod(sa(3), sb(3)))


def _lhs_sums_w(a11, a12, a21, a22):
    s1 = a21 + a22
    s2 = s1 - a11
    return s1, s2, a11 - a21, a12 - s2


def _rhs_sums_w(b11, b12, b21, b22):
    t1 = b12 - b11
    t2 = b22 - t1
    return t1, t2, b22 - b12, t2 - b21


def _winograd(prod, sa, sb, a11, a12, a22, b11, b21, b22, fin):
    p1 = prod(a11, b11)
    fin(0, 0, p1 + prod(a12, b21))
    u2 = p1 + prod(sa(1), sb(1))
    p5 = prod(sa(0), sb(0))
    fin(0, 1, (u2 + p5) + prod(sa(3), b22))
    u3 = u2 + prod(sa(2), sb(2))
    fin(1, 1, u3 + p5)
    fin(1, 0, u3 - prod(a22, sb(3)))


def _balance(work, n):
    jobs = [(lo, hi, sum(it[0] for it in items)) for items, lo, hi in work]
    rate = [None] * n
    while jobs:
        def free(a, b):
            return [p for p in range(a, b) if rate[p] is None]
        dens, a, b = max(
            (sum(w for lo, hi, w in jobs if a <= lo and hi <= b) / max(len(free(a, b)), 1e-9), a, b)
            for a in {j[0] for j in jobs} for b in {j[1] for j in jobs} if a < b)
        while a > 0 and rate[a - 1] is not None:
            a -= 1
        while b < n and rate[b] is not None:
            b += 1
        for p in free(a, b):
            rate[p] = dens
        jobs = [(lo, hi, w) for lo, hi, w in jobs if not (a <= lo and hi <= b)]
        jobs = [(b if a <= lo < b else lo, a if a < hi <= b else hi, w) for lo, hi, w in jobs]
    queues = [[lo * 16, hi * 16, list(items)] for items, lo, hi in work]
    rel = [[] for _ in range(n)]
    budget = 0.0
    for tau in range(n * 16):
        budget += (rate[tau // 16] or 0.0) / 16
        while True:
            ready = [q for q in queues if q[2] and q[0] <= tau]
            if not ready:
                budget = min(budget, 0.0)
                break
            q = min(ready, key=lambda q: q[1])
            if budget < 0 and q[1] - tau > len(q[2]):
                break
            it = q[2].pop(0)
            rel[tau // 16].append((tau % 16, it))
            budget -= it[0]
    assert not any(q[2] for q in queues)
    return rel


def _kernel(x_hbm, k_hbm, v_hbm, skt_hbm, h_hbm, dv_hbm, win_hbm, wsp_hbm, b_hbm,
            wout_hbm, tab_hbm, out_hbm,
            x_v, win_v, wsp_v, wout_v, kv_v, h_v, xn_v, z1_v, z2_v, p_v, as_v, as2_v, bs_v, pq_v, pp_v, ps_v, ws_v,
            kvb_v, pl_v, zz_v, bcol_v, o_v, zta_v, ztb_v, ztc_v, ztd_v, zte_v, ztf_v, xs_v, wi_v, raw_v, tab_v,
            sk_v, dd_v, skt_v, dv_v, b_v, zero_s, sem):
    cp = pltpu.make_async_copy
    x16 = x_v.bitcast(BF16)
    win16 = win_v.bitcast(BF16)
    kv16 = kv_v.bitcast(BF16)
    h16 = h_v.bitcast(BF16)

    xn32, z232, kvb32, zz32, as32, as232, bs32, ws32, xs32, wi32 = (
        r.bitcast(U32)
        for r in (xn_v, z2_v, kvb_v, zz_v, as_v, as2_v, bs_v, ws_v, xs_v, wi_v))
    pp32 = [r.bitcast(U32) for r in pp_v]
    ps32 = [r.bitcast(U32) for r in ps_v]
    wsp16 = wsp_v.bitcast(BF16)

    def wsp_cp(lo, hi, s):
        return cp(wsp_hbm.at[lo:hi, :], wsp16.at[0, lo:hi, :], sem.at[s])

    def x_cp(lo, hi, s):
        return cp(x_hbm.at[0, lo:hi, :], x16.at[0, lo:hi, :], sem.at[s])

    def win_cp(lo, hi, s):
        return cp(win_hbm.at[:, lo:hi], win16.at[0, 0:D, lo:hi], sem.at[s])

    def k_cp(c, s):
        return cp(k_hbm.at[0, :, pl.ds(c * 128, 128)], kv16.at[2 * c, 0:S, :], sem.at[s])

    def v_cp(c, s):
        return cp(v_hbm.at[0, :, pl.ds(c * 128, 128)], kv16.at[2 * c + 1, 0:S, :], sem.at[s])

    def h_cp(c, s):
        return cp(h_hbm.at[pl.ds(c * 128, 128), :], h16.at[c], sem.at[s])

    groups = [
        [cp(b_hbm, b_v, sem.at[0]), cp(skt_hbm, skt_v, sem.at[0]), cp(dv_hbm, dv_v, sem.at[0])],
        [x_cp(0, 256, 1)],
        [win_cp(FH, FH + 256, 2)],
        [win_cp(FH + 256, FH + 512, 3)],
        [win_cp(FH + 512, 2 * FH, 4), win_cp(0, 128, 4)],
        [win_cp(128, 512, 10)],
        [win_cp(512, FH, 5), x_cp(256, 384, 5)],
        [x_cp(384, 6 * T, 6)],
        [x_cp(6 * T, 12 * T, 7), k_cp(0, 7), v_cp(0, 7)],
        [x_cp(12 * T, S, 11), wsp_cp(0, HS // 2, 11), wsp_cp(HS, HS + HS // 2, 11)],
        [cp(tab_hbm, tab_v.bitcast(BF16), sem.at[8]), h_cp(0, 8)],
    ]
    for g in groups:
        for c in g:
            c.start()

    NG = -(-HS // 32 // HF)

    def step_cps(n):
        s = 12 + n
        cps = [k_cp(n + 1, s), v_cp(n + 1, s), h_cp(n + 1, s)]
        if n < HF:
            lo, hi = HS // 2 + n * NG * 16, min(HS // 2 + (n + 1) * NG * 16, HS)
            cps += [wsp_cp(lo, hi, s), wsp_cp(HS + lo, HS + hi, s)]
        return cps

    wout_cp = cp(wout_hbm, wout_v.bitcast(BF16).at[0, 0:FH, :], sem.at[9])
    out_sem = sem.at[5]
    for n in range(NC - 1):
        for d in step_cps(n):
            d.start()
    wout_cp.start()

    def wait(i):
        for c in groups[i]:
            c.wait()

    zero_s[0] = 0
    wait(0)
    skt = skt_v[...].astype(F32)
    dv = dv_v[...].astype(F32).reshape(1, D)
    for c in range(NC):
        sk_v[c] = skt[:, c * 128:(c + 1) * 128]
        dd_v[c] = dv[:, c * 128:(c + 1) * 128]
    brow = b_v[...].astype(F32).reshape(1, S)
    bcol_v[...] = jnp.broadcast_to(brow, (128, S)).T

    def gate_x(tok):
        x_v[0, S // 2:S // 2 + 8, 0:128] = pltpu.bitcast(tok, U32)

    zt_v = (zta_v, ztb_v, ztc_v, ztd_v, zte_v, ztf_v)

    def gate_zt(t):
        def gate(tok):
            zt_v[t % 6][0, T:T + 8, 0:128] = tok
        return gate

    def gate_kv(tok):
        kv_v[0, S // 2:S // 2 + 8, :] = pltpu.bitcast(tok, U32)

    def gate_pl(tok):
        pl_v[0, TOK] = tok

    ndone = [0]

    mode = {'pairs': False}

    def done(val):
        r = (ndone[0] % 8) * 16
        ndone[0] += 1
        if mode['pairs']:
            xs_v[0, 0, 0, r:r + 16, :] = val
        else:
            xn_v[0, S + r:S + r + 16, :] = val

    def lnx_items(t, zero):
        def item(r0):
            def run():
                rs = slice(r0 // 2, r0 // 2 + 8)
                xw = jnp.concatenate([x_v[zero, rs, 0:128], x_v[0, rs, 128:D]], axis=1)
                xn = _layernorm(_up(xw).astype(F32), EPS, _A)
                for c in range(NC):
                    xb = xn[:, c * 128:(c + 1) * 128].astype(BF16)
                    xn_v[c, r0:r0 + 16, :] = xb
                if mode['pairs']:
                    done(xb)
            return (85, gate_x, run)
        return [item(t * T + g * 16) for g in range(T // 16)]

    def lnz_items(t, zero):
        def item(g):
            def run():
                rs = slice(g * 16, (g + 1) * 16)
                z = jnp.concatenate(
                    [zt_v[t % 6][zero, rs, 0:128], zt_v[t % 6][0, rs, 128:FH]], axis=1)
                z = _layernorm(z, 4.0 * _A * _A * EPS)
                r0 = t * T + g * 16
                for n in range(NF):
                    zb = z[:, n * 128:(n + 1) * 128].astype(BF16)
                    z2_v[n, r0:r0 + 16, :] = zb
                done(zb)
            return (90, gate_zt(t), run)
        return [item(g) for g in range(T // 16)]

    def kv_items(c):
        sk = sk_v[c]

        def item(r0):
            def run():
                hs = slice(r0 // 2, (r0 + KR) // 2)
                if r0 == 0:
                    kw = jnp.concatenate(
                        [jnp.zeros((8, 128), F32), _up(kv_v[2 * c, hs, :]).astype(F32)], axis=0)
                else:
                    kw = _up(kv_v[2 * c, r0 // 2 - 8:(r0 + KR) // 2, :]).astype(F32)[8:]
                ks = kw[8:] * sk[0:1, :]
                for t in range(1, KS):
                    ks = ks + pltpu.roll(kw, t, 0)[8:] * sk[t:t + 1, :]
                kvb_v[r0:r0 + KR, :] = (
                    ks * _up(kv_v[2 * c + 1, hs, :]).astype(F32)).astype(BF16)
            return (14 * KR // 8, gate_kv, run)
        return [item(r0) for r0 in range(0, S, KR)]

    def gate_w(tok):
        wsp_v[0, S // 2:S // 2 + 8, 0:128] = pltpu.bitcast(tok, U32)

    def asum_items(r_lo, r_hi):
        def item(zero, r0, c0):
            def run():
                def quad(i, j, c):
                    w = wsp_v[zero, (i * HS + r0) // 2:(i * HS + r0) // 2 + 8,
                              j * HS + c * 128:j * HS + (c + 1) * 128]
                    return _up(w).astype(F32)
                for c in range(c0, c0 + AW):
                    for i, v in enumerate(_lhs_sums_w(
                            quad(0, 0, c), quad(0, 1, c), quad(1, 0, c), quad(1, 1, c))):
                        as_v[i, c, r0:r0 + 16, :] = v.astype(BF16)
            return (20 * AW, gate_w, run)
        return lambda zero: [item(zero, r0, c0) for r0 in range(r_lo * T, r_hi * T, 16)
                             for c0 in range(0, HT, AW)]

    def asum_dyn(g, c):
        def run():
            def quad(i, j):
                r0 = pl.multiple_of(i * (HS // 2) + HS // 4 + g * 8, 8)
                w = wsp_v[0, pl.ds(r0, 8), j * HS + c * 128:j * HS + (c + 1) * 128]
                return _up(w).astype(F32)
            rs = pl.ds(pl.multiple_of(g * 16, 16), 16)
            for i, v in enumerate(_lhs_sums_w(quad(0, 0), quad(0, 1), quad(1, 0), quad(1, 1))):
                as2_v[i, c, rs, :] = v.astype(BF16)
        return (20, gate_w, run)

    def gate_z2(tok):
        z2_v[0, S:S + 8, :] = tok.astype(BF16)

    def bsum(t):
        def item(zero, r0, n):
            def run():
                def quad(i, j):
                    return z2_v[zero + n + j * HF, i * HS + r0:i * HS + r0 + 16, :].astype(F32)
                for i, v in enumerate(_rhs_sums_w(quad(0, 0), quad(0, 1), quad(1, 0), quad(1, 1))):
                    bs_v[i, n, r0:r0 + 16, :] = v.astype(BF16)
            return (21, gate_z2, run)
        return lambda zero: [item(zero, r0, n) for r0 in range((t - HT) * T, (t - HT + 1) * T, 16)
                             for n in range(HF)]

    def gate_xn(tok):
        xn_v[1, S:S + 8, :] = tok.astype(BF16)

    def xsum(u):
        def item(zero, g, c):
            def run():
                def quad(i, j):
                    r0 = (2 * u + i) * T + g * 16
                    return xn_v[zero + c + 2 * j, r0:r0 + 16, :].astype(F32)
                for i, v in enumerate(_lhs_sums(quad(0, 0), quad(0, 1), quad(1, 0), quad(1, 1))):
                    xs_v[u, i, c, g * 16:(g + 1) * 16, :] = v.astype(BF16)
            return (24, gate_xn, run)
        return lambda zero: [item(zero, g, c) for g in range(T // 16) for c in range(2)]

    def gate_wi(tok):
        win_v[0, D // 2:D // 2 + 8, 0:128] = pltpu.bitcast(tok, U32)

    def wisum(zero):
        def item(g, q):
            def run():
                def quad(i, j):
                    r0 = (i * KH + g * 16) // 2
                    c0 = ((q // HF) * NF + q % HF + j * HF) * 128
                    return _up(win_v[zero, r0:r0 + 8, c0:c0 + 128]).astype(F32)
                for i, v in enumerate(_rhs_sums(quad(0, 0), quad(0, 1), quad(1, 0), quad(1, 1))):
                    wi_v[i, q, g * 16:(g + 1) * 16, :] = v.astype(BF16)
            return (23, gate_wi, run)
        return [item(g, (q + HF) % NF) for q in range(NF) for g in range(KH // 16)]

    def taps_of(val):
        rows, cols = val.shape
        return [(lambda i=i, n=n: val[i * 8:(i + 1) * 8, n * 128:(n + 1) * 128])
                for n in range(cols // 128) for i in range(rows // 8)]

    def activate(kind, t, n, z):
        if kind == 2:
            zt_v[t % 6][0, 0:T, n * 128:(n + 1) * 128] = _gelu2(z)
        else:
            z1_v[n, t * T:(t + 1) * T, :] = z.astype(BF16)

    def piece(kind, t, n, zero, defer=False, halves=False):
        col = n * 128 + (FH if kind == 2 else 0)
        xn = jnp.concatenate(
            [_up(xn32[zero if zero is not None and c == 0 else c,
                      t * T // 2:(t + 1) * T // 2, :]) for c in range(NC)], axis=1)
        w = _up(win_v[0, 0:D // 2, col:col + 128])
        if halves:
            z = jnp.concatenate([_dot(xn[:T // 2], w), _dot(xn[T // 2:], w)], axis=0)
        else:
            z = _dot(xn, w)
        if defer:
            raw_v[...] = z
        else:
            activate(kind, t, n, z)
        return taps_of(z)

    def pair_piece(kind, u, m, gate_idx, slot_done):
        def xq(i, cs):
            rows = slice((2 * u + i) * T // 2, (2 * u + i + 1) * T // 2)
            return jnp.concatenate([_up(xn32[c, rows, :]) for c in cs], axis=1)

        def wq(lo, hi, j):
            c0 = ((kind - 1) * NF + m + j * HF) * 128
            return _up(win_v[0, lo // 2:hi // 2, c0:c0 + 128])

        def sa(i):
            return jnp.concatenate(
                [_up(xs32[u + (gate_idx() if c == 0 and i != 4 else 0), i, c])
                 for c in range(2)], axis=1)

        def fin(i, j, c):
            z = c + _dot(xq(i, [NC - 1]), wq(2 * KH, D, j))
            activate(kind, 2 * u + i, m + j * HF, z)
            slot_done(taps_of(z))

        _strassen(_dot, sa, lambda i: _up(wi32[i, (kind - 1) * HF + m]),
                  xq(0, (0, 1)), xq(1, (2, 3)), wq(0, KH, 0), wq(KH, 2 * KH, 1), fin)

    pending = []

    def plan(work, zero, n):
        work = [(mk(zero), lo, hi) for mk, lo, hi in work]
        return [a + b for a, b in zip(
            _balance([w for w in work if w[0][0][0] >= 80], n),
            _balance([w for w in work if w[0][0][0] < 80], n))]

    def pair_block(halves, work, lag):
        zero = zero_s[0]
        mode['pairs'] = True
        if pending:
            activate(*pending.pop(), raw_v[...])
        rel = plan(work, zero, 12 * len(halves))
        taps = []
        state = {'gated': False}

        def release(k):
            for i, (_, gate, run) in sorted(rel[k], key=lambda e: e[0]):
                gate(taps[k][i]())
                run()
                state['gated'] = True

        def slot_done(z):
            taps.append(z)
            if len(taps) > lag:
                release(len(taps) - 1 - lag)

        for kind, u in halves:
            for m in range(HF):
                pair_piece(kind, u, m, lambda: zero if state['gated'] else 0, slot_done)
        for k in range(len(taps) - lag, len(taps)):
            release(k)

    def block(pieces, work, defer=True, free=None):
        zero = zero_s[0]
        if pending:
            activate(*pending.pop(), raw_v[...])
        rel = plan(work, zero, len(pieces))
        taps = []
        gated = False
        for k in range(len(pieces) + LAG):
            if free is not None and k == len(pieces) - 1:
                for _, _, run in free(zero):
                    run()
                gated = True
            if k < len(pieces):
                last = defer and k == len(pieces) - 1
                halves = len(pieces) % 4 == 2 and k == len(pieces) - 1
                taps.append(piece(*pieces[k], zero if gated else None, last, halves))
                if last:
                    pending.append(pieces[k])
            if k >= LAG:
                for i, (_, gate, run) in sorted(rel[k - LAG], key=lambda e: e[0]):
                    gate(taps[k - LAG][i]())
                    run()
                    gated = True

    def cols(kind, t, lo=0, hi=NF):
        return [(kind, t, n) for n in range(lo, hi)]

    def lnx(t):
        return lambda zero: lnx_items(t, zero)

    def lnz(t):
        return lambda zero: lnz_items(t, zero)

    wait(1)
    for it in lnx_items(0, 0) + lnx_items(1, 0):
        it[2]()
    wait(2)
    block(cols(2, 0, 0, 2) + cols(2, 1, 0, 2), [])
    wait(3)
    block(cols(2, 0, 2, 4) + cols(2, 1, 2, 4), [])
    wait(4)
    block(cols(2, 0, 4) + cols(2, 1, 4) + cols(1, 0, 0, 1) + cols(1, 1, 0, 1), [])
    wait(5)
    block(cols(1, 0, 1, 4) + cols(1, 1, 1, 4), [(lnz(0), 0, 1)])
    wait(6)
    block(cols(1, 0, 4) + cols(1, 1, 4), [], free=lnx(2))

    def tiles(lo, hi):
        return [pc for t in range(lo, hi) for pc in cols(2, t) + cols(1, t)]

    wait(7)
    block(tiles(2, 4),
          [(lnx(3), 0, 7), (lnx(4), 0, 14), (lnx(5), 0, 15), (lnz(1), 0, 19),
           (wisum, 0, 24), (xsum(2), 17, 24)])
    wait(8)
    pair_block([(2, 2), (1, 2), (2, 3), (1, 3), (2, 4), (1, 4)],
               [(lnx(6), 0, 10), (lnx(7), 0, 10), (xsum(3), 13, 19),
                (lnx(8), 0, 34), (lnx(9), 0, 34), (xsum(4), 37, 43),
                (lnx(10), 0, 61), (lnx(11), 0, 61), (xsum(5), 64, 72),
                (lnz(2), 0, 43), (lnz(3), 0, 43), (lnz(4), 12, 66), (lnz(5), 12, 66),
                (lnz(6), 36, 66), (lnz(7), 36, 66), (kv_items, 0, 72)], 5)
    wait(9)
    pair_block([(2, 5), (1, 5), (2, 6), (2, 7), (1, 6), (1, 7)],
               [(lnx(12), 0, 11), (lnx(13), 0, 11), (xsum(6), 13, 20),
                (lnx(14), 0, 23), (lnx(15), 0, 23), (xsum(7), 25, 32),
                (lnz(8), 0, 32), (lnz(9), 0, 32), (lnz(10), 12, 44), (lnz(11), 12, 44),
                (lnz(12), 36, 54), (lnz(13), 36, 54), (lnz(14), 48, 63), (lnz(15), 48, 63),
                (bsum(8), 36, 72), (bsum(9), 36, 72), (bsum(10), 48, 72), (bsum(11), 48, 72),
                (bsum(12), 58, 72), (bsum(13), 58, 72), (bsum(14), 67, 72), (bsum(15), 67, 72),
                (asum_items(0, HT // 2), 0, 72)], 4)
    wait(10)

    def unit(n, half, k, tap, put_p):
        def span(start, size):
            if isinstance(start, int):
                return slice(start, start + size)
            return pl.ds(pl.multiple_of(start, size), size)

        r = half * (HT // 2) + k
        top, bot = span(r * T, T), span(HS + r * T, T)
        toph, both = span(r * (T // 2), T // 2), span(HS // 2 + r * (T // 2), T // 2)
        sums, sumh = (as32, as232)[half], span(k * (T // 2), T // 2)

        def prod(lhs, rhs):
            acc = None
            for q in range(HS // KG):
                part = _dot(lhs(q), rhs(q))
                acc = part if acc is None else acc + part
                tap(acc)
            return acc

        def sa(i):
            return lambda q: jnp.concatenate(
                [_up(sums[i, c, sumh, :]) for c in range(q * KG // 128, (q + 1) * KG // 128)],
                axis=1)

        def sb(i):
            return lambda q: _up(bs32[i, n, q * KG // 2:(q + 1) * KG // 2, :])

        def a11(q):
            return _up(wsp_v[0, toph, q * KG:(q + 1) * KG])

        def a12(q):
            return _up(wsp_v[0, toph, HS + q * KG:HS + (q + 1) * KG])

        def b21(q):
            return _up(z232[n, (HS + q * KG) // 2:(HS + (q + 1) * KG) // 2, :])

        def a22(q):
            return _up(wsp_v[0, both, HS + q * KG:HS + (q + 1) * KG])

        def b11(q):
            return _up(z232[n, q * KG // 2:(q + 1) * KG // 2, :])

        def b22(q):
            return _up(z232[n + HF, (HS + q * KG) // 2:(HS + (q + 1) * KG) // 2, :])

        def fin(i, j, c):
            col, rows = n + j * HF, (top, bot)[i]
            put_p(i, j, col, rows, (c + bcol_v[rows, :]).astype(BF16))

        _winograd(prod, sa, sb, a11, a12, a22, b11, b21, b22, fin)

    def p2(n, half):
        nn = jnp.minimum(n + 1, NC - 1)

        for q in range(half * HF, min((half + 1) * HF, NC - 1)):
            @pl.when(n == q)
            def _():
                for d in step_cps(q):
                    d.wait()

        zero = zero_s[0]
        fwd_u = _up(tab_v[0:128, :])
        fwd_h = _up(tab_v[128:256, :])
        dd = dd_v[n]

        def put(slot, val):
            pl_v[:, slot] = val

        def re_im(val):
            val = val.reshape(BLK // 8, 2, 8, 128)
            return val[:, 0], val[:, 1]

        kvi = kv_items(nn)

        def pace_kv(d, val):
            if d % 4 == 3:
                for j in range(8):
                    _, gate, run = kvi[(d // 4) * 8 + j]
                    gate(val[j * 32:j * 32 + 8, :])
                    run()

        for i in range(NB):
            u = _dot(fwd_u, _up(kvb32[i * BLK // 2:(i + 1) * BLK // 2, :]))
            a, b = re_im(u)
            put(UA + i, a)
            put(UB + i, b)
            put(US + i, a + b)
            pace_kv(i, u)
        for i in range(NB):
            hb = _up(h_v[n, :, i * BLK:(i + 1) * BLK])
            hf = jax.lax.dot_general(fwd_h, hb, (((1,), (1,)), ((), ())),
                                     preferred_element_type=F32)
            c, d = re_im(hf)
            if i == 0:
                c, d = c + dd, d + dd
            put(HR + i, c)
            put(HP + i, d - c)
            put(HQ + i, c + d)
            pace_kv(NB + i, hf)

        state = {}

        def mac_item(pos, g0, pi, j0, j1):
            xv, hv = ((US, HR), (UA, HP), (UB, HQ))[pi]
            outs = range(g0, g0 + GRP)
            top = g0 + GRP

            def run():
                pz = zero + pos
                hs = {t: pl_v[pz, hv + t]
                      for t in range(max(g0 - j1 + 1, 0), top - j0)}
                acc = state['acc'] if j0 else {o: None for o in outs}
                for jj in range(j0, j1):
                    xj = pl_v[pz, xv + jj]
                    for o in outs:
                        if o - jj >= 0:
                            t = xj * hs[o - jj]
                            acc[o] = t if acc[o] is None else acc[o] + t
                if j1 < top:
                    state['acc'] = acc
                    return
                r0 = pos * 8
                if pi == 0:
                    state['k1'] = acc
                elif pi == 1:
                    state['im'] = {o: state['k1'][o] + acc[o] for o in outs}
                else:
                    for o in outs:
                        re, im = state['k1'][o] - acc[o], state['im'][o]
                        zr, zi = re, im
                        if o > 0:
                            zr, zi = re - state['prev'][1], im + state['prev'][0]
                        state['prev'] = (re, im)
                        zz_v[n, o, r0:r0 + 8, :] = zr.astype(BF16)
                        zz_v[n, o, BLK + r0:BLK + r0 + 8, :] = zi.astype(BF16)

            nmac = sum(1 for o in outs for jj in range(j0, j1) if o >= jj)
            return (2 * nmac + ((0, GRP, 5 * GRP)[pi] if j1 == top else 0), gate_pl, run)

        items = []
        for pos in range(BLK // 8):
            for g0 in range(0, NB, GRP):
                top = g0 + GRP
                cuts = [0, top] if top <= SPLIT else [0, (top - 1) // 2, top]
                for pi in range(3):
                    for j0, j1 in zip(cuts[:-1], cuts[1:]):
                        items.append(mac_item(pos, g0, pi, j0, j1))

        if half == 0:
            extra = [asum_dyn(jnp.minimum(n * NG + g, HS // 32 - 1), c)
                     for g in range(NG) for c in range(HT)]
            every = len(items) // len(extra)
            items = [it for i, e in enumerate(extra)
                     for it in items[i * every:(i + 1) * every] + [e]
                     ] + items[len(extra) * every:]

        total = sum(c for c, _, _ in items)
        tap_of = []
        cum = 0
        for c, _, _ in items:
            tap_of.append(int(cum * NTAP / total))
            cum += c
        pos = {'tap': 0, 'item': 0}

        def tap(acc):
            t0 = pos['tap']
            pos['tap'] += T // 8
            while pos['item'] < len(items) and tap_of[pos['item']] < pos['tap']:
                i = tap_of[pos['item']] - t0
                _, gate, run = items[pos['item']]
                gate(acc[i * 8:(i + 1) * 8, :])
                run()
                pos['item'] += 1

        def put_p(i, j, col, rows, val):
            p_v[col, rows, :] = val

        for k in range(HT // 2):
            unit(n - half * HF, half, k, tap, put_p)
        assert pos['item'] == len(items)
        return 0

    jax.lax.fori_loop(0, HF, lambda n, c: p2(n, 0), 0)
    jax.lax.fori_loop(HF, NC, lambda n, c: p2(n, 1), 0)

    wout_cp.wait()

    def p3(j, carry):
        inv_p = _up(tab_v[256:288, :])
        inv_m = _up(tab_v[288:320, :])
        rev = 7 - jax.lax.broadcasted_iota(jnp.int32, (8, 128), 0)

        zero = zero_s[0]
        HK = FH // 2

        def rows(k, i):
            tile = i * HT + (k // 2) * (HT // 2) + 2 * j + k % 2
            return (tile, pl.ds(pl.multiple_of(tile * T, T), T),
                    pl.ds(pl.multiple_of(tile * (T // 2), T // 2), T // 2))

        def fresh(k, n):
            return k >= 2 and n % HF == HF - 1

        def p_tile(k, i, n):
            return _up(pp32[k][i + zero, n])

        def gate_p(tok):
            z1_v[0, S:S + 8, :] = tok.astype(BF16)

        def gate_wo(tok):
            wout_v[0, HK:HK + 8, 0:128] = pltpu.bitcast(tok, U32)

        def psum_item(k, n, g):
            def run():
                def quad(i, jj):
                    rs, gs = rows(k, i)[1], slice(g * 16, (g + 1) * 16)
                    if fresh(k, n):
                        gv = pq_v[k - 2, i, jj, gs, :]
                    else:
                        gv = p_v.at[n + jj * HF, rs][gs, :]
                    pv = _gelu2(z1_v.at[n + jj * HF, rs][gs, :].astype(F32)) * gv.astype(F32)
                    pp_v[k][i, n + jj * HF, g * 16:(g + 1) * 16, :] = pv.astype(BF16)
                    return pv
                for i, v in enumerate(_lhs_sums(quad(0, 0), quad(0, 1), quad(1, 0), quad(1, 1))):
                    ps_v[k][i, n, g * 16:(g + 1) * 16, :] = v.astype(BF16)
            return (gate_p, run)

        def wsum_item(m, g):
            def run():
                def quad(i, jj):
                    r0 = (i * HK + g * 16) // 2
                    c0 = (m + 2 * jj) * 128
                    return _up(wout_v[zero, r0:r0 + 8, c0:c0 + 128]).astype(F32)
                for i, v in enumerate(_rhs_sums(quad(0, 0), quad(0, 1), quad(1, 0), quad(1, 1))):
                    ws_v[i, m, g * 16:(g + 1) * 16, :] = v.astype(BF16)
            return (gate_wo, run)

        def psum(k, cols):
            return [psum_item(k, n, g) for n in cols for g in range(T // 16)]

        queue = []

        def tap(val):
            for i in range(min(len(queue), queue_step[0])):
                gate, run = queue.pop(0)
                r = (i * (T // 8)) // queue_step[0] * 8
                gate(val[r:r + 8, :])
                run()

        queue_step = [0]

        def paced(items, ntaps):
            assert not queue
            queue.extend(items)
            queue_step[0] = -(-len(items) // ntaps)

        def do_unit(u):
            def put_q(i, jj, col, rws, val):
                pq_v[u, i, jj] = val
            unit(HF - 1, 1, 2 * j + u, tap, put_q)

        def finish(k, i, c, o):
            tile, rs, hs = rows(k, i)
            cs = slice(c * 128, (c + 1) * 128)
            ye = _dot(inv_p, _up(zz32[c, tile, 0:64, :]))
            yo = _dot(inv_m, _up(zz32[c, tile, 64:128, :]))
            yd = ye - yo
            y = jnp.concatenate(
                [ye + yo] + [
                    jnp.take_along_axis(yd[q * 8:(q + 1) * 8], rev, axis=0,
                                        mode="promise_in_bounds")
                    for q in reversed(range(BLK // 16))], axis=0)
            gate = o * (1.0 + jnp.tanh((0.25 / _A) * o))
            x = _up(x_v[0, hs, cs]).astype(F32)
            xn = xn_v[c, rs, :].astype(F32)
            o_v[rs, cs] = (x + (xn * y) * gate).astype(BF16)

        def do_pair(k, last=False):
            def prod(lhs, rhs):
                res = _dot(lhs, rhs)
                tap(res)
                return res

            def sa(i):
                return jnp.concatenate([_up(ps32[k][i + zero, n]) for n in range(HF)], axis=1)

            a11 = jnp.concatenate([p_tile(k, 0, n) for n in range(HF)], axis=1)
            a22 = jnp.concatenate([p_tile(k, 1, n) for n in range(HF, NF)], axis=1)
            for m in range(2):
                _strassen(
                    prod, sa, lambda i: _up(ws32[i + zero, m]), a11, a22,
                    _up(wout_v[0, 0:HK // 2, m * 128:(m + 1) * 128]),
                    _up(wout_v[0, HK // 2:HK, (m + 2) * 128:(m + 3) * 128]),
                    lambda i, jj, o: finish(k, i, m + 2 * jj, o))
            for i in range(2):
                rs = rows(k, i)[1]
                if last:
                    cp(o_v.at[rs, 0:512], out_hbm.at[0, rs, 0:512], out_sem).start()
            for i in range(2):
                rs = rows(k, i)[1]
                p = jnp.concatenate([p_tile(k, i, n) for n in range(NF)], axis=1)
                finish(k, i, NC - 1, _dot(p, _up(wout_v[0, 0:HK, 512:D])))
                if last:
                    cp(o_v.at[rs, 512:D], out_hbm.at[0, rs, 512:D], out_sem).start()
                else:
                    cp(o_v.at[rs, :], out_hbm.at[0, rs, :], out_sem).start()

        paced(psum(0, (0, 1, 2)) + [wsum_item(m, g) for m in range(2) for g in range(HK // 16)], 12)
        do_unit(0)
        paced(psum(1, (0, 1, 2)), 12)
        do_pair(0)
        paced(psum(2, (0, 1, 2)), 12)
        do_unit(1)
        paced(psum(3, (0, 1, 2)), 12)
        do_pair(1)
        do_pair(2)
        do_pair(3, last=True)
        return carry

    jax.lax.fori_loop(0, P3I, p3, 0)
    cp(o_v, out_hbm.at[0], out_sem).wait()


@jax.jit
def pallas_recurrent_scan__ssm_conv_h3__mixer_gmlp__prompt_kernel(
    A_q: jax.Array,
    A_k: jax.Array,
    A_v: jax.Array,
    A_shift_k: jax.Array,
    A_ssm_k: jax.Array,
    A_ssm_D: jax.Array,
    B_x: jax.Array,
    B_w_in: jax.Array,
    B_w_sp: jax.Array,
    B_b_sp: jax.Array,
    B_w_out: jax.Array,
):
    del B_x
    tab = jnp.asarray(_dft_tables(), dtype=BF16)

    any_spec = pl.BlockSpec(memory_space=pl.ANY)
    return pl.pallas_call(
        _kernel,
        out_shape=jax.ShapeDtypeStruct((1, S, D), BF16),
        in_specs=[any_spec] * 11,
        out_specs=any_spec,
        scratch_shapes=[
            pltpu.VMEM((1, S // 2 + 32, D), U32),
            pltpu.VMEM((1, D // 2 + 8, 2 * FH), U32),
            pltpu.VMEM((1, S // 2 + 8, S), U32),
            pltpu.VMEM((1, FH // 2 + 32, D), U32),
            pltpu.VMEM((2 * NC, S // 2 + 32, 128), U32),
            pltpu.VMEM((NC, 64, S), U32),
            pltpu.VMEM((NC, S + 256, 128), BF16),
            pltpu.VMEM((NF, S + 64, 128), BF16),
            pltpu.VMEM((NF, S + 64, 128), BF16),
            pltpu.VMEM((NF, S, 128), BF16),
            pltpu.VMEM((4, HT, HS // 2, 128), BF16),
            pltpu.VMEM((4, HT, HS // 2, 128), BF16),
            pltpu.VMEM((4, HF, HS, 128), BF16),
            pltpu.VMEM((2, 2, 2, T, 128), BF16),
            [pltpu.VMEM((2, NF, T, 128), BF16)] * 4,
            [pltpu.VMEM((5, HF, T, 128), BF16)] * 4,
            pltpu.VMEM((5, 2, FH // 2, 128), BF16),
            pltpu.VMEM((S, 128), BF16),
            pltpu.VMEM((BLK // 8, 6 * NB + 1, 8, 128), F32),
            pltpu.VMEM((NC, NB, 2 * BLK, 128), BF16),
            pltpu.VMEM((S, 128), F32),
            pltpu.VMEM((S, D), BF16),
            pltpu.VMEM((1, T + 16, FH), F32),
            pltpu.VMEM((1, T + 16, FH), F32),
            pltpu.VMEM((1, T + 16, FH), F32),
            pltpu.VMEM((1, T + 16, FH), F32),
            pltpu.VMEM((1, T + 16, FH), F32),
            pltpu.VMEM((1, T + 16, FH), F32),
            pltpu.VMEM((NT // 2, 5, 2, T, 128), BF16),
            pltpu.VMEM((5, NF, KH, 128), BF16),
            pltpu.VMEM((T, 128), F32),
            pltpu.VMEM((320, 128), U32),
            pltpu.VMEM((NC, KS, 128), F32),
            pltpu.VMEM((NC + 2, 1, 128), F32),
            pltpu.VMEM((KS, D), BF16),
            pltpu.VMEM((D,), BF16),
            pltpu.VMEM((S,), BF16),
            pltpu.SMEM((1,), jnp.int32),
            pltpu.SemaphoreType.DMA((16,)),
        ],
        compiler_params=pltpu.CompilerParams(
            vmem_limit_bytes=100 * 1024 * 1024, disable_bounds_checks=True),
    )(A_q, A_k, A_v, A_shift_k.T, A_ssm_k, A_ssm_D, B_w_in, B_w_sp, B_b_sp, B_w_out, tab)
```

```python
import jax
import jax.numpy as jnp
import numpy as np
import jax.experimental.pallas as pl
import jax.experimental.pallas.tpu as pltpu

F32 = jnp.float32
BF16 = jnp.bfloat16
U32 = jnp.uint32

S = 2048
D = 640
FH = 768
KS = 4
BLK = 128
NB = S // BLK
NC = D // 128
NF = FH // 128
T = 128
NT = S // T
EPS = 1e-5
GRP = 4
SPLIT = 8
AW = 2
KG = 512
KR = 32
UA, UB, US, HP, HQ, HR, TOK = (i * NB for i in range(7))
LAG = 4
NTAP = 888
HS = S // 2
HT = HS // T
HF = NF // 2
KH = 256
P3I = 2

_GELU_C0 = float(np.sqrt(2.0 / np.pi))
_GELU_C1 = _GELU_C0 * 0.044715
_A = _GELU_C1 ** (1.0 / 3.0)
_K = _GELU_C0 / _A


def _dft_tables():
    m = np.arange(BLK)[:, None]
    n = np.arange(BLK)[None, :]
    th = 2.0 * np.pi * (((4 * m + 1) * n) % (4 * BLK)) / (4 * BLK)
    ph = 2.0 * np.pi * (((4 * m + 1) * (2 * n + 1)) % (8 * BLK)) / (8 * BLK)
    fu = np.concatenate([np.cos(ph), -np.sin(ph)], axis=0)
    fh = np.concatenate([np.cos(th) + np.sin(th), np.cos(th) - np.sin(th)], axis=0)
    fu, fh = (f.reshape(2, BLK // 8, 8, BLK).transpose(1, 0, 2, 3).reshape(2 * BLK, BLK)
              for f in (fu, fh))
    cp = (np.cos(ph) + np.sin(ph)).T[:BLK // 2] / (8.0 * BLK * _A * _A)
    cm = (np.cos(ph) - np.sin(ph)).T[:BLK // 2] / (8.0 * BLK * _A * _A)
    return np.concatenate([fu, fh, cp, cm], axis=0).astype(np.float32)


def _layernorm(x, eps, scale=1.0):
    m = jnp.mean(x, axis=-1, keepdims=True)
    d = x - m
    v = jnp.sum(d * d, axis=-1, keepdims=True) * (1.0 / (x.shape[-1] * scale * scale))
    return d * jax.lax.rsqrt(v + eps / (scale * scale))


def _gelu2(y):
    return y * (1.0 + jnp.tanh(y * (y * y + _K)))


def _up(x):
    return pltpu.bitcast(x, BF16)


def _dot(a, b):
    return jnp.dot(a, b, preferred_element_type=F32)


def _lhs_sums(a11, a12, a21, a22):
    return a11 + a22, a21 + a22, a11 + a12, a21 - a11, a12 - a22


def _rhs_sums(b11, b12, b21, b22):
    return b11 + b22, b12 - b22, b21 - b11, b11 + b12, b21 + b22


def _strassen(prod, sa, sb, a11, a22, b11, b22, fin):
    m2 = prod(sa(1), b11)
    m4 = prod(a22, sb(2))
    fin(1, 0, m2 + m4)
    m5 = prod(sa(2), b22)
    c11 = m4 - m5
    m3 = prod(a11, sb(1))
    fin(0, 1, m3 + m5)
    c22 = m3 - m2
    m1 = prod(sa(0), sb(0))
    c11, c22 = c11 + m1, c22 + m1
    fin(0, 0, c11 + prod(sa(4), sb(4)))
    fin(1, 1, c22 + prod(sa(3), sb(3)))


def _lhs_sums_w(a11, a12, a21, a22):
    s1 = a21 + a22
    s2 = s1 - a11
    return s1, s2, a11 - a21, a12 - s2


def _rhs_sums_w(b11, b12, b21, b22):
    t1 = b12 - b11
    t2 = b22 - t1
    return t1, t2, b22 - b12, t2 - b21


def _winograd(prod, sa, sb, a11, a12, a22, b11, b21, b22, fin):
    p1 = prod(a11, b11)
    fin(0, 0, p1 + prod(a12, b21))
    u2 = p1 + prod(sa(1), sb(1))
    p5 = prod(sa(0), sb(0))
    fin(0, 1, (u2 + p5) + prod(sa(3), b22))
    u3 = u2 + prod(sa(2), sb(2))
    fin(1, 1, u3 + p5)
    fin(1, 0, u3 - prod(a22, sb(3)))


def _balance(work, n):
    jobs = [(lo, hi, sum(it[0] for it in items)) for items, lo, hi in work]
    rate = [None] * n
    while jobs:
        def free(a, b):
            return [p for p in range(a, b) if rate[p] is None]
        dens, a, b = max(
            (sum(w for lo, hi, w in jobs if a <= lo and hi <= b) / max(len(free(a, b)), 1e-9), a, b)
            for a in {j[0] for j in jobs} for b in {j[1] for j in jobs} if a < b)
        while a > 0 and rate[a - 1] is not None:
            a -= 1
        while b < n and rate[b] is not None:
            b += 1
        for p in free(a, b):
            rate[p] = dens
        jobs = [(lo, hi, w) for lo, hi, w in jobs if not (a <= lo and hi <= b)]
        jobs = [(b if a <= lo < b else lo, a if a < hi <= b else hi, w) for lo, hi, w in jobs]
    queues = [[lo * 16, hi * 16, list(items)] for items, lo, hi in work]
    rel = [[] for _ in range(n)]
    budget = 0.0
    for tau in range(n * 16):
        budget += (rate[tau // 16] or 0.0) / 16
        while True:
            ready = [q for q in queues if q[2] and q[0] <= tau]
            if not ready:
                budget = min(budget, 0.0)
                break
            q = min(ready, key=lambda q: q[1])
            if budget < 0 and q[1] - tau > len(q[2]):
                break
            it = q[2].pop(0)
            rel[tau // 16].append((tau % 16, it))
            budget -= it[0]
    assert not any(q[2] for q in queues)
    return rel


def _kernel(x_hbm, k_hbm, v_hbm, skt_hbm, h_hbm, dv_hbm, win_hbm, wsp_hbm, b_hbm,
            wout_hbm, tab_hbm, out_hbm,
            x_v, win_v, wsp_v, wout_v, kv_v, h_v, xn_v, z1_v, z2_v, z2b_v, p_v, as_v, as2_v, bs_v, pq_v, pp_v, ps_v, ws_v,
            kvb_v, pl_v, zz_v, bcol_v, o_v, zta_v, ztb_v, ztc_v, ztd_v, zte_v, ztf_v, xs_v, wi_v, raw_v, tab_v,
            sk_v, dd_v, skt_v, dv_v, b_v, zero_s, sem):
    cp = pltpu.make_async_copy
    x16 = x_v.bitcast(BF16)
    win16 = win_v.bitcast(BF16)
    kv16 = kv_v.bitcast(BF16)
    h16 = h_v.bitcast(BF16)

    xn32, z232, kvb32, zz32, as32, as232, bs32, ws32, xs32, wi32 = (
        r.bitcast(U32)
        for r in (xn_v, z2_v, kvb_v, zz_v, as_v, as2_v, bs_v, ws_v, xs_v, wi_v))
    z2b32 = z2b_v.bitcast(U32)
    pp32 = [r.bitcast(U32) for r in pp_v]
    ps32 = [r.bitcast(U32) for r in ps_v]
    wsp16 = wsp_v.bitcast(BF16)

    def wsp_cp(lo, hi, s):
        return cp(wsp_hbm.at[lo:hi, :], wsp16.at[0, lo:hi, :], sem.at[s])

    def x_cp(lo, hi, s):
        return cp(x_hbm.at[0, lo:hi, :], x16.at[0, lo:hi, :], sem.at[s])

    def win_cp(lo, hi, s):
        return cp(win_hbm.at[:, lo:hi], win16.at[0, 0:D, lo:hi], sem.at[s])

    def k_cp(c, s):
        return cp(k_hbm.at[0, :, pl.ds(c * 128, 128)], kv16.at[2 * c, 0:S, :], sem.at[s])

    def v_cp(c, s):
        return cp(v_hbm.at[0, :, pl.ds(c * 128, 128)], kv16.at[2 * c + 1, 0:S, :], sem.at[s])

    def h_cp(c, s):
        return cp(h_hbm.at[pl.ds(c * 128, 128), :], h16.at[c], sem.at[s])

    groups = [
        [cp(b_hbm, b_v, sem.at[0]), cp(skt_hbm, skt_v, sem.at[0]), cp(dv_hbm, dv_v, sem.at[0])],
        [x_cp(0, 256, 1)],
        [win_cp(FH, FH + 256, 2)],
        [win_cp(FH + 256, FH + 512, 3)],
        [win_cp(FH + 512, 2 * FH, 4), win_cp(0, 128, 4)],
        [win_cp(128, 512, 10)],
        [win_cp(512, FH, 5), x_cp(256, 384, 5)],
        [x_cp(384, 6 * T, 6)],
        [x_cp(6 * T, 12 * T, 7), k_cp(0, 7), v_cp(0, 7)],
        [x_cp(12 * T, S, 11), wsp_cp(0, HS // 2, 11), wsp_cp(HS, HS + HS // 2, 11)],
        [cp(tab_hbm, tab_v.bitcast(BF16), sem.at[8]), h_cp(0, 8)],
    ]
    for g in groups:
        for c in g:
            c.start()

    NG = -(-HS // 32 // HF)

    def step_cps(n):
        s = 12 + n
        cps = [k_cp(n + 1, s), v_cp(n + 1, s), h_cp(n + 1, s)]
        if n < HF:
            lo, hi = HS // 2 + n * NG * 16, min(HS // 2 + (n + 1) * NG * 16, HS)
            cps += [wsp_cp(lo, hi, s), wsp_cp(HS + lo, HS + hi, s)]
        return cps

    wout_cp = cp(wout_hbm, wout_v.bitcast(BF16).at[0, 0:FH, :], sem.at[9])
    out_sem = sem.at[5]
    for n in range(NC - 1):
        for d in step_cps(n):
            d.start()
    wout_cp.start()

    def wait(i):
        for c in groups[i]:
            c.wait()

    zero_s[0] = 0
    wait(0)
    skt = skt_v[...].astype(F32)
    dv = dv_v[...].astype(F32).reshape(1, D)
    for c in range(NC):
        sk_v[c] = skt[:, c * 128:(c + 1) * 128]
        dd_v[c] = dv[:, c * 128:(c + 1) * 128]
    brow = b_v[...].astype(F32).reshape(1, S)
    bcol_v[...] = jnp.broadcast_to(brow, (128, S)).T

    def gate_x(tok):
        x_v[0, S // 2:S // 2 + 8, 0:128] = pltpu.bitcast(tok, U32)

    zt_v = (zta_v, ztb_v, ztc_v, ztd_v, zte_v, ztf_v)

    def gate_zt(t):
        def gate(tok):
            zt_v[t % 6][0, T:T + 8, 0:128] = tok
        return gate

    def gate_kv(tok):
        kv_v[0, S // 2:S // 2 + 8, :] = pltpu.bitcast(tok, U32)

    def gate_pl(tok):
        pl_v[0, TOK] = tok

    ndone = [0]

    mode = {'pairs': False}

    def done(val):
        r = (ndone[0] % 8) * 16
        ndone[0] += 1
        if mode['pairs']:
            xs_v[0, 0, 0, r:r + 16, :] = val
        else:
            xn_v[0, S + r:S + r + 16, :] = val

    def lnx_items(t, zero):
        def item(r0):
            def run():
                rs = slice(r0 // 2, r0 // 2 + 8)
                xw = jnp.concatenate([x_v[zero, rs, 0:128], x_v[0, rs, 128:D]], axis=1)
                xn = _layernorm(_up(xw).astype(F32), EPS, _A)
                for c in range(NC):
                    xb = xn[:, c * 128:(c + 1) * 128].astype(BF16)
                    xn_v[c, r0:r0 + 16, :] = xb
                if mode['pairs']:
                    done(xb)
            return (85, gate_x, run)
        return [item(t * T + g * 16) for g in range(T // 16)]

    def lnz_items(t, zero):
        def item(g):
            def run():
                rs = slice(g * 16, (g + 1) * 16)
                z = jnp.concatenate(
                    [zt_v[t % 6][zero, rs, 0:128], zt_v[t % 6][0, rs, 128:FH]], axis=1)
                z = _layernorm(z, 4.0 * _A * _A * EPS)
                r0 = t * T + g * 16
                for n in range(NF):
                    zb = z[:, n * 128:(n + 1) * 128].astype(BF16)
                    (z2_v, z2b_v)[t // HT][n, r0 % HS:r0 % HS + 16, :] = zb
                done(zb)
            return (90, gate_zt(t), run)
        return [item(g) for g in range(T // 16)]

    def kv_items(c):
        sk = sk_v[c]

        def item(r0):
            def run():
                hs = slice(r0 // 2, (r0 + KR) // 2)
                if r0 == 0:
                    kw = jnp.concatenate(
                        [jnp.zeros((8, 128), F32), _up(kv_v[2 * c, hs, :]).astype(F32)], axis=0)
                else:
                    kw = _up(kv_v[2 * c, r0 // 2 - 8:(r0 + KR) // 2, :]).astype(F32)[8:]
                ks = kw[8:] * sk[0:1, :]
                for t in range(1, KS):
                    ks = ks + pltpu.roll(kw, t, 0)[8:] * sk[t:t + 1, :]
                kvb_v[r0:r0 + KR, :] = (
                    ks * _up(kv_v[2 * c + 1, hs, :]).astype(F32)).astype(BF16)
            return (14 * KR // 8, gate_kv, run)
        return [item(r0) for r0 in range(0, S, KR)]

    def gate_w(tok):
        wsp_v[0, S // 2:S // 2 + 8, 0:128] = pltpu.bitcast(tok, U32)

    def asum_items(r_lo, r_hi):
        def item(zero, r0, c0):
            def run():
                def quad(i, j, c):
                    w = wsp_v[zero, (i * HS + r0) // 2:(i * HS + r0) // 2 + 8,
                              j * HS + c * 128:j * HS + (c + 1) * 128]
                    return _up(w).astype(F32)
                for c in range(c0, c0 + AW):
                    for i, v in enumerate(_lhs_sums_w(
                            quad(0, 0, c), quad(0, 1, c), quad(1, 0, c), quad(1, 1, c))):
                        as_v[i, c, r0:r0 + 16, :] = v.astype(BF16)
            return (20 * AW, gate_w, run)
        return lambda zero: [item(zero, r0, c0) for r0 in range(r_lo * T, r_hi * T, 16)
                             for c0 in range(0, HT, AW)]

    def asum_dyn(g, c):
        def run():
            def quad(i, j):
                r0 = pl.multiple_of(i * (HS // 2) + HS // 4 + g * 8, 8)
                w = wsp_v[0, pl.ds(r0, 8), j * HS + c * 128:j * HS + (c + 1) * 128]
                return _up(w).astype(F32)
            rs = pl.ds(pl.multiple_of(g * 16, 16), 16)
            for i, v in enumerate(_lhs_sums_w(quad(0, 0), quad(0, 1), quad(1, 0), quad(1, 1))):
                as2_v[i, c, rs, :] = v.astype(BF16)
        return (20, gate_w, run)

    def gate_z2(tok):
        z2_v[0, HS:HS + 8, :] = tok.astype(BF16)

    def bsum(t):
        def item(zero, r0, n):
            def run():
                def quad(i, j):
                    if i:
                        return z2b_v[n + j * HF, r0:r0 + 16, :].astype(F32)
                    return z2_v[zero + n + j * HF, r0:r0 + 16, :].astype(F32)
                for i, v in enumerate(_rhs_sums_w(quad(0, 0), quad(0, 1), quad(1, 0), quad(1, 1))):
                    bs_v[i, n, r0:r0 + 16, :] = v.astype(BF16)
            return (21, gate_z2, run)
        return lambda zero: [item(zero, r0, n) for r0 in range((t - HT) * T, (t - HT + 1) * T, 16)
                             for n in range(HF)]

    def gate_xn(tok):
        xn_v[1, S:S + 8, :] = tok.astype(BF16)

    def xsum(u):
        def item(zero, g, c):
            def run():
                def quad(i, j):
                    r0 = (2 * u + i) * T + g * 16
                    return xn_v[zero + c + 2 * j, r0:r0 + 16, :].astype(F32)
                for i, v in enumerate(_lhs_sums(quad(0, 0), quad(0, 1), quad(1, 0), quad(1, 1))):
                    xs_v[u, i, c, g * 16:(g + 1) * 16, :] = v.astype(BF16)
            return (24, gate_xn, run)
        return lambda zero: [item(zero, g, c) for g in range(T // 16) for c in range(2)]

    def gate_wi(tok):
        win_v[0, D // 2:D // 2 + 8, 0:128] = pltpu.bitcast(tok, U32)

    def wisum(zero):
        def item(g, q):
            def run():
                def quad(i, j):
                    r0 = (i * KH + g * 16) // 2
                    c0 = ((q // HF) * NF + q % HF + j * HF) * 128
                    return _up(win_v[zero, r0:r0 + 8, c0:c0 + 128]).astype(F32)
                for i, v in enumerate(_rhs_sums(quad(0, 0), quad(0, 1), quad(1, 0), quad(1, 1))):
                    wi_v[i, q, g * 16:(g + 1) * 16, :] = v.astype(BF16)
            return (23, gate_wi, run)
        return [item(g, (q + HF) % NF) for q in range(NF) for g in range(KH // 16)]

    def taps_of(val):
        rows, cols = val.shape
        return [(lambda i=i, n=n: val[i * 8:(i + 1) * 8, n * 128:(n + 1) * 128])
                for n in range(cols // 128) for i in range(rows // 8)]

    def activate(kind, t, n, z):
        if kind == 2:
            zt_v[t % 6][0, 0:T, n * 128:(n + 1) * 128] = _gelu2(z)
        else:
            z1_v[n, t * T:(t + 1) * T, :] = z.astype(BF16)

    def piece(kind, t, n, zero, defer=False, halves=False):
        col = n * 128 + (FH if kind == 2 else 0)
        xn = jnp.concatenate(
            [_up(xn32[zero if zero is not None and c == 0 else c,
                      t * T // 2:(t + 1) * T // 2, :]) for c in range(NC)], axis=1)
        w = _up(win_v[0, 0:D // 2, col:col + 128])
        if halves:
            z = jnp.concatenate([_dot(xn[:T // 2], w), _dot(xn[T // 2:], w)], axis=0)
        else:
            z = _dot(xn, w)
        if defer:
            raw_v[...] = z
        else:
            activate(kind, t, n, z)
        return taps_of(z)

    def pair_piece(kind, u, m, gate_idx, slot_done):
        def xq(i, cs):
            rows = slice((2 * u + i) * T // 2, (2 * u + i + 1) * T // 2)
            return jnp.concatenate([_up(xn32[c, rows, :]) for c in cs], axis=1)

        def wq(lo, hi, j):
            c0 = ((kind - 1) * NF + m + j * HF) * 128
            return _up(win_v[0, lo // 2:hi // 2, c0:c0 + 128])

        def sa(i):
            return jnp.concatenate(
                [_up(xs32[u + (gate_idx() if c == 0 and i != 4 else 0), i, c])
                 for c in range(2)], axis=1)

        def fin(i, j, c):
            z = c + _dot(xq(i, [NC - 1]), wq(2 * KH, D, j))
            activate(kind, 2 * u + i, m + j * HF, z)
            slot_done(taps_of(z))

        _strassen(_dot, sa, lambda i: _up(wi32[i, (kind - 1) * HF + m]),
                  xq(0, (0, 1)), xq(1, (2, 3)), wq(0, KH, 0), wq(KH, 2 * KH, 1), fin)

    pending = []

    def plan(work, zero, n):
        work = [(mk(zero), lo, hi) for mk, lo, hi in work]
        return [a + b for a, b in zip(
            _balance([w for w in work if w[0][0][0] >= 80], n),
            _balance([w for w in work if w[0][0][0] < 80], n))]

    def pair_block(halves, work, lag):
        zero = zero_s[0]
        mode['pairs'] = True
        if pending:
            activate(*pending.pop(), raw_v[...])
        rel = plan(work, zero, 12 * len(halves))
        taps = []
        state = {'gated': False}

        def release(k):
            for i, (_, gate, run) in sorted(rel[k], key=lambda e: e[0]):
                gate(taps[k][i]())
                run()
                state['gated'] = True

        def slot_done(z):
            taps.append(z)
            if len(taps) > lag:
                release(len(taps) - 1 - lag)

        for kind, u in halves:
            for m in range(HF):
                pair_piece(kind, u, m, lambda: zero if state['gated'] else 0, slot_done)
        for k in range(len(taps) - lag, len(taps)):
            release(k)

    def block(pieces, work, defer=True, free=None):
        zero = zero_s[0]
        if pending:
            activate(*pending.pop(), raw_v[...])
        rel = plan(work, zero, len(pieces))
        taps = []
        gated = False
        for k in range(len(pieces) + LAG):
            if free is not None and k == len(pieces) - 1:
                for _, _, run in free(zero):
                    run()
                gated = True
            if k < len(pieces):
                last = defer and k == len(pieces) - 1
                halves = len(pieces) % 4 == 2 and k == len(pieces) - 1
                taps.append(piece(*pieces[k], zero if gated else None, last, halves))
                if last:
                    pending.append(pieces[k])
            if k >= LAG:
                for i, (_, gate, run) in sorted(rel[k - LAG], key=lambda e: e[0]):
                    gate(taps[k - LAG][i]())
                    run()
                    gated = True

    def cols(kind, t, lo=0, hi=NF):
        return [(kind, t, n) for n in range(lo, hi)]

    def lnx(t):
        return lambda zero: lnx_items(t, zero)

    def lnz(t):
        return lambda zero: lnz_items(t, zero)

    wait(1)
    for it in lnx_items(0, 0) + lnx_items(1, 0):
        it[2]()
    wait(2)
    block(cols(2, 0, 0, 2) + cols(2, 1, 0, 2), [])
    wait(3)
    block(cols(2, 0, 2, 4) + cols(2, 1, 2, 4), [])
    wait(4)
    block(cols(2, 0, 4) + cols(2, 1, 4) + cols(1, 0, 0, 1) + cols(1, 1, 0, 1), [])
    wait(5)
    block(cols(1, 0, 1, 4) + cols(1, 1, 1, 4), [(lnz(0), 0, 1)])
    wait(6)
    block(cols(1, 0, 4) + cols(1, 1, 4), [], free=lnx(2))

    def tiles(lo, hi):
        return [pc for t in range(lo, hi) for pc in cols(2, t) + cols(1, t)]

    wait(7)
    block(tiles(2, 4),
          [(lnx(3), 0, 7), (lnx(4), 0, 14), (lnx(5), 0, 15), (lnz(1), 0, 19),
           (wisum, 0, 24), (xsum(2), 17, 24)])
    wait(8)
    pair_block([(2, 2), (1, 2), (2, 3), (1, 3), (2, 4), (1, 4)],
               [(lnx(6), 0, 10), (lnx(7), 0, 10), (xsum(3), 13, 19),
                (lnx(8), 0, 34), (lnx(9), 0, 34), (xsum(4), 37, 43),
                (lnx(10), 0, 61), (lnx(11), 0, 61), (xsum(5), 64, 72),
                (lnz(2), 0, 43), (lnz(3), 0, 43), (lnz(4), 12, 66), (lnz(5), 12, 66),
                (lnz(6), 36, 66), (lnz(7), 36, 66), (kv_items, 0, 72)], 5)
    wait(9)
    pair_block([(2, 5), (1, 5), (2, 6), (2, 7), (1, 6), (1, 7)],
               [(lnx(12), 0, 11), (lnx(13), 0, 11), (xsum(6), 13, 20),
                (lnx(14), 0, 23), (lnx(15), 0, 23), (xsum(7), 25, 32),
                (lnz(8), 0, 32), (lnz(9), 0, 32), (lnz(10), 12, 44), (lnz(11), 12, 44),
                (lnz(12), 36, 54), (lnz(13), 36, 54), (lnz(14), 48, 63), (lnz(15), 48, 63),
                (bsum(8), 36, 72), (bsum(9), 36, 72), (bsum(10), 48, 72), (bsum(11), 48, 72),
                (bsum(12), 58, 72), (bsum(13), 58, 72), (bsum(14), 67, 72), (bsum(15), 67, 72),
                (asum_items(0, HT // 2), 0, 72)], 4)
    wait(10)

    def unit(n, half, k, tap, put_p):
        def span(start, size):
            if isinstance(start, int):
                return slice(start, start + size)
            return pl.ds(pl.multiple_of(start, size), size)

        r = half * (HT // 2) + k
        top, bot = span(r * T, T), span(HS + r * T, T)
        toph, both = span(r * (T // 2), T // 2), span(HS // 2 + r * (T // 2), T // 2)
        sums, sumh = (as32, as232)[half], span(k * (T // 2), T // 2)

        def prod(lhs, rhs):
            acc = None
            for q in range(HS // KG):
                part = _dot(lhs(q), rhs(q))
                acc = part if acc is None else acc + part
                tap(acc)
            return acc

        def sa(i):
            return lambda q: jnp.concatenate(
                [_up(sums[i, c, sumh, :]) for c in range(q * KG // 128, (q + 1) * KG // 128)],
                axis=1)

        def sb(i):
            return lambda q: _up(bs32[i, n, q * KG // 2:(q + 1) * KG // 2, :])

        def a11(q):
            return _up(wsp_v[0, toph, q * KG:(q + 1) * KG])

        def a12(q):
            return _up(wsp_v[0, toph, HS + q * KG:HS + (q + 1) * KG])

        def b21(q):
            return _up(z2b32[n, q * KG // 2:(q + 1) * KG // 2, :])

        def a22(q):
            return _up(wsp_v[0, both, HS + q * KG:HS + (q + 1) * KG])

        def b11(q):
            return _up(z232[n, q * KG // 2:(q + 1) * KG // 2, :])

        def b22(q):
            return _up(z2b32[n + HF, q * KG // 2:(q + 1) * KG // 2, :])

        def fin(i, j, c):
            col, rows = n + j * HF, (top, bot)[i]
            put_p(i, j, col, rows, (c + bcol_v[rows, :]).astype(BF16))

        _winograd(prod, sa, sb, a11, a12, a22, b11, b21, b22, fin)

    def p2(n, half):
        nn = jnp.minimum(n + 1, NC - 1)

        for q in range(half * HF, min((half + 1) * HF, NC - 1)):
            @pl.when(n == q)
            def _():
                for d in step_cps(q):
                    d.wait()

        zero = zero_s[0]
        fwd_u = _up(tab_v[0:128, :])
        fwd_h = _up(tab_v[128:256, :])
        dd = dd_v[n]

        def put(slot, val):
            pl_v[:, slot] = val

        def re_im(val):
            val = val.reshape(BLK // 8, 2, 8, 128)
            return val[:, 0], val[:, 1]

        kvi = kv_items(nn)

        def pace_kv(d, val):
            if d % 4 == 3:
                for j in range(8):
                    _, gate, run = kvi[(d // 4) * 8 + j]
                    gate(val[j * 32:j * 32 + 8, :])
                    run()

        for i in range(NB):
            u = _dot(fwd_u, _up(kvb32[i * BLK // 2:(i + 1) * BLK // 2, :]))
            a, b = re_im(u)
            put(UA + i, a)
            put(UB + i, b)
            put(US + i, a + b)
            pace_kv(i, u)
        for i in range(NB):
            hb = _up(h_v[n, :, i * BLK:(i + 1) * BLK])
            hf = jax.lax.dot_general(fwd_h, hb, (((1,), (1,)), ((), ())),
                                     preferred_element_type=F32)
            c, d = re_im(hf)
            if i == 0:
                c, d = c + dd, d + dd
            put(HR + i, c)
            put(HP + i, d - c)
            put(HQ + i, c + d)
            pace_kv(NB + i, hf)

        state = {}

        def mac_item(pos, g0, pi, j0, j1):
            xv, hv = ((US, HR), (UA, HP), (UB, HQ))[pi]
            outs = range(g0, g0 + GRP)
            top = g0 + GRP

            def run():
                pz = zero + pos
                hs = {t: pl_v[pz, hv + t]
                      for t in range(max(g0 - j1 + 1, 0), top - j0)}
                acc = state['acc'] if j0 else {o: None for o in outs}
                for jj in range(j0, j1):
                    xj = pl_v[pz, xv + jj]
                    for o in outs:
                        if o - jj >= 0:
                            t = xj * hs[o - jj]
                            acc[o] = t if acc[o] is None else acc[o] + t
                if j1 < top:
                    state['acc'] = acc
                    return
                r0 = pos * 8
                if pi == 0:
                    state['k1'] = acc
                elif pi == 1:
                    state['im'] = {o: state['k1'][o] + acc[o] for o in outs}
                else:
                    for o in outs:
                        re, im = state['k1'][o] - acc[o], state['im'][o]
                        zr, zi = re, im
                        if o > 0:
                            zr, zi = re - state['prev'][1], im + state['prev'][0]
                        state['prev'] = (re, im)
                        zz_v[n, o, r0:r0 + 8, :] = zr.astype(BF16)
                        zz_v[n, o, BLK + r0:BLK + r0 + 8, :] = zi.astype(BF16)

            nmac = sum(1 for o in outs for jj in range(j0, j1) if o >= jj)
            return (2 * nmac + ((0, GRP, 5 * GRP)[pi] if j1 == top else 0), gate_pl, run)

        items = []
        for pos in range(BLK // 8):
            for g0 in range(0, NB, GRP):
                top = g0 + GRP
                cuts = [0, top] if top <= SPLIT else [0, (top - 1) // 2, top]
                for pi in range(3):
                    for j0, j1 in zip(cuts[:-1], cuts[1:]):
                        items.append(mac_item(pos, g0, pi, j0, j1))

        if half == 0:
            extra = [asum_dyn(jnp.minimum(n * NG + g, HS // 32 - 1), c)
                     for g in range(NG) for c in range(HT)]
            every = len(items) // len(extra)
            items = [it for i, e in enumerate(extra)
                     for it in items[i * every:(i + 1) * every] + [e]
                     ] + items[len(extra) * every:]

        total = sum(c for c, _, _ in items)
        tap_of = []
        cum = 0
        for c, _, _ in items:
            tap_of.append(int(cum * NTAP / total))
            cum += c
        pos = {'tap': 0, 'item': 0}

        def tap(acc):
            t0 = pos['tap']
            pos['tap'] += T // 8
            while pos['item'] < len(items) and tap_of[pos['item']] < pos['tap']:
                i = tap_of[pos['item']] - t0
                _, gate, run = items[pos['item']]
                gate(acc[i * 8:(i + 1) * 8, :])
                run()
                pos['item'] += 1

        def put_p(i, j, col, rows, val):
            p_v[col, rows, :] = val

        for k in range(HT // 2):
            unit(n - half * HF, half, k, tap, put_p)
        assert pos['item'] == len(items)
        return 0

    jax.lax.fori_loop(0, HF, lambda n, c: p2(n, 0), 0)
    jax.lax.fori_loop(HF, NC, lambda n, c: p2(n, 1), 0)

    wout_cp.wait()

    def p3(j, carry):
        inv_p = _up(tab_v[256:288, :])
        inv_m = _up(tab_v[288:320, :])
        rev = 7 - jax.lax.broadcasted_iota(jnp.int32, (8, 128), 0)

        zero = zero_s[0]
        HK = FH // 2

        def rows(k, i):
            tile = i * HT + (k // 2) * (HT // 2) + 2 * j + k % 2
            return (tile, pl.ds(pl.multiple_of(tile * T, T), T),
                    pl.ds(pl.multiple_of(tile * (T // 2), T // 2), T // 2))

        def fresh(k, n):
            return k >= 2 and n % HF == HF - 1

        def p_tile(k, i, n):
            return _up(pp32[k][i + zero, n])

        def gate_p(tok):
            z1_v[0, S:S + 8, :] = tok.astype(BF16)

        def gate_wo(tok):
            wout_v[0, HK:HK + 8, 0:128] = pltpu.bitcast(tok, U32)

        def psum_item(k, n, g):
            def run():
                def quad(i, jj):
                    rs, gs = rows(k, i)[1], slice(g * 16, (g + 1) * 16)
                    if fresh(k, n):
                        gv = pq_v[k - 2, i, jj, gs, :]
                    else:
                        gv = p_v.at[n + jj * HF, rs][gs, :]
                    pv = _gelu2(z1_v.at[n + jj * HF, rs][gs, :].astype(F32)) * gv.astype(F32)
                    pp_v[k][i, n + jj * HF, g * 16:(g + 1) * 16, :] = pv.astype(BF16)
                    return pv
                for i, v in enumerate(_lhs_sums(quad(0, 0), quad(0, 1), quad(1, 0), quad(1, 1))):
                    ps_v[k][i, n, g * 16:(g + 1) * 16, :] = v.astype(BF16)
            return (gate_p, run)

        def wsum_item(m, g):
            def run():
                def quad(i, jj):
                    r0 = (i * HK + g * 16) // 2
                    c0 = (m + 2 * jj) * 128
                    return _up(wout_v[zero, r0:r0 + 8, c0:c0 + 128]).astype(F32)
                for i, v in enumerate(_rhs_sums(quad(0, 0), quad(0, 1), quad(1, 0), quad(1, 1))):
                    ws_v[i, m, g * 16:(g + 1) * 16, :] = v.astype(BF16)
            return (gate_wo, run)

        def psum(k, cols):
            return [psum_item(k, n, g) for n in cols for g in range(T // 16)]

        queue = []

        def tap(val):
            for i in range(min(len(queue), queue_step[0])):
                gate, run = queue.pop(0)
                r = (i * (T // 8)) // queue_step[0] * 8
                gate(val[r:r + 8, :])
                run()

        queue_step = [0]

        def paced(items, ntaps):
            assert not queue
            queue.extend(items)
            queue_step[0] = -(-len(items) // ntaps)

        def do_unit(u):
            def put_q(i, jj, col, rws, val):
                pq_v[u, i, jj] = val
            unit(HF - 1, 1, 2 * j + u, tap, put_q)

        def finish(k, i, c, o):
            tile, rs, hs = rows(k, i)
            cs = slice(c * 128, (c + 1) * 128)
            ye = _dot(inv_p, _up(zz32[c, tile, 0:64, :]))
            yo = _dot(inv_m, _up(zz32[c, tile, 64:128, :]))
            yd = ye - yo
            y = jnp.concatenate(
                [ye + yo] + [
                    jnp.take_along_axis(yd[q * 8:(q + 1) * 8], rev, axis=0,
                                        mode="promise_in_bounds")
                    for q in reversed(range(BLK // 16))], axis=0)
            gate = o * (1.0 + jnp.tanh((0.25 / _A) * o))
            x = _up(x_v[0, hs, cs]).astype(F32)
            xn = xn_v[c, rs, :].astype(F32)
            o_v[rs, cs] = (x + (xn * y) * gate).astype(BF16)

        def do_pair(k, last=False):
            def prod(lhs, rhs):
                res = _dot(lhs, rhs)
                tap(res)
                return res

            def sa(i):
                return jnp.concatenate([_up(ps32[k][i + zero, n]) for n in range(HF)], axis=1)

            a11 = jnp.concatenate([p_tile(k, 0, n) for n in range(HF)], axis=1)
            a22 = jnp.concatenate([p_tile(k, 1, n) for n in range(HF, NF)], axis=1)
            for m in range(2):
                _strassen(
                    prod, sa, lambda i: _up(ws32[i + zero, m]), a11, a22,
                    _up(wout_v[0, 0:HK // 2, m * 128:(m + 1) * 128]),
                    _up(wout_v[0, HK // 2:HK, (m + 2) * 128:(m + 3) * 128]),
                    lambda i, jj, o: finish(k, i, m + 2 * jj, o))
            for i in range(2):
                rs = rows(k, i)[1]
                if last:
                    cp(o_v.at[rs, 0:512], out_hbm.at[0, rs, 0:512], out_sem).start()
            for i in range(2):
                rs = rows(k, i)[1]
                p = jnp.concatenate([p_tile(k, i, n) for n in range(NF)], axis=1)
                finish(k, i, NC - 1, _dot(p, _up(wout_v[0, 0:HK, 512:D])))
                if last:
                    cp(o_v.at[rs, 512:D], out_hbm.at[0, rs, 512:D], out_sem).start()
                else:
                    cp(o_v.at[rs, :], out_hbm.at[0, rs, :], out_sem).start()

        paced(psum(0, (0, 1, 2)) + [wsum_item(m, g) for m in range(2) for g in range(HK // 16)], 12)
        do_unit(0)
        paced(psum(1, (0, 1, 2)), 12)
        do_pair(0)
        paced(psum(2, (0, 1, 2)), 12)
        do_unit(1)
        paced(psum(3, (0, 1, 2)), 12)
        do_pair(1)
        do_pair(2)
        do_pair(3, last=True)
        return carry

    jax.lax.fori_loop(0, P3I, p3, 0)
    cp(o_v, out_hbm.at[0], out_sem).wait()


@jax.jit
def pallas_recurrent_scan__ssm_conv_h3__mixer_gmlp__prompt_kernel(
    A_q: jax.Array,
    A_k: jax.Array,
    A_v: jax.Array,
    A_shift_k: jax.Array,
    A_ssm_k: jax.Array,
    A_ssm_D: jax.Array,
    B_x: jax.Array,
    B_w_in: jax.Array,
    B_w_sp: jax.Array,
    B_b_sp: jax.Array,
    B_w_out: jax.Array,
):
    del B_x
    tab = jnp.asarray(_dft_tables(), dtype=BF16)

    any_spec = pl.BlockSpec(memory_space=pl.ANY)
    return pl.pallas_call(
        _kernel,
        out_shape=jax.ShapeDtypeStruct((1, S, D), BF16),
        in_specs=[any_spec] * 11,
        out_specs=any_spec,
        scratch_shapes=[
            pltpu.VMEM((1, S // 2 + 32, D), U32),
            pltpu.VMEM((1, D // 2 + 8, 2 * FH), U32),
            pltpu.VMEM((1, S // 2 + 8, S), U32),
            pltpu.VMEM((1, FH // 2 + 32, D), U32),
            pltpu.VMEM((2 * NC, S // 2 + 32, 128), U32),
            pltpu.VMEM((NC, 64, S), U32),
            pltpu.VMEM((NC, S + 256, 128), BF16),
            pltpu.VMEM((NF, S + 64, 128), BF16),
            pltpu.VMEM((NF, HS + 64, 128), BF16),
            pltpu.VMEM((NF, HS, 128), BF16),
            pltpu.VMEM((NF, S, 128), BF16),
            pltpu.VMEM((4, HT, HS // 2, 128), BF16),
            pltpu.VMEM((4, HT, HS // 2, 128), BF16),
            pltpu.VMEM((4, HF, HS, 128), BF16),
            pltpu.VMEM((2, 2, 2, T, 128), BF16),
            [pltpu.VMEM((2, NF, T, 128), BF16)] * 4,
            [pltpu.VMEM((5, HF, T, 128), BF16)] * 4,
            pltpu.VMEM((5, 2, FH // 2, 128), BF16),
            pltpu.VMEM((S, 128), BF16),
            pltpu.VMEM((BLK // 8, 6 * NB + 1, 8, 128), F32),
            pltpu.VMEM((NC, NB, 2 * BLK, 128), BF16),
            pltpu.VMEM((S, 128), F32),
            pltpu.VMEM((S, D), BF16),
            pltpu.VMEM((1, T + 16, FH), F32),
            pltpu.VMEM((1, T + 16, FH), F32),
            pltpu.VMEM((1, T + 16, FH), F32),
            pltpu.VMEM((1, T + 16, FH), F32),
            pltpu.VMEM((1, T + 16, FH), F32),
            pltpu.VMEM((1, T + 16, FH), F32),
            pltpu.VMEM((NT // 2, 5, 2, T, 128), BF16),
            pltpu.VMEM((5, NF, KH, 128), BF16),
            pltpu.VMEM((T, 128), F32),
            pltpu.VMEM((320, 128), U32),
            pltpu.VMEM((NC, KS, 128), F32),
            pltpu.VMEM((NC + 2, 1, 128), F32),
            pltpu.VMEM((KS, D), BF16),
            pltpu.VMEM((D,), BF16),
            pltpu.VMEM((S,), BF16),
            pltpu.SMEM((1,), jnp.int32),
            pltpu.SemaphoreType.DMA((16,)),
        ],
        compiler_params=pltpu.CompilerParams(
            vmem_limit_bytes=100 * 1024 * 1024, disable_bounds_checks=True),
    )(A_q, A_k, A_v, A_shift_k.T, A_ssm_k, A_ssm_D, B_w_in, B_w_sp, B_b_sp, B_w_out, tab)
```

```python
import jax
import jax.numpy as jnp
import numpy as np
import jax.experimental.pallas as pl
import jax.experimental.pallas.tpu as pltpu

F32 = jnp.float32
BF16 = jnp.bfloat16
U32 = jnp.uint32

S = 2048
D = 640
FH = 768
KS = 4
BLK = 128
NB = S // BLK
NC = D // 128
NF = FH // 128
T = 128
NT = S // T
EPS = 1e-5
GRP = 4
SPLIT = 8
AW = 2
KG = 512
KR = 32
UA, UB, US, HP, HQ, HR, TOK = (i * NB for i in range(7))
LAG = 4
NTAP = 888
HS = S // 2
HT = HS // T
HF = NF // 2
KH = 256
P3I = 2

_GELU_C0 = float(np.sqrt(2.0 / np.pi))
_GELU_C1 = _GELU_C0 * 0.044715
_A = _GELU_C1 ** (1.0 / 3.0)
_K = _GELU_C0 / _A


def _dft_tables():
    m = np.arange(BLK)[:, None]
    n = np.arange(BLK)[None, :]
    th = 2.0 * np.pi * (((4 * m + 1) * n) % (4 * BLK)) / (4 * BLK)
    ph = 2.0 * np.pi * (((4 * m + 1) * (2 * n + 1)) % (8 * BLK)) / (8 * BLK)
    fu = np.concatenate([np.cos(ph), -np.sin(ph)], axis=0)
    fh = np.concatenate([np.cos(th) + np.sin(th), np.cos(th) - np.sin(th)], axis=0)
    fu, fh = (f.reshape(2, BLK // 8, 8, BLK).transpose(1, 0, 2, 3).reshape(2 * BLK, BLK)
              for f in (fu, fh))
    cp = (np.cos(ph) + np.sin(ph)).T[:BLK // 2] / (8.0 * BLK * _A * _A)
    cm = (np.cos(ph) - np.sin(ph)).T[:BLK // 2] / (8.0 * BLK * _A * _A)
    return np.concatenate([fu, fh, cp, cm], axis=0).astype(np.float32)


def _layernorm(x, eps, scale=1.0):
    m = jnp.mean(x, axis=-1, keepdims=True)
    d = x - m
    v = jnp.sum(d * d, axis=-1, keepdims=True) * (1.0 / (x.shape[-1] * scale * scale))
    return d * jax.lax.rsqrt(v + eps / (scale * scale))


def _gelu2(y):
    return y * (1.0 + jnp.tanh(y * (y * y + _K)))


def _up(x):
    return pltpu.bitcast(x, BF16)


def _dot(a, b):
    return jnp.dot(a, b, preferred_element_type=F32)


def _lhs_sums(a11, a12, a21, a22):
    return a11 + a22, a21 + a22, a11 + a12, a21 - a11, a12 - a22


def _rhs_sums(b11, b12, b21, b22):
    return b11 + b22, b12 - b22, b21 - b11, b11 + b12, b21 + b22


def _strassen(prod, sa, sb, a11, a22, b11, b22, fin):
    m2 = prod(sa(1), b11)
    m4 = prod(a22, sb(2))
    fin(1, 0, m2 + m4)
    m5 = prod(sa(2), b22)
    c11 = m4 - m5
    m3 = prod(a11, sb(1))
    fin(0, 1, m3 + m5)
    c22 = m3 - m2
    m1 = prod(sa(0), sb(0))
    c11, c22 = c11 + m1, c22 + m1
    fin(0, 0, c11 + prod(sa(4), sb(4)))
    fin(1, 1, c22 + prod(sa(3), sb(3)))


def _lhs_sums_w(a11, a12, a21, a22):
    s1 = a21 + a22
    s2 = s1 - a11
    return s1, s2, a11 - a21, a12 - s2


def _rhs_sums_w(b11, b12, b21, b22):
    t1 = b12 - b11
    t2 = b22 - t1
    return t1, t2, b22 - b12, t2 - b21


def _winograd(prod, sa, sb, a11, a12, a22, b11, b21, b22, fin):
    p1 = prod(a11, b11)
    fin(0, 0, p1 + prod(a12, b21))
    u2 = p1 + prod(sa(1), sb(1))
    p5 = prod(sa(0), sb(0))
    fin(0, 1, (u2 + p5) + prod(sa(3), b22))
    u3 = u2 + prod(sa(2), sb(2))
    fin(1, 1, u3 + p5)
    fin(1, 0, u3 - prod(a22, sb(3)))


def _balance(work, n):
    jobs = [(lo, hi, sum(it[0] for it in items)) for items, lo, hi in work]
    rate = [None] * n
    while jobs:
        def free(a, b):
            return [p for p in range(a, b) if rate[p] is None]
        dens, a, b = max(
            (sum(w for lo, hi, w in jobs if a <= lo and hi <= b) / max(len(free(a, b)), 1e-9), a, b)
            for a in {j[0] for j in jobs} for b in {j[1] for j in jobs} if a < b)
        while a > 0 and rate[a - 1] is not None:
            a -= 1
        while b < n and rate[b] is not None:
            b += 1
        for p in free(a, b):
            rate[p] = dens
        jobs = [(lo, hi, w) for lo, hi, w in jobs if not (a <= lo and hi <= b)]
        jobs = [(b if a <= lo < b else lo, a if a < hi <= b else hi, w) for lo, hi, w in jobs]
    queues = [[lo * 16, hi * 16, list(items)] for items, lo, hi in work]
    rel = [[] for _ in range(n)]
    budget = 0.0
    for tau in range(n * 16):
        budget += (rate[tau // 16] or 0.0) / 16
        while True:
            ready = [q for q in queues if q[2] and q[0] <= tau]
            if not ready:
                budget = min(budget, 0.0)
                break
            q = min(ready, key=lambda q: q[1])
            if budget < 0 and q[1] - tau > len(q[2]):
                break
            it = q[2].pop(0)
            rel[tau // 16].append((tau % 16, it))
            budget -= it[0]
    assert not any(q[2] for q in queues)
    return rel


def _kernel(x_hbm, k_hbm, v_hbm, skt_hbm, h_hbm, dv_hbm, win_hbm, wsp_hbm, b_hbm,
            wout_hbm, tab_hbm, out_hbm,
            x_v, win_v, wsp_v, wout_v, kv_v, h_v, xn_v, z1_v, z2_v, z2b_v, g_v,
            as_v, as2_v, bs_v, gq_v, pp_v, ps_v, ws_v, kvb_v, pl_v, zz_v, bcol_v, o_v,
            zt_v, xs_v, wi_v, raw_v, tab_v,
            sk_v, dd_v, skt_v, dv_v, b_v, zero_s, sem):
    cp = pltpu.make_async_copy
    x16 = x_v.bitcast(BF16)
    win16 = win_v.bitcast(BF16)
    kv16 = kv_v.bitcast(BF16)
    h16 = h_v.bitcast(BF16)

    xn32, z232, kvb32, zz32, as32, as232, bs32, ws32, xs32, wi32 = (
        r.bitcast(U32)
        for r in (xn_v, z2_v, kvb_v, zz_v, as_v, as2_v, bs_v, ws_v, xs_v, wi_v))
    z2b32 = z2b_v.bitcast(U32)
    pp32 = [r.bitcast(U32) for r in pp_v]
    ps32 = [r.bitcast(U32) for r in ps_v]
    wsp16 = wsp_v.bitcast(BF16)

    def wsp_cp(lo, hi, s):
        return cp(wsp_hbm.at[lo:hi, :], wsp16.at[0, lo:hi, :], sem.at[s])

    def x_cp(lo, hi, s):
        return cp(x_hbm.at[0, lo:hi, :], x16.at[0, lo:hi, :], sem.at[s])

    def win_cp(lo, hi, s):
        return cp(win_hbm.at[:, lo:hi], win16.at[0, 0:D, lo:hi], sem.at[s])

    def k_cp(c, s):
        return cp(k_hbm.at[0, :, pl.ds(c * 128, 128)], kv16.at[2 * c, 0:S, :], sem.at[s])

    def v_cp(c, s):
        return cp(v_hbm.at[0, :, pl.ds(c * 128, 128)], kv16.at[2 * c + 1, 0:S, :], sem.at[s])

    def h_cp(c, s):
        return cp(h_hbm.at[pl.ds(c * 128, 128), :], h16.at[c], sem.at[s])

    groups = [
        [cp(b_hbm, b_v, sem.at[0]), cp(skt_hbm, skt_v, sem.at[0]), cp(dv_hbm, dv_v, sem.at[0])],
        [x_cp(0, 256, 1)],
        [win_cp(FH, FH + 256, 2)],
        [win_cp(FH + 256, FH + 512, 3)],
        [win_cp(FH + 512, 2 * FH, 4), win_cp(0, 128, 4)],
        [win_cp(128, 512, 10)],
        [win_cp(512, FH, 5), x_cp(256, 384, 5)],
        [x_cp(384, 6 * T, 6)],
        [x_cp(6 * T, 12 * T, 7), k_cp(0, 7), v_cp(0, 7)],
        [x_cp(12 * T, S, 11), wsp_cp(0, HS // 2, 11), wsp_cp(HS, HS + HS // 2, 11)],
        [cp(tab_hbm, tab_v.bitcast(BF16), sem.at[8]), h_cp(0, 8)],
    ]
    for g in groups:
        for c in g:
            c.start()

    NG = -(-HS // 32 // HF)

    def step_cps(n):
        s = 12 + n
        cps = [k_cp(n + 1, s), v_cp(n + 1, s), h_cp(n + 1, s)]
        if n < HF:
            lo, hi = HS // 2 + n * NG * 16, min(HS // 2 + (n + 1) * NG * 16, HS)
            cps += [wsp_cp(lo, hi, s), wsp_cp(HS + lo, HS + hi, s)]
        return cps

    wout_cp = cp(wout_hbm, wout_v.bitcast(BF16).at[0, 0:FH, :], sem.at[9])
    out_sem = sem.at[5]
    for n in range(NC - 1):
        for d in step_cps(n):
            d.start()
    wout_cp.start()

    def wait(i):
        for c in groups[i]:
            c.wait()

    zero_s[0] = 0
    wait(0)
    skt = skt_v[...].astype(F32)
    dv = dv_v[...].astype(F32).reshape(1, D)
    for c in range(NC):
        sk_v[c] = skt[:, c * 128:(c + 1) * 128]
        dd_v[c] = dv[:, c * 128:(c + 1) * 128]
    brow = b_v[...].astype(F32).reshape(1, S)
    bcol_v[...] = jnp.broadcast_to(brow, (128, S)).T

    def gate_x(tok):
        x_v[0, S // 2:S // 2 + 8, 0:128] = pltpu.bitcast(tok, U32)

    def gate_zt(t):
        def gate(tok):
            zt_v[t % 6][0, T:T + 8, 0:128] = tok
        return gate

    def gate_kv(tok):
        kv_v[0, S // 2:S // 2 + 8, :] = pltpu.bitcast(tok, U32)

    def gate_pl(tok):
        pl_v[0, TOK] = tok

    ndone = [0]
    mode = {'pairs': False}

    def done(val):
        r = (ndone[0] % 8) * 16
        ndone[0] += 1
        if mode['pairs']:
            xs_v[0, 0, 0, r:r + 16, :] = val
        else:
            xn_v[0, S + r:S + r + 16, :] = val

    def lnx_items(t, zero):
        def item(r0):
            def run():
                rs = slice(r0 // 2, r0 // 2 + 8)
                xw = jnp.concatenate([x_v[zero, rs, 0:128], x_v[0, rs, 128:D]], axis=1)
                xn = _layernorm(_up(xw).astype(F32), EPS, _A)
                for c in range(NC):
                    xb = xn[:, c * 128:(c + 1) * 128].astype(BF16)
                    xn_v[c, r0:r0 + 16, :] = xb
                if mode['pairs']:
                    done(xb)
            return (85, gate_x, run)
        return [item(t * T + g * 16) for g in range(T // 16)]

    def lnz_items(t, zero):
        def item(g):
            def run():
                rs = slice(g * 16, (g + 1) * 16)
                z = jnp.concatenate(
                    [zt_v[t % 6][zero, rs, 0:128], zt_v[t % 6][0, rs, 128:FH]], axis=1)
                z = _layernorm(z, 4.0 * _A * _A * EPS)
                r0 = t * T + g * 16
                for n in range(NF):
                    zb = z[:, n * 128:(n + 1) * 128].astype(BF16)
                    (z2_v, z2b_v)[t // HT][n, r0 % HS:r0 % HS + 16, :] = zb
                done(zb)
            return (90, gate_zt(t), run)
        return [item(g) for g in range(T // 16)]

    def kv_items(c):
        sk = sk_v[c]

        def item(r0):
            def run():
                hs = slice(r0 // 2, (r0 + KR) // 2)
                if r0 == 0:
                    kw = jnp.concatenate(
                        [jnp.zeros((8, 128), F32), _up(kv_v[2 * c, hs, :]).astype(F32)], axis=0)
                else:
                    kw = _up(kv_v[2 * c, r0 // 2 - 8:(r0 + KR) // 2, :]).astype(F32)[8:]
                ks = kw[8:] * sk[0:1, :]
                for t in range(1, KS):
                    ks = ks + pltpu.roll(kw, t, 0)[8:] * sk[t:t + 1, :]
                kvb_v[r0:r0 + KR, :] = (
                    ks * _up(kv_v[2 * c + 1, hs, :]).astype(F32)).astype(BF16)
            return (14 * KR // 8, gate_kv, run)
        return [item(r0) for r0 in range(0, S, KR)]

    def gate_w(tok):
        wsp_v[0, S // 2:S // 2 + 8, 0:128] = pltpu.bitcast(tok, U32)

    def asum_items(r_lo, r_hi):
        def item(zero, r0, c0):
            def run():
                def quad(i, j, c):
                    w = wsp_v[zero, (i * HS + r0) // 2:(i * HS + r0) // 2 + 8,
                              j * HS + c * 128:j * HS + (c + 1) * 128]
                    return _up(w).astype(F32)
                for c in range(c0, c0 + AW):
                    for i, v in enumerate(_lhs_sums_w(
                            quad(0, 0, c), quad(0, 1, c), quad(1, 0, c), quad(1, 1, c))):
                        as_v[i, c, r0:r0 + 16, :] = v.astype(BF16)
            return (20 * AW, gate_w, run)
        return lambda zero: [item(zero, r0, c0) for r0 in range(r_lo * T, r_hi * T, 16)
                             for c0 in range(0, HT, AW)]

    def asum_dyn(g, c):
        def run():
            def quad(i, j):
                r0 = pl.multiple_of(i * (HS // 2) + HS // 4 + g * 8, 8)
                w = wsp_v[0, pl.ds(r0, 8), j * HS + c * 128:j * HS + (c + 1) * 128]
                return _up(w).astype(F32)
            rs = pl.ds(pl.multiple_of(g * 16, 16), 16)
            for i, v in enumerate(_lhs_sums_w(quad(0, 0), quad(0, 1), quad(1, 0), quad(1, 1))):
                as2_v[i, c, rs, :] = v.astype(BF16)
        return (20, gate_w, run)

    def gate_z2(tok):
        z2_v[0, HS:HS + 8, :] = tok.astype(BF16)

    def bsum(t):
        def item(zero, r0, n):
            def run():
                def quad(i, j):
                    if i:
                        return z2b_v[n + j * HF, r0:r0 + 16, :].astype(F32)
                    return z2_v[zero + n + j * HF, r0:r0 + 16, :].astype(F32)
                for i, v in enumerate(_rhs_sums_w(quad(0, 0), quad(0, 1), quad(1, 0), quad(1, 1))):
                    bs_v[i, n, r0:r0 + 16, :] = v.astype(BF16)
            return (21, gate_z2, run)
        return lambda zero: [item(zero, r0, n) for r0 in range((t - HT) * T, (t - HT + 1) * T, 16)
                             for n in range(HF)]

    def gate_xn(tok):
        xn_v[1, S:S + 8, :] = tok.astype(BF16)

    def xsum(u):
        def item(zero, g, c):
            def run():
                def quad(i, j):
                    r0 = (2 * u + i) * T + g * 16
                    return xn_v[zero + c + 2 * j, r0:r0 + 16, :].astype(F32)
                for i, v in enumerate(_lhs_sums(quad(0, 0), quad(0, 1), quad(1, 0), quad(1, 1))):
                    xs_v[u, i, c, g * 16:(g + 1) * 16, :] = v.astype(BF16)
            return (24, gate_xn, run)
        return lambda zero: [item(zero, g, c) for g in range(T // 16) for c in range(2)]

    def gate_wi(tok):
        win_v[0, D // 2:D // 2 + 8, 0:128] = pltpu.bitcast(tok, U32)

    def wisum(zero):
        def item(g, q):
            def run():
                def quad(i, j):
                    r0 = (i * KH + g * 16) // 2
                    c0 = ((q // HF) * NF + q % HF + j * HF) * 128
                    return _up(win_v[zero, r0:r0 + 8, c0:c0 + 128]).astype(F32)
                for i, v in enumerate(_rhs_sums(quad(0, 0), quad(0, 1), quad(1, 0), quad(1, 1))):
                    wi_v[i, q, g * 16:(g + 1) * 16, :] = v.astype(BF16)
            return (23, gate_wi, run)
        return [item(g, (q + HF) % NF) for q in range(NF) for g in range(KH // 16)]

    def taps_of(val):
        rows, cols = val.shape
        return [(lambda i=i, n=n: val[i * 8:(i + 1) * 8, n * 128:(n + 1) * 128])
                for n in range(cols // 128) for i in range(rows // 8)]

    def activate(kind, t, n, z):
        if kind == 2:
            zt_v[t % 6][0, 0:T, n * 128:(n + 1) * 128] = _gelu2(z)
        else:
            z1_v[n, t * T:(t + 1) * T, :] = z.astype(BF16)

    def piece(kind, t, n, zero, defer=False, halves=False):
        col = n * 128 + (FH if kind == 2 else 0)
        xn = jnp.concatenate(
            [_up(xn32[zero if zero is not None and c == 0 else c,
                      t * T // 2:(t + 1) * T // 2, :]) for c in range(NC)], axis=1)
        w = _up(win_v[0, 0:D // 2, col:col + 128])
        if halves:
            z = jnp.concatenate([_dot(xn[:T // 2], w), _dot(xn[T // 2:], w)], axis=0)
        else:
            z = _dot(xn, w)
        if defer:
            raw_v[...] = z
        else:
            activate(kind, t, n, z)
        return taps_of(z)

    def pair_piece(kind, u, m, gate_idx, slot_done):
        def xq(i, cs):
            rows = slice((2 * u + i) * T // 2, (2 * u + i + 1) * T // 2)
            return jnp.concatenate([_up(xn32[c, rows, :]) for c in cs], axis=1)

        def wq(lo, hi, j):
            c0 = ((kind - 1) * NF + m + j * HF) * 128
            return _up(win_v[0, lo // 2:hi // 2, c0:c0 + 128])

        def sa(i):
            return jnp.concatenate(
                [_up(xs32[u + (gate_idx() if c == 0 and i != 4 else 0), i, c])
                 for c in range(2)], axis=1)

        def fin(i, j, c):
            z = c + _dot(xq(i, [NC - 1]), wq(2 * KH, D, j))
            activate(kind, 2 * u + i, m + j * HF, z)
            slot_done(taps_of(z))

        _strassen(_dot, sa, lambda i: _up(wi32[i, (kind - 1) * HF + m]),
                  xq(0, (0, 1)), xq(1, (2, 3)), wq(0, KH, 0), wq(KH, 2 * KH, 1), fin)

    pending = []

    def plan(work, zero, n):
        work = [(mk(zero), lo, hi) for mk, lo, hi in work]
        return [a + b for a, b in zip(
            _balance([w for w in work if w[0][0][0] >= 80], n),
            _balance([w for w in work if w[0][0][0] < 80], n))]

    def pair_block(halves, work, lag):
        zero = zero_s[0]
        mode['pairs'] = True
        if pending:
            activate(*pending.pop(), raw_v[...])
        rel = plan(work, zero, 12 * len(halves))
        taps = []
        state = {'gated': False}

        def release(k):
            for i, (_, gate, run) in sorted(rel[k], key=lambda e: e[0]):
                gate(taps[k][i]())
                run()
                state['gated'] = True

        def slot_done(z):
            taps.append(z)
            if len(taps) > lag:
                release(len(taps) - 1 - lag)

        for kind, u in halves:
            for m in range(HF):
                pair_piece(kind, u, m, lambda: zero if state['gated'] else 0, slot_done)
        for k in range(len(taps) - lag, len(taps)):
            release(k)

    def block(pieces, work, defer=True, free=None):
        zero = zero_s[0]
        if pending:
            activate(*pending.pop(), raw_v[...])
        rel = plan(work, zero, len(pieces))
        taps = []
        gated = False
        for k in range(len(pieces) + LAG):
            if free is not None and k == len(pieces) - 1:
                for _, _, run in free(zero):
                    run()
                gated = True
            if k < len(pieces):
                last = defer and k == len(pieces) - 1
                halves = len(pieces) % 4 == 2 and k == len(pieces) - 1
                taps.append(piece(*pieces[k], zero if gated else None, last, halves))
                if last:
                    pending.append(pieces[k])
            if k >= LAG:
                for i, (_, gate, run) in sorted(rel[k - LAG], key=lambda e: e[0]):
                    gate(taps[k - LAG][i]())
                    run()
                    gated = True

    def cols(kind, t, lo=0, hi=NF):
        return [(kind, t, n) for n in range(lo, hi)]

    def lnx(t):
        return lambda zero: lnx_items(t, zero)

    def lnz(t):
        return lambda zero: lnz_items(t, zero)

    wait(1)
    for it in lnx_items(0, 0) + lnx_items(1, 0):
        it[2]()
    wait(2)
    block(cols(2, 0, 0, 2) + cols(2, 1, 0, 2), [])
    wait(3)
    block(cols(2, 0, 2, 4) + cols(2, 1, 2, 4), [])
    wait(4)
    block(cols(2, 0, 4) + cols(2, 1, 4) + cols(1, 0, 0, 1) + cols(1, 1, 0, 1), [])
    wait(5)
    block(cols(1, 0, 1, 4) + cols(1, 1, 1, 4), [(lnz(0), 0, 1)])
    wait(6)
    block(cols(1, 0, 4) + cols(1, 1, 4), [], free=lnx(2))

    def tiles(lo, hi):
        return [pc for t in range(lo, hi) for pc in cols(2, t) + cols(1, t)]

    wait(7)
    block(tiles(2, 4),
          [(lnx(3), 0, 7), (lnx(4), 0, 14), (lnx(5), 0, 15), (lnz(1), 0, 19),
           (wisum, 0, 24), (xsum(2), 17, 24)])
    wait(8)
    pair_block([(2, 2), (1, 2), (2, 3), (1, 3), (2, 4), (1, 4)],
               [(lnx(6), 0, 10), (lnx(7), 0, 10), (xsum(3), 13, 19),
                (lnx(8), 0, 34), (lnx(9), 0, 34), (xsum(4), 37, 43),
                (lnx(10), 0, 61), (lnx(11), 0, 61), (xsum(5), 64, 72),
                (lnz(2), 0, 43), (lnz(3), 0, 43), (lnz(4), 12, 66), (lnz(5), 12, 66),
                (lnz(6), 36, 66), (lnz(7), 36, 66), (kv_items, 0, 72)], 5)
    wait(9)
    pair_block([(2, 5), (1, 5), (2, 6), (2, 7), (1, 6), (1, 7)],
               [(lnx(12), 0, 11), (lnx(13), 0, 11), (xsum(6), 13, 20),
                (lnx(14), 0, 23), (lnx(15), 0, 23), (xsum(7), 25, 32),
                (lnz(8), 0, 32), (lnz(9), 0, 32), (lnz(10), 12, 44), (lnz(11), 12, 44),
                (lnz(12), 36, 54), (lnz(13), 36, 54), (lnz(14), 48, 63), (lnz(15), 48, 63),
                (bsum(8), 36, 72), (bsum(9), 36, 72), (bsum(10), 48, 72), (bsum(11), 48, 72),
                (bsum(12), 58, 72), (bsum(13), 58, 72), (bsum(14), 67, 72), (bsum(15), 67, 72),
                (asum_items(0, HT // 2), 0, 72)], 4)
    wait(10)

    def unit(n, half, k, tap, put_g):
        def span(start, size):
            if isinstance(start, int):
                return slice(start, start + size)
            return pl.ds(pl.multiple_of(start, size), size)

        r = half * (HT // 2) + k
        top, bot = span(r * T, T), span(HS + r * T, T)
        toph, both = span(r * (T // 2), T // 2), span(HS // 2 + r * (T // 2), T // 2)
        sums, sumh = (as32, as232)[half], span(k * (T // 2), T // 2)

        def prod(lhs, rhs):
            acc = None
            for q in range(HS // KG):
                part = _dot(lhs(q), rhs(q))
                acc = part if acc is None else acc + part
                tap(acc)
            return acc

        def sa(i):
            return lambda q: jnp.concatenate(
                [_up(sums[i, c, sumh, :]) for c in range(q * KG // 128, (q + 1) * KG // 128)],
                axis=1)

        def sb(i):
            return lambda q: _up(bs32[i, n, q * KG // 2:(q + 1) * KG // 2, :])

        def a11(q):
            return _up(wsp_v[0, toph, q * KG:(q + 1) * KG])

        def a12(q):
            return _up(wsp_v[0, toph, HS + q * KG:HS + (q + 1) * KG])

        def b21(q):
            return _up(z2b32[n, q * KG // 2:(q + 1) * KG // 2, :])

        def a22(q):
            return _up(wsp_v[0, both, HS + q * KG:HS + (q + 1) * KG])

        def b11(q):
            return _up(z232[n, q * KG // 2:(q + 1) * KG // 2, :])

        def b22(q):
            return _up(z2b32[n + HF, q * KG // 2:(q + 1) * KG // 2, :])

        def fin(i, j, c):
            col, rows = n + j * HF, (top, bot)[i]
            put_g(i, j, col, rows, (c + bcol_v[rows, :]).astype(BF16))

        _winograd(prod, sa, sb, a11, a12, a22, b11, b21, b22, fin)

    def p2(n, half):
        nn = jnp.minimum(n + 1, NC - 1)

        for q in range(half * HF, min((half + 1) * HF, NC - 1)):
            @pl.when(n == q)
            def _():
                for d in step_cps(q):
                    d.wait()

        zero = zero_s[0]
        fwd_u = _up(tab_v[0:128, :])
        fwd_h = _up(tab_v[128:256, :])
        dd = dd_v[n]

        def put(slot, val):
            pl_v[:, slot] = val

        def re_im(val):
            val = val.reshape(BLK // 8, 2, 8, 128)
            return val[:, 0], val[:, 1]

        kvi = kv_items(nn)

        def pace_kv(d, val):
            if d % 4 == 3:
                for j in range(8):
                    _, gate, run = kvi[(d // 4) * 8 + j]
                    gate(val[j * 32:j * 32 + 8, :])
                    run()

        for i in range(NB):
            u = _dot(fwd_u, _up(kvb32[i * BLK // 2:(i + 1) * BLK // 2, :]))
            a, b = re_im(u)
            put(UA + i, a)
            put(UB + i, b)
            put(US + i, a + b)
            pace_kv(i, u)
        for i in range(NB):
            hb = _up(h_v[n, :, i * BLK:(i + 1) * BLK])
            hf = jax.lax.dot_general(fwd_h, hb, (((1,), (1,)), ((), ())),
                                     preferred_element_type=F32)
            c, d = re_im(hf)
            if i == 0:
                c, d = c + dd, d + dd
            put(HR + i, c)
            put(HP + i, d - c)
            put(HQ + i, c + d)
            pace_kv(NB + i, hf)

        state = {}

        def mac_item(pos, g0, pi, j0, j1):
            xv, hv = ((US, HR), (UA, HP), (UB, HQ))[pi]
            outs = range(g0, g0 + GRP)
            top = g0 + GRP

            def run():
                pz = zero + pos
                hs = {t: pl_v[pz, hv + t]
                      for t in range(max(g0 - j1 + 1, 0), top - j0)}
                acc = state['acc'] if j0 else {o: None for o in outs}
                for jj in range(j0, j1):
                    xj = pl_v[pz, xv + jj]
                    for o in outs:
                        if o - jj >= 0:
                            t = xj * hs[o - jj]
                            acc[o] = t if acc[o] is None else acc[o] + t
                if j1 < top:
                    state['acc'] = acc
                    return
                r0 = pos * 8
                if pi == 0:
                    state['k1'] = acc
                elif pi == 1:
                    state['im'] = {o: state['k1'][o] + acc[o] for o in outs}
                else:
                    for o in outs:
                        re, im = state['k1'][o] - acc[o], state['im'][o]
                        zr, zi = re, im
                        if o > 0:
                            zr, zi = re - state['prev'][1], im + state['prev'][0]
                        state['prev'] = (re, im)
                        zz_v[n, o, r0:r0 + 8, :] = zr.astype(BF16)
                        zz_v[n, o, BLK + r0:BLK + r0 + 8, :] = zi.astype(BF16)

            nmac = sum(1 for o in outs for jj in range(j0, j1) if o >= jj)
            return (2 * nmac + ((0, GRP, 5 * GRP)[pi] if j1 == top else 0), gate_pl, run)

        items = []
        for pos in range(BLK // 8):
            for g0 in range(0, NB, GRP):
                top = g0 + GRP
                cuts = [0, top] if top <= SPLIT else [0, (top - 1) // 2, top]
                for pi in range(3):
                    for j0, j1 in zip(cuts[:-1], cuts[1:]):
                        items.append(mac_item(pos, g0, pi, j0, j1))

        if half == 0:
            extra = [asum_dyn(jnp.minimum(n * NG + g, HS // 32 - 1), c)
                     for g in range(NG) for c in range(HT)]
            every = len(items) // len(extra)
            items = [it for i, e in enumerate(extra)
                     for it in items[i * every:(i + 1) * every] + [e]
                     ] + items[len(extra) * every:]

        total = sum(c for c, _, _ in items)
        tap_of = []
        cum = 0
        for c, _, _ in items:
            tap_of.append(int(cum * NTAP / total))
            cum += c
        pos = {'tap': 0, 'item': 0}

        def tap(acc):
            t0 = pos['tap']
            pos['tap'] += T // 8
            while pos['item'] < len(items) and tap_of[pos['item']] < pos['tap']:
                i = tap_of[pos['item']] - t0
                _, gate, run = items[pos['item']]
                gate(acc[i * 8:(i + 1) * 8, :])
                run()
                pos['item'] += 1

        def put_g(i, j, col, rows, val):
            g_v[col, rows, :] = val

        for k in range(HT // 2):
            unit(n - half * HF, half, k, tap, put_g)
        assert pos['item'] == len(items)
        return 0

    jax.lax.fori_loop(0, HF, lambda n, c: p2(n, 0), 0)
    jax.lax.fori_loop(HF, NC, lambda n, c: p2(n, 1), 0)

    wout_cp.wait()

    def p3(j, carry):
        inv_p = _up(tab_v[256:288, :])
        inv_m = _up(tab_v[288:320, :])
        rev = 7 - jax.lax.broadcasted_iota(jnp.int32, (8, 128), 0)

        zero = zero_s[0]
        HK = FH // 2

        def rows(k, i):
            tile = i * HT + (k // 2) * (HT // 2) + 2 * j + k % 2
            return (tile, pl.ds(pl.multiple_of(tile * T, T), T),
                    pl.ds(pl.multiple_of(tile * (T // 2), T // 2), T // 2))

        def fresh(k, n):
            return k >= 2 and n % HF == HF - 1

        def p_tile(k, i, n):
            return _up(pp32[k][i + zero, n])

        def gate_p(tok):
            z1_v[0, S:S + 8, :] = tok.astype(BF16)

        def gate_wo(tok):
            wout_v[0, HK:HK + 8, 0:128] = pltpu.bitcast(tok, U32)

        def psum_item(k, n, g):
            def run():
                def quad(i, jj):
                    rs, gs = rows(k, i)[1], slice(g * 16, (g + 1) * 16)
                    if fresh(k, n):
                        gv = gq_v[k - 2, i, jj, gs, :]
                    else:
                        gv = g_v.at[n + jj * HF, rs][gs, :]
                    pv = _gelu2(z1_v.at[n + jj * HF, rs][gs, :].astype(F32)) * gv.astype(F32)
                    pp_v[k][i, n + jj * HF, g * 16:(g + 1) * 16, :] = pv.astype(BF16)
                    return pv
                for i, v in enumerate(_lhs_sums(quad(0, 0), quad(0, 1), quad(1, 0), quad(1, 1))):
                    ps_v[k][i, n, g * 16:(g + 1) * 16, :] = v.astype(BF16)
            return (gate_p, run)

        def wsum_item(m, g):
            def run():
                def quad(i, jj):
                    r0 = (i * HK + g * 16) // 2
                    c0 = (m + 2 * jj) * 128
                    return _up(wout_v[zero, r0:r0 + 8, c0:c0 + 128]).astype(F32)
                for i, v in enumerate(_rhs_sums(quad(0, 0), quad(0, 1), quad(1, 0), quad(1, 1))):
                    ws_v[i, m, g * 16:(g + 1) * 16, :] = v.astype(BF16)
            return (gate_wo, run)

        def psum(k, cols):
            return [psum_item(k, n, g) for n in cols for g in range(T // 16)]

        queue = []

        def tap(val):
            for i in range(min(len(queue), queue_step[0])):
                gate, run = queue.pop(0)
                r = (i * (T // 8)) // queue_step[0] * 8
                gate(val[r:r + 8, :])
                run()

        queue_step = [0]

        def paced(items, ntaps):
            assert not queue
            queue.extend(items)
            queue_step[0] = -(-len(items) // ntaps)

        def do_unit(u):
            def put_q(i, jj, col, rws, val):
                gq_v[u, i, jj] = val
            unit(HF - 1, 1, 2 * j + u, tap, put_q)

        def finish(k, i, c, o):
            tile, rs, hs = rows(k, i)
            cs = slice(c * 128, (c + 1) * 128)
            ye = _dot(inv_p, _up(zz32[c, tile, 0:64, :]))
            yo = _dot(inv_m, _up(zz32[c, tile, 64:128, :]))
            yd = ye - yo
            y = jnp.concatenate(
                [ye + yo] + [
                    jnp.take_along_axis(yd[q * 8:(q + 1) * 8], rev, axis=0,
                                        mode="promise_in_bounds")
                    for q in reversed(range(BLK // 16))], axis=0)
            gate = o * (1.0 + jnp.tanh((0.25 / _A) * o))
            x = _up(x_v[0, hs, cs]).astype(F32)
            xn = xn_v[c, rs, :].astype(F32)
            o_v[rs, cs] = (x + (xn * y) * gate).astype(BF16)

        def do_pair(k, last=False):
            def prod(lhs, rhs):
                res = _dot(lhs, rhs)
                tap(res)
                return res

            def sa(i):
                return jnp.concatenate([_up(ps32[k][i + zero, n]) for n in range(HF)], axis=1)

            a11 = jnp.concatenate([p_tile(k, 0, n) for n in range(HF)], axis=1)
            a22 = jnp.concatenate([p_tile(k, 1, n) for n in range(HF, NF)], axis=1)
            for m in range(2):
                _strassen(
                    prod, sa, lambda i: _up(ws32[i + zero, m]), a11, a22,
                    _up(wout_v[0, 0:HK // 2, m * 128:(m + 1) * 128]),
                    _up(wout_v[0, HK // 2:HK, (m + 2) * 128:(m + 3) * 128]),
                    lambda i, jj, o: finish(k, i, m + 2 * jj, o))
            for i in range(2):
                rs = rows(k, i)[1]
                if last:
                    cp(o_v.at[rs, 0:512], out_hbm.at[0, rs, 0:512], out_sem).start()
            for i in range(2):
                rs = rows(k, i)[1]
                p = jnp.concatenate([p_tile(k, i, n) for n in range(NF)], axis=1)
                finish(k, i, NC - 1, _dot(p, _up(wout_v[0, 0:HK, 512:D])))
                if last:
                    cp(o_v.at[rs, 512:D], out_hbm.at[0, rs, 512:D], out_sem).start()
                else:
                    cp(o_v.at[rs, :], out_hbm.at[0, rs, :], out_sem).start()

        paced(psum(0, (0, 1, 2)) + [wsum_item(m, g) for m in range(2) for g in range(HK // 16)], 12)
        do_unit(0)
        paced(psum(1, (0, 1, 2)), 12)
        do_pair(0)
        paced(psum(2, (0, 1, 2)), 12)
        do_unit(1)
        paced(psum(3, (0, 1, 2)), 12)
        do_pair(1)
        do_pair(2)
        do_pair(3, last=True)
        return carry

    jax.lax.fori_loop(0, P3I, p3, 0)
    cp(o_v, out_hbm.at[0], out_sem).wait()


@jax.jit
def pallas_recurrent_scan__ssm_conv_h3__mixer_gmlp__prompt_kernel(
    A_q: jax.Array,
    A_k: jax.Array,
    A_v: jax.Array,
    A_shift_k: jax.Array,
    A_ssm_k: jax.Array,
    A_ssm_D: jax.Array,
    B_x: jax.Array,
    B_w_in: jax.Array,
    B_w_sp: jax.Array,
    B_b_sp: jax.Array,
    B_w_out: jax.Array,
):
    del B_x
    tab = jnp.asarray(_dft_tables(), dtype=BF16)

    any_spec = pl.BlockSpec(memory_space=pl.ANY)
    return pl.pallas_call(
        _kernel,
        out_shape=jax.ShapeDtypeStruct((1, S, D), BF16),
        in_specs=[any_spec] * 11,
        out_specs=any_spec,
        scratch_shapes=[
            pltpu.VMEM((1, S // 2 + 32, D), U32),
            pltpu.VMEM((1, D // 2 + 8, 2 * FH), U32),
            pltpu.VMEM((1, S // 2 + 8, S), U32),
            pltpu.VMEM((1, FH // 2 + 32, D), U32),
            pltpu.VMEM((2 * NC, S // 2 + 32, 128), U32),
            pltpu.VMEM((NC, 64, S), U32),
            pltpu.VMEM((NC, S + 256, 128), BF16),
            pltpu.VMEM((NF, S + 64, 128), BF16),
            pltpu.VMEM((NF, HS + 64, 128), BF16),
            pltpu.VMEM((NF, HS, 128), BF16),
            pltpu.VMEM((NF, S, 128), BF16),
            pltpu.VMEM((4, HT, HS // 2, 128), BF16),
            pltpu.VMEM((4, HT, HS // 2, 128), BF16),
            pltpu.VMEM((4, HF, HS, 128), BF16),
            pltpu.VMEM((2, 2, 2, T, 128), BF16),
            [pltpu.VMEM((2, NF, T, 128), BF16)] * 4,
            [pltpu.VMEM((5, HF, T, 128), BF16)] * 4,
            pltpu.VMEM((5, 2, FH // 2, 128), BF16),
            pltpu.VMEM((S, 128), BF16),
            pltpu.VMEM((BLK // 8, 6 * NB + 1, 8, 128), F32),
            pltpu.VMEM((NC, NB, 2 * BLK, 128), BF16),
            pltpu.VMEM((S, 128), F32),
            pltpu.VMEM((S, D), BF16),
            [pltpu.VMEM((1, T + 16, FH), F32)] * 6,
            pltpu.VMEM((NT // 2, 5, 2, T, 128), BF16),
            pltpu.VMEM((5, NF, KH, 128), BF16),
            pltpu.VMEM((T, 128), F32),
            pltpu.VMEM((320, 128), U32),
            pltpu.VMEM((NC, KS, 128), F32),
            pltpu.VMEM((NC + 2, 1, 128), F32),
            pltpu.VMEM((KS, D), BF16),
            pltpu.VMEM((D,), BF16),
            pltpu.VMEM((S,), BF16),
            pltpu.SMEM((1,), jnp.int32),
            pltpu.SemaphoreType.DMA((16,)),
        ],
        compiler_params=pltpu.CompilerParams(
            vmem_limit_bytes=100 * 1024 * 1024, disable_bounds_checks=True),
    )(A_q, A_k, A_v, A_shift_k.T, A_ssm_k, A_ssm_D, B_w_in, B_w_sp, B_b_sp, B_w_out, tab)
```
